```python
import jax
import jax.numpy as jnp

def _softmax(x, axis=-1):
    return jax.nn.softmax(x, axis=axis)
def _gelu(x):
    return jax.nn.gelu(x, approximate=True)
def _silu(x):
    return jax.nn.silu(x)
def _sigmoid(x):
    return jax.nn.sigmoid(x)
def _layernorm(x, axis=-1, eps=1e-5):
    m = jnp.mean(x, axis=axis, keepdims=True)
    v = jnp.var(x, axis=axis, keepdims=True)
    return (x - m) / jnp.sqrt(v + eps)
def _scatter_add(tgt, idx, src, axis=0):
    return tgt.at[idx].add(src)
def _segment_sum(src, seg, n):
    return jax.ops.segment_sum(src, seg, n)
class _Rng:
    def __init__(self, key):
        self._k = key
    def _next(self):
        self._k, sub = jax.random.split(self._k)
        return sub
    def normal(self, shape):
        return jax.random.normal(self._next(), shape, dtype=jnp.bfloat16)
    def randint(self, lo, hi, shape):
        return jax.random.randint(self._next(), shape, lo, hi, dtype=jnp.int32)
    def uniform(self, shape, lo=0.0, hi=1.0):
        return jax.random.uniform(self._next(), shape, jnp.bfloat16, lo, hi)
    def permutation(self, n):
        return jax.random.permutation(self._next(), n)


kernel_name = 'gated_mix__compressed_kv_cla__moe_arch_mod__prompt'

def setup_inputs():
    _rng = _Rng(jax.random.key(int.from_bytes(__import__("os").urandom(4), "little")))
    _w = (lambda a: (lambda t: t.astype(jnp.bfloat16) if jnp.issubdtype(t.dtype, jnp.floating) else t)(jnp.asarray(a)))
    def _A_setup():
        B, H, Sq, Sk, D, M = 1, 16, 2048, 2048, 256, 448
        Dc = 4 * D
        return {
            "x": _w((lambda *s: _rng.normal(s) * 0.05)(B, Sq, M)),
            "c_kv": _w((lambda *s: _rng.normal(s) * 0.05)(B, Sk, Dc)),
            "w_q": _w((lambda *s: _rng.normal(s) * 0.05)(M, H, D) * (M ** -0.5)),
            "w_uk": _w((lambda *s: _rng.normal(s) * 0.05)(Dc, H, D) * (Dc ** -0.5)),
            "w_uv": _w((lambda *s: _rng.normal(s) * 0.05)(Dc, H, D) * (Dc ** -0.5)),
            "w_o": _w((lambda *s: _rng.normal(s) * 0.05)(H, D, M) * ((H * D) ** -0.5)),
        }
    _A_in = _A_setup()

    def _B_setup():
        B, S, D, F, C = 1, 2048, 448, 1792, 2
        return {
            "x": _w((lambda *s: _rng.normal(s) * 0.05)(B, S, D)),
            "w_r": _w((lambda *s: _rng.normal(s) * 0.05)(D)),
            "w_gate": _w((lambda *s: _rng.normal(s) * 0.05)(D, F)),
            "w_up": _w((lambda *s: _rng.normal(s) * 0.05)(D, F)),
            "w_down": _w((lambda *s: _rng.normal(s) * 0.05)(F, D)),
        }
    _B_in = _B_setup()

    return {
        "A_x": _A_in["x"],
        "A_c_kv": _A_in["c_kv"],
        "A_w_q": _A_in["w_q"],
        "A_w_uk": _A_in["w_uk"],
        "A_w_uv": _A_in["w_uv"],
        "A_w_o": _A_in["w_o"],
        "B_x": _B_in["x"],
        "B_w_r": _B_in["w_r"],
        "B_w_gate": _B_in["w_gate"],
        "B_w_up": _B_in["w_up"],
        "B_w_down": _B_in["w_down"],
        "gate_w": _w((lambda *s: _rng.normal(s) * 0.05)(448)),
    }

def reference(A_x, A_c_kv, A_w_q, A_w_uk, A_w_uv, A_w_o, B_x, B_w_r, B_w_gate, B_w_up, B_w_down, gate_w):
    def _A_ref(x, c_kv, w_q, w_uk, w_uv, w_o):
        B, Sq, M = x.shape[0], x.shape[1], x.shape[2]
        Sk = c_kv.shape[1]
        H, D = w_q.shape[1], w_q.shape[2]
        q = jnp.einsum("bqm,mhd->bhqd", x, w_q)
        k = jnp.einsum("bkc,chd->bhkd", c_kv, w_uk)
        v = jnp.einsum("bkc,chd->bhkd", c_kv, w_uv)
        scores = jnp.einsum("bhqd,bhkd->bhqk", q, k) * (D ** -0.5)
        off = Sk - Sq
        qi = jnp.arange(Sq)[:, None]
        kj = jnp.arange(Sk)[None, :]
        cmask = kj <= (qi + off)
        scores = jnp.where(cmask[None, None], scores, -1e9)
        p = _softmax(scores, axis=-1)
        ctx = jnp.einsum("bhqk,bhkd->bhqd", p, v)
        return jnp.einsum("bhqd,hdm->bqm", ctx, w_o)

    def _B_ref(x, w_r, w_gate, w_up, w_down):
        B, S, D = x.shape
        C = 2
        r = x @ w_r
        idx = jnp.argsort(-r, axis=-1)[:, :C]
        idx_e = jnp.repeat(idx.reshape(B, C, 1), D, axis=2)
        x_sel = jnp.take_along_axis(x, idx_e, axis=1)
        g = _silu(x_sel @ w_gate)
        u = x_sel @ w_up
        y = (g * u) @ w_down
        r_sel = _sigmoid(jnp.take_along_axis(r, idx, axis=1))
        y = y * r_sel.reshape(B, C, 1)
        b_off = (jnp.arange(B) * S).reshape(B, 1)
        flat_idx = (idx + b_off).reshape(B * C)
        zero = (x * 0.0).reshape(B * S, D)
        upd = _scatter_add(zero, flat_idx, y.reshape(B * C, D), axis=0)
        return x + upd.reshape(B, S, D)

    x = A_x
    g = _sigmoid((x * gate_w).sum(-1, keepdims=True))
    a = _A_ref(x, A_c_kv, A_w_q, A_w_uk, A_w_uv, A_w_o)
    b = _B_ref(x, B_w_r, B_w_gate, B_w_up, B_w_down)
    return g * a + (1 - g) * b
```

```python
import math

import jax
import jax.numpy as jnp
import jax.experimental.pallas as pl
import jax.experimental.pallas.tpu as pltpu

F32 = jnp.float32
BF16 = jnp.bfloat16
U32 = jnp.uint32
NT = (((1,), (1,)), ((), ()))

LANES = 128
TQ = 256
RC = 512
NCH = 4

S_X, S_Q0, S_Q1, S_K, S_V, S_MISC, S_OUT = 0, 4, 8, 12, 16, 20, 28
N_SEM = 32


def _to_u32(x_f32):
    return pltpu.bitcast(x_f32.astype(BF16), U32)


def _as_bf16(x_u32):
    return pltpu.bitcast(x_u32, BF16)


def _relayout(raw_ref, dst_ref, gs, p0, npairs, pitch, lo, hi):
    for g in gs:
        blk = pltpu.bitcast(raw_ref[pl.ds(2 * p0, 2 * npairs), g], U32)
        for i in range(npairs):
            e, o = blk[2 * i], blk[2 * i + 1]
            dst_ref[2 * g, pl.ds(p0 + i, 8, stride=pitch), :] = (e & lo) | (o << 16)
            dst_ref[2 * g + 1, pl.ds(p0 + i, 8, stride=pitch), :] = (e >> 16) | (o & hi)


def _head_weight(dst_ref, h, nrows, pitch):
    sel = ((h >> 3) << 1) + (h & 1)
    r = (h >> 1) & 3
    return jnp.concatenate(
        [_as_bf16(dst_ref[sel, pl.ds((dt * 4 + r) * pitch, nrows), :]) for dt in range(2)], axis=1)


def _kernel(xT_hbm, c_hbm, wq_hbm, wk_hbm, wv_hbm, wo_hbm, wr_hbm, gw_hbm, wg_hbm, wu_hbm, wd_hbm,
            o_hbm,
            xT_s, c_s, wq_r, wk_r, wv_r, wo_s, wr_s, gw_s, wg_s, wu_s, wd_s,
            x_s, wq_s, wk_s, wv_s, q_s, k_s, v_s, g_s, o_s, sem, *, S, M, DC, H, D):
    nq = S // TQ
    pq = M // 2 + 1
    pk = DC // 2 + 1
    qscale = (D ** -0.5) * math.log2(math.e)
    neg = -1e9 * math.log2(math.e)
    LO = jnp.uint32(0xFFFF)
    HI = jnp.uint32(0xFFFF0000)
    mq = M // NCH
    mk = DC // NCH

    def x_copy(j):
        return pltpu.make_async_copy(xT_hbm.at[:, pl.ds(j * RC, RC)], xT_s.at[:, pl.ds(j * RC, RC)],
                                     sem.at[S_X + j])

    def wq_copy(g, j):
        return pltpu.make_async_copy(wq_hbm.at[pl.ds(j * mq, mq), g], wq_r.at[pl.ds(j * mq, mq), g],
                                     sem.at[(S_Q1 if g else S_Q0) + j])

    def wkv_copy(src, dst, s0, j):
        return pltpu.make_async_copy(src.at[pl.ds(j * mk, mk)], dst.at[pl.ds(j * mk, mk)], sem.at[s0 + j])

    misc = [pltpu.make_async_copy(a, b, sem.at[S_MISC + i]) for i, (a, b) in enumerate(
        [(wr_hbm, wr_s), (gw_hbm, gw_s), (c_hbm, c_s), (wg_hbm, wg_s), (wu_hbm, wu_s), (wd_hbm, wd_s),
         (wo_hbm, wo_s)])]

    def out_copy(j):
        return pltpu.make_async_copy(o_s.at[:, pl.ds(j * RC, RC)], o_hbm.at[:, pl.ds(j * RC, RC)],
                                     sem.at[S_OUT + j])

    x_copy(0).start()
    for j in range(NCH):
        wq_copy(0, j).start()
    for j in range(NCH):
        if j + 1 < NCH:
            x_copy(j + 1).start()
        wq_copy(1, j).start()
    misc[0].start()
    misc[1].start()
    for j in range(NCH):
        wkv_copy(wk_hbm, wk_r, S_K, j).start()
        wkv_copy(wv_hbm, wv_r, S_V, j).start()
    for cp in misc[2:]:
        cp.start()

    def transpose_x(j):
        c0 = j * RC if isinstance(j, int) else pl.multiple_of(j * RC, RC)
        r0 = j * (RC // 2) if isinstance(j, int) else pl.multiple_of(j * (RC // 2), RC // 2)
        for t in range(RC // TQ):
            xt = xT_s[:, pl.ds(c0 + t * TQ, TQ)]
            x_s[pl.ds(r0 + t * (TQ // 2), TQ // 2), :] = pltpu.bitcast(xt.T, U32)

    x_copy(0).wait()
    transpose_x(0)
    for j in range(NCH):
        wq_copy(0, j).wait()
        _relayout(wq_r, wq_s, (0,), j * (mq // 2), mq // 2, pq, LO, HI)

    def q_step(g, j, side):
        r0 = pl.multiple_of(j * (RC // 2), RC // 2)
        xb = _as_bf16(x_s[pl.ds(r0, RC // 2), :])
        never = jax.lax.broadcasted_iota(jnp.int32, (8, LANES), 0) < (j >> 10)
        for hh in range(8):
            h = 8 * g + hh
            q = jnp.dot(xb, _head_weight(wq_s, h, M // 2, pq), preferred_element_type=F32) * qscale
            q_s[h, pl.ds(r0, RC // 2), :] = _to_u32(q)
            for k in range(8):
                piece = pltpu.bitcast(q[(k % 4) * LANES:(k % 4) * LANES + 8,
                                        (k // 4) * LANES:(k // 4 + 1) * LANES], U32)
                side(hh * 8 + k, jnp.where(never, piece, LO), jnp.where(never, piece, HI))

    def q_lo(j, _):
        @pl.when(j + 1 < NCH)
        def _():
            x_copy(j + 1).wait()
        wq_copy(1, j).wait()

        def side(k, lo, hi):
            if k < mq // 2:
                _relayout(wq_r, wq_s, (1,), j * (mq // 2) + k, 1, pq, lo, hi)
        q_step(0, j, side)
        transpose_x((j + 1) & (NCH - 1))
        return 0
    jax.lax.fori_loop(0, NCH, q_lo, 0)

    def q_hi(j, _):
        wkv_copy(wk_hbm, wk_r, S_K, j).wait()
        wkv_copy(wv_hbm, wv_r, S_V, j).wait()
        n = mk // 2 // 64

        def side(k, lo, hi):
            p0 = j * (mk // 2) + k * n
            _relayout(wk_r, wk_s, (0, 1), p0, n, pk, lo, hi)
            _relayout(wv_r, wv_s, (0, 1), p0, n, pk, lo, hi)
        q_step(1, j, side)
        return 0
    jax.lax.fori_loop(0, NCH, q_hi, 0)

    for cp in misc[:6]:
        cp.wait()
    rid = jax.lax.broadcasted_iota(jnp.int32, (8, M), 0)
    wr = jnp.broadcast_to(wr_s[...].reshape(1, M).astype(F32), (8, M))
    gw = jnp.broadcast_to(gw_s[...].reshape(1, M).astype(F32), (8, M))
    w8 = jnp.where(rid == 0, wr, gw).astype(BF16)
    rg = jnp.dot(w8, xT_s[...], preferred_element_type=F32)
    g_s[...] = jax.nn.sigmoid(rg[1:2])
    r = rg[0:1].astype(BF16).astype(F32)
    lane = jax.lax.broadcasted_iota(jnp.int32, (1, S), 1)
    m1 = jnp.max(r, axis=1, keepdims=True)
    i1 = jnp.min(jnp.where(r == m1, lane, S - 1), axis=1, keepdims=True)
    r2 = jnp.where(lane == i1, -jnp.inf, r)
    m2 = jnp.max(r2, axis=1, keepdims=True)
    i2 = jnp.min(jnp.where(jnp.logical_and(r2 == m2, lane != i1), lane, S - 1), axis=1, keepdims=True)
    idx = [i1[0, 0], i2[0, 0]]
    rows = []
    for i in idx:
        w = x_s[pl.ds(i >> 1, 1), :]
        w = jnp.where((i & 1) == 1, w & HI, w << 16)
        rows.append(pltpu.bitcast(w, F32))
    xsel = jnp.where(rid == 0, rows[0], rows[1]).astype(BF16)
    gate = jnp.dot(xsel, wg_s[...], preferred_element_type=F32)
    up = jnp.dot(xsel, wu_s[...], preferred_element_type=F32)
    hid = (jax.nn.silu(gate) * up).astype(BF16)
    y = jax.lax.dot_general(hid, wd_s[...], NT, preferred_element_type=F32)
    rid1 = jax.lax.broadcasted_iota(jnp.int32, (8, 1), 0)
    y = y * jax.nn.sigmoid(jnp.where(rid1 == 0, m1, m2))
    MP = -(-M // LANES) * LANES
    y = jnp.concatenate([y, jnp.zeros((8, MP - M), F32)], axis=1)
    yT = jnp.concatenate([y, jnp.zeros((LANES - 8, MP), F32)], axis=0).T
    ln = jax.lax.broadcasted_iota(jnp.int32, (M, LANES), 1)
    for t, i in enumerate(idx):
        c0 = pl.multiple_of((i >> 7) << 7, LANES)
        blk = xT_s[:, pl.ds(c0, LANES)].astype(F32)
        upd = jnp.where(ln == (i & (LANES - 1)), yT[:M, t:t + 1], 0.0)
        xT_s[:, pl.ds(c0, LANES)] = (blk + upd).astype(BF16)

    row = jax.lax.broadcasted_iota(jnp.int32, (LANES, LANES), 0)
    col = jax.lax.broadcasted_iota(jnp.int32, (LANES, LANES), 1)
    tri = col <= row
    hq = TQ // 2

    def head(h, _):
        wkv = jnp.concatenate([_head_weight(wk_s, h, DC // 2, pk),
                               _head_weight(wv_s, h, DC // 2, pk)], axis=1)

        def proj(i):
            kv = jnp.dot(c_s[i * TQ:(i + 1) * TQ, :], wkv, preferred_element_type=F32)
            k_s[i * hq:(i + 1) * hq, :] = _to_u32(kv[:, :D])
            v_s[i * hq:(i + 1) * hq, :] = _to_u32(kv[:, D:])

        def qk(i):
            q = _as_bf16(q_s[h, i * hq:(i + 1) * hq, :])
            n0 = i * TQ
            n1 = n0 + LANES
            s1 = jax.lax.dot_general(q, _as_bf16(k_s[0:n1 // 2, :]), NT, preferred_element_type=F32)
            s2 = jax.lax.dot_general(q[LANES:], _as_bf16(k_s[n1 // 2:(n1 + LANES) // 2, :]), NT,
                                     preferred_element_type=F32)
            top = jnp.where(tri, s1[:LANES, n0:], neg)
            if n0:
                top = jnp.concatenate([s1[:LANES, :n0], top], axis=1)
            bot = jnp.concatenate([s1[LANES:], jnp.where(tri, s2, neg)], axis=1)
            return top, bot

        def probs(s):
            m = jnp.max(s, axis=1, keepdims=True)
            l = jnp.sum(jnp.exp2(s - m), axis=1, keepdims=True)
            return jnp.exp2(s - (m + jnp.log2(l)))

        def softmax(i, top, bot):
            n1 = i * TQ + LANES
            p_top, p_bot = probs(top), probs(bot)
            return (jnp.concatenate([p_top, p_bot[:, :n1]], axis=0).astype(BF16),
                    p_bot[:, n1:].astype(BF16))

        def pv(i, p1, p2):
            n1 = i * TQ + LANES
            c1 = jnp.dot(p1, _as_bf16(v_s[0:n1 // 2, :]), preferred_element_type=F32)
            c2 = jnp.dot(p2, _as_bf16(v_s[n1 // 2:(n1 + LANES) // 2, :]), preferred_element_type=F32)
            q_s[h, i * hq:i * hq + hq // 2, :] = _to_u32(c1[:LANES])
            q_s[h, i * hq + hq // 2:(i + 1) * hq, :] = _to_u32(c1[LANES:] + c2)

        proj(0)
        proj(1)
        for i in range(nq - 2):
            s = qk(i)
            proj(i + 2)
            pv(i, *softmax(i, *s))
        sa = qk(nq - 2)
        sb = qk(nq - 1)
        pv(nq - 2, *softmax(nq - 2, *sa))
        pv(nq - 1, *softmax(nq - 1, *sb))
        return 0
    jax.lax.fori_loop(0, H, head, 0)

    misc[6].wait()

    def out_step(j, _):
        c0 = pl.multiple_of(j * RC, RC)
        r0 = pl.multiple_of(j * (RC // 2), RC // 2)
        wo = jnp.concatenate([wo_s[h] for h in range(H)], axis=1)
        for t in range(RC // TQ):
            ctx = jnp.concatenate([_as_bf16(q_s[h, pl.ds(r0 + t * hq, hq), :]) for h in range(H)], axis=1)
            a = jax.lax.dot_general(wo, ctx, NT, preferred_element_type=F32)
            gj = g_s[:, pl.ds(c0 + t * TQ, TQ)]
            b = xT_s[:, pl.ds(c0 + t * TQ, TQ)].astype(F32)
            o_s[:, pl.ds(c0 + t * TQ, TQ)] = (gj * a + (1.0 - gj) * b).astype(BF16)
        out_copy(j).start()
        return 0
    jax.lax.fori_loop(0, S // RC, out_step, 0)
    for j in range(S // RC):
        out_copy(j).wait()


def _tile_view(w):
    c, h, d = w.shape
    w = w.reshape(c, h // 8, 8, d // LANES, LANES).transpose(0, 1, 3, 2, 4)
    return w.reshape(c, h // 8, 8 * (d // LANES), LANES)


@jax.jit
def pallas_gated_mix__compressed_kv_cla__moe_arch_mod__prompt_kernel(
    A_x: jax.Array,
    A_c_kv: jax.Array,
    A_w_q: jax.Array,
    A_w_uk: jax.Array,
    A_w_uv: jax.Array,
    A_w_o: jax.Array,
    B_x: jax.Array,
    B_w_r: jax.Array,
    B_w_gate: jax.Array,
    B_w_up: jax.Array,
    B_w_down: jax.Array,
    gate_w: jax.Array,
):
    _, S, M = A_x.shape
    DC = A_c_kv.shape[2]
    H, D = A_w_q.shape[1], A_w_q.shape[2]
    args = (jnp.transpose(A_x[0]), A_c_kv[0], _tile_view(A_w_q), _tile_view(A_w_uk), _tile_view(A_w_uv),
            jnp.transpose(A_w_o, (0, 2, 1)), B_w_r, gate_w, B_w_gate, B_w_up, jnp.transpose(B_w_down))

    def kern(*refs):
        _kernel(*refs, S=S, M=M, DC=DC, H=H, D=D)

    hbm = pl.BlockSpec(memory_space=pl.ANY)
    oT = pl.pallas_call(
        kern,
        out_shape=jax.ShapeDtypeStruct((M, S), A_x.dtype),
        in_specs=[hbm] * len(args),
        out_specs=hbm,
        scratch_shapes=[pltpu.VMEM(a.shape, a.dtype) for a in args] + [
            pltpu.VMEM((S // 2, M), U32),
            pltpu.VMEM((4, 8 * (M // 2 + 1), LANES), U32),
            pltpu.VMEM((4, 8 * (DC // 2 + 1), LANES), U32),
            pltpu.VMEM((4, 8 * (DC // 2 + 1), LANES), U32),
            pltpu.VMEM((H, S // 2, D), U32),
            pltpu.VMEM((S // 2, D), U32),
            pltpu.VMEM((S // 2, D), U32),
            pltpu.VMEM((1, S), F32),
            pltpu.VMEM((M, S), BF16),
            pltpu.SemaphoreType.DMA((N_SEM,)),
        ],
        compiler_params=pltpu.CompilerParams(vmem_limit_bytes=120 * 1024 * 1024),
    )(*args)
    return jnp.transpose(oT)[None]
```

```python
import math

import jax
import jax.numpy as jnp
import jax.experimental.pallas as pl
import jax.experimental.pallas.tpu as pltpu

F32 = jnp.float32
BF16 = jnp.bfloat16
U32 = jnp.uint32
NT = (((1,), (1,)), ((), ()))

LANES = 128
TQ = 256
RC = 512
NCH = 4

S_X, S_Q0, S_Q1, S_K, S_V, S_C, S_MISC, S_OUT = 0, 4, 8, 12, 16, 20, 24, 30
N_SEM = 34


def _to_u32(x_f32):
    return pltpu.bitcast(x_f32.astype(BF16), U32)


def _as_bf16(x_u32):
    return pltpu.bitcast(x_u32, BF16)


def _relayout(raw_ref, dst_ref, gs, p0, npairs, pitch, lo, hi):
    for g in gs:
        blk = pltpu.bitcast(raw_ref[pl.ds(2 * p0, 2 * npairs), g], U32)
        for i in range(npairs):
            e, o = blk[2 * i], blk[2 * i + 1]
            dst_ref[2 * g, pl.ds(p0 + i, 8, stride=pitch), :] = (e & lo) | (o << 16)
            dst_ref[2 * g + 1, pl.ds(p0 + i, 8, stride=pitch), :] = (e >> 16) | (o & hi)


def _head_weight(dst_ref, h, nrows, pitch):
    sel = ((h >> 3) << 1) + (h & 1)
    r = (h >> 1) & 3
    return jnp.concatenate(
        [_as_bf16(dst_ref[sel, pl.ds((dt * 4 + r) * pitch, nrows), :]) for dt in range(2)], axis=1)


def _kernel(xT_hbm, c_hbm, wq_hbm, wk_hbm, wv_hbm, wo_hbm, wr_hbm, gw_hbm, wg_hbm, wu_hbm, wd_hbm,
            o_hbm,
            xT_s, c_s, wq_r, wk_r, wv_r, wo_s, wr_s, gw_s, wg_s, wu_s, wd_s,
            x_s, wq_s, a_s, b_s, q_s, k_s, v_s, g_s, o_s, sem, *, S, M, DC, H, D):
    nq = S // TQ
    pq = M // 2 + 1
    pb = DC // 4 + 1
    qscale = (D ** -0.5) * math.log2(math.e)
    neg = -1e9 * math.log2(math.e)
    LO = jnp.uint32(0xFFFF)
    HI = jnp.uint32(0xFFFF0000)
    mq = M // NCH
    mk = DC // NCH

    def x_copy(j):
        return pltpu.make_async_copy(xT_hbm.at[:, pl.ds(j * RC, RC)], xT_s.at[:, pl.ds(j * RC, RC)],
                                     sem.at[S_X + j])

    def wq_copy(g, j):
        return pltpu.make_async_copy(wq_hbm.at[pl.ds(j * mq, mq), g], wq_r.at[pl.ds(j * mq, mq), g],
                                     sem.at[(S_Q1 if g else S_Q0) + j])

    def wkv_copy(src, dst, s0, j):
        return pltpu.make_async_copy(src.at[pl.ds(j * mk, mk)], dst.at[pl.ds(j * mk, mk)], sem.at[s0 + j])

    misc = [pltpu.make_async_copy(a, b, sem.at[S_MISC + i]) for i, (a, b) in enumerate(
        [(wr_hbm, wr_s), (gw_hbm, gw_s), (wg_hbm, wg_s), (wu_hbm, wu_s), (wd_hbm, wd_s), (wo_hbm, wo_s)])]

    def c_copy(j):
        return pltpu.make_async_copy(c_hbm.at[pl.ds(j * RC, RC)], c_s.at[pl.ds(j * RC, RC)], sem.at[S_C + j])

    def out_copy(j):
        return pltpu.make_async_copy(o_s.at[:, pl.ds(j * RC, RC)], o_hbm.at[:, pl.ds(j * RC, RC)],
                                     sem.at[S_OUT + j])

    x_copy(0).start()
    for j in range(NCH):
        wq_copy(0, j).start()
    for j in range(NCH):
        if j + 1 < NCH:
            x_copy(j + 1).start()
        wq_copy(1, j).start()
    misc[0].start()
    misc[1].start()
    for j in range(NCH):
        c_copy(j).start()
        wkv_copy(wk_hbm, wk_r, S_K, j).start()
        wkv_copy(wv_hbm, wv_r, S_V, j).start()
    for cp in misc[2:]:
        cp.start()

    def transpose_x(j):
        c0 = j * RC if isinstance(j, int) else pl.multiple_of(j * RC, RC)
        r0 = j * (RC // 2) if isinstance(j, int) else pl.multiple_of(j * (RC // 2), RC // 2)
        for t in range(RC // TQ):
            xt = xT_s[:, pl.ds(c0 + t * TQ, TQ)]
            x_s[pl.ds(r0 + t * (TQ // 2), TQ // 2), :] = pltpu.bitcast(xt.T, U32)

    x_copy(0).wait()
    transpose_x(0)
    for j in range(NCH):
        wq_copy(0, j).wait()
        _relayout(wq_r, wq_s, (0,), j * (mq // 2), mq // 2, pq, LO, HI)

    def q_step(g, j, side):
        r0 = pl.multiple_of(j * (RC // 2), RC // 2)
        xb = _as_bf16(x_s[pl.ds(r0, RC // 2), :])
        for hh in range(8):
            h = 8 * g + hh
            q = jnp.dot(xb, _head_weight(wq_s, h, M // 2, pq), preferred_element_type=F32) * qscale
            q_s[h, pl.ds(r0, RC // 2), :] = _to_u32(q)
            for k in range(8):
                side(hh * 8 + k, q[(k % 4) * LANES:(k % 4) * LANES + 8,
                                   (k // 4) * LANES:(k // 4 + 1) * LANES])

    def q_lo(j, _):
        @pl.when(j + 1 < NCH)
        def _():
            x_copy(j + 1).wait()
        wq_copy(1, j).wait()

        never = jax.lax.broadcasted_iota(jnp.int32, (8, LANES), 0) < (j >> 10)

        def side(k, piece):
            if k < mq // 2:
                piece = pltpu.bitcast(piece, U32)
                _relayout(wq_r, wq_s, (1,), j * (mq // 2) + k, 1, pq,
                          jnp.where(never, piece, LO), jnp.where(never, piece, HI))
        q_step(0, j, side)
        transpose_x((j + 1) & (NCH - 1))
        return 0
    jax.lax.fori_loop(0, NCH, q_lo, 0)

    def unpack(w, par):
        return pltpu.unpack_elementwise(w, index=par, packed_dtype=BF16, unpacked_dtype=F32)

    def q_hi(j, _):
        c_copy(j).wait()
        wkv_copy(wk_hbm, wk_r, S_K, j).wait()
        wkv_copy(wv_hbm, wv_r, S_V, j).wait()
        never = jax.lax.broadcasted_iota(jnp.int32, (8, LANES), 0) < (j >> 10)

        def side(k, piece):
            rg, t = k // 4, k % 4
            a = []
            for rb in range(2):
                r0 = pl.multiple_of(j * RC + rb * TQ + rg * 16, 16)
                for ch in range(2):
                    a.append(c_s[pl.ds(r0, 16), (2 * t + ch) * LANES:(2 * t + ch + 1) * LANES].astype(F32))
            a11, a12, a21, a22 = a
            a11 = jnp.where(jnp.concatenate([never, never], axis=0),
                            jnp.concatenate([piece, piece], axis=0), a11)
            ops = [_to_u32(o) for o in (a11 + a22, a21 + a22, a11, a22, a11 + a12, a21 - a11, a12 - a22)]
            d0 = pl.multiple_of(j * (TQ // 2) + rg * 8, 8)
            for n, o in enumerate(ops):
                a_s[n, pl.ds(d0, 8), t * LANES:(t + 1) * LANES] = o
            link = ops[0] | ops[4] | ops[5] | ops[1] | ops[6]
            c0 = j * mk + 2 * k
            for g in range(2):
                w = [pltpu.bitcast(r[pl.ds(c0 + o, 2), g], U32) for o in (0, LANES) for r in (wk_r, wv_r)]
                w = [[x[0], x[1]] for x in w]
                w[0][0] = jnp.where(never, link, w[0][0])
                for par in range(2):
                    outs = []
                    for e in range(2):
                        b11, b12, b21, b22 = [unpack(x[e], par) for x in w]
                        outs.append((b11 + b22, b11, b12 - b22, b21 - b11, b22, b11 + b12, b21 + b22))
                    for n in range(7):
                        b_s[n, 2 * g + par, pl.ds(j * (mk // 4) + k, 8, stride=pb), :] = pltpu.bitcast(
                            pltpu.pack_elementwise([outs[0][n], outs[1][n]], packed_dtype=BF16), U32)
        q_step(1, j, side)
        return 0
    jax.lax.fori_loop(0, NCH, q_hi, 0)

    for cp in misc[:5]:
        cp.wait()
    rid = jax.lax.broadcasted_iota(jnp.int32, (8, M), 0)
    wr = jnp.broadcast_to(wr_s[...].reshape(1, M).astype(F32), (8, M))
    gw = jnp.broadcast_to(gw_s[...].reshape(1, M).astype(F32), (8, M))
    w8 = jnp.where(rid == 0, wr, gw).astype(BF16)
    rg = jnp.dot(w8, xT_s[...], preferred_element_type=F32)
    g_s[...] = jax.nn.sigmoid(rg[1:2])
    r = rg[0:1].astype(BF16).astype(F32)
    lane = jax.lax.broadcasted_iota(jnp.int32, (1, S), 1)
    m1 = jnp.max(r, axis=1, keepdims=True)
    i1 = jnp.min(jnp.where(r == m1, lane, S - 1), axis=1, keepdims=True)
    r2 = jnp.where(lane == i1, -jnp.inf, r)
    m2 = jnp.max(r2, axis=1, keepdims=True)
    i2 = jnp.min(jnp.where(jnp.logical_and(r2 == m2, lane != i1), lane, S - 1), axis=1, keepdims=True)
    idx = [i1[0, 0], i2[0, 0]]
    rows = []
    for i in idx:
        w = x_s[pl.ds(i >> 1, 1), :]
        w = jnp.where((i & 1) == 1, w & HI, w << 16)
        rows.append(pltpu.bitcast(w, F32))
    xsel = jnp.where(rid == 0, rows[0], rows[1]).astype(BF16)
    gate = jnp.dot(xsel, wg_s[...], preferred_element_type=F32)
    up = jnp.dot(xsel, wu_s[...], preferred_element_type=F32)
    hid = (jax.nn.silu(gate) * up).astype(BF16)
    y = jax.lax.dot_general(hid, wd_s[...], NT, preferred_element_type=F32)
    rid1 = jax.lax.broadcasted_iota(jnp.int32, (8, 1), 0)
    y = y * jax.nn.sigmoid(jnp.where(rid1 == 0, m1, m2))
    MP = -(-M // LANES) * LANES
    y = jnp.concatenate([y, jnp.zeros((8, MP - M), F32)], axis=1)
    yT = jnp.concatenate([y, jnp.zeros((LANES - 8, MP), F32)], axis=0).T
    ln = jax.lax.broadcasted_iota(jnp.int32, (M, LANES), 1)
    for t, i in enumerate(idx):
        c0 = pl.multiple_of((i >> 7) << 7, LANES)
        blk = xT_s[:, pl.ds(c0, LANES)].astype(F32)
        upd = jnp.where(ln == (i & (LANES - 1)), yT[:M, t:t + 1], 0.0)
        xT_s[:, pl.ds(c0, LANES)] = (blk + upd).astype(BF16)

    row = jax.lax.broadcasted_iota(jnp.int32, (LANES, LANES), 0)
    col = jax.lax.broadcasted_iota(jnp.int32, (LANES, LANES), 1)
    tri = col <= row
    hq = TQ // 2

    def head(h, _):
        sel = ((h >> 3) << 1) + (h & 1)
        r = (h >> 1) & 3
        never = jax.lax.broadcasted_iota(jnp.int32, (8, LANES), 0) < (h >> 10)
        never2 = jnp.concatenate([never, never], axis=0)
        prods = {}

        def spots(v, cols):
            return [v[rr:rr + 8, n * LANES:(n + 1) * LANES] for n in cols for rr in (0, 64, 128, 192)]

        def proj(k, part):
            pieces = []
            for n in ((0, 3, 4, 6), (1, 2, 5))[part]:
                w = jnp.concatenate([_as_bf16(b_s[n, sel, pl.ds((dt * 4 + r) * pb, DC // 4), :])
                                     for dt in range(2)], axis=1)
                prods[n + 1] = jnp.dot(_as_bf16(a_s[n, k * hq:(k + 1) * hq, :]), w,
                                       preferred_element_type=F32)
                pieces += spots(prods[n + 1], (0, 1))
            m = prods
            t0, t1 = 2 * k * hq, (2 * k + 1) * hq
            if part == 0:
                k_s[t0:t0 + hq, :] = _to_u32((m[1] + m[4]) + (m[7] - m[5]))
            else:
                k_s[t1:t1 + hq, :] = _to_u32(m[2] + m[4])
                v_s[t0:t0 + hq, :] = _to_u32(m[3] + m[5])
                v_s[t1:t1 + hq, :] = _to_u32((m[1] - m[2]) + (m[3] + m[6]))
            return pieces

        def qk(i):
            q = _as_bf16(q_s[h, i * hq:(i + 1) * hq, :])
            n0 = i * TQ
            n1 = n0 + LANES
            s1 = jax.lax.dot_general(q, _as_bf16(k_s[0:n1 // 2, :]), NT, preferred_element_type=F32)
            s2 = jax.lax.dot_general(q[LANES:], _as_bf16(k_s[n1 // 2:(n1 + LANES) // 2, :]), NT,
                                     preferred_element_type=F32)
            top = jnp.where(tri, s1[:LANES, n0:], neg)
            if n0:
                top = jnp.concatenate([s1[:LANES, :n0], top], axis=1)
            bot = jnp.concatenate([s1[LANES:], jnp.where(tri, s2, neg)], axis=1)
            return (top, bot), spots(s1, range(n0 // LANES))

        def softmax(i, top, bot, pieces):
            n1 = i * TQ + LANES
            G = 16
            ps, prev = [], None
            for k in range(TQ // G):
                r0 = (k * G) % LANES
                s = (top if k * G < LANES else bot)[r0:r0 + G]
                tiles = [s[:, t:t + LANES] for t in range(0, s.shape[1], LANES)]
                link = pieces[int(0.8 * k / 16 * len(pieces))]
                if prev is not None:
                    link = jnp.where(never, link, prev)
                m = jnp.broadcast_to(jnp.max(s, axis=1, keepdims=True), (G, LANES))
                m = jnp.where(never2, jnp.concatenate([link, link], axis=0), m)
                acc = None
                for t in tiles:
                    e = jnp.exp2(t - m)
                    acc = e if acc is None else acc + e
                prev = acc[8:]
                m = m + jnp.log2(jnp.sum(acc, axis=1, keepdims=True))
                ps.append(jnp.concatenate([jnp.exp2(t - m) for t in tiles], axis=1))
            nh = LANES // G
            return (jnp.concatenate(ps[:nh] + [p[:, :n1] for p in ps[nh:]], axis=0).astype(BF16),
                    jnp.concatenate([p[:, n1:] for p in ps[nh:]], axis=0).astype(BF16))

        def pv(i, p1, p2):
            n1 = i * TQ + LANES
            c1, pieces = None, []
            for c0 in range(0, n1, 512):
                ce = min(c0 + 512, n1)
                part = jnp.dot(p1[:, c0:ce], _as_bf16(v_s[c0 // 2:ce // 2, :]), preferred_element_type=F32)
                c1 = part if c1 is None else c1 + part
                pieces += spots(c1, (0, 1))
            c2 = jnp.dot(p2, _as_bf16(v_s[n1 // 2:(n1 + LANES) // 2, :]), preferred_element_type=F32)
            q_s[h, i * hq:i * hq + hq // 2, :] = _to_u32(c1[:LANES])
            q_s[h, i * hq + hq // 2:(i + 1) * hq, :] = _to_u32(c1[LANES:] + c2)
            return pieces

        proj(0, 0)
        proj(0, 1)
        for i in range(nq - 2):
            s, _ = qk(i)
            pieces = proj((i + 2) // 2, i % 2)
            pv(i, *softmax(i, *s, pieces))
        sa, _ = qk(nq - 2)
        sb, pieces = qk(nq - 1)
        pieces = pv(nq - 2, *softmax(nq - 2, *sa, pieces))
        pv(nq - 1, *softmax(nq - 1, *sb, pieces))
        return 0
    jax.lax.fori_loop(0, H, head, 0)

    misc[5].wait()

    def out_step(j, _):
        c0 = pl.multiple_of(j * RC, RC)
        r0 = pl.multiple_of(j * (RC // 2), RC // 2)
        wo = jnp.concatenate([wo_s[h] for h in range(H)], axis=1)
        for t in range(RC // TQ):
            ctx = jnp.concatenate([_as_bf16(q_s[h, pl.ds(r0 + t * hq, hq), :]) for h in range(H)], axis=1)
            a = jax.lax.dot_general(wo, ctx, NT, preferred_element_type=F32)
            gj = g_s[:, pl.ds(c0 + t * TQ, TQ)]
            b = xT_s[:, pl.ds(c0 + t * TQ, TQ)].astype(F32)
            o_s[:, pl.ds(c0 + t * TQ, TQ)] = (gj * a + (1.0 - gj) * b).astype(BF16)
        out_copy(j).start()
        return 0
    jax.lax.fori_loop(0, S // RC, out_step, 0)
    for j in range(S // RC):
        out_copy(j).wait()


def _tile_view(w):
    c, h, d = w.shape
    w = w.reshape(c, h // 8, 8, d // LANES, LANES).transpose(0, 1, 3, 2, 4)
    return w.reshape(c, h // 8, 8 * (d // LANES), LANES)


@jax.jit
def pallas_gated_mix__compressed_kv_cla__moe_arch_mod__prompt_kernel(
    A_x: jax.Array,
    A_c_kv: jax.Array,
    A_w_q: jax.Array,
    A_w_uk: jax.Array,
    A_w_uv: jax.Array,
    A_w_o: jax.Array,
    B_x: jax.Array,
    B_w_r: jax.Array,
    B_w_gate: jax.Array,
    B_w_up: jax.Array,
    B_w_down: jax.Array,
    gate_w: jax.Array,
):
    _, S, M = A_x.shape
    DC = A_c_kv.shape[2]
    H, D = A_w_q.shape[1], A_w_q.shape[2]
    args = (jnp.transpose(A_x[0]), A_c_kv[0], _tile_view(A_w_q), _tile_view(A_w_uk), _tile_view(A_w_uv),
            jnp.transpose(A_w_o, (0, 2, 1)), B_w_r, gate_w, B_w_gate, B_w_up, jnp.transpose(B_w_down))

    def kern(*refs):
        _kernel(*refs, S=S, M=M, DC=DC, H=H, D=D)

    hbm = pl.BlockSpec(memory_space=pl.ANY)
    oT = pl.pallas_call(
        kern,
        out_shape=jax.ShapeDtypeStruct((M, S), A_x.dtype),
        in_specs=[hbm] * len(args),
        out_specs=hbm,
        scratch_shapes=[pltpu.VMEM(a.shape, a.dtype) for a in args] + [
            pltpu.VMEM((S // 2, M), U32),
            pltpu.VMEM((4, 8 * (M // 2 + 1), LANES), U32),
            pltpu.VMEM((7, S // 4, DC // 2), U32),
            pltpu.VMEM((7, 4, 8 * (DC // 4 + 1), LANES), U32),
            pltpu.VMEM((H, S // 2, D), U32),
            pltpu.VMEM((S // 2, D), U32),
            pltpu.VMEM((S // 2, D), U32),
            pltpu.VMEM((1, S), F32),
            pltpu.VMEM((M, S), BF16),
            pltpu.SemaphoreType.DMA((N_SEM,)),
        ],
        compiler_params=pltpu.CompilerParams(vmem_limit_bytes=120 * 1024 * 1024),
    )(*args)
    return jnp.transpose(oT)[None]
```

```python
import math

import jax
import jax.numpy as jnp
import jax.experimental.pallas as pl
import jax.experimental.pallas.tpu as pltpu

F32 = jnp.float32
BF16 = jnp.bfloat16
U32 = jnp.uint32
NT = (((1,), (1,)), ((), ()))

L = 128
TQ = 256
HQ = TQ // 2
RC = 512
NCH = 4

S_X, S_Q0, S_Q1, S_K, S_V, S_C, S_MISC, S_OUT = 0, 4, 8, 12, 16, 20, 24, 30
N_SEM = 34

LOOP_ORDER = ("Q7 a3 S7 V7 Q6 b3 S6 V6 w3 Q5 a2 S5 V5 Q4 b2 S4 V4 w2 "
              "Q3 a1 S3 V3 Q2 b1 S2 V2 w1 Q1 a0 S1 V1 Q0 b0 S0 V0 w0")
LAST_ORDER = "Q7 Q6 S7 Q5 S6 V7 Q4 S5 V6 Q3 S4 V5 Q2 S3 V4 Q1 S2 V3 Q0 S1 V2 S0 V1 V0"


def _to_u32(x_f32):
    return pltpu.bitcast(x_f32.astype(BF16), U32)


def _as_bf16(x_u32):
    return pltpu.bitcast(x_u32, BF16)


def _left(a11, a12, a21, a22):
    return (a11 + a22, a21 + a22, a11, a22, a11 + a12, a21 - a11, a12 - a22)


def _right(b11, b12, b21, b22):
    return (b11 + b22, b11, b12 - b22, b21 - b11, b22, b11 + b12, b21 + b22)


def _c11(m):
    return (m[0] + m[3]) + (m[6] - m[4])


def _c12(m):
    return m[2] + m[4]


def _c21(m):
    return m[1] + m[3]


def _c22(m):
    return (m[0] - m[1]) + (m[2] + m[5])


def _never(i):
    return jax.lax.broadcasted_iota(jnp.int32, (8, L), 0) < (i >> 10)


def _or_all(xs):
    out = xs[0]
    for x in xs[1:]:
        out = out | x
    return out


def _relayout(raw_ref, dst_ref, g, p0, npairs, pitch, lo, hi):
    blk = pltpu.bitcast(raw_ref[pl.ds(2 * p0, 2 * npairs), g], U32)
    for i in range(npairs):
        e, o = blk[2 * i], blk[2 * i + 1]
        dst_ref[2 * g, pl.ds(p0 + i, 8, stride=pitch), :] = (e & lo) | (o << 16)
        dst_ref[2 * g + 1, pl.ds(p0 + i, 8, stride=pitch), :] = (e >> 16) | (o & hi)


def _head_weight(ref, h, nrows, pitch):
    sel = ((h >> 3) << 1) + (h & 1)
    r = (h >> 1) & 3
    return jnp.concatenate(
        [_as_bf16(ref[sel, pl.ds((dt * 4 + r) * pitch, nrows), :]) for dt in range(2)], axis=1)


def _kernel(xT_hbm, c_hbm, wq_hbm, wk_hbm, wv_hbm, wo_hbm, wr_hbm, gw_hbm, wg_hbm, wu_hbm, wd_hbm,
            o_hbm,
            xT_s, wo_s, a_s, b_s, q_s, k_s, v_s, v5_s, wo7_s, g_s, o_s, sem, *, S, M, DC, H, D):
    nq = S // TQ
    pq = M // 2 + 1
    pb = DC // 4 + 1
    mq = M // NCH
    mk = DC // NCH
    qscale = (D ** -0.5) * math.log2(math.e)
    neg = -1e9 * math.log2(math.e)
    LO = jnp.uint32(0xFFFF)
    HI = jnp.uint32(0xFFFF0000)
    wo_copy = pltpu.make_async_copy(wo_hbm, wo_s, sem.at[S_MISC + 5])

    def out_copy(j):
        return pltpu.make_async_copy(o_s.at[:, pl.ds(j * RC, RC)], o_hbm.at[:, pl.ds(j * RC, RC)],
                                     sem.at[S_OUT + j])

    tri = (jax.lax.broadcasted_iota(jnp.int32, (L, L), 1) <= jax.lax.broadcasted_iota(jnp.int32, (L, L), 0))

    def head_program(order, h, hn, x7_s, two_pass, hooks=None):
        never = _never(hn)
        never2 = jnp.concatenate([never, never], axis=0)
        prods, held, waiting = {}, {}, []

        def spots(v, cols, rows=(0, 64, 128, 192)):
            return [v[r:r + 8, n * L:(n + 1) * L] for n in cols for r in rows]

        def tie(lhs, links, every):
            rows = []
            for rg in range(lhs.shape[0] // 8):
                blk = lhs[rg * 8:(rg + 1) * 8]
                if links and rg % every == 0:
                    blk = jnp.concatenate([jnp.where(never, links.pop(0), blk[:, :L]), blk[:, L:]], axis=1)
                rows.append(blk)
            return jnp.concatenate(rows, axis=0)

        def proj(k, part):
            ns = ((0, 3, 4, 6), (1, 2, 5))[part]
            links = list(waiting)
            del waiting[:]
            per = -(-len(links) // len(ns))
            pieces = []
            for n in ns:
                lhs = a_s[n, k * HQ:(k + 1) * HQ, :]
                mine, links = links[:per], links[per:]
                if mine:
                    lhs = tie(lhs, mine, 16 // per)
                prods[n] = jnp.dot(_as_bf16(lhs), _head_weight(b_s.at[n], hn, DC // 4, pb),
                                   preferred_element_type=F32)
                pieces += spots(prods[n], (0, 1))
            if part == 0:
                held[2 * k, "k"] = _to_u32(_c11(prods))
            else:
                held[2 * k + 1, "k"] = _to_u32(_c21(prods))
                for ch, v in ((2 * k, _c12(prods)), (2 * k + 1, _c22(prods))):
                    held[ch, "v"] = _to_u32(v)
                    if ch < nq - 1:
                        ops = _right(v[:L, :L], v[:L, L:], v[L:, :L], v[L:, L:])
                        held[ch, "r"] = [_to_u32(ops[n]) for n in (0, 2, 3, 5, 6)]
            return pieces

        def write_kv(k):
            for ch in (2 * k, 2 * k + 1):
                k_s[ch * HQ:(ch + 1) * HQ, :] = held[ch, "k"]
                v_s[ch * HQ:(ch + 1) * HQ, :] = held[ch, "v"]
                for n, o in enumerate(held.get((ch, "r"), ())):
                    v5_s[n, ch * 64:(ch + 1) * 64, :] = o

        def qk(i):
            q = _as_bf16(q_s[h, i * HQ:(i + 1) * HQ, :])
            n0 = i * TQ
            n1 = n0 + L
            s1 = jax.lax.dot_general(q, _as_bf16(k_s[0:n1 // 2, :]), NT, preferred_element_type=F32)
            s2 = jax.lax.dot_general(q[L:], _as_bf16(k_s[n1 // 2:(n1 + L) // 2, :]), NT,
                                     preferred_element_type=F32)
            top = jnp.where(tri, s1[:L, n0:], neg)
            if n0:
                top = jnp.concatenate([s1[:L, :n0], top], axis=1)
            bot = jnp.concatenate([s1[L:], jnp.where(tri, s2, neg)], axis=1)
            return (top, bot), spots(s1, range(max(1, n0 // L)))

        def softmax(i, top, bot, pieces):
            G = 16
            lo = 0.0 if two_pass else 0.15
            p, sums, prev = ([], []), ([], []), None
            for k in range(TQ // G):
                half = k % 2
                s = (top, bot)[half][(k // 2) * G:(k // 2 + 1) * G]
                tiles = [s[:, t:t + L] for t in range(0, s.shape[1], L)]
                link = pieces[int((lo + (0.8 - lo) * k / 16) * len(pieces))]
                if prev is not None:
                    link = jnp.where(never, link, prev)
                m = jnp.broadcast_to(jnp.max(s, axis=1, keepdims=True), (G, L))
                m = jnp.where(never2, jnp.concatenate([link, link], axis=0), m)
                e = [jnp.exp2(t - m) for t in tiles]
                acc = e[0]
                for x in e[1:]:
                    acc = acc + x
                prev = acc[8:]
                if two_pass:
                    m = m + jnp.log2(jnp.sum(acc, axis=1, keepdims=True))
                    e = [jnp.exp2(t - m) for t in tiles]
                sums[half].append(acc)
                p[half].append(jnp.concatenate(e, axis=1))
            pt, pb_ = jnp.concatenate(p[0], axis=0), jnp.concatenate(p[1], axis=0)

            def tile(x, t):
                return x[:, t * L:(t + 1) * L]
            ops = [_left(tile(pt, 2 * c), tile(pt, 2 * c + 1), tile(pb_, 2 * c), tile(pb_, 2 * c + 1))
                   for c in range(i)]
            left = [jnp.concatenate([o[n] for o in ops], axis=1).astype(BF16) for n in range(7)] if i else None
            inv = None if two_pass else [
                pl.reciprocal(jnp.sum(jnp.concatenate(x, axis=0), axis=1, keepdims=True), approx=True)
                for x in sums]
            return (left, jnp.concatenate([tile(pt, 2 * i), tile(pb_, 2 * i)], axis=0).astype(BF16),
                    tile(pb_, 2 * i + 1).astype(BF16), inv)

        def pv(i, left, p1, p2, inv):
            r0 = i * HQ
            m, pieces = {}, []
            for n in (2, 3, 0, 4, 1, 5, 6) if i else ():
                if n == 1:
                    w = jnp.concatenate([_as_bf16(v_s[c * HQ:c * HQ + 64, :L]) for c in range(i)], axis=0)
                elif n == 4:
                    w = jnp.concatenate([_as_bf16(v_s[c * HQ + 64:(c + 1) * HQ, L:]) for c in range(i)], axis=0)
                else:
                    w = _as_bf16(v5_s[(0, 2, 3, 5, 6).index(n), 0:i * 64, :])
                m[n] = jnp.dot(left[n], w, preferred_element_type=F32)
                pieces += spots(m[n], (0,), (0, 32, 64, 96))
            c1 = jnp.dot(p1, _as_bf16(v_s[r0:r0 + 64, :]), preferred_element_type=F32)
            c2 = jnp.dot(p2, _as_bf16(v_s[r0 + 64:r0 + HQ, :]), preferred_element_type=F32)
            top, bot = c1[:L], c1[L:] + c2
            if i:
                top = top + jnp.concatenate([_c11(m), _c12(m)], axis=1)
                bot = bot + jnp.concatenate([_c21(m), _c22(m)], axis=1)
            else:
                pieces = spots(c1, (0, 1))
            if inv is not None:
                top, bot = top * inv[0], bot * inv[1]
            us = [_to_u32(o) for o in _right(top[:, :L], bot[:, :L], top[:, L:], bot[:, L:])]
            for n in range(7):
                x7_s[n, h, i * 64:(i + 1) * 64, :] = us[n]
            waiting.extend(_or_all([us[n][g * 8:(g + 1) * 8] for n in (0, 2, 3, 5, 6)]) for g in range(8))
            return pieces

        def wo_operands():
            for rg in range(M // 32):
                a = [wo_s[h, hf * (M // 2) + rg * 16:hf * (M // 2) + (rg + 1) * 16, ch * L:(ch + 1) * L].astype(F32)
                     for hf in range(2) for ch in range(2)]
                us = [_to_u32(o) for o in _left(*a)]
                for n in range(7):
                    wo7_s[n, h, rg * 8:(rg + 1) * 8, :] = us[n]
                waiting.append(_or_all([us[n] for n in (0, 1, 4, 5, 6)]))

        if h is not None:
            wo_operands()
        scores, probs, pieces = {}, {}, None
        for op in order.split():
            i = int(op[1:])
            if op[0] in "ab":
                pieces = proj(i, "ab".index(op[0]))
            elif op[0] == "w":
                write_kv(i)
            elif op[0] == "Q":
                scores[i], pieces = qk(i)
            elif op[0] == "S":
                probs[i] = softmax(i, *scores.pop(i), pieces)
            elif op[0] == "V":
                pieces = pv(i, *probs.pop(i))
            else:
                hooks[i]()

    def phase1(c_s, wq_r, wk_r, wv_r, wr_s, gw_s, wg_s, wu_s, wd_s, x_s, wq_s):
        def x_copy(j):
            return pltpu.make_async_copy(xT_hbm.at[:, pl.ds(j * RC, RC)], xT_s.at[:, pl.ds(j * RC, RC)],
                                         sem.at[S_X + j])

        def wq_copy(g, j):
            return pltpu.make_async_copy(wq_hbm.at[pl.ds(j * mq, mq), g], wq_r.at[pl.ds(j * mq, mq), g],
                                         sem.at[(S_Q1 if g else S_Q0) + j])

        def kv_copies(j):
            return [pltpu.make_async_copy(src.at[pl.ds(j * n, n)], dst.at[pl.ds(j * n, n)], sem.at[s0 + j])
                    for src, dst, s0, n in ((c_hbm, c_s, S_C, RC), (wk_hbm, wk_r, S_K, mk), (wv_hbm, wv_r, S_V, mk))]

        misc = [pltpu.make_async_copy(a, b, sem.at[S_MISC + i]) for i, (a, b) in enumerate(
            [(wr_hbm, wr_s), (gw_hbm, gw_s), (wg_hbm, wg_s), (wu_hbm, wu_s), (wd_hbm, wd_s)])]

        x_copy(0).start()
        for j in range(NCH):
            wq_copy(0, j).start()
        for j in range(NCH):
            if j + 1 < NCH:
                x_copy(j + 1).start()
            wq_copy(1, j).start()
        misc[0].start()
        misc[1].start()
        for j in range(NCH):
            for cp in kv_copies(j):
                cp.start()
        for cp in misc[2:]:
            cp.start()
        wo_copy.start()

        def transpose_x(j):
            c0 = j * RC if isinstance(j, int) else pl.multiple_of(j * RC, RC)
            r0 = j * (RC // 2) if isinstance(j, int) else pl.multiple_of(j * (RC // 2), RC // 2)
            for t in range(RC // TQ):
                xt = xT_s[:, pl.ds(c0 + t * TQ, TQ)]
                x_s[pl.ds(r0 + t * HQ, HQ), :] = pltpu.bitcast(xt.T, U32)

        x_copy(0).wait()
        transpose_x(0)
        for j in range(NCH):
            wq_copy(0, j).wait()
            _relayout(wq_r, wq_s, 0, j * (mq // 2), mq // 2, pq, LO, HI)

        def q_step(g, j, side):
            r0 = pl.multiple_of(j * (RC // 2), RC // 2)
            xb = _as_bf16(x_s[pl.ds(r0, RC // 2), :])
            for hh in range(8):
                h = 8 * g + hh
                q = jnp.dot(xb, _head_weight(wq_s, h, M // 2, pq), preferred_element_type=F32) * qscale
                q_s[h, pl.ds(r0, RC // 2), :] = _to_u32(q)
                for k in range(8):
                    side(hh * 8 + k, q[(k % 4) * L:(k % 4) * L + 8, (k // 4) * L:(k // 4 + 1) * L])

        def q_lo(j, _):
            @pl.when(j + 1 < NCH)
            def _():
                x_copy(j + 1).wait()
            wq_copy(1, j).wait()
            never = _never(j)

            def side(k, piece):
                if k < mq // 2:
                    piece = pltpu.bitcast(piece, U32)
                    _relayout(wq_r, wq_s, 1, j * (mq // 2) + k, 1, pq,
                              jnp.where(never, piece, LO), jnp.where(never, piece, HI))
            q_step(0, j, side)
            transpose_x((j + 1) & (NCH - 1))
            return 0
        jax.lax.fori_loop(0, NCH, q_lo, 0)

        def q_hi(j, _):
            for cp in kv_copies(j):
                cp.wait()
            never = _never(j)

            def side(k, piece):
                rg, t = k // 4, k % 4
                a = []
                for rb in range(2):
                    r0 = pl.multiple_of(j * RC + rb * TQ + rg * 16, 16)
                    for ch in range(2):
                        a.append(c_s[pl.ds(r0, 16), (2 * t + ch) * L:(2 * t + ch + 1) * L].astype(F32))
                a[0] = jnp.where(jnp.concatenate([never, never], axis=0),
                                 jnp.concatenate([piece, piece], axis=0), a[0])
                us = [_to_u32(o) for o in _left(*a)]
                d0 = pl.multiple_of(j * HQ + rg * 8, 8)
                for n in range(7):
                    a_s[n, pl.ds(d0, 8), t * L:(t + 1) * L] = us[n]
                link = _or_all([us[n] for n in (0, 1, 4, 5, 6)])
                c0 = j * mk + 2 * k
                for g in range(2):
                    w = [pltpu.bitcast(r[pl.ds(c0 + o, 2), g], U32) for o in (0, L) for r in (wk_r, wv_r)]
                    w = [[x[0], x[1]] for x in w]
                    w[0][0] = jnp.where(never, link, w[0][0])
                    for par in range(2):
                        rows = [_right(*[pltpu.unpack_elementwise(x[e], index=par, packed_dtype=BF16,
                                                                  unpacked_dtype=F32) for x in w])
                                for e in range(2)]
                        for n in range(7):
                            b_s[n, 2 * g + par, pl.ds(j * (mk // 4) + k, 8, stride=pb), :] = pltpu.bitcast(
                                pltpu.pack_elementwise([rows[0][n], rows[1][n]], packed_dtype=BF16), U32)
            q_step(1, j, side)
            return 0
        jax.lax.fori_loop(0, NCH, q_hi, 0)

        for cp in misc:
            cp.wait()
        st = {}
        rid = jax.lax.broadcasted_iota(jnp.int32, (8, M), 0)

        def route():
            wr = jnp.broadcast_to(wr_s[...].reshape(1, M).astype(F32), (8, M))
            gw = jnp.broadcast_to(gw_s[...].reshape(1, M).astype(F32), (8, M))
            rg = jnp.dot(jnp.where(rid == 0, wr, gw).astype(BF16), xT_s[...], preferred_element_type=F32)
            g_s[...] = jax.nn.sigmoid(rg[1:2])
            r = rg[0:1].astype(BF16).astype(F32)
            lane = jax.lax.broadcasted_iota(jnp.int32, (1, S), 1)
            m1 = jnp.max(r, axis=1, keepdims=True)
            i1 = jnp.min(jnp.where(r == m1, lane, S - 1), axis=1, keepdims=True)
            r2 = jnp.where(lane == i1, -jnp.inf, r)
            m2 = jnp.max(r2, axis=1, keepdims=True)
            i2 = jnp.min(jnp.where(jnp.logical_and(r2 == m2, lane != i1), lane, S - 1), axis=1, keepdims=True)
            st["idx"] = [i1[0, 0], i2[0, 0]]
            rows = []
            for i in st["idx"]:
                w = x_s[pl.ds(i >> 1, 1), :]
                rows.append(pltpu.bitcast(jnp.where((i & 1) == 1, w & HI, w << 16), F32))
            st["x"] = jnp.where(rid == 0, rows[0], rows[1]).astype(BF16)
            st["r"] = jax.nn.sigmoid(jnp.where(rid[:, :1] == 0, m1, m2))

        def hidden():
            gate = jnp.dot(st["x"], wg_s[...], preferred_element_type=F32)
            up = jnp.dot(st["x"], wu_s[...], preferred_element_type=F32)
            st["h"] = (jax.nn.silu(gate) * up).astype(BF16)

        def patch():
            y = jax.lax.dot_general(st["h"], wd_s[...], NT, preferred_element_type=F32) * st["r"]
            mp = -(-M // L) * L
            y = jnp.concatenate([y, jnp.zeros((8, mp - M), F32)], axis=1)
            yT = jnp.concatenate([y, jnp.zeros((L - 8, mp), F32)], axis=0).T
            ln = jax.lax.broadcasted_iota(jnp.int32, (M, L), 1)
            for t, i in enumerate(st["idx"]):
                c0 = pl.multiple_of((i >> 7) << 7, L)
                blk = xT_s[:, pl.ds(c0, L)].astype(F32)
                upd = jnp.where(ln == (i & (L - 1)), yT[:M, t:t + 1], 0.0)
                xT_s[:, pl.ds(c0, L)] = (blk + upd).astype(BF16)

        head_program("h0 a0 h1 b0 w0 h2 a1 b1 w1 a2 b2 w2 a3 b3 w3", None, 0, None, False,
                     hooks=(route, hidden, patch))

    def phase2(x7_s):
        wo_copy.wait()

        def head(h, _):
            head_program(LOOP_ORDER, h, h + 1, x7_s, False)
            return 0
        jax.lax.fori_loop(0, H - 1, head, 0)
        head_program(LAST_ORDER, H - 1, pl.program_id(0), x7_s, True)

        def out_step(j, _):
            c0 = pl.multiple_of(j * RC, RC)
            for t in range(RC // TQ):
                r0 = pl.multiple_of(j * (RC // 4) + t * 64, 64)
                m = {}
                for n in range(7):
                    left = jnp.concatenate([_as_bf16(wo7_s[n, h]) for h in range(H)], axis=1)
                    right = jnp.concatenate([_as_bf16(x7_s[n, h, pl.ds(r0, 64), :]) for h in range(H)], axis=1)
                    m[n] = jax.lax.dot_general(left, right, NT, preferred_element_type=F32)
                a = jnp.concatenate([jnp.concatenate([_c11(m), _c12(m)], axis=1),
                                     jnp.concatenate([_c21(m), _c22(m)], axis=1)], axis=0)
                gj = g_s[:, pl.ds(c0 + t * TQ, TQ)]
                b = xT_s[:, pl.ds(c0 + t * TQ, TQ)].astype(F32)
                o_s[:, pl.ds(c0 + t * TQ, TQ)] = (gj * a + (1.0 - gj) * b).astype(BF16)
            out_copy(j).start()
            return 0
        jax.lax.fori_loop(0, S // RC, out_step, 0)
        for j in range(S // RC):
            out_copy(j).wait()

    pl.run_scoped(
        phase1,
        *[pltpu.VMEM(r.shape, r.dtype) for r in (c_hbm, wq_hbm, wk_hbm, wv_hbm, wr_hbm, gw_hbm,
                                                 wg_hbm, wu_hbm, wd_hbm)],
        pltpu.VMEM((S // 2, M), U32),
        pltpu.VMEM((4, 8 * pq, L), U32))
    pl.run_scoped(phase2, pltpu.VMEM((7, H, S // 4, L), U32))


def _tile_view(w):
    c, h, d = w.shape
    w = w.reshape(c, h // 8, 8, d // L, L).transpose(0, 1, 3, 2, 4)
    return w.reshape(c, h // 8, 8 * (d // L), L)


@jax.jit
def pallas_gated_mix__compressed_kv_cla__moe_arch_mod__prompt_kernel(
    A_x: jax.Array,
    A_c_kv: jax.Array,
    A_w_q: jax.Array,
    A_w_uk: jax.Array,
    A_w_uv: jax.Array,
    A_w_o: jax.Array,
    B_x: jax.Array,
    B_w_r: jax.Array,
    B_w_gate: jax.Array,
    B_w_up: jax.Array,
    B_w_down: jax.Array,
    gate_w: jax.Array,
):
    _, S, M = A_x.shape
    DC = A_c_kv.shape[2]
    H, D = A_w_q.shape[1], A_w_q.shape[2]
    args = (jnp.transpose(A_x[0]), A_c_kv[0], _tile_view(A_w_q), _tile_view(A_w_uk), _tile_view(A_w_uv),
            jnp.transpose(A_w_o, (0, 2, 1)), B_w_r, gate_w, B_w_gate, B_w_up, jnp.transpose(B_w_down))

    def kern(*refs):
        _kernel(*refs, S=S, M=M, DC=DC, H=H, D=D)

    hbm = pl.BlockSpec(memory_space=pl.ANY)
    oT = pl.pallas_call(
        kern,
        grid=(1,),
        out_shape=jax.ShapeDtypeStruct((M, S), A_x.dtype),
        in_specs=[hbm] * len(args),
        out_specs=hbm,
        scratch_shapes=[
            pltpu.VMEM((M, S), BF16),
            pltpu.VMEM((H, M, D), BF16),
            pltpu.VMEM((7, S // 4, DC // 2), U32),
            pltpu.VMEM((7, 4, 8 * (DC // 4 + 1), L), U32),
            pltpu.VMEM((H, S // 2, D), U32),
            pltpu.VMEM((S // 2, D), U32),
            pltpu.VMEM((S // 2, D), U32),
            pltpu.VMEM((5, S // 4, L), U32),
            pltpu.VMEM((7, H, M // 4, L), U32),
            pltpu.VMEM((1, S), F32),
            pltpu.VMEM((M, S), BF16),
            pltpu.SemaphoreType.DMA((N_SEM,)),
        ],
        compiler_params=pltpu.CompilerParams(vmem_limit_bytes=124 * 1024 * 1024),
    )(*args)
    return jnp.transpose(oT)[None]
```

```python
import math

import jax
import jax.numpy as jnp
import jax.experimental.pallas as pl
import jax.experimental.pallas.tpu as pltpu

F32 = jnp.float32
BF16 = jnp.bfloat16
U32 = jnp.uint32
NT = (((1,), (1,)), ((), ()))

L = 128
TQ = 256
HQ = TQ // 2
RC = 512
NCH = 4

S_X, S_Q0, S_Q1, S_K, S_V, S_C, S_MISC, S_OUT = 0, 4, 8, 12, 16, 20, 24, 30
N_SEM = 34

LOOP_ORDER = ("Q7 G0 S7 V7 Q6 G3 S6 V6 Q5 G4 S5 V5 Q4 G6 S4 V4 Q3 G1 S3 V3 Q2 G2 S2 V2 "
              "Q1 Q0 G5 S1 S0 V1 V0 w0")
LAST_ORDER = "Q7 Q6 S7 Q5 S6 V7 Q4 S5 V6 Q3 S4 V5 Q2 S3 V4 Q1 S2 V3 Q0 S1 V2 S0 V1 V0"


def _to_u32(x_f32):
    return pltpu.bitcast(x_f32.astype(BF16), U32)


def _as_bf16(x_u32):
    return pltpu.bitcast(x_u32, BF16)


def _left(a11, a12, a21, a22):
    return (a11 + a22, a21 + a22, a11, a22, a11 + a12, a21 - a11, a12 - a22)


def _right(b11, b12, b21, b22):
    return (b11 + b22, b11, b12 - b22, b21 - b11, b22, b11 + b12, b21 + b22)


def _c11(m):
    return (m[0] + m[3]) + (m[6] - m[4])


def _c12(m):
    return m[2] + m[4]


def _c21(m):
    return m[1] + m[3]


def _c22(m):
    return (m[0] - m[1]) + (m[2] + m[5])


def _never(i):
    return jax.lax.broadcasted_iota(jnp.int32, (8, L), 0) < (i >> 10)


def _or_all(xs):
    out = xs[0]
    for x in xs[1:]:
        out = out | x
    return out


def _relayout(raw_ref, dst_ref, g, p0, npairs, pitch, lo, hi):
    blk = pltpu.bitcast(raw_ref[pl.ds(2 * p0, 2 * npairs), g], U32)
    for i in range(npairs):
        e, o = blk[2 * i], blk[2 * i + 1]
        dst_ref[2 * g, pl.ds(p0 + i, 8, stride=pitch), :] = (e & lo) | (o << 16)
        dst_ref[2 * g + 1, pl.ds(p0 + i, 8, stride=pitch), :] = (e >> 16) | (o & hi)


def _head_weight(ref, h, nrows, pitch):
    sel = ((h >> 3) << 1) + (h & 1)
    r = (h >> 1) & 3
    return jnp.concatenate(
        [_as_bf16(ref[sel, pl.ds((dt * 4 + r) * pitch, nrows), :]) for dt in range(2)], axis=1)


def _kernel(xT_hbm, c_hbm, wq_hbm, wk_hbm, wv_hbm, wo_hbm, wr_hbm, gw_hbm, wg_hbm, wu_hbm, wd_hbm,
            o_hbm,
            xT_s, wo_s, a_s, b_s, q_s, k_s, v_s, v5_s, wo7_s, g_s, o_s, sem, *, S, M, DC, H, D):
    nq = S // TQ
    pq = M // 2 + 1
    pb = DC // 4 + 1
    mq = M // NCH
    mk = DC // NCH
    qscale = (D ** -0.5) * math.log2(math.e)
    neg = -1e9 * math.log2(math.e)
    LO = jnp.uint32(0xFFFF)
    HI = jnp.uint32(0xFFFF0000)
    wo_copy = pltpu.make_async_copy(wo_hbm, wo_s, sem.at[S_MISC + 5])

    def out_copy(j):
        return pltpu.make_async_copy(o_s.at[:, pl.ds(j * RC, RC)], o_hbm.at[:, pl.ds(j * RC, RC)],
                                     sem.at[S_OUT + j])

    tri = (jax.lax.broadcasted_iota(jnp.int32, (L, L), 1) <= jax.lax.broadcasted_iota(jnp.int32, (L, L), 0))

    def head_program(order, h, hn, x7_s, two_pass, hooks=None):
        never = _never(hn)
        prods, held, waiting = {}, {}, []

        def spots(v, cols, rows=(0, 64, 128, 192)):
            return [v[r:r + 8, n * L:(n + 1) * L] for n in cols for r in rows]

        def tie(lhs, links, every):
            rows = []
            for rg in range(lhs.shape[0] // 8):
                blk = lhs[rg * 8:(rg + 1) * 8]
                if links and rg % every == 0:
                    blk = jnp.concatenate([jnp.where(never, links.pop(0), blk[:, :L]), blk[:, L:]], axis=1)
                rows.append(blk)
            return jnp.concatenate(rows, axis=0)

        def proj(n):
            lhs = a_s[n]
            if waiting:
                lhs = tie(lhs, list(waiting), lhs.shape[0] // 8 // len(waiting))
                del waiting[:]
            prods[n] = jnp.dot(_as_bf16(lhs), _head_weight(b_s.at[n], hn, DC // 4, pb),
                               preferred_element_type=F32)
            for key, odd, comb, needs in (("k", 0, _c11, (0, 3, 4, 6)), ("k", 1, _c21, (1, 3)),
                                          ("v", 0, _c12, (2, 4)), ("v", 1, _c22, (0, 1, 2, 5))):
                if n in needs and all(x in prods for x in needs):
                    for k in range(nq // 2):
                        c = comb({x: prods[x][k * TQ:(k + 1) * TQ] for x in needs})
                        held[2 * k + odd, key] = _to_u32(c)
                        if key == "v" and 2 * k + odd < nq - 1:
                            ops = _right(c[:L, :L], c[:L, L:], c[L:, :L], c[L:, L:])
                            held[2 * k + odd, "r"] = [_to_u32(ops[x]) for x in (0, 2, 3, 5, 6)]
            return spots(prods[n], (0, 1), range(0, S // 2, 32))

        def write_kv():
            for ch in reversed(range(nq)):
                k_s[ch * HQ:(ch + 1) * HQ, :] = held[ch, "k"]
                v_s[ch * HQ:(ch + 1) * HQ, :] = held[ch, "v"]
                for n, o in enumerate(held.get((ch, "r"), ())):
                    v5_s[n, ch * 64:(ch + 1) * 64, :] = o

        def qk(i):
            q = _as_bf16(q_s[h, i * HQ:(i + 1) * HQ, :])
            n0 = i * TQ
            n1 = n0 + L
            s1 = jax.lax.dot_general(q, _as_bf16(k_s[0:n1 // 2, :]), NT, preferred_element_type=F32)
            s2 = jax.lax.dot_general(q[L:], _as_bf16(k_s[n1 // 2:(n1 + L) // 2, :]), NT,
                                     preferred_element_type=F32)
            top = jnp.where(tri, s1[:L, n0:], neg)
            if n0:
                top = jnp.concatenate([s1[:L, :n0], top], axis=1)
            bot = jnp.concatenate([s1[L:], jnp.where(tri, s2, neg)], axis=1)
            return (top, bot), spots(s1, range(max(1, n0 // L)))

        def softmax(i, top, bot, pieces):
            G, span = (16, 0.8) if two_pass else (8, 0.9)
            p, sums, prev = ([], []), ([], []), None
            for k in range(TQ // G):
                half = k % 2
                s = (top, bot)[half][(k // 2) * G:(k // 2 + 1) * G]
                tiles = [s[:, t:t + L] for t in range(0, s.shape[1], L)]
                link = pieces[int(span * k * G / TQ * len(pieces))]
                if prev is not None:
                    link = jnp.where(never, link, prev)
                m = jnp.broadcast_to(jnp.max(s, axis=1, keepdims=True), (G, L))
                m = jnp.where(jnp.concatenate([never] * (G // 8), axis=0),
                              jnp.concatenate([link] * (G // 8), axis=0), m)
                e = [jnp.exp2(t - m) for t in tiles]
                acc = e[0]
                for x in e[1:]:
                    acc = acc + x
                prev = acc[G - 8:]
                if two_pass:
                    m = m + jnp.log2(jnp.sum(acc, axis=1, keepdims=True))
                    e = [jnp.exp2(t - m) for t in tiles]
                sums[half].append(acc)
                p[half].append(jnp.concatenate(e, axis=1))
            pt, pb_ = jnp.concatenate(p[0], axis=0), jnp.concatenate(p[1], axis=0)

            def tile(x, t):
                return x[:, t * L:(t + 1) * L]
            ops = [_left(tile(pt, 2 * c), tile(pt, 2 * c + 1), tile(pb_, 2 * c), tile(pb_, 2 * c + 1))
                   for c in range(i)]
            left = [jnp.concatenate([o[n] for o in ops], axis=1).astype(BF16) for n in range(7)] if i else None
            inv = None if two_pass else [
                pl.reciprocal(jnp.sum(jnp.concatenate(x, axis=0), axis=1, keepdims=True), approx=True)
                for x in sums]
            return (left, jnp.concatenate([tile(pt, 2 * i), tile(pb_, 2 * i)], axis=0).astype(BF16),
                    tile(pb_, 2 * i + 1).astype(BF16), inv)

        def pv(i, left, p1, p2, inv):
            r0 = i * HQ
            m, pieces = {}, []
            for n in (2, 3, 0, 4, 1, 5, 6) if i else ():
                if n == 1:
                    w = jnp.concatenate([_as_bf16(v_s[c * HQ:c * HQ + 64, :L]) for c in range(i)], axis=0)
                elif n == 4:
                    w = jnp.concatenate([_as_bf16(v_s[c * HQ + 64:(c + 1) * HQ, L:]) for c in range(i)], axis=0)
                else:
                    w = _as_bf16(v5_s[(0, 2, 3, 5, 6).index(n), 0:i * 64, :])
                m[n] = jnp.dot(left[n], w, preferred_element_type=F32)
                pieces += spots(m[n], (0,), (0, 32, 64, 96))
            c1 = jnp.dot(p1, _as_bf16(v_s[r0:r0 + 64, :]), preferred_element_type=F32)
            c2 = jnp.dot(p2, _as_bf16(v_s[r0 + 64:r0 + HQ, :]), preferred_element_type=F32)
            top, bot = c1[:L], c1[L:] + c2
            if i:
                top = top + jnp.concatenate([_c11(m), _c12(m)], axis=1)
                bot = bot + jnp.concatenate([_c21(m), _c22(m)], axis=1)
            else:
                pieces = spots(c1, (0, 1))
            if inv is not None:
                top, bot = top * inv[0], bot * inv[1]
            us = [_to_u32(o) for o in _right(top[:, :L], bot[:, :L], top[:, L:], bot[:, L:])]
            for n in range(7):
                x7_s[n, h, i * 64:(i + 1) * 64, :] = us[n]
            waiting.extend(_or_all([us[n][g * 8:(g + 1) * 8] for n in (0, 2, 3, 5, 6)]) for g in range(8))
            return pieces

        def wo_operands():
            for rg in range(M // 32):
                a = [wo_s[h, hf * (M // 2) + rg * 16:hf * (M // 2) + (rg + 1) * 16, ch * L:(ch + 1) * L].astype(F32)
                     for hf in range(2) for ch in range(2)]
                us = [_to_u32(o) for o in _left(*a)]
                for n in range(7):
                    wo7_s[n, h, rg * 8:(rg + 1) * 8, :] = us[n]
                waiting.append(_or_all([us[n] for n in (0, 1, 4, 5, 6)]))

        if h is not None:
            wo_operands()
        scores, probs, pieces = {}, {}, None
        for op in order.split():
            i = int(op[1:])
            if op[0] == "G":
                pieces = proj(i)
            elif op[0] == "w":
                write_kv()
            elif op[0] == "Q":
                scores[i], pieces = qk(i)
            elif op[0] == "S":
                probs[i] = softmax(i, *scores.pop(i), pieces)
            elif op[0] == "V":
                pieces = pv(i, *probs.pop(i))
            else:
                hooks[i]()

    def phase1(c_s, wq_r, wk_r, wv_r, wr_s, gw_s, wg_s, wu_s, wd_s, x_s, wq_s):
        def x_copy(j):
            return pltpu.make_async_copy(xT_hbm.at[:, pl.ds(j * RC, RC)], xT_s.at[:, pl.ds(j * RC, RC)],
                                         sem.at[S_X + j])

        def wq_copy(g, j):
            return pltpu.make_async_copy(wq_hbm.at[pl.ds(j * mq, mq), g], wq_r.at[pl.ds(j * mq, mq), g],
                                         sem.at[(S_Q1 if g else S_Q0) + j])

        def kv_copies(j):
            return [pltpu.make_async_copy(src.at[pl.ds(j * n, n)], dst.at[pl.ds(j * n, n)], sem.at[s0 + j])
                    for src, dst, s0, n in ((c_hbm, c_s, S_C, RC), (wk_hbm, wk_r, S_K, mk), (wv_hbm, wv_r, S_V, mk))]

        misc = [pltpu.make_async_copy(a, b, sem.at[S_MISC + i]) for i, (a, b) in enumerate(
            [(wr_hbm, wr_s), (gw_hbm, gw_s), (wg_hbm, wg_s), (wu_hbm, wu_s), (wd_hbm, wd_s)])]

        x_copy(0).start()
        for j in range(NCH):
            wq_copy(0, j).start()
        for j in range(NCH):
            if j + 1 < NCH:
                x_copy(j + 1).start()
            wq_copy(1, j).start()
        misc[0].start()
        misc[1].start()
        for j in range(NCH):
            for cp in kv_copies(j):
                cp.start()
        for cp in misc[2:]:
            cp.start()
        wo_copy.start()

        def transpose_x(j):
            c0 = j * RC if isinstance(j, int) else pl.multiple_of(j * RC, RC)
            r0 = j * (RC // 2) if isinstance(j, int) else pl.multiple_of(j * (RC // 2), RC // 2)
            for t in range(RC // TQ):
                xt = xT_s[:, pl.ds(c0 + t * TQ, TQ)]
                x_s[pl.ds(r0 + t * HQ, HQ), :] = pltpu.bitcast(xt.T, U32)

        x_copy(0).wait()
        transpose_x(0)
        for j in range(NCH):
            wq_copy(0, j).wait()
            _relayout(wq_r, wq_s, 0, j * (mq // 2), mq // 2, pq, LO, HI)

        def q_step(g, j, side):
            r0 = pl.multiple_of(j * (RC // 2), RC // 2)
            xb = _as_bf16(x_s[pl.ds(r0, RC // 2), :])
            for hh in range(8):
                h = 8 * g + hh
                q = jnp.dot(xb, _head_weight(wq_s, h, M // 2, pq), preferred_element_type=F32) * qscale
                q_s[h, pl.ds(r0, RC // 2), :] = _to_u32(q)
                for k in range(8):
                    side(hh * 8 + k, q[(k % 4) * L:(k % 4) * L + 8, (k // 4) * L:(k // 4 + 1) * L])

        def q_lo(j, _):
            @pl.when(j + 1 < NCH)
            def _():
                x_copy(j + 1).wait()
            wq_copy(1, j).wait()
            never = _never(j)

            def side(k, piece):
                if k < mq // 2:
                    piece = pltpu.bitcast(piece, U32)
                    _relayout(wq_r, wq_s, 1, j * (mq // 2) + k, 1, pq,
                              jnp.where(never, piece, LO), jnp.where(never, piece, HI))
            q_step(0, j, side)
            transpose_x((j + 1) & (NCH - 1))
            return 0
        jax.lax.fori_loop(0, NCH, q_lo, 0)

        def q_hi(j, _):
            for cp in kv_copies(j):
                cp.wait()
            never = _never(j)

            def side(k, piece):
                rg, t = k // 4, k % 4
                a = []
                for rb in range(2):
                    r0 = pl.multiple_of(j * RC + rb * TQ + rg * 16, 16)
                    for ch in range(2):
                        a.append(c_s[pl.ds(r0, 16), (2 * t + ch) * L:(2 * t + ch + 1) * L].astype(F32))
                a[0] = jnp.where(jnp.concatenate([never, never], axis=0),
                                 jnp.concatenate([piece, piece], axis=0), a[0])
                us = [_to_u32(o) for o in _left(*a)]
                d0 = pl.multiple_of(j * HQ + rg * 8, 8)
                for n in range(7):
                    a_s[n, pl.ds(d0, 8), t * L:(t + 1) * L] = us[n]
                link = _or_all([us[n] for n in (0, 1, 4, 5, 6)])
                c0 = j * mk + 2 * k
                for g in range(2):
                    w = [pltpu.bitcast(r[pl.ds(c0 + o, 2), g], U32) for o in (0, L) for r in (wk_r, wv_r)]
                    w = [[x[0], x[1]] for x in w]
                    w[0][0] = jnp.where(never, link, w[0][0])
                    for par in range(2):
                        rows = [_right(*[pltpu.unpack_elementwise(x[e], index=par, packed_dtype=BF16,
                                                                  unpacked_dtype=F32) for x in w])
                                for e in range(2)]
                        for n in range(7):
                            b_s[n, 2 * g + par, pl.ds(j * (mk // 4) + k, 8, stride=pb), :] = pltpu.bitcast(
                                pltpu.pack_elementwise([rows[0][n], rows[1][n]], packed_dtype=BF16), U32)
            q_step(1, j, side)
            return 0
        jax.lax.fori_loop(0, NCH, q_hi, 0)

        for cp in misc:
            cp.wait()
        st = {}
        rid = jax.lax.broadcasted_iota(jnp.int32, (8, M), 0)

        def route():
            wr = jnp.broadcast_to(wr_s[...].reshape(1, M).astype(F32), (8, M))
            gw = jnp.broadcast_to(gw_s[...].reshape(1, M).astype(F32), (8, M))
            rg = jnp.dot(jnp.where(rid == 0, wr, gw).astype(BF16), xT_s[...], preferred_element_type=F32)
            g_s[...] = jax.nn.sigmoid(rg[1:2])
            r = rg[0:1].astype(BF16).astype(F32)
            lane = jax.lax.broadcasted_iota(jnp.int32, (1, S), 1)
            m1 = jnp.max(r, axis=1, keepdims=True)
            i1 = jnp.min(jnp.where(r == m1, lane, S - 1), axis=1, keepdims=True)
            r2 = jnp.where(lane == i1, -jnp.inf, r)
            m2 = jnp.max(r2, axis=1, keepdims=True)
            i2 = jnp.min(jnp.where(jnp.logical_and(r2 == m2, lane != i1), lane, S - 1), axis=1, keepdims=True)
            st["idx"] = [i1[0, 0], i2[0, 0]]
            rows = []
            for i in st["idx"]:
                w = x_s[pl.ds(i >> 1, 1), :]
                rows.append(pltpu.bitcast(jnp.where((i & 1) == 1, w & HI, w << 16), F32))
            st["x"] = jnp.where(rid == 0, rows[0], rows[1]).astype(BF16)
            st["r"] = jax.nn.sigmoid(jnp.where(rid[:, :1] == 0, m1, m2))

        def hidden():
            gate = jnp.dot(st["x"], wg_s[...], preferred_element_type=F32)
            up = jnp.dot(st["x"], wu_s[...], preferred_element_type=F32)
            st["h"] = (jax.nn.silu(gate) * up).astype(BF16)

        def patch():
            y = jax.lax.dot_general(st["h"], wd_s[...], NT, preferred_element_type=F32) * st["r"]
            mp = -(-M // L) * L
            y = jnp.concatenate([y, jnp.zeros((8, mp - M), F32)], axis=1)
            yT = jnp.concatenate([y, jnp.zeros((L - 8, mp), F32)], axis=0).T
            ln = jax.lax.broadcasted_iota(jnp.int32, (M, L), 1)
            for t, i in enumerate(st["idx"]):
                c0 = pl.multiple_of((i >> 7) << 7, L)
                blk = xT_s[:, pl.ds(c0, L)].astype(F32)
                upd = jnp.where(ln == (i & (L - 1)), yT[:M, t:t + 1], 0.0)
                xT_s[:, pl.ds(c0, L)] = (blk + upd).astype(BF16)

        head_program("h0 G0 h1 G3 h2 G4 G6 G1 G2 G5 w0", None, 0, None, False,
                     hooks=(route, hidden, patch))

    def phase2(x7_s):
        wo_copy.wait()

        def head(h, _):
            head_program(LOOP_ORDER, h, h + 1, x7_s, False)
            return 0
        jax.lax.fori_loop(0, H - 1, head, 0)
        head_program(LAST_ORDER, H - 1, pl.program_id(0), x7_s, True)

        def out_step(j, _):
            c0 = pl.multiple_of(j * RC, RC)
            for t in range(RC // TQ):
                r0 = pl.multiple_of(j * (RC // 4) + t * 64, 64)
                m = {}
                for n in range(7):
                    left = jnp.concatenate([_as_bf16(wo7_s[n, h, :M // 4]) for h in range(H)], axis=1)
                    right = jnp.concatenate([_as_bf16(x7_s[n, h, pl.ds(r0, 64), :]) for h in range(H)], axis=1)
                    m[n] = jax.lax.dot_general(left, right, NT, preferred_element_type=F32)
                a = jnp.concatenate([jnp.concatenate([_c11(m), _c12(m)], axis=1),
                                     jnp.concatenate([_c21(m), _c22(m)], axis=1)], axis=0)
                gj = g_s[:, pl.ds(c0 + t * TQ, TQ)]
                b = xT_s[:, pl.ds(c0 + t * TQ, TQ)].astype(F32)
                o_s[:, pl.ds(c0 + t * TQ, TQ)] = (gj * a + (1.0 - gj) * b).astype(BF16)
            out_copy(j).start()
            return 0
        jax.lax.fori_loop(0, S // RC, out_step, 0)
        for j in range(S // RC):
            out_copy(j).wait()

    pl.run_scoped(
        phase1,
        *[pltpu.VMEM(r.shape, r.dtype) for r in (c_hbm, wq_hbm, wk_hbm, wv_hbm, wr_hbm, gw_hbm,
                                                 wg_hbm, wu_hbm, wd_hbm)],
        pltpu.VMEM((S // 2, M), U32),
        pltpu.VMEM((4, 8 * pq, L), U32))
    pl.run_scoped(phase2, pltpu.VMEM((7, H, S // 4, L), U32))


def _tile_view(w):
    c, h, d = w.shape
    w = w.reshape(c, h // 8, 8, d // L, L).transpose(0, 1, 3, 2, 4)
    return w.reshape(c, h // 8, 8 * (d // L), L)


@jax.jit
def pallas_gated_mix__compressed_kv_cla__moe_arch_mod__prompt_kernel(
    A_x: jax.Array,
    A_c_kv: jax.Array,
    A_w_q: jax.Array,
    A_w_uk: jax.Array,
    A_w_uv: jax.Array,
    A_w_o: jax.Array,
    B_x: jax.Array,
    B_w_r: jax.Array,
    B_w_gate: jax.Array,
    B_w_up: jax.Array,
    B_w_down: jax.Array,
    gate_w: jax.Array,
):
    _, S, M = A_x.shape
    DC = A_c_kv.shape[2]
    H, D = A_w_q.shape[1], A_w_q.shape[2]
    args = (jnp.transpose(A_x[0]), A_c_kv[0], _tile_view(A_w_q), _tile_view(A_w_uk), _tile_view(A_w_uv),
            jnp.transpose(A_w_o, (0, 2, 1)), B_w_r, gate_w, B_w_gate, B_w_up, jnp.transpose(B_w_down))

    def kern(*refs):
        _kernel(*refs, S=S, M=M, DC=DC, H=H, D=D)

    hbm = pl.BlockSpec(memory_space=pl.ANY)
    oT = pl.pallas_call(
        kern,
        grid=(1,),
        out_shape=jax.ShapeDtypeStruct((M, S), A_x.dtype),
        in_specs=[hbm] * len(args),
        out_specs=hbm,
        scratch_shapes=[
            pltpu.VMEM((M, S), BF16),
            pltpu.VMEM((H, M, D), BF16),
            pltpu.VMEM((7, S // 4, DC // 2), U32),
            pltpu.VMEM((7, 4, 8 * (DC // 4 + 1), L), U32),
            pltpu.VMEM((H, S // 2, D), U32),
            pltpu.VMEM((S // 2, D), U32),
            pltpu.VMEM((S // 2, D), U32),
            pltpu.VMEM((5, S // 4, L), U32),
            pltpu.VMEM((7, H, L, L), U32),
            pltpu.VMEM((1, S), F32),
            pltpu.VMEM((M, S), BF16),
            pltpu.SemaphoreType.DMA((N_SEM,)),
        ],
        compiler_params=pltpu.CompilerParams(vmem_limit_bytes=124 * 1024 * 1024),
    )(*args)
    return jnp.transpose(oT)[None]
```

```python
import math

import jax
import jax.numpy as jnp
import jax.experimental.pallas as pl
import jax.experimental.pallas.tpu as pltpu

F32 = jnp.float32
BF16 = jnp.bfloat16
U32 = jnp.uint32
NT = (((1,), (1,)), ((), ()))

L = 128
TQ = 256
HQ = TQ // 2
RC = 512
NCH = 4

S_X, S_Q0, S_Q1, S_K, S_V, S_C, S_MISC, S_OUT = 0, 4, 8, 12, 16, 20, 24, 30
N_SEM = 34

LOOP_ORDER = ("Q7 G0 S7 V7 Q6 G3 S6 V6 Q5 G4 S5 V5 Q4 G6 S4 V4 Q3 G1 S3 V3 Q2 G2 S2 V2 "
              "Q1 Q0 G5 S1 S0 V1 V0 w0")
LAST_ORDER = "Q7 Q6 S7 Q5 S6 V7 Q4 S5 V6 Q3 S4 V5 Q2 S3 V4 Q1 S2 V3 Q0 S1 V2 S0 V1 V0"


def _to_u32(x_f32):
    return pltpu.bitcast(x_f32.astype(BF16), U32)


def _as_bf16(x_u32):
    return pltpu.bitcast(x_u32, BF16)


def _left(a11, a12, a21, a22):
    return (a11 + a22, a21 + a22, a11, a22, a11 + a12, a21 - a11, a12 - a22)


def _right(b11, b12, b21, b22):
    return (b11 + b22, b11, b12 - b22, b21 - b11, b22, b11 + b12, b21 + b22)


def _c11(m):
    return (m[0] + m[3]) + (m[6] - m[4])


def _c12(m):
    return m[2] + m[4]


def _c21(m):
    return m[1] + m[3]


def _c22(m):
    return (m[0] - m[1]) + (m[2] + m[5])


def _never(i):
    return jax.lax.broadcasted_iota(jnp.int32, (8, L), 0) < (i >> 10)


def _or_all(xs):
    out = xs[0]
    for x in xs[1:]:
        out = out | x
    return out


def _unpack(w, par):
    return pltpu.unpack_elementwise(w, index=par, packed_dtype=BF16, unpacked_dtype=F32)


def _pack(even, odd):
    return pltpu.bitcast(pltpu.pack_elementwise([even, odd], packed_dtype=BF16), U32)


def _head_weight(ref, h, nrows, pitch):
    sel = ((h >> 3) << 1) + (h & 1)
    r = (h >> 1) & 3
    return jnp.concatenate(
        [_as_bf16(ref[sel, pl.ds((dt * 4 + r) * pitch, nrows), :]) for dt in range(2)], axis=1)


def _kernel(xT_hbm, c_hbm, wq_hbm, wk_hbm, wv_hbm, wo_hbm, wr_hbm, gw_hbm, wg_hbm, wu_hbm, wd_hbm,
            o_hbm,
            xT_s, wo_s, a_s, b_s, q_s, k_s, v_s, v5_s, wo7_s, g_s, o_s, sem, *, S, M, DC, H, D):
    nq = S // TQ
    mh = M // 2
    pq = mh // 2 + 1
    pb = DC // 4 + 1
    mq = mh // NCH
    mk = DC // NCH
    qscale = (D ** -0.5) * math.log2(math.e)
    neg = -1e9 * math.log2(math.e)
    wo_copy = pltpu.make_async_copy(wo_hbm, wo_s, sem.at[S_MISC + 5])

    def out_copy(j):
        return pltpu.make_async_copy(o_s.at[:, pl.ds(j * RC, RC)], o_hbm.at[:, pl.ds(j * RC, RC)],
                                     sem.at[S_OUT + j])

    tri = (jax.lax.broadcasted_iota(jnp.int32, (L, L), 1) <= jax.lax.broadcasted_iota(jnp.int32, (L, L), 0))

    def head_program(order, h, hn, x7_s, two_pass, hooks=None):
        never = _never(hn)
        prods, held, waiting = {}, {}, []

        def spots(v, cols, rows=(0, 64, 128, 192)):
            return [v[r:r + 8, n * L:(n + 1) * L] for n in cols for r in rows]

        def tie(lhs, links, every):
            rows = []
            for rg in range(lhs.shape[0] // 8):
                blk = lhs[rg * 8:(rg + 1) * 8]
                if links and rg % every == 0:
                    blk = jnp.concatenate([jnp.where(never, links.pop(0), blk[:, :L]), blk[:, L:]], axis=1)
                rows.append(blk)
            return jnp.concatenate(rows, axis=0)

        def proj(n):
            lhs = a_s[n]
            if waiting:
                lhs = tie(lhs, list(waiting), lhs.shape[0] // 8 // len(waiting))
                del waiting[:]
            prods[n] = jnp.dot(_as_bf16(lhs), _head_weight(b_s.at[n], hn, DC // 4, pb),
                               preferred_element_type=F32)
            for key, odd, comb, needs in (("k", 0, _c11, (0, 3, 4, 6)), ("k", 1, _c21, (1, 3)),
                                          ("v", 0, _c12, (2, 4)), ("v", 1, _c22, (0, 1, 2, 5))):
                if n in needs and all(x in prods for x in needs):
                    for k in range(nq // 2):
                        c = comb({x: prods[x][k * TQ:(k + 1) * TQ] for x in needs})
                        held[2 * k + odd, key] = _to_u32(c)
                        if key == "v" and 2 * k + odd < nq - 1:
                            ops = _right(c[:L, :L], c[:L, L:], c[L:, :L], c[L:, L:])
                            held[2 * k + odd, "r"] = [_to_u32(ops[x]) for x in (0, 2, 3, 5, 6)]
            return spots(prods[n], (0, 1), range(0, S // 2, 32))

        def write_kv():
            for ch in reversed(range(nq)):
                k_s[ch * HQ:(ch + 1) * HQ, :] = held[ch, "k"]
                v_s[ch * HQ:(ch + 1) * HQ, :] = held[ch, "v"]
                for n, o in enumerate(held.get((ch, "r"), ())):
                    v5_s[n, ch * 64:(ch + 1) * 64, :] = o

        def qk(i):
            q = _as_bf16(q_s[h, i * HQ:(i + 1) * HQ, :])
            n0 = i * TQ
            n1 = n0 + L
            s1 = jax.lax.dot_general(q, _as_bf16(k_s[0:n1 // 2, :]), NT, preferred_element_type=F32)
            s2 = jax.lax.dot_general(q[L:], _as_bf16(k_s[n1 // 2:(n1 + L) // 2, :]), NT,
                                     preferred_element_type=F32)
            top = jnp.where(tri, s1[:L, n0:], neg)
            if n0:
                top = jnp.concatenate([s1[:L, :n0], top], axis=1)
            bot = jnp.concatenate([s1[L:], jnp.where(tri, s2, neg)], axis=1)
            return (top, bot), spots(s1, range(max(1, n0 // L)))

        def softmax(i, top, bot, pieces):
            G, span = (16, 0.8) if two_pass else (8, 0.9)
            p, sums, prev = ([], []), ([], []), None
            for k in range(TQ // G):
                half = k % 2
                s = (top, bot)[half][(k // 2) * G:(k // 2 + 1) * G]
                tiles = [s[:, t:t + L] for t in range(0, s.shape[1], L)]
                link = pieces[int(span * k * G / TQ * len(pieces))]
                if prev is not None:
                    link = jnp.where(never, link, prev)
                m = jnp.broadcast_to(jnp.max(s, axis=1, keepdims=True), (G, L))
                m = jnp.where(jnp.concatenate([never] * (G // 8), axis=0),
                              jnp.concatenate([link] * (G // 8), axis=0), m)
                e = [jnp.exp2(t - m) for t in tiles]
                acc = e[0]
                for x in e[1:]:
                    acc = acc + x
                prev = acc[G - 8:]
                if two_pass:
                    m = m + jnp.log2(jnp.sum(acc, axis=1, keepdims=True))
                    e = [jnp.exp2(t - m) for t in tiles]
                sums[half].append(acc)
                p[half].append(jnp.concatenate(e, axis=1))
            pt, pb_ = jnp.concatenate(p[0], axis=0), jnp.concatenate(p[1], axis=0)

            def tile(x, t):
                return x[:, t * L:(t + 1) * L]
            ops = [_left(tile(pt, 2 * c), tile(pt, 2 * c + 1), tile(pb_, 2 * c), tile(pb_, 2 * c + 1))
                   for c in range(i)]
            left = [jnp.concatenate([o[n] for o in ops], axis=1).astype(BF16) for n in range(7)] if i else None
            inv = None if two_pass else [
                pl.reciprocal(jnp.sum(jnp.concatenate(x, axis=0), axis=1, keepdims=True), approx=True)
                for x in sums]
            return (left, jnp.concatenate([tile(pt, 2 * i), tile(pb_, 2 * i)], axis=0).astype(BF16),
                    tile(pb_, 2 * i + 1).astype(BF16), inv)

        def pv(i, left, p1, p2, inv):
            r0 = i * HQ
            m, pieces = {}, []
            for n in (2, 3, 0, 4, 1, 5, 6) if i else ():
                if n == 1:
                    w = jnp.concatenate([_as_bf16(v_s[c * HQ:c * HQ + 64, :L]) for c in range(i)], axis=0)
                elif n == 4:
                    w = jnp.concatenate([_as_bf16(v_s[c * HQ + 64:(c + 1) * HQ, L:]) for c in range(i)], axis=0)
                else:
                    w = _as_bf16(v5_s[(0, 2, 3, 5, 6).index(n), 0:i * 64, :])
                m[n] = jnp.dot(left[n], w, preferred_element_type=F32)
                pieces += spots(m[n], (0,), (0, 32, 64, 96))
            c1 = jnp.dot(p1, _as_bf16(v_s[r0:r0 + 64, :]), preferred_element_type=F32)
            c2 = jnp.dot(p2, _as_bf16(v_s[r0 + 64:r0 + HQ, :]), preferred_element_type=F32)
            top, bot = c1[:L], c1[L:] + c2
            if i:
                top = top + jnp.concatenate([_c11(m), _c12(m)], axis=1)
                bot = bot + jnp.concatenate([_c21(m), _c22(m)], axis=1)
            else:
                pieces = spots(c1, (0, 1))
            if inv is not None:
                top, bot = top * inv[0], bot * inv[1]
            us = [_to_u32(o) for o in _right(top[:, :L], bot[:, :L], top[:, L:], bot[:, L:])]
            for n in range(7):
                x7_s[n, h, i * 64:(i + 1) * 64, :] = us[n]
            waiting.extend(_or_all([us[n][g * 8:(g + 1) * 8] for n in (0, 2, 3, 5, 6)]) for g in range(8))
            return pieces

        def wo_operands():
            for rg in range(M // 32):
                a = [wo_s[h, hf * (M // 2) + rg * 16:hf * (M // 2) + (rg + 1) * 16, ch * L:(ch + 1) * L].astype(F32)
                     for hf in range(2) for ch in range(2)]
                us = [_to_u32(o) for o in _left(*a)]
                for n in range(7):
                    wo7_s[n, h, rg * 8:(rg + 1) * 8, :] = us[n]
                waiting.append(_or_all([us[n] for n in (0, 1, 4, 5, 6)]))

        if h is not None:
            wo_operands()
        scores, probs, pieces = {}, {}, None
        for op in order.split():
            i = int(op[1:])
            if op[0] == "G":
                pieces = proj(i)
            elif op[0] == "w":
                write_kv()
            elif op[0] == "Q":
                scores[i], pieces = qk(i)
            elif op[0] == "S":
                probs[i] = softmax(i, *scores.pop(i), pieces)
            elif op[0] == "V":
                pieces = pv(i, *probs.pop(i))
            else:
                hooks[i]()

    def phase1(c_s, wq_r, wk_r, wv_r, wr_s, gw_s, wg_s, wu_s, wd_s, xa_s, wq0_s, wq1_s):
        def x_copy(j):
            return pltpu.make_async_copy(xT_hbm.at[:, pl.ds(j * RC, RC)], xT_s.at[:, pl.ds(j * RC, RC)],
                                         sem.at[S_X + j])

        def wq_copy(g, j):
            return pltpu.make_async_copy(wq_hbm.at[:, pl.ds(j * mq, mq), g], wq_r.at[:, pl.ds(j * mq, mq), g],
                                         sem.at[(S_Q1 if g else S_Q0) + j])

        def kv_copies(j):
            return [pltpu.make_async_copy(src.at[pl.ds(j * n, n)], dst.at[pl.ds(j * n, n)], sem.at[s0 + j])
                    for src, dst, s0, n in ((c_hbm, c_s, S_C, RC), (wk_hbm, wk_r, S_K, mk), (wv_hbm, wv_r, S_V, mk))]

        misc = [pltpu.make_async_copy(a, b, sem.at[S_MISC + i]) for i, (a, b) in enumerate(
            [(wr_hbm, wr_s), (gw_hbm, gw_s), (wg_hbm, wg_s), (wu_hbm, wu_s), (wd_hbm, wd_s)])]

        x_copy(0).start()
        for j in range(NCH):
            wq_copy(0, j).start()

        def start_rest():
            for j in range(NCH):
                if j + 1 < NCH:
                    x_copy(j + 1).start()
                wq_copy(1, j).start()
            misc[0].start()
            misc[1].start()
            for j in range(NCH):
                for cp in kv_copies(j):
                    cp.start()
            for cp in misc[2:]:
                cp.start()
            wo_copy.start()

        start_rest()

        def x_operands(j):
            c0 = j * RC if isinstance(j, int) else pl.multiple_of(j * RC, RC)
            r0 = j * HQ if isinstance(j, int) else pl.multiple_of(j * HQ, HQ)
            a = [xT_s[kh * mh:(kh + 1) * mh, pl.ds(c0 + rb * TQ, TQ)].astype(F32)
                 for rb in range(2) for kh in range(2)]
            for n, o in enumerate(_left(*a)):
                xa_s[n, pl.ds(r0, HQ), :] = pltpu.bitcast(o.astype(BF16).T, U32)

        def wq_operands(g, p, never=None, link=None):
            w = [pltpu.bitcast(wq_r[kh, pl.ds(2 * p, 2), g], U32) for kh in range(2)]
            w = [[x[0], x[1]] for x in w]
            if link is not None:
                w[0][0] = jnp.where(never, link, w[0][0])
            rows = [_right(*[_unpack(w[kh][e], par) for kh in range(2) for par in range(2)]) for e in range(2)]
            for n in range(7):
                (wq0_s, wq1_s)[g][n, pl.ds(p, 8, stride=pq), :] = _pack(rows[0][n], rows[1][n])

        x_copy(0).wait()
        x_operands(0)

        def first_half(j, _):
            wq_copy(0, j).wait()
            for k in range(mq // 2):
                wq_operands(0, j * (mq // 2) + k)
            return 0
        jax.lax.fori_loop(0, NCH, first_half, 0)

        def q_step(g, j, side):
            pieces = []
            for r in range(4):
                m = {}
                for n in (0, 3, 4, 6, 1, 2, 5):
                    w = jnp.concatenate([_as_bf16((wq0_s, wq1_s)[g][n, pl.ds((dt * 4 + r) * pq, mh // 2), :])
                                         for dt in range(2)], axis=1)
                    m[n] = jnp.dot(_as_bf16(xa_s[n, pl.ds(pl.multiple_of(j * HQ, HQ), HQ), :]), w,
                                   preferred_element_type=F32)
                    for k in range(5):
                        pieces.append(m[n][k * 48:k * 48 + 8, (k % 2) * L:(k % 2 + 1) * L])
                        side(len(pieces) - 1, pieces[-1])
                for par, rb, comb in ((0, 0, _c11), (0, 1, _c21), (1, 0, _c12), (1, 1, _c22)):
                    r0 = pl.multiple_of(j * TQ + rb * HQ, HQ)
                    q_s[8 * g + 2 * r + par, pl.ds(r0, HQ), :] = _to_u32(comb(m) * qscale)

        def q_lo(j, _):
            never = _never(j)

            def side(k, piece):
                if k == 35:
                    @pl.when(j + 1 < NCH)
                    def _():
                        x_copy(j + 1).wait()
                    wq_copy(1, j).wait()
                if k >= 42 and k % 3 == 0 and (k - 42) // 3 < mq // 2:
                    wq_operands(1, j * (mq // 2) + (k - 42) // 3, never, pltpu.bitcast(piece, U32))
            q_step(0, j, side)
            x_operands((j + 1) & (NCH - 1))
            return 0
        jax.lax.fori_loop(0, NCH, q_lo, 0)

        def q_hi(j, _):
            for cp in kv_copies(j):
                cp.wait()
            never = _never(j)

            def side(kk, piece):
                if kk >= 128:
                    return
                k, g = kk // 2, kk % 2
                link = pltpu.bitcast(piece, U32)
                if g == 0:
                    rg, t = k // 4, k % 4
                    a = []
                    for rb in range(2):
                        r0 = pl.multiple_of(j * RC + rb * TQ + rg * 16, 16)
                        for ch in range(2):
                            a.append(c_s[pl.ds(r0, 16), (2 * t + ch) * L:(2 * t + ch + 1) * L].astype(F32))
                    a[0] = jnp.where(jnp.concatenate([never, never], axis=0),
                                     jnp.concatenate([piece, piece], axis=0), a[0])
                    us = [_to_u32(o) for o in _left(*a)]
                    d0 = pl.multiple_of(j * HQ + rg * 8, 8)
                    for n in range(7):
                        a_s[n, pl.ds(d0, 8), t * L:(t + 1) * L] = us[n]
                    link = _or_all([us[n] for n in (0, 1, 4, 5, 6)])
                c0 = j * mk + 2 * k
                w = [pltpu.bitcast(r[pl.ds(c0 + o, 2), g], U32) for o in (0, L) for r in (wk_r, wv_r)]
                w = [[x[0], x[1]] for x in w]
                w[0][0] = jnp.where(never, link, w[0][0])
                for par in range(2):
                    rows = [_right(*[_unpack(x[e], par) for x in w]) for e in range(2)]
                    for n in range(7):
                        b_s[n, 2 * g + par, pl.ds(j * (mk // 4) + k, 8, stride=pb), :] = _pack(
                            rows[0][n], rows[1][n])
            q_step(1, j, side)
            return 0
        jax.lax.fori_loop(0, NCH, q_hi, 0)

        for cp in misc:
            cp.wait()
        st = {}
        rid = jax.lax.broadcasted_iota(jnp.int32, (8, M), 0)

        def route():
            wr = jnp.broadcast_to(wr_s[...].reshape(1, M).astype(F32), (8, M))
            gw = jnp.broadcast_to(gw_s[...].reshape(1, M).astype(F32), (8, M))
            rg = jnp.dot(jnp.where(rid == 0, wr, gw).astype(BF16), xT_s[...], preferred_element_type=F32)
            g_s[...] = jax.nn.sigmoid(rg[1:2])
            r = rg[0:1].astype(BF16).astype(F32)
            lane = jax.lax.broadcasted_iota(jnp.int32, (1, S), 1)
            m1 = jnp.max(r, axis=1, keepdims=True)
            i1 = jnp.min(jnp.where(r == m1, lane, S - 1), axis=1, keepdims=True)
            r2 = jnp.where(lane == i1, -jnp.inf, r)
            m2 = jnp.max(r2, axis=1, keepdims=True)
            i2 = jnp.min(jnp.where(jnp.logical_and(r2 == m2, lane != i1), lane, S - 1), axis=1, keepdims=True)
            st["idx"] = [i1[0, 0], i2[0, 0]]
            st["r"] = jax.nn.sigmoid(jnp.where(rid[:, :1] == 0, m1, m2))

        def gather():
            ln = jax.lax.broadcasted_iota(jnp.int32, (8, L), 1)
            xs = None
            for t, i in enumerate(st["idx"]):
                pick = jnp.where(jnp.logical_and(rid[:, :L] == t, ln == (i & (L - 1))), 1.0, 0.0)
                blk = xT_s[:, pl.ds(pl.multiple_of((i >> 7) << 7, L), L)]
                x = jax.lax.dot_general(pick.astype(BF16), blk, NT, preferred_element_type=F32)
                xs = x if xs is None else xs + x
            st["x"] = xs.astype(BF16)

        def hidden():
            gate = jnp.dot(st["x"], wg_s[...], preferred_element_type=F32)
            up = jnp.dot(st["x"], wu_s[...], preferred_element_type=F32)
            st["h"] = (jax.nn.silu(gate) * up).astype(BF16)

        def patch():
            y = jax.lax.dot_general(st["h"], wd_s[...], NT, preferred_element_type=F32) * st["r"]
            mp = -(-M // L) * L
            y = jnp.concatenate([y, jnp.zeros((8, mp - M), F32)], axis=1)
            yT = jnp.concatenate([y, jnp.zeros((L - 8, mp), F32)], axis=0).T
            ln = jax.lax.broadcasted_iota(jnp.int32, (M, L), 1)
            for t, i in enumerate(st["idx"]):
                c0 = pl.multiple_of((i >> 7) << 7, L)
                blk = xT_s[:, pl.ds(c0, L)].astype(F32)
                upd = jnp.where(ln == (i & (L - 1)), yT[:M, t:t + 1], 0.0)
                xT_s[:, pl.ds(c0, L)] = (blk + upd).astype(BF16)

        head_program("h0 G0 h1 G3 h2 G4 h3 G6 G1 G2 G5 w0", None, 0, None, False,
                     hooks=(route, gather, hidden, patch))

    def phase2(x7_s):
        wo_copy.wait()

        def head(h, _):
            head_program(LOOP_ORDER, h, h + 1, x7_s, False)
            return 0
        jax.lax.fori_loop(0, H - 1, head, 0)
        head_program(LAST_ORDER, H - 1, pl.program_id(0), x7_s, True)

        def out_step(j, _):
            c0 = pl.multiple_of(j * RC, RC)
            for t in range(RC // TQ):
                r0 = pl.multiple_of(j * (RC // 4) + t * 64, 64)
                m = {}
                for n in range(7):
                    left = jnp.concatenate([_as_bf16(wo7_s[n, h, :M // 4]) for h in range(H)], axis=1)
                    right = jnp.concatenate([_as_bf16(x7_s[n, h, pl.ds(r0, 64), :]) for h in range(H)], axis=1)
                    m[n] = jax.lax.dot_general(left, right, NT, preferred_element_type=F32)
                a = jnp.concatenate([jnp.concatenate([_c11(m), _c12(m)], axis=1),
                                     jnp.concatenate([_c21(m), _c22(m)], axis=1)], axis=0)
                gj = g_s[:, pl.ds(c0 + t * TQ, TQ)]
                b = xT_s[:, pl.ds(c0 + t * TQ, TQ)].astype(F32)
                o_s[:, pl.ds(c0 + t * TQ, TQ)] = (gj * a + (1.0 - gj) * b).astype(BF16)
            out_copy(j).start()
            return 0
        jax.lax.fori_loop(0, S // RC, out_step, 0)
        for j in range(S // RC):
            out_copy(j).wait()

    pl.run_scoped(
        phase1,
        *[pltpu.VMEM(r.shape, r.dtype) for r in (c_hbm, wq_hbm, wk_hbm, wv_hbm, wr_hbm, gw_hbm,
                                                 wg_hbm, wu_hbm, wd_hbm)],
        pltpu.VMEM((7, S // 4, mh), U32),
        pltpu.VMEM((7, 8 * pq, L), U32),
        pltpu.VMEM((7, 8 * pq, L), U32))
    pl.run_scoped(phase2, pltpu.VMEM((7, H, S // 4, L), U32))


def _tile_view(w):
    c, h, d = w.shape
    w = w.reshape(c, h // 8, 8, d // L, L).transpose(0, 1, 3, 2, 4)
    return w.reshape(c, h // 8, 8 * (d // L), L)


@jax.jit
def pallas_gated_mix__compressed_kv_cla__moe_arch_mod__prompt_kernel(
    A_x: jax.Array,
    A_c_kv: jax.Array,
    A_w_q: jax.Array,
    A_w_uk: jax.Array,
    A_w_uv: jax.Array,
    A_w_o: jax.Array,
    B_x: jax.Array,
    B_w_r: jax.Array,
    B_w_gate: jax.Array,
    B_w_up: jax.Array,
    B_w_down: jax.Array,
    gate_w: jax.Array,
):
    _, S, M = A_x.shape
    DC = A_c_kv.shape[2]
    H, D = A_w_q.shape[1], A_w_q.shape[2]
    args = (jnp.transpose(A_x[0]), A_c_kv[0], _tile_view(A_w_q).reshape(2, M // 2, 2, 16, L),
            _tile_view(A_w_uk), _tile_view(A_w_uv),
            jnp.transpose(A_w_o, (0, 2, 1)), B_w_r, gate_w, B_w_gate, B_w_up, jnp.transpose(B_w_down))

    def kern(*refs):
        _kernel(*refs, S=S, M=M, DC=DC, H=H, D=D)

    hbm = pl.BlockSpec(memory_space=pl.ANY)
    oT = pl.pallas_call(
        kern,
        grid=(1,),
        out_shape=jax.ShapeDtypeStruct((M, S), A_x.dtype),
        in_specs=[hbm] * len(args),
        out_specs=hbm,
        scratch_shapes=[
            pltpu.VMEM((M, S), BF16),
            pltpu.VMEM((H, M, D), BF16),
            pltpu.VMEM((7, S // 4, DC // 2), U32),
            pltpu.VMEM((7, 4, 8 * (DC // 4 + 1), L), U32),
            pltpu.VMEM((H, S // 2, D), U32),
            pltpu.VMEM((S // 2, D), U32),
            pltpu.VMEM((S // 2, D), U32),
            pltpu.VMEM((5, S // 4, L), U32),
            pltpu.VMEM((7, H, L, L), U32),
            pltpu.VMEM((1, S), F32),
            pltpu.VMEM((M, S), BF16),
            pltpu.SemaphoreType.DMA((N_SEM,)),
        ],
        compiler_params=pltpu.CompilerParams(vmem_limit_bytes=124 * 1024 * 1024),
    )(*args)
    return jnp.transpose(oT)[None]
```

```python
import math

import jax
import jax.numpy as jnp
import jax.experimental.pallas as pl
import jax.experimental.pallas.tpu as pltpu

F32 = jnp.float32
BF16 = jnp.bfloat16
U32 = jnp.uint32
NT = (((1,), (1,)), ((), ()))

L = 128
TQ = 256
HQ = TQ // 2
RC = 512
NCH = 4

PAD_TILES = 3
PAD_V = 16

S_X, S_Q0, S_Q1, S_K, S_V, S_C, S_MISC, S_OUT = 0, 4, 8, 12, 16, 20, 24, 30
N_SEM = 34

LOOP_ORDER = ("Q7 G0 S7 V7 Q6 G3 S6 V6 Q5 G4 S5 V5 Q4 G6 S4 V4 Q3 G1 S3 V3 Q2 G2 S2 V2 "
              "Q1 Q0 G5 S1 S0 V1 V0 w0")
LAST_ORDER = "Q7 Q6 S7 Q5 S6 V7 Q4 S5 V6 Q3 S4 V5 Q2 S3 V4 Q1 S2 V3 Q0 S1 V2 S0 V1 V0"


def _to_u32(x_f32):
    return pltpu.bitcast(x_f32.astype(BF16), U32)


def _as_bf16(x_u32):
    return pltpu.bitcast(x_u32, BF16)


def _left(a11, a12, a21, a22):
    return (a11 + a22, a21 + a22, a11, a22, a11 + a12, a21 - a11, a12 - a22)


def _right(b11, b12, b21, b22):
    return (b11 + b22, b11, b12 - b22, b21 - b11, b22, b11 + b12, b21 + b22)


def _c11(m):
    return (m[0] + m[3]) + (m[6] - m[4])


def _c12(m):
    return m[2] + m[4]


def _c21(m):
    return m[1] + m[3]


def _c22(m):
    return (m[0] - m[1]) + (m[2] + m[5])


def _never(i):
    return jax.lax.broadcasted_iota(jnp.int32, (8, L), 0) < (i >> 10)


def _or_all(xs):
    out = xs[0]
    for x in xs[1:]:
        out = out | x
    return out


def _unpack(w, par):
    return pltpu.unpack_elementwise(w, index=par, packed_dtype=BF16, unpacked_dtype=F32)


def _pack(even, odd):
    return pltpu.bitcast(pltpu.pack_elementwise([even, odd], packed_dtype=BF16), U32)


def _head_weight(ref, h, nrows, pitch):
    sel = ((h >> 3) << 1) + (h & 1)
    r = (h >> 1) & 3
    return jnp.concatenate(
        [_as_bf16(ref[sel, pl.ds((dt * 4 + r) * pitch, nrows), :]) for dt in range(2)], axis=1)


def _kernel(xT_hbm, c_hbm, wq_hbm, wk_hbm, wv_hbm, wo_hbm, wr_hbm, gw_hbm, wg_hbm, wu_hbm, wd_hbm,
            o_hbm,
            g_s, xT_s, wo_s, a_s, b_s, q_s, k_s, v_s, wo7_s, o_s, v5_s, sem, *, S, M, DC, H, D):
    nq = S // TQ
    mh = M // 2
    pq = mh // 2 + 1
    pb = DC // 4 + 1
    mq = mh // NCH
    mk = DC // NCH
    qscale = (D ** -0.5) * math.log2(math.e)
    neg = -1e9 * math.log2(math.e)
    wo_copy = pltpu.make_async_copy(wo_hbm, wo_s, sem.at[S_MISC + 5])

    def out_copy(j):
        return pltpu.make_async_copy(o_s.at[:, pl.ds(j * RC, RC)], o_hbm.at[:, pl.ds(j * RC, RC)],
                                     sem.at[S_OUT + j])

    tri = (jax.lax.broadcasted_iota(jnp.int32, (L, L), 1) <= jax.lax.broadcasted_iota(jnp.int32, (L, L), 0))

    def head_program(order, h, hn, x7_s, two_pass, hooks=None):
        never = _never(hn)
        prods, held, waiting = {}, {}, []

        def spots(v, cols, rows=(0, 64, 128, 192)):
            return [v[r:r + 8, n * L:(n + 1) * L] for n in cols for r in rows]

        def tie(lhs, links, every):
            rows = []
            for rg in range(lhs.shape[0] // 8):
                blk = lhs[rg * 8:(rg + 1) * 8]
                if links and rg % every == 0:
                    blk = jnp.concatenate([jnp.where(never, links.pop(0), blk[:, :L]), blk[:, L:]], axis=1)
                rows.append(blk)
            return jnp.concatenate(rows, axis=0)

        def proj(n):
            lhs = a_s[n]
            if waiting:
                lhs = tie(lhs, list(waiting), lhs.shape[0] // 8 // len(waiting))
                del waiting[:]
            prods[n] = jnp.dot(_as_bf16(lhs), _head_weight(b_s.at[n], hn, DC // 4, pb),
                               preferred_element_type=F32)
            for key, odd, comb, needs in (("k", 0, _c11, (0, 3, 4, 6)), ("k", 1, _c21, (1, 3)),
                                          ("v", 0, _c12, (2, 4)), ("v", 1, _c22, (0, 1, 2, 5))):
                if n in needs and all(x in prods for x in needs):
                    for k in range(nq // 2):
                        c = comb({x: prods[x][k * TQ:(k + 1) * TQ] for x in needs})
                        held[2 * k + odd, key] = _to_u32(c)
                        if key == "v" and 2 * k + odd < nq - 1:
                            ops = _right(c[:L, :L], c[:L, L:], c[L:, :L], c[L:, L:])
                            held[2 * k + odd, "r"] = [_to_u32(ops[x]) for x in (0, 2, 3, 5, 6)]
            return spots(prods[n], (0, 1), range(0, S // 2, 32))

        def write_kv():
            for ch in reversed(range(nq)):
                k_s[ch * HQ:(ch + 1) * HQ, :] = held[ch, "k"]
                v_s[ch * HQ:(ch + 1) * HQ, :] = held[ch, "v"]
                for n, o in enumerate(held.get((ch, "r"), ())):
                    v5_s[n, ch * 64:(ch + 1) * 64, :] = o

        def qk(i):
            q = _as_bf16(q_s[h, i * HQ:(i + 1) * HQ, :])
            n0 = i * TQ
            n1 = n0 + L
            s1 = jax.lax.dot_general(q, _as_bf16(k_s[0:n1 // 2, :]), NT, preferred_element_type=F32)
            s2 = jax.lax.dot_general(q[L:], _as_bf16(k_s[n1 // 2:(n1 + L) // 2, :]), NT,
                                     preferred_element_type=F32)
            top = jnp.where(tri, s1[:L, n0:], neg)
            if n0:
                top = jnp.concatenate([s1[:L, :n0], top], axis=1)
            bot = jnp.concatenate([s1[L:], jnp.where(tri, s2, neg)], axis=1)
            return (top, bot), spots(s1, range(max(1, n0 // L)))

        def softmax(i, top, bot, pieces):
            G, span = (16, 0.8) if two_pass else (8, 0.9)
            p, sums, prev = ([], []), ([], []), None
            for k in range(TQ // G):
                half = k % 2
                s = (top, bot)[half][(k // 2) * G:(k // 2 + 1) * G]
                tiles = [s[:, t:t + L] for t in range(0, s.shape[1], L)]
                link = pieces[int(span * k * G / TQ * len(pieces))]
                if prev is not None:
                    link = jnp.where(never, link, prev)
                m = jnp.broadcast_to(jnp.max(s, axis=1, keepdims=True), (G, L))
                m = jnp.where(jnp.concatenate([never] * (G // 8), axis=0),
                              jnp.concatenate([link] * (G // 8), axis=0), m)
                e = [jnp.exp2(t - m) for t in tiles]
                acc = e[0]
                for x in e[1:]:
                    acc = acc + x
                prev = acc[G - 8:]
                if two_pass:
                    m = m + jnp.log2(jnp.sum(acc, axis=1, keepdims=True))
                    e = [jnp.exp2(t - m) for t in tiles]
                sums[half].append(acc)
                p[half].append(jnp.concatenate(e, axis=1))
            pt, pb_ = jnp.concatenate(p[0], axis=0), jnp.concatenate(p[1], axis=0)

            def tile(x, t):
                return x[:, t * L:(t + 1) * L]
            ops = [_left(tile(pt, 2 * c), tile(pt, 2 * c + 1), tile(pb_, 2 * c), tile(pb_, 2 * c + 1))
                   for c in range(i)]
            left = [jnp.concatenate([o[n] for o in ops], axis=1).astype(BF16) for n in range(7)] if i else None
            inv = None if two_pass else [
                pl.reciprocal(jnp.sum(jnp.concatenate(x, axis=0), axis=1, keepdims=True), approx=True)
                for x in sums]
            return (left, jnp.concatenate([tile(pt, 2 * i), tile(pb_, 2 * i)], axis=0).astype(BF16),
                    tile(pb_, 2 * i + 1).astype(BF16), inv)

        def pv(i, left, p1, p2, inv):
            r0 = i * HQ
            m, pieces = {}, []
            for n in (2, 3, 0, 4, 1, 5, 6) if i else ():
                if n == 1:
                    w = jnp.concatenate([_as_bf16(v_s[c * HQ:c * HQ + 64, :L]) for c in range(i)], axis=0)
                elif n == 4:
                    w = jnp.concatenate([_as_bf16(v_s[c * HQ + 64:(c + 1) * HQ, L:]) for c in range(i)], axis=0)
                else:
                    w = _as_bf16(v5_s[(0, 2, 3, 5, 6).index(n), 0:i * 64, :])
                m[n] = jnp.dot(left[n], w, preferred_element_type=F32)
                pieces += spots(m[n], (0,), (0, 32, 64, 96))
            c1 = jnp.dot(p1, _as_bf16(v_s[r0:r0 + 64, :]), preferred_element_type=F32)
            c2 = jnp.dot(p2, _as_bf16(v_s[r0 + 64:r0 + HQ, :]), preferred_element_type=F32)
            top, bot = c1[:L], c1[L:] + c2
            if i:
                top = top + jnp.concatenate([_c11(m), _c12(m)], axis=1)
                bot = bot + jnp.concatenate([_c21(m), _c22(m)], axis=1)
            else:
                pieces = spots(c1, (0, 1))
            if inv is not None:
                top, bot = top * inv[0], bot * inv[1]
            us = [_to_u32(o) for o in _right(top[:, :L], bot[:, :L], top[:, L:], bot[:, L:])]
            for n in range(7):
                x7_s[n, h, i * 64:(i + 1) * 64, :] = us[n]
            waiting.extend(_or_all([us[n][g * 8:(g + 1) * 8] for n in (0, 2, 3, 5, 6)]) for g in range(8))
            return pieces

        def wo_operands():
            for rg in range(M // 32):
                a = [wo_s[h, hf * (M // 2) + rg * 16:hf * (M // 2) + (rg + 1) * 16, ch * L:(ch + 1) * L].astype(F32)
                     for hf in range(2) for ch in range(2)]
                us = [_to_u32(o) for o in _left(*a)]
                for n in range(7):
                    wo7_s[n, h, rg * 8:(rg + 1) * 8, :] = us[n]
                waiting.append(_or_all([us[n] for n in (0, 1, 4, 5, 6)]))

        if h is not None:
            wo_operands()
        scores, probs, pieces = {}, {}, None
        for op in order.split():
            i = int(op[1:])
            if op[0] == "G":
                pieces = proj(i)
            elif op[0] == "w":
                write_kv()
            elif op[0] == "Q":
                scores[i], pieces = qk(i)
            elif op[0] == "S":
                probs[i] = softmax(i, *scores.pop(i), pieces)
            elif op[0] == "V":
                pieces = pv(i, *probs.pop(i))
            else:
                hooks[i]()

    def phase1(c_s, wq_r, wk_r, wv_r, wg_s, wu_s, wd_s, xa_s, wq0_s, wq1_s, wr_s, gw_s):
        def x_copy(j):
            return pltpu.make_async_copy(xT_hbm.at[:, pl.ds(j * RC, RC)], xT_s.at[:, pl.ds(j * RC, RC)],
                                         sem.at[S_X + j])

        def wq_copy(g, j):
            return pltpu.make_async_copy(wq_hbm.at[:, pl.ds(j * mq, mq), g], wq_r.at[:, pl.ds(j * mq, mq), g],
                                         sem.at[(S_Q1 if g else S_Q0) + j])

        def kv_copies(j):
            return [pltpu.make_async_copy(src.at[pl.ds(j * n, n)], dst.at[pl.ds(j * n, n)], sem.at[s0 + j])
                    for src, dst, s0, n in ((c_hbm, c_s, S_C, RC), (wk_hbm, wk_r, S_K, mk), (wv_hbm, wv_r, S_V, mk))]

        misc = [pltpu.make_async_copy(a, b, sem.at[S_MISC + i]) for i, (a, b) in enumerate(
            [(wr_hbm, wr_s), (gw_hbm, gw_s), (wg_hbm, wg_s), (wu_hbm, wu_s), (wd_hbm, wd_s)])]

        x_copy(0).start()
        for j in range(NCH):
            wq_copy(0, j).start()

        def start_rest():
            for j in range(NCH):
                if j + 1 < NCH:
                    x_copy(j + 1).start()
                wq_copy(1, j).start()
            misc[0].start()
            misc[1].start()
            for j in range(NCH):
                for cp in kv_copies(j):
                    cp.start()
            for cp in misc[2:]:
                cp.start()
            wo_copy.start()

        start_rest()

        def x_operands(j):
            c0 = j * RC if isinstance(j, int) else pl.multiple_of(j * RC, RC)
            r0 = j * HQ if isinstance(j, int) else pl.multiple_of(j * HQ, HQ)
            a = [xT_s[kh * mh:(kh + 1) * mh, pl.ds(c0 + rb * TQ, TQ)].astype(F32)
                 for rb in range(2) for kh in range(2)]
            for n, o in enumerate(_left(*a)):
                xa_s[n, pl.ds(r0, HQ), :] = pltpu.bitcast(o.astype(BF16).T, U32)

        def wq_operands(g, p, never=None, link=None):
            w = [pltpu.bitcast(wq_r[kh, pl.ds(2 * p, 2), g], U32) for kh in range(2)]
            w = [[x[0], x[1]] for x in w]
            if link is not None:
                w[0][0] = jnp.where(never, link, w[0][0])
            rows = [_right(*[_unpack(w[kh][e], par) for kh in range(2) for par in range(2)]) for e in range(2)]
            for n in range(7):
                (wq0_s, wq1_s)[g][n, pl.ds(p, 8, stride=pq), :] = _pack(rows[0][n], rows[1][n])

        x_copy(0).wait()
        x_operands(0)

        def first_half(j, _):
            wq_copy(0, j).wait()
            for k in range(mq // 2):
                wq_operands(0, j * (mq // 2) + k)
            return 0
        jax.lax.fori_loop(0, NCH, first_half, 0)

        def q_step(g, j, side):
            pieces = []
            for r in range(4):
                m = {}
                for n in (0, 3, 4, 6, 1, 2, 5):
                    w = jnp.concatenate([_as_bf16((wq0_s, wq1_s)[g][n, pl.ds((dt * 4 + r) * pq, mh // 2), :])
                                         for dt in range(2)], axis=1)
                    m[n] = jnp.dot(_as_bf16(xa_s[n, pl.ds(pl.multiple_of(j * HQ, HQ), HQ), :]), w,
                                   preferred_element_type=F32)
                    for k in range(5):
                        pieces.append(m[n][k * 48:k * 48 + 8, (k % 2) * L:(k % 2 + 1) * L])
                        side(len(pieces) - 1, pieces[-1])
                for par, rb, comb in ((0, 0, _c11), (0, 1, _c21), (1, 0, _c12), (1, 1, _c22)):
                    r0 = pl.multiple_of(j * TQ + rb * HQ, HQ)
                    q_s[8 * g + 2 * r + par, pl.ds(r0, HQ), :] = _to_u32(comb(m) * qscale)

        def q_lo(j, _):
            never = _never(j)

            def side(k, piece):
                if k == 35:
                    @pl.when(j + 1 < NCH)
                    def _():
                        x_copy(j + 1).wait()
                    wq_copy(1, j).wait()
                if k >= 42 and k % 3 == 0 and (k - 42) // 3 < mq // 2:
                    wq_operands(1, j * (mq // 2) + (k - 42) // 3, never, pltpu.bitcast(piece, U32))
            q_step(0, j, side)
            x_operands((j + 1) & (NCH - 1))
            return 0
        jax.lax.fori_loop(0, NCH, q_lo, 0)

        def q_hi(j, _):
            for cp in kv_copies(j):
                cp.wait()
            never = _never(j)

            def side(kk, piece):
                if kk >= 128:
                    return
                k, g = kk // 2, kk % 2
                link = pltpu.bitcast(piece, U32)
                if g == 0:
                    rg, t = k // 4, k % 4
                    a = []
                    for rb in range(2):
                        r0 = pl.multiple_of(j * RC + rb * TQ + rg * 16, 16)
                        for ch in range(2):
                            a.append(c_s[pl.ds(r0, 16), (2 * t + ch) * L:(2 * t + ch + 1) * L].astype(F32))
                    a[0] = jnp.where(jnp.concatenate([never, never], axis=0),
                                     jnp.concatenate([piece, piece], axis=0), a[0])
                    us = [_to_u32(o) for o in _left(*a)]
                    d0 = pl.multiple_of(j * HQ + rg * 8, 8)
                    for n in range(7):
                        a_s[n, pl.ds(d0, 8), t * L:(t + 1) * L] = us[n]
                    link = _or_all([us[n] for n in (0, 1, 4, 5, 6)])
                c0 = j * mk + 2 * k
                w = [pltpu.bitcast(r[pl.ds(c0 + o, 2), g], U32) for o in (0, L) for r in (wk_r, wv_r)]
                w = [[x[0], x[1]] for x in w]
                w[0][0] = jnp.where(never, link, w[0][0])
                for par in range(2):
                    rows = [_right(*[_unpack(x[e], par) for x in w]) for e in range(2)]
                    for n in range(7):
                        b_s[n, 2 * g + par, pl.ds(j * (mk // 4) + k, 8, stride=pb), :] = _pack(
                            rows[0][n], rows[1][n])
            q_step(1, j, side)
            return 0
        jax.lax.fori_loop(0, NCH, q_hi, 0)

        for cp in misc:
            cp.wait()
        st = {}
        rid = jax.lax.broadcasted_iota(jnp.int32, (8, M), 0)

        def route():
            wr = jnp.broadcast_to(wr_s[...].reshape(1, M).astype(F32), (8, M))
            gw = jnp.broadcast_to(gw_s[...].reshape(1, M).astype(F32), (8, M))
            rg = jnp.dot(jnp.where(rid == 0, wr, gw).astype(BF16), xT_s[...], preferred_element_type=F32)
            g_s[0:1, :S] = jax.nn.sigmoid(rg[1:2])
            r = rg[0:1].astype(BF16).astype(F32)
            lane = jax.lax.broadcasted_iota(jnp.int32, (1, S), 1)
            m1 = jnp.max(r, axis=1, keepdims=True)
            i1 = jnp.min(jnp.where(r == m1, lane, S - 1), axis=1, keepdims=True)
            r2 = jnp.where(lane == i1, -jnp.inf, r)
            m2 = jnp.max(r2, axis=1, keepdims=True)
            i2 = jnp.min(jnp.where(jnp.logical_and(r2 == m2, lane != i1), lane, S - 1), axis=1, keepdims=True)
            st["idx"] = [i1[0, 0], i2[0, 0]]
            st["r"] = jax.nn.sigmoid(jnp.where(rid[:, :1] == 0, m1, m2))

        def gather():
            ln = jax.lax.broadcasted_iota(jnp.int32, (8, L), 1)
            xs = None
            for t, i in enumerate(st["idx"]):
                pick = jnp.where(jnp.logical_and(rid[:, :L] == t, ln == (i & (L - 1))), 1.0, 0.0)
                blk = xT_s[:, pl.ds(pl.multiple_of((i >> 7) << 7, L), L)]
                x = jax.lax.dot_general(pick.astype(BF16), blk, NT, preferred_element_type=F32)
                xs = x if xs is None else xs + x
            st["x"] = xs.astype(BF16)

        def hidden():
            gate = jnp.dot(st["x"], wg_s[...], preferred_element_type=F32)
            up = jnp.dot(st["x"], wu_s[...], preferred_element_type=F32)
            st["h"] = (jax.nn.silu(gate) * up).astype(BF16)

        def patch():
            y = jax.lax.dot_general(st["h"], wd_s[...], NT, preferred_element_type=F32) * st["r"]
            mp = -(-M // L) * L
            y = jnp.concatenate([y, jnp.zeros((8, mp - M), F32)], axis=1)
            yT = jnp.concatenate([y, jnp.zeros((L - 8, mp), F32)], axis=0).T
            ln = jax.lax.broadcasted_iota(jnp.int32, (M, L), 1)
            for t, i in enumerate(st["idx"]):
                c0 = pl.multiple_of((i >> 7) << 7, L)
                blk = xT_s[:, pl.ds(c0, L)].astype(F32)
                upd = jnp.where(ln == (i & (L - 1)), yT[:M, t:t + 1], 0.0)
                xT_s[:, pl.ds(c0, L)] = (blk + upd).astype(BF16)

        head_program("h0 G0 h1 G3 h2 G4 h3 G6 G1 G2 G5 w0", None, 0, None, False,
                     hooks=(route, gather, hidden, patch))

    def phase2(x7_s):
        wo_copy.wait()

        def head(h, _):
            head_program(LOOP_ORDER, h, h + 1, x7_s, False)
            return 0
        jax.lax.fori_loop(0, H - 1, head, 0)
        head_program(LAST_ORDER, H - 1, pl.program_id(0), x7_s, True)

        def out_step(j, _):
            c0 = pl.multiple_of(j * RC, RC)
            for t in range(RC // TQ):
                r0 = pl.multiple_of(j * (RC // 4) + t * 64, 64)
                m = {}
                for n in range(7):
                    left = jnp.concatenate([_as_bf16(wo7_s[n, h, :M // 4]) for h in range(H)], axis=1)
                    right = jnp.concatenate([_as_bf16(x7_s[n, h, pl.ds(r0, 64), :]) for h in range(H)], axis=1)
                    m[n] = jax.lax.dot_general(left, right, NT, preferred_element_type=F32)
                a = jnp.concatenate([jnp.concatenate([_c11(m), _c12(m)], axis=1),
                                     jnp.concatenate([_c21(m), _c22(m)], axis=1)], axis=0)
                gj = g_s[0:1, pl.ds(c0 + t * TQ, TQ)]
                b = xT_s[:, pl.ds(c0 + t * TQ, TQ)].astype(F32)
                o_s[:, pl.ds(c0 + t * TQ, TQ)] = (gj * a + (1.0 - gj) * b).astype(BF16)
            out_copy(j).start()
            return 0
        jax.lax.fori_loop(0, S // RC, out_step, 0)
        for j in range(S // RC):
            out_copy(j).wait()

    pl.run_scoped(
        phase1,
        *[pltpu.VMEM(r.shape, r.dtype) for r in (c_hbm, wq_hbm, wk_hbm, wv_hbm, wg_hbm, wu_hbm, wd_hbm)],
        pltpu.VMEM((7, S // 4, mh), U32),
        pltpu.VMEM((7, -(-pq // 4) * 32, L), U32),
        pltpu.VMEM((7, -(-pq // 4) * 32, L), U32),
        pltpu.VMEM((M,), BF16),
        pltpu.VMEM((M,), BF16))
    pl.run_scoped(phase2, pltpu.VMEM((7, H, S // 4, L), U32))


def _tile_view(w):
    c, h, d = w.shape
    w = w.reshape(c, h // 8, 8, d // L, L).transpose(0, 1, 3, 2, 4)
    return w.reshape(c, h // 8, 8 * (d // L), L)


@jax.jit
def pallas_gated_mix__compressed_kv_cla__moe_arch_mod__prompt_kernel(
    A_x: jax.Array,
    A_c_kv: jax.Array,
    A_w_q: jax.Array,
    A_w_uk: jax.Array,
    A_w_uv: jax.Array,
    A_w_o: jax.Array,
    B_x: jax.Array,
    B_w_r: jax.Array,
    B_w_gate: jax.Array,
    B_w_up: jax.Array,
    B_w_down: jax.Array,
    gate_w: jax.Array,
):
    _, S, M = A_x.shape
    DC = A_c_kv.shape[2]
    H, D = A_w_q.shape[1], A_w_q.shape[2]
    args = (jnp.transpose(A_x[0]), A_c_kv[0], _tile_view(A_w_q).reshape(2, M // 2, 2, 16, L),
            _tile_view(A_w_uk), _tile_view(A_w_uv),
            jnp.transpose(A_w_o, (0, 2, 1)), B_w_r, gate_w, B_w_gate, B_w_up, jnp.transpose(B_w_down))

    def kern(*refs):
        _kernel(*refs, S=S, M=M, DC=DC, H=H, D=D)

    hbm = pl.BlockSpec(memory_space=pl.ANY)
    oT = pl.pallas_call(
        kern,
        grid=(1,),
        out_shape=jax.ShapeDtypeStruct((M, S), A_x.dtype),
        in_specs=[hbm] * len(args),
        out_specs=hbm,
        scratch_shapes=[
            pltpu.VMEM((8, S + PAD_TILES * L), F32),
            pltpu.VMEM((M, S), BF16),
            pltpu.VMEM((H, M, D), BF16),
            pltpu.VMEM((7, S // 4, DC // 2), U32),
            pltpu.VMEM((7, 4, 8 * (DC // 4 + 1), L), U32),
            pltpu.VMEM((H, S // 2, D), U32),
            pltpu.VMEM((S // 2, D), U32),
            pltpu.VMEM((S // 2, D), U32),
            pltpu.VMEM((7, H, L, L), U32),
            pltpu.VMEM((M, S), BF16),
            pltpu.VMEM((5, S // 4 + PAD_V, L), U32),
            pltpu.SemaphoreType.DMA((N_SEM,)),
        ],
        compiler_params=pltpu.CompilerParams(vmem_limit_bytes=124 * 1024 * 1024),
    )(*args)
    return jnp.transpose(oT)[None]
```

```python
import math

import jax
import jax.numpy as jnp
import jax.experimental.pallas as pl
import jax.experimental.pallas.tpu as pltpu

F32 = jnp.float32
BF16 = jnp.bfloat16
U32 = jnp.uint32
NT = (((1,), (1,)), ((), ()))

L = 128
TQ = 256
HQ = TQ // 2
RC = 512
NCH = 4

PAD_TILES = 3
PAD_V = 16

S_X, S_Q0, S_Q1, S_K, S_V, S_C, S_MISC, S_OUT = 0, 4, 8, 12, 16, 20, 24, 30
N_SEM = 38

LOOP_ORDER = ("Q7 G0 S7 V7 Q6 G3 S6 V6 Q5 G4 S5 V5 Q4 G6 S4 V4 Q3 G1 S3 V3 Q2 G2 S2 V2 "
              "Q1 Q0 G5 S1 S0 V1 V0 w0")
LAST_ORDER = "Q7 Q6 q5 s7 V7 S6 Q4 V6 S5 r3 V5 S4 r2 V4 S3 r1 V3 S2 r0 V2 S1 S0 V1 V0"
SPAN = 0.9


def _to_u32(x_f32):
    return pltpu.bitcast(x_f32.astype(BF16), U32)


def _as_bf16(x_u32):
    return pltpu.bitcast(x_u32, BF16)


def _left(a11, a12, a21, a22):
    return (a11 + a22, a21 + a22, a11, a22, a11 + a12, a21 - a11, a12 - a22)


def _right(b11, b12, b21, b22):
    return (b11 + b22, b11, b12 - b22, b21 - b11, b22, b11 + b12, b21 + b22)


def _c11(m):
    return (m[0] + m[3]) + (m[6] - m[4])


def _c12(m):
    return m[2] + m[4]


def _c21(m):
    return m[1] + m[3]


def _c22(m):
    return (m[0] - m[1]) + (m[2] + m[5])


def _never(i):
    return jax.lax.broadcasted_iota(jnp.int32, (8, L), 0) < (i >> 10)


def _or_all(xs):
    out = xs[0]
    for x in xs[1:]:
        out = out | x
    return out


def _unpack(w, par):
    return pltpu.unpack_elementwise(w, index=par, packed_dtype=BF16, unpacked_dtype=F32)


def _pack(even, odd):
    return pltpu.bitcast(pltpu.pack_elementwise([even, odd], packed_dtype=BF16), U32)


def _head_weight(ref, h, nrows, pitch):
    sel = ((h >> 3) << 1) + (h & 1)
    r = (h >> 1) & 3
    return jnp.concatenate(
        [_as_bf16(ref[sel, pl.ds((dt * 4 + r) * pitch, nrows), :]) for dt in range(2)], axis=1)


def _kernel(xT_hbm, c_hbm, wq_hbm, wk_hbm, wv_hbm, wo_hbm, wr_hbm, gw_hbm, wg_hbm, wu_hbm, wd_hbm,
            o_hbm,
            g_s, xT_s, wo_s, a_s, b_s, q_s, k_s, v_s, wo7_s, o_s, v5_s, sem, *, S, M, DC, H, D):
    nq = S // TQ
    mh = M // 2
    pq = mh // 2 + 1
    pb = DC // 4 + 1
    mq = mh // NCH
    mk = DC // NCH
    qscale = (D ** -0.5) * math.log2(math.e)
    neg = -1e9 * math.log2(math.e)
    wo_copy = pltpu.make_async_copy(wo_hbm, wo_s, sem.at[S_MISC + 5])

    def out_copy(j):
        return pltpu.make_async_copy(o_s.at[:, pl.ds(j * TQ, TQ)], o_hbm.at[:, pl.ds(j * TQ, TQ)],
                                     sem.at[S_OUT + j])

    tri = (jax.lax.broadcasted_iota(jnp.int32, (L, L), 1) <= jax.lax.broadcasted_iota(jnp.int32, (L, L), 0))

    def head_program(order, h, hn, x7_s, hooks=None):
        never = _never(hn)
        prods, held, waiting = {}, {}, []

        def spots(v, cols, rows=(0, 64, 128, 192)):
            return [v[r:r + 8, n * L:(n + 1) * L] for n in cols for r in rows]

        def tie(lhs, links, every):
            rows = []
            for rg in range(lhs.shape[0] // 8):
                blk = lhs[rg * 8:(rg + 1) * 8]
                if links and rg % every == 0:
                    blk = jnp.concatenate([jnp.where(never, links.pop(0), blk[:, :L]), blk[:, L:]], axis=1)
                rows.append(blk)
            return jnp.concatenate(rows, axis=0)

        def proj(n):
            lhs = a_s[n]
            if waiting:
                lhs = tie(lhs, list(waiting), lhs.shape[0] // 8 // len(waiting))
                del waiting[:]
            prods[n] = jnp.dot(_as_bf16(lhs), _head_weight(b_s.at[n], hn, DC // 4, pb),
                               preferred_element_type=F32)
            for key, odd, comb, needs in (("k", 0, _c11, (0, 3, 4, 6)), ("k", 1, _c21, (1, 3)),
                                          ("v", 0, _c12, (2, 4)), ("v", 1, _c22, (0, 1, 2, 5))):
                if n in needs and all(x in prods for x in needs):
                    for k in range(nq // 2):
                        c = comb({x: prods[x][k * TQ:(k + 1) * TQ] for x in needs})
                        held[2 * k + odd, key] = _to_u32(c)
                        if key == "v" and 2 * k + odd < nq - 1:
                            ops = _right(c[:L, :L], c[:L, L:], c[L:, :L], c[L:, L:])
                            held[2 * k + odd, "r"] = [_to_u32(ops[x]) for x in (0, 2, 3, 5, 6)]
            return spots(prods[n], (0, 1), range(0, S // 2, 32))

        def write_kv():
            for ch in reversed(range(nq)):
                k_s[ch * HQ:(ch + 1) * HQ, :] = held[ch, "k"]
                v_s[ch * HQ:(ch + 1) * HQ, :] = held[ch, "v"]
                for n, o in enumerate(held.get((ch, "r"), ())):
                    v5_s[n, ch * 64:(ch + 1) * 64, :] = o

        def qk(i, tied):
            q = q_s[h, i * HQ:(i + 1) * HQ, :]
            if tied:
                n = len(waiting) - tied + 1
                q = tie(q, waiting[:n], 16 // n)
                del waiting[:n]
            q = _as_bf16(q)
            n0 = i * TQ
            n1 = n0 + L
            s1 = jax.lax.dot_general(q, _as_bf16(k_s[0:n1 // 2, :]), NT, preferred_element_type=F32)
            s2 = jax.lax.dot_general(q[L:], _as_bf16(k_s[n1 // 2:(n1 + L) // 2, :]), NT,
                                     preferred_element_type=F32)
            top = jnp.where(tri, s1[:L, n0:], neg)
            if n0:
                top = jnp.concatenate([s1[:L, :n0], top], axis=1)
            bot = jnp.concatenate([s1[L:], jnp.where(tri, s2, neg)], axis=1)
            return (top, bot), spots(s1, range(max(1, n0 // L)))

        def softmax(i, top, bot, pieces):
            p, sums, prev = ([], []), ([], []), None
            for k in range(TQ // 8):
                half = k % 2
                s = (top, bot)[half][(k // 2) * 8:(k // 2 + 1) * 8]
                link = pieces[int(SPAN * k * 8 / TQ * len(pieces))]
                if prev is not None:
                    link = jnp.where(never, link, prev)
                m = jnp.broadcast_to(jnp.max(s, axis=1, keepdims=True), (8, L))
                m = jnp.where(never, link, m)
                e = [jnp.exp2(s[:, t:t + L] - m) for t in range(0, s.shape[1], L)]
                prev = e[0]
                for x in e[1:]:
                    prev = prev + x
                sums[half].append(prev)
                p[half].append(jnp.concatenate(e, axis=1))
            pt, pb_ = jnp.concatenate(p[0], axis=0), jnp.concatenate(p[1], axis=0)

            def tile(x, t):
                return x[:, t * L:(t + 1) * L]
            ops = [_left(tile(pt, 2 * c), tile(pt, 2 * c + 1), tile(pb_, 2 * c), tile(pb_, 2 * c + 1))
                   for c in range(i)]
            left = [jnp.concatenate([o[n] for o in ops], axis=1).astype(BF16) for n in range(7)] if i else None
            inv = [pl.reciprocal(jnp.sum(jnp.concatenate(x, axis=0), axis=1, keepdims=True), approx=True)
                   for x in sums]
            return (left, jnp.concatenate([tile(pt, 2 * i), tile(pb_, 2 * i)], axis=0).astype(BF16),
                    tile(pb_, 2 * i + 1).astype(BF16), inv)

        def pv(i, left, p1, p2, inv):
            r0 = i * HQ
            m, pieces = {}, []
            for n in (2, 3, 0, 4, 1, 5, 6) if i else ():
                if n == 1:
                    w = jnp.concatenate([_as_bf16(v_s[c * HQ:c * HQ + 64, :L]) for c in range(i)], axis=0)
                elif n == 4:
                    w = jnp.concatenate([_as_bf16(v_s[c * HQ + 64:(c + 1) * HQ, L:]) for c in range(i)], axis=0)
                else:
                    w = _as_bf16(v5_s[(0, 2, 3, 5, 6).index(n), 0:i * 64, :])
                m[n] = jnp.dot(left[n], w, preferred_element_type=F32)
                pieces += spots(m[n], (0,), (0, 32, 64, 96))
            c1 = jnp.dot(p1, _as_bf16(v_s[r0:r0 + 64, :]), preferred_element_type=F32)
            c2 = jnp.dot(p2, _as_bf16(v_s[r0 + 64:r0 + HQ, :]), preferred_element_type=F32)
            top, bot = c1[:L], c1[L:] + c2
            if i:
                top = top + jnp.concatenate([_c11(m), _c12(m)], axis=1)
                bot = bot + jnp.concatenate([_c21(m), _c22(m)], axis=1)
            else:
                pieces = spots(c1, (0, 1))
            top, bot = top * inv[0], bot * inv[1]
            us = [_to_u32(o) for o in _right(top[:, :L], bot[:, :L], top[:, L:], bot[:, L:])]
            for n in range(7):
                x7_s[n, h, i * 64:(i + 1) * 64, :] = us[n]
            waiting.extend(_or_all([us[n][g * 8:(g + 1) * 8] for n in (0, 2, 3, 5, 6)]) for g in range(8))
            return pieces

        def wo_operands():
            for rg in range(M // 32):
                a = [wo_s[h, hf * (M // 2) + rg * 16:hf * (M // 2) + (rg + 1) * 16, ch * L:(ch + 1) * L].astype(F32)
                     for hf in range(2) for ch in range(2)]
                us = [_to_u32(o) for o in _left(*a)]
                for n in range(7):
                    wo7_s[n, h, rg * 8:(rg + 1) * 8, :] = us[n]
                waiting.append(_or_all([us[n] for n in (0, 1, 4, 5, 6)]))

        if h is not None:
            wo_operands()
        scores, probs, pieces = {}, {}, []
        for op in order.split():
            i = int(op[1:])
            if op[0] == "G":
                pieces.append(proj(i))
            elif op[0] == "w":
                write_kv()
            elif op[0] in "Qqr":
                scores[i], new = qk(i, {"Q": 0, "q": 1, "r": 9}[op[0]])
                pieces.append(new)
            elif op[0] in "Ss":
                probs[i] = softmax(i, *scores.pop(i), pieces[-1] if op[0] == "S" else pieces[-2] + pieces[-1])
            elif op[0] == "V":
                pieces.append(pv(i, *probs.pop(i)))
            else:
                hooks[i]()

    def phase1(c_s, wq_r, wk_r, wv_r, wg_s, wu_s, wd_s, xa_s, wq0_s, wq1_s, wr_s, gw_s):
        def x_copy(j):
            return pltpu.make_async_copy(xT_hbm.at[:, pl.ds(j * RC, RC)], xT_s.at[:, pl.ds(j * RC, RC)],
                                         sem.at[S_X + j])

        def wq_copy(g, j):
            return pltpu.make_async_copy(wq_hbm.at[:, pl.ds(j * mq, mq), g], wq_r.at[:, pl.ds(j * mq, mq), g],
                                         sem.at[(S_Q1 if g else S_Q0) + j])

        def kv_copies(j):
            return [pltpu.make_async_copy(src.at[pl.ds(j * n, n)], dst.at[pl.ds(j * n, n)], sem.at[s0 + j])
                    for src, dst, s0, n in ((c_hbm, c_s, S_C, RC), (wk_hbm, wk_r, S_K, mk), (wv_hbm, wv_r, S_V, mk))]

        misc = [pltpu.make_async_copy(a, b, sem.at[S_MISC + i]) for i, (a, b) in enumerate(
            [(wr_hbm, wr_s), (gw_hbm, gw_s), (wg_hbm, wg_s), (wu_hbm, wu_s), (wd_hbm, wd_s)])]

        x_copy(0).start()
        for j in range(NCH):
            wq_copy(0, j).start()

        def start_rest():
            for j in range(NCH):
                if j + 1 < NCH:
                    x_copy(j + 1).start()
                wq_copy(1, j).start()
            misc[0].start()
            misc[1].start()
            for j in range(NCH):
                for cp in kv_copies(j):
                    cp.start()
            for cp in misc[2:]:
                cp.start()
            wo_copy.start()

        start_rest()

        def x_operands(j):
            c0 = j * RC if isinstance(j, int) else pl.multiple_of(j * RC, RC)
            r0 = j * HQ if isinstance(j, int) else pl.multiple_of(j * HQ, HQ)
            a = [xT_s[kh * mh:(kh + 1) * mh, pl.ds(c0 + rb * TQ, TQ)].astype(F32)
                 for rb in range(2) for kh in range(2)]
            for n, o in enumerate(_left(*a)):
                xa_s[n, pl.ds(r0, HQ), :] = pltpu.bitcast(o.astype(BF16).T, U32)

        def wq_operands(g, p, never=None, link=None):
            w = [pltpu.bitcast(wq_r[kh, pl.ds(2 * p, 2), g], U32) for kh in range(2)]
            w = [[x[0], x[1]] for x in w]
            if link is not None:
                w[0][0] = jnp.where(never, link, w[0][0])
            rows = [_right(*[_unpack(w[kh][e], par) for kh in range(2) for par in range(2)]) for e in range(2)]
            for n in range(7):
                (wq0_s, wq1_s)[g][n, pl.ds(p, 8, stride=pq), :] = _pack(rows[0][n], rows[1][n])

        x_copy(0).wait()
        x_operands(0)

        def first_half(j, _):
            wq_copy(0, j).wait()
            for k in range(mq // 2):
                wq_operands(0, j * (mq // 2) + k)
            return 0
        jax.lax.fori_loop(0, NCH, first_half, 0)

        def q_step(g, j, side):
            pieces = []
            for r in range(4):
                m = {}
                for n in (0, 3, 4, 6, 1, 2, 5):
                    w = jnp.concatenate([_as_bf16((wq0_s, wq1_s)[g][n, pl.ds((dt * 4 + r) * pq, mh // 2), :])
                                         for dt in range(2)], axis=1)
                    m[n] = jnp.dot(_as_bf16(xa_s[n, pl.ds(pl.multiple_of(j * HQ, HQ), HQ), :]), w,
                                   preferred_element_type=F32)
                    for k in range(5):
                        pieces.append(m[n][k * 48:k * 48 + 8, (k % 2) * L:(k % 2 + 1) * L])
                        side(len(pieces) - 1, pieces[-1])
                for par, rb, comb in ((0, 0, _c11), (0, 1, _c21), (1, 0, _c12), (1, 1, _c22)):
                    r0 = pl.multiple_of(j * TQ + rb * HQ, HQ)
                    q_s[8 * g + 2 * r + par, pl.ds(r0, HQ), :] = _to_u32(comb(m) * qscale)

        def q_lo(j, _):
            never = _never(j)

            def side(k, piece):
                if k == 35:
                    @pl.when(j + 1 < NCH)
                    def _():
                        x_copy(j + 1).wait()
                    wq_copy(1, j).wait()
                if k >= 42 and k % 3 == 0 and (k - 42) // 3 < mq // 2:
                    wq_operands(1, j * (mq // 2) + (k - 42) // 3, never, pltpu.bitcast(piece, U32))
            q_step(0, j, side)
            x_operands((j + 1) & (NCH - 1))
            return 0
        jax.lax.fori_loop(0, NCH, q_lo, 0)

        def q_hi(j, _):
            for cp in kv_copies(j):
                cp.wait()
            never = _never(j)

            def side(kk, piece):
                if kk >= 128:
                    return
                k, g = kk // 2, kk % 2
                link = pltpu.bitcast(piece, U32)
                if g == 0:
                    rg, t = k // 4, k % 4
                    a = []
                    for rb in range(2):
                        r0 = pl.multiple_of(j * RC + rb * TQ + rg * 16, 16)
                        for ch in range(2):
                            a.append(c_s[pl.ds(r0, 16), (2 * t + ch) * L:(2 * t + ch + 1) * L].astype(F32))
                    a[0] = jnp.where(jnp.concatenate([never, never], axis=0),
                                     jnp.concatenate([piece, piece], axis=0), a[0])
                    us = [_to_u32(o) for o in _left(*a)]
                    d0 = pl.multiple_of(j * HQ + rg * 8, 8)
                    for n in range(7):
                        a_s[n, pl.ds(d0, 8), t * L:(t + 1) * L] = us[n]
                    link = _or_all([us[n] for n in (0, 1, 4, 5, 6)])
                c0 = j * mk + 2 * k
                w = [pltpu.bitcast(r[pl.ds(c0 + o, 2), g], U32) for o in (0, L) for r in (wk_r, wv_r)]
                w = [[x[0], x[1]] for x in w]
                w[0][0] = jnp.where(never, link, w[0][0])
                for par in range(2):
                    rows = [_right(*[_unpack(x[e], par) for x in w]) for e in range(2)]
                    for n in range(7):
                        b_s[n, 2 * g + par, pl.ds(j * (mk // 4) + k, 8, stride=pb), :] = _pack(
                            rows[0][n], rows[1][n])
            q_step(1, j, side)
            return 0
        jax.lax.fori_loop(0, NCH, q_hi, 0)

        for cp in misc:
            cp.wait()
        st = {}
        rid = jax.lax.broadcasted_iota(jnp.int32, (8, M), 0)

        def route():
            wr = jnp.broadcast_to(wr_s[...].reshape(1, M).astype(F32), (8, M))
            gw = jnp.broadcast_to(gw_s[...].reshape(1, M).astype(F32), (8, M))
            rg = jnp.dot(jnp.where(rid == 0, wr, gw).astype(BF16), xT_s[...], preferred_element_type=F32)
            g_s[0:1, :S] = jax.nn.sigmoid(rg[1:2])
            r = rg[0:1].astype(BF16).astype(F32)
            lane = jax.lax.broadcasted_iota(jnp.int32, (1, S), 1)
            m1 = jnp.max(r, axis=1, keepdims=True)
            i1 = jnp.min(jnp.where(r == m1, lane, S - 1), axis=1, keepdims=True)
            r2 = jnp.where(lane == i1, -jnp.inf, r)
            m2 = jnp.max(r2, axis=1, keepdims=True)
            i2 = jnp.min(jnp.where(jnp.logical_and(r2 == m2, lane != i1), lane, S - 1), axis=1, keepdims=True)
            st["idx"] = [i1[0, 0], i2[0, 0]]
            st["r"] = jax.nn.sigmoid(jnp.where(rid[:, :1] == 0, m1, m2))

        def gather():
            ln = jax.lax.broadcasted_iota(jnp.int32, (8, L), 1)
            xs = None
            for t, i in enumerate(st["idx"]):
                pick = jnp.where(jnp.logical_and(rid[:, :L] == t, ln == (i & (L - 1))), 1.0, 0.0)
                blk = xT_s[:, pl.ds(pl.multiple_of((i >> 7) << 7, L), L)]
                x = jax.lax.dot_general(pick.astype(BF16), blk, NT, preferred_element_type=F32)
                xs = x if xs is None else xs + x
            st["x"] = xs.astype(BF16)

        def hidden():
            gate = jnp.dot(st["x"], wg_s[...], preferred_element_type=F32)
            up = jnp.dot(st["x"], wu_s[...], preferred_element_type=F32)
            st["h"] = (jax.nn.silu(gate) * up).astype(BF16)

        def patch():
            y = jax.lax.dot_general(st["h"], wd_s[...], NT, preferred_element_type=F32) * st["r"]
            mp = -(-M // L) * L
            y = jnp.concatenate([y, jnp.zeros((8, mp - M), F32)], axis=1)
            yT = jnp.concatenate([y, jnp.zeros((L - 8, mp), F32)], axis=0).T
            ln = jax.lax.broadcasted_iota(jnp.int32, (M, L), 1)
            for t, i in enumerate(st["idx"]):
                c0 = pl.multiple_of((i >> 7) << 7, L)
                blk = xT_s[:, pl.ds(c0, L)].astype(F32)
                upd = jnp.where(ln == (i & (L - 1)), yT[:M, t:t + 1], 0.0)
                xT_s[:, pl.ds(c0, L)] = (blk + upd).astype(BF16)

        head_program("h0 G0 h1 G3 h2 G4 h3 G6 G1 G2 G5 w0", None, 0, None,
                     hooks=(route, gather, hidden, patch))

    def phase2(x7_s):
        wo_copy.wait()

        def head(h, _):
            head_program(LOOP_ORDER, h, h + 1, x7_s)
            return h
        last = jax.lax.fori_loop(0, H - 1, head, 0)
        head_program(LAST_ORDER, H - 1, last, x7_s)

        def out_step(j, _):
            c0 = pl.multiple_of(j * RC, RC)
            for t in range(RC // TQ):
                r0 = pl.multiple_of(j * (RC // 4) + t * 64, 64)
                m = {}
                for n in range(7):
                    left = jnp.concatenate([_as_bf16(wo7_s[n, h, :M // 4]) for h in range(H)], axis=1)
                    right = jnp.concatenate([_as_bf16(x7_s[n, h, pl.ds(r0, 64), :]) for h in range(H)], axis=1)
                    m[n] = jax.lax.dot_general(left, right, NT, preferred_element_type=F32)
                a = jnp.concatenate([jnp.concatenate([_c11(m), _c12(m)], axis=1),
                                     jnp.concatenate([_c21(m), _c22(m)], axis=1)], axis=0)
                gj = g_s[0:1, pl.ds(c0 + t * TQ, TQ)]
                b = xT_s[:, pl.ds(c0 + t * TQ, TQ)].astype(F32)
                o_s[:, pl.ds(c0 + t * TQ, TQ)] = (gj * a + (1.0 - gj) * b).astype(BF16)
                out_copy(j * (RC // TQ) + t).start()
            return 0
        jax.lax.fori_loop(0, S // RC, out_step, 0)
        for j in range(nq):
            out_copy(j).wait()

    pl.run_scoped(
        phase1,
        *[pltpu.VMEM(r.shape, r.dtype) for r in (c_hbm, wq_hbm, wk_hbm, wv_hbm, wg_hbm, wu_hbm, wd_hbm)],
        pltpu.VMEM((7, S // 4, mh), U32),
        pltpu.VMEM((7, -(-pq // 4) * 32, L), U32),
        pltpu.VMEM((7, -(-pq // 4) * 32, L), U32),
        pltpu.VMEM((M,), BF16),
        pltpu.VMEM((M,), BF16))
    pl.run_scoped(phase2, pltpu.VMEM((7, H, S // 4, L), U32))


def _tile_view(w):
    c, h, d = w.shape
    w = w.reshape(c, h // 8, 8, d // L, L).transpose(0, 1, 3, 2, 4)
    return w.reshape(c, h // 8, 8 * (d // L), L)


@jax.jit
def pallas_gated_mix__compressed_kv_cla__moe_arch_mod__prompt_kernel(
    A_x: jax.Array,
    A_c_kv: jax.Array,
    A_w_q: jax.Array,
    A_w_uk: jax.Array,
    A_w_uv: jax.Array,
    A_w_o: jax.Array,
    B_x: jax.Array,
    B_w_r: jax.Array,
    B_w_gate: jax.Array,
    B_w_up: jax.Array,
    B_w_down: jax.Array,
    gate_w: jax.Array,
):
    _, S, M = A_x.shape
    DC = A_c_kv.shape[2]
    H, D = A_w_q.shape[1], A_w_q.shape[2]
    args = (jnp.transpose(A_x[0]), A_c_kv[0], _tile_view(A_w_q).reshape(2, M // 2, 2, 16, L),
            _tile_view(A_w_uk), _tile_view(A_w_uv),
            jnp.transpose(A_w_o, (0, 2, 1)), B_w_r, gate_w, B_w_gate, B_w_up, jnp.transpose(B_w_down))

    def kern(*refs):
        _kernel(*refs, S=S, M=M, DC=DC, H=H, D=D)

    hbm = pl.BlockSpec(memory_space=pl.ANY)
    oT = pl.pallas_call(
        kern,
        out_shape=jax.ShapeDtypeStruct((M, S), A_x.dtype),
        in_specs=[hbm] * len(args),
        out_specs=hbm,
        scratch_shapes=[
            pltpu.VMEM((8, S + PAD_TILES * L), F32),
            pltpu.VMEM((M, S), BF16),
            pltpu.VMEM((H, M, D), BF16),
            pltpu.VMEM((7, S // 4, DC // 2), U32),
            pltpu.VMEM((7, 4, 8 * (DC // 4 + 1), L), U32),
            pltpu.VMEM((H, S // 2, D), U32),
            pltpu.VMEM((S // 2, D), U32),
            pltpu.VMEM((S // 2, D), U32),
            pltpu.VMEM((7, H, L, L), U32),
            pltpu.VMEM((M, S), BF16),
            pltpu.VMEM((5, S // 4 + PAD_V, L), U32),
            pltpu.SemaphoreType.DMA((N_SEM,)),
        ],
        compiler_params=pltpu.CompilerParams(vmem_limit_bytes=124 * 1024 * 1024),
    )(*args)
    return jnp.transpose(oT)[None]
```

```python
import math

import jax
import jax.numpy as jnp
import jax.experimental.pallas as pl
import jax.experimental.pallas.tpu as pltpu

F32 = jnp.float32
BF16 = jnp.bfloat16
U32 = jnp.uint32
NT = (((1,), (1,)), ((), ()))

L = 128
TQ = 256
HQ = TQ // 2
RC = 512
NCH = 4

PAD_TILES = 3
PAD_V = 16

S_X, S_Q0, S_Q1, S_K, S_V, S_C, S_MISC, S_OUT = 0, 4, 8, 12, 16, 20, 24, 30
N_SEM = 38

LOOP_ORDER = ("Q0 Q7 S0 G0 S7 V0 V7 Q6 G3 S6 V6 Q5 G4 S5 V5 Q4 G6 S4 V4 Q3 G1 S3 V3 Q2 G2 S2 V2 "
              "Q1 G5 S1 V1 w0")
LAST_ORDER = "Q7 Q6 q5 s7 V7 S6 Q4 V6 S5 r3 V5 S4 r2 V4 S3 r1 V3 S2 r0 V2 S1 S0 V1 V0"


def _to_u32(x_f32):
    return pltpu.bitcast(x_f32.astype(BF16), U32)


def _as_bf16(x_u32):
    return pltpu.bitcast(x_u32, BF16)


def _left(a11, a12, a21, a22):
    return (a11 + a22, a21 + a22, a11, a22, a11 + a12, a21 - a11, a12 - a22)


def _right(b11, b12, b21, b22):
    return (b11 + b22, b11, b12 - b22, b21 - b11, b22, b11 + b12, b21 + b22)


def _c11(m):
    return (m[0] + m[3]) + (m[6] - m[4])


def _c12(m):
    return m[2] + m[4]


def _c21(m):
    return m[1] + m[3]


def _c22(m):
    return (m[0] - m[1]) + (m[2] + m[5])


def _never(i):
    return jax.lax.broadcasted_iota(jnp.int32, (8, L), 0) < (i >> 10)


def _or_all(xs):
    out = xs[0]
    for x in xs[1:]:
        out = out | x
    return out


def _unpack(w, par):
    return pltpu.unpack_elementwise(w, index=par, packed_dtype=BF16, unpacked_dtype=F32)


def _pack(even, odd):
    return pltpu.bitcast(pltpu.pack_elementwise([even, odd], packed_dtype=BF16), U32)


def _head_weight(ref, h, nrows, pitch):
    sel = ((h >> 3) << 1) + (h & 1)
    r = (h >> 1) & 3
    return jnp.concatenate(
        [_as_bf16(ref[sel, pl.ds((dt * 4 + r) * pitch, nrows), :]) for dt in range(2)], axis=1)


def _kernel(xT_hbm, c_hbm, wq_hbm, wk_hbm, wv_hbm, wo_hbm, wr_hbm, gw_hbm, wg_hbm, wu_hbm, wd_hbm,
            o_hbm,
            g_s, xT_s, wo_s, a_s, b_s, q_s, k_s, v_s, wo7_s, o_s, v5_s, sem, *, S, M, DC, H, D):
    nq = S // TQ
    mh = M // 2
    pq = mh // 2 + 1
    pb = DC // 4 + 1
    mq = mh // NCH
    mk = DC // NCH
    qscale = (D ** -0.5) * math.log2(math.e)
    neg = -1e9 * math.log2(math.e)
    wo_copy = pltpu.make_async_copy(wo_hbm, wo_s, sem.at[S_MISC + 5])

    def out_copy(j):
        return pltpu.make_async_copy(o_s.at[:, pl.ds(j * TQ, TQ)], o_hbm.at[:, pl.ds(j * TQ, TQ)],
                                     sem.at[S_OUT + j])

    tri = (jax.lax.broadcasted_iota(jnp.int32, (L, L), 1) <= jax.lax.broadcasted_iota(jnp.int32, (L, L), 0))

    def head_program(order, h, hn, x7_s, span=0.9, hooks=None):
        never = _never(hn)
        prods, held, waiting = {}, {}, []

        def spots(v, cols, rows=(0, 64, 128, 192)):
            return [v[r:r + 8, n * L:(n + 1) * L] for n in cols for r in rows]

        def tie(lhs, links, every):
            rows = []
            for rg in range(lhs.shape[0] // 8):
                blk = lhs[rg * 8:(rg + 1) * 8]
                if links and rg % every == 0:
                    blk = jnp.concatenate([jnp.where(never, links.pop(0), blk[:, :L]), blk[:, L:]], axis=1)
                rows.append(blk)
            return jnp.concatenate(rows, axis=0)

        def proj(n):
            lhs = a_s[n]
            if waiting:
                lhs = tie(lhs, list(waiting), lhs.shape[0] // 8 // len(waiting))
                del waiting[:]
            prods[n] = jnp.dot(_as_bf16(lhs), _head_weight(b_s.at[n], hn, DC // 4, pb),
                               preferred_element_type=F32)
            for key, odd, comb, needs in (("k", 0, _c11, (0, 3, 4, 6)), ("k", 1, _c21, (1, 3)),
                                          ("v", 0, _c12, (2, 4)), ("v", 1, _c22, (0, 1, 2, 5))):
                if n in needs and all(x in prods for x in needs):
                    for k in range(nq // 2):
                        c = comb({x: prods[x][k * TQ:(k + 1) * TQ] for x in needs})
                        held[2 * k + odd, key] = _to_u32(c)
                        if key == "v" and 2 * k + odd < nq - 1:
                            ops = _right(c[:L, :L], c[:L, L:], c[L:, :L], c[L:, L:])
                            held[2 * k + odd, "r"] = [_to_u32(ops[x]) for x in (0, 2, 3, 5, 6)]
            return spots(prods[n], (0, 1), range(0, S // 2, 32))

        def write_kv():
            for ch in reversed(range(nq)):
                k_s[ch * HQ:(ch + 1) * HQ, :] = held[ch, "k"]
                v_s[ch * HQ:(ch + 1) * HQ, :] = held[ch, "v"]
                for n, o in enumerate(held.get((ch, "r"), ())):
                    v5_s[n, ch * 64:(ch + 1) * 64, :] = o

        def qk(i, tied):
            q = q_s[h, i * HQ:(i + 1) * HQ, :]
            if tied:
                n = len(waiting) - tied + 1
                q = tie(q, waiting[:n], 16 // n)
                del waiting[:n]
            q = _as_bf16(q)
            n0 = i * TQ
            n1 = n0 + L
            s1 = jax.lax.dot_general(q, _as_bf16(k_s[0:n1 // 2, :]), NT, preferred_element_type=F32)
            s2 = jax.lax.dot_general(q[L:], _as_bf16(k_s[n1 // 2:(n1 + L) // 2, :]), NT,
                                     preferred_element_type=F32)
            top = jnp.where(tri, s1[:L, n0:], neg)
            if n0:
                top = jnp.concatenate([s1[:L, :n0], top], axis=1)
            bot = jnp.concatenate([s1[L:], jnp.where(tri, s2, neg)], axis=1)
            return (top, bot), spots(s1, range(max(1, n0 // L)))

        def softmax(i, top, bot, pieces):
            p, sums, prev = ([], []), ([], []), None
            for k in range(TQ // 8):
                half = k % 2
                s = (top, bot)[half][(k // 2) * 8:(k // 2 + 1) * 8]
                link = pieces[int(span * k * 8 / TQ * len(pieces))]
                if prev is not None:
                    link = jnp.where(never, link, prev)
                m = jnp.broadcast_to(jnp.max(s, axis=1, keepdims=True), (8, L))
                m = jnp.where(never, link, m)
                e = [jnp.exp2(s[:, t:t + L] - m) for t in range(0, s.shape[1], L)]
                prev = e[0]
                for x in e[1:]:
                    prev = prev + x
                sums[half].append(prev)
                p[half].append(jnp.concatenate(e, axis=1))
            pt, pb_ = jnp.concatenate(p[0], axis=0), jnp.concatenate(p[1], axis=0)

            def tile(x, t):
                return x[:, t * L:(t + 1) * L]
            ops = [_left(tile(pt, 2 * c), tile(pt, 2 * c + 1), tile(pb_, 2 * c), tile(pb_, 2 * c + 1))
                   for c in range(i)]
            left = [jnp.concatenate([o[n] for o in ops], axis=1).astype(BF16) for n in range(7)] if i else None
            inv = []
            for x in sums:
                l = jnp.sum(jnp.concatenate(x, axis=0), axis=1, keepdims=True)
                r = pl.reciprocal(l, approx=True)
                inv.append(r * (2.0 - l * r))
            return (left, jnp.concatenate([tile(pt, 2 * i), tile(pb_, 2 * i)], axis=0).astype(BF16),
                    tile(pb_, 2 * i + 1).astype(BF16), inv)

        def pv(i, left, p1, p2, inv):
            r0 = i * HQ
            m, pieces = {}, []
            for n in (2, 3, 0, 4, 1, 5, 6) if i else ():
                if n == 1:
                    w = jnp.concatenate([_as_bf16(v_s[c * HQ:c * HQ + 64, :L]) for c in range(i)], axis=0)
                elif n == 4:
                    w = jnp.concatenate([_as_bf16(v_s[c * HQ + 64:(c + 1) * HQ, L:]) for c in range(i)], axis=0)
                else:
                    w = _as_bf16(v5_s[(0, 2, 3, 5, 6).index(n), 0:i * 64, :])
                m[n] = jnp.dot(left[n], w, preferred_element_type=F32)
                pieces += spots(m[n], (0,), (0, 32, 64, 96))
            c1 = jnp.dot(p1, _as_bf16(v_s[r0:r0 + 64, :]), preferred_element_type=F32)
            c2 = jnp.dot(p2, _as_bf16(v_s[r0 + 64:r0 + HQ, :]), preferred_element_type=F32)
            top, bot = c1[:L], c1[L:] + c2
            if i:
                top = top + jnp.concatenate([_c11(m), _c12(m)], axis=1)
                bot = bot + jnp.concatenate([_c21(m), _c22(m)], axis=1)
            else:
                pieces = spots(c1, (0, 1))
            top, bot = top * inv[0], bot * inv[1]
            us = [_to_u32(o) for o in _right(top[:, :L], bot[:, :L], top[:, L:], bot[:, L:])]
            for n in range(7):
                x7_s[n, h, i * 64:(i + 1) * 64, :] = us[n]
            waiting.extend(_or_all([us[n][g * 8:(g + 1) * 8] for n in (0, 2, 3, 5, 6)]) for g in range(8))
            return pieces

        def wo_operands():
            for rg in range(M // 32):
                a = [wo_s[h, hf * (M // 2) + rg * 16:hf * (M // 2) + (rg + 1) * 16, ch * L:(ch + 1) * L].astype(F32)
                     for hf in range(2) for ch in range(2)]
                us = [_to_u32(o) for o in _left(*a)]
                for n in range(7):
                    wo7_s[n, h, rg * 8:(rg + 1) * 8, :] = us[n]
                waiting.append(_or_all([us[n] for n in (0, 1, 4, 5, 6)]))

        if h is not None:
            wo_operands()
        scores, probs, pieces = {}, {}, []
        for op in order.split():
            i = int(op[1:])
            if op[0] == "G":
                pieces.append(proj(i))
            elif op[0] == "w":
                write_kv()
            elif op[0] in "Qqr":
                scores[i], new = qk(i, {"Q": 0, "q": 1, "r": 9}[op[0]])
                pieces.append(new)
            elif op[0] in "Ss":
                probs[i] = softmax(i, *scores.pop(i), pieces[-1] if op[0] == "S" else pieces[-2] + pieces[-1])
            elif op[0] == "V":
                pieces.append(pv(i, *probs.pop(i)))
            else:
                hooks[i]()

    def phase1(c_s, wq_r, wk_r, wv_r, wg_s, wu_s, wd_s, xa_s, wq0_s, wq1_s, wr_s, gw_s):
        def x_copy(j):
            return pltpu.make_async_copy(xT_hbm.at[:, pl.ds(j * RC, RC)], xT_s.at[:, pl.ds(j * RC, RC)],
                                         sem.at[S_X + j])

        def wq_copy(g, j):
            return pltpu.make_async_copy(wq_hbm.at[:, pl.ds(j * mq, mq), g], wq_r.at[:, pl.ds(j * mq, mq), g],
                                         sem.at[(S_Q1 if g else S_Q0) + j])

        def kv_copies(j):
            return [pltpu.make_async_copy(src.at[pl.ds(j * n, n)], dst.at[pl.ds(j * n, n)], sem.at[s0 + j])
                    for src, dst, s0, n in ((c_hbm, c_s, S_C, RC), (wk_hbm, wk_r, S_K, mk), (wv_hbm, wv_r, S_V, mk))]

        misc = [pltpu.make_async_copy(a, b, sem.at[S_MISC + i]) for i, (a, b) in enumerate(
            [(wr_hbm, wr_s), (gw_hbm, gw_s), (wg_hbm, wg_s), (wu_hbm, wu_s), (wd_hbm, wd_s)])]

        x_copy(0).start()
        for j in range(NCH):
            wq_copy(0, j).start()

        def start_rest():
            for j in range(NCH):
                if j + 1 < NCH:
                    x_copy(j + 1).start()
                wq_copy(1, j).start()
            misc[0].start()
            misc[1].start()
            for j in range(NCH):
                for cp in kv_copies(j):
                    cp.start()
            for cp in misc[2:]:
                cp.start()
            wo_copy.start()

        start_rest()

        def x_operands(j):
            c0 = j * RC if isinstance(j, int) else pl.multiple_of(j * RC, RC)
            r0 = j * HQ if isinstance(j, int) else pl.multiple_of(j * HQ, HQ)
            a = [xT_s[kh * mh:(kh + 1) * mh, pl.ds(c0 + rb * TQ, TQ)].astype(F32)
                 for rb in range(2) for kh in range(2)]
            for n, o in enumerate(_left(*a)):
                xa_s[n, pl.ds(r0, HQ), :] = pltpu.bitcast(o.astype(BF16).T, U32)

        def wq_operands(g, p, never=None, link=None):
            w = [pltpu.bitcast(wq_r[kh, pl.ds(2 * p, 2), g], U32) for kh in range(2)]
            w = [[x[0], x[1]] for x in w]
            if link is not None:
                w[0][0] = jnp.where(never, link, w[0][0])
            rows = [_right(*[_unpack(w[kh][e], par) for kh in range(2) for par in range(2)]) for e in range(2)]
            for n in range(7):
                (wq0_s, wq1_s)[g][n, pl.ds(p, 8, stride=pq), :] = _pack(rows[0][n], rows[1][n])

        x_copy(0).wait()
        x_operands(0)

        def first_half(j, _):
            wq_copy(0, j).wait()
            for k in range(mq // 2):
                wq_operands(0, j * (mq // 2) + k)
            return 0
        jax.lax.fori_loop(0, NCH, first_half, 0)

        def q_step(g, j, side):
            pieces = []
            for r in range(4):
                m = {}
                for n in (0, 3, 4, 6, 1, 2, 5):
                    w = jnp.concatenate([_as_bf16((wq0_s, wq1_s)[g][n, pl.ds((dt * 4 + r) * pq, mh // 2), :])
                                         for dt in range(2)], axis=1)
                    m[n] = jnp.dot(_as_bf16(xa_s[n, pl.ds(pl.multiple_of(j * HQ, HQ), HQ), :]), w,
                                   preferred_element_type=F32)
                    for k in range(5):
                        pieces.append(m[n][k * 48:k * 48 + 8, (k % 2) * L:(k % 2 + 1) * L])
                        side(len(pieces) - 1, pieces[-1])
                for par, rb, comb in ((0, 0, _c11), (0, 1, _c21), (1, 0, _c12), (1, 1, _c22)):
                    r0 = pl.multiple_of(j * TQ + rb * HQ, HQ)
                    q_s[8 * g + 2 * r + par, pl.ds(r0, HQ), :] = _to_u32(comb(m) * qscale)

        def q_lo(j, _):
            never = _never(j)

            def side(k, piece):
                if k == 35:
                    @pl.when(j + 1 < NCH)
                    def _():
                        x_copy(j + 1).wait()
                    wq_copy(1, j).wait()
                if k >= 42 and k % 3 == 0 and (k - 42) // 3 < mq // 2:
                    wq_operands(1, j * (mq // 2) + (k - 42) // 3, never, pltpu.bitcast(piece, U32))
            q_step(0, j, side)
            x_operands((j + 1) & (NCH - 1))
            return 0
        jax.lax.fori_loop(0, NCH, q_lo, 0)

        def q_hi(j, _):
            for cp in kv_copies(j):
                cp.wait()
            never = _never(j)

            def side(kk, piece):
                if kk >= 128:
                    return
                k, g = kk // 2, kk % 2
                link = pltpu.bitcast(piece, U32)
                if g == 0:
                    rg, t = k // 4, k % 4
                    a = []
                    for rb in range(2):
                        r0 = pl.multiple_of(j * RC + rb * TQ + rg * 16, 16)
                        for ch in range(2):
                            a.append(c_s[pl.ds(r0, 16), (2 * t + ch) * L:(2 * t + ch + 1) * L].astype(F32))
                    a[0] = jnp.where(jnp.concatenate([never, never], axis=0),
                                     jnp.concatenate([piece, piece], axis=0), a[0])
                    us = [_to_u32(o) for o in _left(*a)]
                    d0 = pl.multiple_of(j * HQ + rg * 8, 8)
                    for n in range(7):
                        a_s[n, pl.ds(d0, 8), t * L:(t + 1) * L] = us[n]
                    link = _or_all([us[n] for n in (0, 1, 4, 5, 6)])
                c0 = j * mk + 2 * k
                w = [pltpu.bitcast(r[pl.ds(c0 + o, 2), g], U32) for o in (0, L) for r in (wk_r, wv_r)]
                w = [[x[0], x[1]] for x in w]
                w[0][0] = jnp.where(never, link, w[0][0])
                for par in range(2):
                    rows = [_right(*[_unpack(x[e], par) for x in w]) for e in range(2)]
                    for n in range(7):
                        b_s[n, 2 * g + par, pl.ds(j * (mk // 4) + k, 8, stride=pb), :] = _pack(
                            rows[0][n], rows[1][n])
            q_step(1, j, side)
            return 0
        jax.lax.fori_loop(0, NCH, q_hi, 0)

        for cp in misc:
            cp.wait()
        st = {}
        rid = jax.lax.broadcasted_iota(jnp.int32, (8, M), 0)

        def route():
            wr = jnp.broadcast_to(wr_s[...].reshape(1, M).astype(F32), (8, M))
            gw = jnp.broadcast_to(gw_s[...].reshape(1, M).astype(F32), (8, M))
            rg = jnp.dot(jnp.where(rid == 0, wr, gw).astype(BF16), xT_s[...], preferred_element_type=F32)
            g_s[0:1, :S] = jax.nn.sigmoid(rg[1:2])
            r = rg[0:1].astype(BF16).astype(F32)
            lane = jax.lax.broadcasted_iota(jnp.int32, (1, S), 1)
            m1 = jnp.max(r, axis=1, keepdims=True)
            i1 = jnp.min(jnp.where(r == m1, lane, S - 1), axis=1, keepdims=True)
            r2 = jnp.where(lane == i1, -jnp.inf, r)
            m2 = jnp.max(r2, axis=1, keepdims=True)
            i2 = jnp.min(jnp.where(jnp.logical_and(r2 == m2, lane != i1), lane, S - 1), axis=1, keepdims=True)
            st["idx"] = [i1[0, 0], i2[0, 0]]
            st["r"] = jax.nn.sigmoid(jnp.where(rid[:, :1] == 0, m1, m2))

        def gather():
            ln = jax.lax.broadcasted_iota(jnp.int32, (8, L), 1)
            xs = None
            for t, i in enumerate(st["idx"]):
                pick = jnp.where(jnp.logical_and(rid[:, :L] == t, ln == (i & (L - 1))), 1.0, 0.0)
                blk = xT_s[:, pl.ds(pl.multiple_of((i >> 7) << 7, L), L)]
                x = jax.lax.dot_general(pick.astype(BF16), blk, NT, preferred_element_type=F32)
                xs = x if xs is None else xs + x
            st["x"] = xs.astype(BF16)

        def hidden():
            gate = jnp.dot(st["x"], wg_s[...], preferred_element_type=F32)
            up = jnp.dot(st["x"], wu_s[...], preferred_element_type=F32)
            st["h"] = (jax.nn.silu(gate) * up).astype(BF16)

        def patch():
            y = jax.lax.dot_general(st["h"], wd_s[...], NT, preferred_element_type=F32) * st["r"]
            mp = -(-M // L) * L
            y = jnp.concatenate([y, jnp.zeros((8, mp - M), F32)], axis=1)
            yT = jnp.concatenate([y, jnp.zeros((L - 8, mp), F32)], axis=0).T
            ln = jax.lax.broadcasted_iota(jnp.int32, (M, L), 1)
            for t, i in enumerate(st["idx"]):
                c0 = pl.multiple_of((i >> 7) << 7, L)
                blk = xT_s[:, pl.ds(c0, L)].astype(F32)
                upd = jnp.where(ln == (i & (L - 1)), yT[:M, t:t + 1], 0.0)
                xT_s[:, pl.ds(c0, L)] = (blk + upd).astype(BF16)

        head_program("h0 G0 h1 G3 h2 G4 h3 G6 G1 G2 G5 w0", None, 0, None,
                     hooks=(route, gather, hidden, patch))

    def phase2(x7_s):
        wo_copy.wait()

        def head(h, _):
            head_program(LOOP_ORDER, h, h + 1, x7_s, span=0.96)
            return h
        last = jax.lax.fori_loop(0, H - 1, head, 0)
        head_program(LAST_ORDER, H - 1, last, x7_s)

        def out_step(j, _):
            c0 = pl.multiple_of(j * RC, RC)
            for t in range(RC // TQ):
                r0 = pl.multiple_of(j * (RC // 4) + t * 64, 64)
                m = {}
                for n in range(7):
                    left = jnp.concatenate([_as_bf16(wo7_s[n, h, :M // 4]) for h in range(H)], axis=1)
                    right = jnp.concatenate([_as_bf16(x7_s[n, h, pl.ds(r0, 64), :]) for h in range(H)], axis=1)
                    m[n] = jax.lax.dot_general(left, right, NT, preferred_element_type=F32)
                a = jnp.concatenate([jnp.concatenate([_c11(m), _c12(m)], axis=1),
                                     jnp.concatenate([_c21(m), _c22(m)], axis=1)], axis=0)
                gj = g_s[0:1, pl.ds(c0 + t * TQ, TQ)]
                b = xT_s[:, pl.ds(c0 + t * TQ, TQ)].astype(F32)
                o_s[:, pl.ds(c0 + t * TQ, TQ)] = (gj * a + (1.0 - gj) * b).astype(BF16)
                out_copy(j * (RC // TQ) + t).start()
            return 0
        jax.lax.fori_loop(0, S // RC, out_step, 0)
        for j in range(nq):
            out_copy(j).wait()

    pl.run_scoped(
        phase1,
        *[pltpu.VMEM(r.shape, r.dtype) for r in (c_hbm, wq_hbm, wk_hbm, wv_hbm, wg_hbm, wu_hbm, wd_hbm)],
        pltpu.VMEM((7, S // 4, mh), U32),
        pltpu.VMEM((7, -(-pq // 4) * 32, L), U32),
        pltpu.VMEM((7, -(-pq // 4) * 32, L), U32),
        pltpu.VMEM((M,), BF16),
        pltpu.VMEM((M,), BF16))
    pl.run_scoped(phase2, pltpu.VMEM((7, H, S // 4, L), U32))


def _tile_view(w):
    c, h, d = w.shape
    w = w.reshape(c, h // 8, 8, d // L, L).transpose(0, 1, 3, 2, 4)
    return w.reshape(c, h // 8, 8 * (d // L), L)


@jax.jit
def pallas_gated_mix__compressed_kv_cla__moe_arch_mod__prompt_kernel(
    A_x: jax.Array,
    A_c_kv: jax.Array,
    A_w_q: jax.Array,
    A_w_uk: jax.Array,
    A_w_uv: jax.Array,
    A_w_o: jax.Array,
    B_x: jax.Array,
    B_w_r: jax.Array,
    B_w_gate: jax.Array,
    B_w_up: jax.Array,
    B_w_down: jax.Array,
    gate_w: jax.Array,
):
    _, S, M = A_x.shape
    DC = A_c_kv.shape[2]
    H, D = A_w_q.shape[1], A_w_q.shape[2]
    args = (jnp.transpose(A_x[0]), A_c_kv[0], _tile_view(A_w_q).reshape(2, M // 2, 2, 16, L),
            _tile_view(A_w_uk), _tile_view(A_w_uv),
            jnp.transpose(A_w_o, (0, 2, 1)), B_w_r, gate_w, B_w_gate, B_w_up, jnp.transpose(B_w_down))

    def kern(*refs):
        _kernel(*refs, S=S, M=M, DC=DC, H=H, D=D)

    hbm = pl.BlockSpec(memory_space=pl.ANY)
    oT = pl.pallas_call(
        kern,
        out_shape=jax.ShapeDtypeStruct((M, S), A_x.dtype),
        in_specs=[hbm] * len(args),
        out_specs=hbm,
        scratch_shapes=[
            pltpu.VMEM((8, S + PAD_TILES * L), F32),
            pltpu.VMEM((M, S), BF16),
            pltpu.VMEM((H, M, D), BF16),
            pltpu.VMEM((7, S // 4, DC // 2), U32),
            pltpu.VMEM((7, 4, 8 * (DC // 4 + 1), L), U32),
            pltpu.VMEM((H, S // 2, D), U32),
            pltpu.VMEM((S // 2, D), U32),
            pltpu.VMEM((S // 2, D), U32),
            pltpu.VMEM((7, H, L, L), U32),
            pltpu.VMEM((M, S), BF16),
            pltpu.VMEM((5, S // 4 + PAD_V, L), U32),
            pltpu.SemaphoreType.DMA((N_SEM,)),
        ],
        compiler_params=pltpu.CompilerParams(vmem_limit_bytes=124 * 1024 * 1024),
    )(*args)
    return jnp.transpose(oT)[None]
```

```python
import math

import jax
import jax.numpy as jnp
import jax.experimental.pallas as pl
import jax.experimental.pallas.tpu as pltpu

F32 = jnp.float32
BF16 = jnp.bfloat16
U32 = jnp.uint32
NT = (((1,), (1,)), ((), ()))

L = 128
TQ = 256
HQ = TQ // 2
RC = 512
NCH = 4

PAD_TILES = 3
PAD_V = 16

S_X, S_Q0, S_Q1, S_K, S_V, S_C, S_MISC, S_OUT = 0, 4, 8, 12, 16, 20, 24, 30
N_SEM = 38

LOOP_ORDER = ("Q0 Q7 S0 G0 S7 V0 V7 Q6 G3 S6 V6 Q5 G4 S5 V5 Q4 G6 S4 V4 Q3 G1 S3 V3 Q2 G2 S2 V2 "
              "Q1 G5 S1 V1 w0")
FIRST_ORDER = "h0 G0 G3 G4 G6 h1 G1 G2 h2 G5 w0"
LAST_ORDER = "Q7 Q6 q5 s7 V7 S6 Q4 V6 S5 r3 V5 S4 r2 V4 S3 r1 V3 S2 r0 V2 S1 S0 V1 V0"


def _to_u32(x_f32):
    return pltpu.bitcast(x_f32.astype(BF16), U32)


def _as_bf16(x_u32):
    return pltpu.bitcast(x_u32, BF16)


def _left(a11, a12, a21, a22):
    return (a11 + a22, a21 + a22, a11, a22, a11 + a12, a21 - a11, a12 - a22)


def _right(b11, b12, b21, b22):
    return (b11 + b22, b11, b12 - b22, b21 - b11, b22, b11 + b12, b21 + b22)


def _c11(m):
    return (m[0] + m[3]) + (m[6] - m[4])


def _c12(m):
    return m[2] + m[4]


def _c21(m):
    return m[1] + m[3]


def _c22(m):
    return (m[0] - m[1]) + (m[2] + m[5])


def _never(i):
    return jax.lax.broadcasted_iota(jnp.int32, (8, L), 0) < (i >> 10)


def _or_all(xs):
    out = xs[0]
    for x in xs[1:]:
        out = out | x
    return out


def _unpack(w, par):
    return pltpu.unpack_elementwise(w, index=par, packed_dtype=BF16, unpacked_dtype=F32)


def _pack(even, odd):
    return pltpu.bitcast(pltpu.pack_elementwise([even, odd], packed_dtype=BF16), U32)


def _head_weight(ref, h, nrows, pitch):
    sel = ((h >> 3) << 1) + (h & 1)
    r = (h >> 1) & 3
    return jnp.concatenate(
        [_as_bf16(ref[sel, pl.ds((dt * 4 + r) * pitch, nrows), :]) for dt in range(2)], axis=1)


def _kernel(xT_hbm, c_hbm, wq_hbm, wk_hbm, wv_hbm, wo_hbm, wr_hbm, gw_hbm, wg_hbm, wu_hbm, wd_hbm,
            o_hbm,
            g_s, xT_s, wo_s, a_s, b_s, q_s, k_s, v_s, wo7_s, o_s, v5_s, sem, *, S, M, DC, H, D):
    nq = S // TQ
    mh = M // 2
    pq = mh // 2 + 1
    pb = DC // 4 + 1
    mq = mh // NCH
    mk = DC // NCH
    qscale = (D ** -0.5) * math.log2(math.e)
    neg = -1e9 * math.log2(math.e)
    wo_copy = pltpu.make_async_copy(wo_hbm, wo_s, sem.at[S_MISC + 5])

    def out_copy(j):
        return pltpu.make_async_copy(o_s.at[:, pl.ds(j * TQ, TQ)], o_hbm.at[:, pl.ds(j * TQ, TQ)],
                                     sem.at[S_OUT + j])

    tri = (jax.lax.broadcasted_iota(jnp.int32, (L, L), 1) <= jax.lax.broadcasted_iota(jnp.int32, (L, L), 0))

    def head_program(order, h, hn, never, x7_s, span=0.9, hooks=None):
        prods, held, waiting = {}, {}, []

        def spots(v, cols, rows=(0, 64, 128, 192)):
            return [v[r:r + 8, n * L:(n + 1) * L] for n in cols for r in rows]

        def tie(lhs, links, every):
            rows = []
            for rg in range(lhs.shape[0] // 8):
                blk = lhs[rg * 8:(rg + 1) * 8]
                if links and rg % every == 0:
                    blk = jnp.concatenate([jnp.where(never, links.pop(0), blk[:, :L]), blk[:, L:]], axis=1)
                rows.append(blk)
            return jnp.concatenate(rows, axis=0)

        def proj(n):
            lhs = a_s[n]
            if waiting:
                lhs = tie(lhs, list(waiting), lhs.shape[0] // 8 // len(waiting))
                del waiting[:]
            prods[n] = jnp.dot(_as_bf16(lhs), _head_weight(b_s.at[n], hn, DC // 4, pb),
                               preferred_element_type=F32)
            for key, odd, comb, needs in (("k", 0, _c11, (0, 3, 4, 6)), ("k", 1, _c21, (1, 3)),
                                          ("v", 0, _c12, (2, 4)), ("v", 1, _c22, (0, 1, 2, 5))):
                if n in needs and all(x in prods for x in needs):
                    for k in range(nq // 2):
                        c = comb({x: prods[x][k * TQ:(k + 1) * TQ] for x in needs})
                        held[2 * k + odd, key] = _to_u32(c)
                        if key == "v" and 2 * k + odd < nq - 1:
                            ops = _right(c[:L, :L], c[:L, L:], c[L:, :L], c[L:, L:])
                            held[2 * k + odd, "r"] = [_to_u32(ops[x]) for x in (0, 2, 3, 5, 6)]
            return spots(prods[n], (0, 1), range(0, S // 2, 32))

        def write_kv():
            for ch in reversed(range(nq)):
                k_s[ch * HQ:(ch + 1) * HQ, :] = held[ch, "k"]
                v_s[ch * HQ:(ch + 1) * HQ, :] = held[ch, "v"]
                for n, o in enumerate(held.get((ch, "r"), ())):
                    v5_s[n, ch * 64:(ch + 1) * 64, :] = o

        def qk(i, tied):
            q = q_s[h, i * HQ:(i + 1) * HQ, :]
            if tied:
                n = len(waiting) - tied + 1
                q = tie(q, waiting[:n], 16 // n)
                del waiting[:n]
            q = _as_bf16(q)
            n0 = i * TQ
            n1 = n0 + L
            s1 = jax.lax.dot_general(q, _as_bf16(k_s[0:n1 // 2, :]), NT, preferred_element_type=F32)
            s2 = jax.lax.dot_general(q[L:], _as_bf16(k_s[n1 // 2:(n1 + L) // 2, :]), NT,
                                     preferred_element_type=F32)
            top = jnp.where(tri, s1[:L, n0:], neg)
            if n0:
                top = jnp.concatenate([s1[:L, :n0], top], axis=1)
            bot = jnp.concatenate([s1[L:], jnp.where(tri, s2, neg)], axis=1)
            return (top, bot), spots(s1, range(max(1, n0 // L)))

        def softmax(i, top, bot, pieces):
            p, sums, prev = ([], []), ([], []), None
            for k in range(TQ // 8):
                half = k % 2
                s = (top, bot)[half][(k // 2) * 8:(k // 2 + 1) * 8]
                link = pieces[int(span * k * 8 / TQ * len(pieces))]
                if prev is not None:
                    link = jnp.where(never, link, prev)
                m = jnp.broadcast_to(jnp.max(s, axis=1, keepdims=True), (8, L))
                m = jnp.where(never, link, m)
                e = [jnp.exp2(s[:, t:t + L] - m) for t in range(0, s.shape[1], L)]
                prev = e[0]
                for x in e[1:]:
                    prev = prev + x
                sums[half].append(prev)
                p[half].append(jnp.concatenate(e, axis=1))
            pt, pb_ = jnp.concatenate(p[0], axis=0), jnp.concatenate(p[1], axis=0)

            def tile(x, t):
                return x[:, t * L:(t + 1) * L]
            ops = [_left(tile(pt, 2 * c), tile(pt, 2 * c + 1), tile(pb_, 2 * c), tile(pb_, 2 * c + 1))
                   for c in range(i)]
            left = [jnp.concatenate([o[n] for o in ops], axis=1).astype(BF16) for n in range(7)] if i else None
            inv = []
            for x in sums:
                l = jnp.sum(jnp.concatenate(x, axis=0), axis=1, keepdims=True)
                r = pl.reciprocal(l, approx=True)
                inv.append(r * (2.0 - l * r))
            return (left, jnp.concatenate([tile(pt, 2 * i), tile(pb_, 2 * i)], axis=0).astype(BF16),
                    tile(pb_, 2 * i + 1).astype(BF16), inv)

        def pv(i, left, p1, p2, inv):
            r0 = i * HQ
            m, pieces = {}, []
            for n in (2, 3, 0, 4, 1, 5, 6) if i else ():
                if n == 1:
                    w = jnp.concatenate([_as_bf16(v_s[c * HQ:c * HQ + 64, :L]) for c in range(i)], axis=0)
                elif n == 4:
                    w = jnp.concatenate([_as_bf16(v_s[c * HQ + 64:(c + 1) * HQ, L:]) for c in range(i)], axis=0)
                else:
                    w = _as_bf16(v5_s[(0, 2, 3, 5, 6).index(n), 0:i * 64, :])
                m[n] = jnp.dot(left[n], w, preferred_element_type=F32)
                pieces += spots(m[n], (0,), (0, 32, 64, 96))
            c1 = jnp.dot(p1, _as_bf16(v_s[r0:r0 + 64, :]), preferred_element_type=F32)
            c2 = jnp.dot(p2, _as_bf16(v_s[r0 + 64:r0 + HQ, :]), preferred_element_type=F32)
            top, bot = c1[:L], c1[L:] + c2
            if i:
                top = top + jnp.concatenate([_c11(m), _c12(m)], axis=1)
                bot = bot + jnp.concatenate([_c21(m), _c22(m)], axis=1)
            else:
                pieces = spots(c1, (0, 1))
            top, bot = top * inv[0], bot * inv[1]
            us = [_to_u32(o) for o in _right(top[:, :L], bot[:, :L], top[:, L:], bot[:, L:])]
            for n in range(7):
                x7_s[n, h, i * 64:(i + 1) * 64, :] = us[n]
            waiting.extend(_or_all([us[n][g * 8:(g + 1) * 8] for n in (0, 2, 3, 5, 6)]) for g in range(8))
            return pieces

        def wo_operands():
            for rg in range(M // 32):
                a = [wo_s[h, hf * (M // 2) + rg * 16:hf * (M // 2) + (rg + 1) * 16, ch * L:(ch + 1) * L].astype(F32)
                     for hf in range(2) for ch in range(2)]
                us = [_to_u32(o) for o in _left(*a)]
                for n in range(7):
                    wo7_s[n, h, rg * 8:(rg + 1) * 8, :] = us[n]
                waiting.append(_or_all([us[n] for n in (0, 1, 4, 5, 6)]))

        if h is not None:
            wo_operands()
        scores, probs, pieces = {}, {}, []
        for op in order.split():
            i = int(op[1:])
            if op[0] == "G":
                pieces.append(proj(i))
            elif op[0] == "w":
                write_kv()
            elif op[0] in "Qqr":
                scores[i], new = qk(i, {"Q": 0, "q": 1, "r": 9}[op[0]])
                pieces.append(new)
            elif op[0] in "Ss":
                probs[i] = softmax(i, *scores.pop(i), pieces[-1] if op[0] == "S" else pieces[-2] + pieces[-1])
            elif op[0] == "V":
                pieces.append(pv(i, *probs.pop(i)))
            else:
                hooks[i](pieces)

    def phase1(c_s, wq_r, wk_r, wv_r, wg_s, wu_s, wd_s, xa_s, wq0_s, wq1_s, wr_s, gw_s):
        def x_copy(j):
            return pltpu.make_async_copy(xT_hbm.at[:, pl.ds(j * RC, RC)], xT_s.at[:, pl.ds(j * RC, RC)],
                                         sem.at[S_X + j])

        def wq_copy(g, j):
            return pltpu.make_async_copy(wq_hbm.at[:, pl.ds(j * mq, mq), g], wq_r.at[:, pl.ds(j * mq, mq), g],
                                         sem.at[(S_Q1 if g else S_Q0) + j])

        def kv_copies(j):
            return [pltpu.make_async_copy(src.at[pl.ds(j * n, n)], dst.at[pl.ds(j * n, n)], sem.at[s0 + j])
                    for src, dst, s0, n in ((c_hbm, c_s, S_C, RC), (wk_hbm, wk_r, S_K, mk), (wv_hbm, wv_r, S_V, mk))]

        misc = [pltpu.make_async_copy(a, b, sem.at[S_MISC + i]) for i, (a, b) in enumerate(
            [(wr_hbm, wr_s), (gw_hbm, gw_s), (wg_hbm, wg_s), (wu_hbm, wu_s), (wd_hbm, wd_s)])]

        x_copy(0).start()
        for j in range(NCH):
            wq_copy(0, j).start()

        def start_rest():
            for j in range(NCH):
                if j + 1 < NCH:
                    x_copy(j + 1).start()
                wq_copy(1, j).start()
            misc[0].start()
            misc[1].start()
            for j in range(NCH):
                for cp in kv_copies(j):
                    cp.start()
            for cp in misc[2:]:
                cp.start()
            wo_copy.start()

        start_rest()

        def x_operands(j):
            c0 = j * RC if isinstance(j, int) else pl.multiple_of(j * RC, RC)
            r0 = j * HQ if isinstance(j, int) else pl.multiple_of(j * HQ, HQ)
            a = [xT_s[kh * mh:(kh + 1) * mh, pl.ds(c0 + rb * TQ, TQ)].astype(F32)
                 for rb in range(2) for kh in range(2)]
            for n, o in enumerate(_left(*a)):
                xa_s[n, pl.ds(r0, HQ), :] = pltpu.bitcast(o.astype(BF16).T, U32)

        def wq_operands(g, p, never=None, link=None):
            w = [pltpu.bitcast(wq_r[kh, pl.ds(2 * p, 2), g], U32) for kh in range(2)]
            w = [[x[0], x[1]] for x in w]
            if link is not None:
                w[0][0] = jnp.where(never, link, w[0][0])
            rows = [_right(*[_unpack(w[kh][e], par) for kh in range(2) for par in range(2)]) for e in range(2)]
            for n in range(7):
                (wq0_s, wq1_s)[g][n, pl.ds(p, 8, stride=pq), :] = _pack(rows[0][n], rows[1][n])

        x_copy(0).wait()
        x_operands(0)

        def first_half(j, _):
            wq_copy(0, j).wait()
            for k in range(mq // 2):
                wq_operands(0, j * (mq // 2) + k)
            return 0
        jax.lax.fori_loop(0, NCH, first_half, 0)

        def q_step(g, j, side):
            pieces = []
            for r in range(4):
                m = {}
                for n in (0, 3, 4, 6, 1, 2, 5):
                    w = jnp.concatenate([_as_bf16((wq0_s, wq1_s)[g][n, pl.ds((dt * 4 + r) * pq, mh // 2), :])
                                         for dt in range(2)], axis=1)
                    m[n] = jnp.dot(_as_bf16(xa_s[n, pl.ds(pl.multiple_of(j * HQ, HQ), HQ), :]), w,
                                   preferred_element_type=F32)
                    for k in range(5):
                        pieces.append(m[n][k * 48:k * 48 + 8, (k % 2) * L:(k % 2 + 1) * L])
                        side(len(pieces) - 1, pieces[-1])
                for par, rb, comb in ((0, 0, _c11), (0, 1, _c21), (1, 0, _c12), (1, 1, _c22)):
                    r0 = pl.multiple_of(j * TQ + rb * HQ, HQ)
                    q_s[8 * g + 2 * r + par, pl.ds(r0, HQ), :] = _to_u32(comb(m) * qscale)

        def q_lo(j, _):
            never = _never(j)

            def side(k, piece):
                if k == 35:
                    @pl.when(j + 1 < NCH)
                    def _():
                        x_copy(j + 1).wait()
                    wq_copy(1, j).wait()
                if k >= 42 and k % 3 == 0 and (k - 42) // 3 < mq // 2:
                    wq_operands(1, j * (mq // 2) + (k - 42) // 3, never, pltpu.bitcast(piece, U32))
            q_step(0, j, side)
            x_operands((j + 1) & (NCH - 1))
            return 0
        jax.lax.fori_loop(0, NCH, q_lo, 0)

        def q_hi(j, _):
            for cp in kv_copies(j):
                cp.wait()
            never = _never(j)

            def side(kk, piece):
                if kk >= 128:
                    return
                k, g = kk // 2, kk % 2
                link = pltpu.bitcast(piece, U32)
                if g == 0:
                    rg, t = k // 4, k % 4
                    a = []
                    for rb in range(2):
                        r0 = pl.multiple_of(j * RC + rb * TQ + rg * 16, 16)
                        for ch in range(2):
                            a.append(c_s[pl.ds(r0, 16), (2 * t + ch) * L:(2 * t + ch + 1) * L].astype(F32))
                    a[0] = jnp.where(jnp.concatenate([never, never], axis=0),
                                     jnp.concatenate([piece, piece], axis=0), a[0])
                    us = [_to_u32(o) for o in _left(*a)]
                    d0 = pl.multiple_of(j * HQ + rg * 8, 8)
                    for n in range(7):
                        a_s[n, pl.ds(d0, 8), t * L:(t + 1) * L] = us[n]
                    link = _or_all([us[n] for n in (0, 1, 4, 5, 6)])
                c0 = j * mk + 2 * k
                w = [pltpu.bitcast(r[pl.ds(c0 + o, 2), g], U32) for o in (0, L) for r in (wk_r, wv_r)]
                w = [[x[0], x[1]] for x in w]
                w[0][0] = jnp.where(never, link, w[0][0])
                for par in range(2):
                    rows = [_right(*[_unpack(x[e], par) for x in w]) for e in range(2)]
                    for n in range(7):
                        b_s[n, 2 * g + par, pl.ds(j * (mk // 4) + k, 8, stride=pb), :] = _pack(
                            rows[0][n], rows[1][n])
            q_step(1, j, side)
            return j
        never = _never(jax.lax.fori_loop(0, NCH, q_hi, 0))

        for cp in misc:
            cp.wait()
        st = {}
        rid = jax.lax.broadcasted_iota(jnp.int32, (8, M), 0)

        F = wg_s.shape[1]

        def route(_):
            wr = jnp.broadcast_to(wr_s[...].reshape(1, M).astype(F32), (8, M))
            gw = jnp.broadcast_to(gw_s[...].reshape(1, M).astype(F32), (8, M))
            rg = jnp.dot(jnp.where(rid == 0, wr, gw).astype(BF16), xT_s[...], preferred_element_type=F32)
            g_s[0:1, :S] = jax.nn.sigmoid(rg[1:2])
            r = rg[0:1].astype(BF16).astype(F32)
            lane = jax.lax.broadcasted_iota(jnp.int32, (1, S), 1)
            m1 = jnp.max(r, axis=1, keepdims=True)
            i1 = jnp.min(jnp.where(r == m1, lane, S - 1), axis=1, keepdims=True)
            r2 = jnp.where(lane == i1, -jnp.inf, r)
            m2 = jnp.max(r2, axis=1, keepdims=True)
            i2 = jnp.min(jnp.where(jnp.logical_and(r2 == m2, lane != i1), lane, S - 1), axis=1, keepdims=True)
            ln = jax.lax.broadcasted_iota(jnp.int32, (M, L), 1)
            st["c0"] = [pl.multiple_of((i[0, 0] >> 7) << 7, L) for i in (i1, i2)]
            st["hit"] = [ln == (i & (L - 1)) for i in (i1, i2)]
            st["r"] = [jax.nn.sigmoid(m1), jax.nn.sigmoid(m2)]
            st["x"] = [jnp.broadcast_to(jnp.sum(jnp.where(hit, xT_s[:, pl.ds(c0, L)].astype(F32), 0.0),
                                                axis=1, keepdims=True), (M, L))
                       for c0, hit in zip(st["c0"], st["hit"])]

        def fold(v, axis_len):
            parts = [v[k * 8:(k + 1) * 8] if axis_len == 0 else v[:, k * L:(k + 1) * L]
                     for k in range(v.shape[axis_len] // (8, L)[axis_len])]
            while len(parts) > 1:
                parts = [parts[k] + parts[k + 1] if k + 1 < len(parts) else parts[k]
                         for k in range(0, len(parts), 2)]
            return parts[0]

        def linked(w, link):
            w = pltpu.bitcast(w, U32)
            reps = (w.shape[0] // 8, w.shape[1] // L)
            w = jnp.where(jnp.tile(never, reps), jnp.tile(pltpu.bitcast(link, U32), reps), w)
            return _as_bf16(w).astype(F32)

        def hidden(pieces):
            pieces = pieces[-3] + pieces[-2] + pieces[-1]
            nr, rows = 4, M // 4
            total = 2 * (F // L) * nr
            out, k, prev = [], 0, None
            for w_s in (wg_s, wu_s):
                cols = ([], [])
                for ct in range(F // L):
                    acc = [None, None]
                    for q in range(nr):
                        link = pieces[int(0.9 * k / total * len(pieces))]
                        if prev is not None:
                            link = jnp.where(never, link, prev)
                        k += 1
                        w = linked(w_s[q * rows:(q + 1) * rows, ct * L:(ct + 1) * L], link)
                        for t in range(2):
                            part = fold(w * st["x"][t][q * rows:(q + 1) * rows], 0)
                            acc[t] = part if acc[t] is None else acc[t] + part
                        prev = acc[0] + acc[1]
                    for t in range(2):
                        cols[t].append(jnp.sum(acc[t], axis=0, keepdims=True))
                out.append([jnp.concatenate(c, axis=1) for c in cols])
            st["h"] = [(jax.nn.silu(out[0][t]) * out[1][t]).astype(BF16).astype(F32) for t in range(2)]

        def patch(pieces):
            pieces = pieces[-2] + pieces[-1]
            half = F // 2
            ys, k, prev = ([], []), 0, None
            for rg in range(M // 16):
                acc = [None, None]
                for hf in range(2):
                    link = pieces[int((0.1 + 0.8 * k / (M // 8)) * len(pieces))]
                    if prev is not None:
                        link = jnp.where(never, link, prev)
                    k += 1
                    w = linked(wd_s[rg * 16:(rg + 1) * 16, hf * half:(hf + 1) * half], link)
                    for t in range(2):
                        part = fold(w * st["h"][t][:, hf * half:(hf + 1) * half], 1)
                        acc[t] = part if acc[t] is None else acc[t] + part
                    prev = fold(acc[0] + acc[1], 0)
                for t in range(2):
                    ys[t].append(jnp.sum(acc[t], axis=1, keepdims=True))
            for t in range(2):
                y = jnp.concatenate(ys[t], axis=0) * st["r"][t]
                blk = xT_s[:, pl.ds(st["c0"][t], L)].astype(F32)
                xT_s[:, pl.ds(st["c0"][t], L)] = (blk + jnp.where(st["hit"][t], y, 0.0)).astype(BF16)

        head_program(FIRST_ORDER, None, 0, never, None, hooks=(route, hidden, patch))

    def phase2(x7_s):
        wo_copy.wait()

        def head(h, _):
            head_program(LOOP_ORDER, h, h + 1, _never(h), x7_s, span=0.96)
            return h
        last = jax.lax.fori_loop(0, H - 1, head, 0)
        head_program(LAST_ORDER, H - 1, None, _never(last), x7_s)

        def out_step(j, _):
            c0 = pl.multiple_of(j * RC, RC)
            for t in range(RC // TQ):
                r0 = pl.multiple_of(j * (RC // 4) + t * 64, 64)
                m = {}
                for n in range(7):
                    left = jnp.concatenate([_as_bf16(wo7_s[n, h, :M // 4]) for h in range(H)], axis=1)
                    right = jnp.concatenate([_as_bf16(x7_s[n, h, pl.ds(r0, 64), :]) for h in range(H)], axis=1)
                    m[n] = jax.lax.dot_general(left, right, NT, preferred_element_type=F32)
                a = jnp.concatenate([jnp.concatenate([_c11(m), _c12(m)], axis=1),
                                     jnp.concatenate([_c21(m), _c22(m)], axis=1)], axis=0)
                gj = g_s[0:1, pl.ds(c0 + t * TQ, TQ)]
                b = xT_s[:, pl.ds(c0 + t * TQ, TQ)].astype(F32)
                o_s[:, pl.ds(c0 + t * TQ, TQ)] = (gj * a + (1.0 - gj) * b).astype(BF16)
                out_copy(j * (RC // TQ) + t).start()
            return 0
        jax.lax.fori_loop(0, S // RC, out_step, 0)
        for j in range(nq):
            out_copy(j).wait()

    pl.run_scoped(
        phase1,
        *[pltpu.VMEM(r.shape, r.dtype) for r in (c_hbm, wq_hbm, wk_hbm, wv_hbm, wg_hbm, wu_hbm, wd_hbm)],
        pltpu.VMEM((7, S // 4, mh), U32),
        pltpu.VMEM((7, -(-pq // 4) * 32, L), U32),
        pltpu.VMEM((7, -(-pq // 4) * 32, L), U32),
        pltpu.VMEM((M,), BF16),
        pltpu.VMEM((M,), BF16))
    pl.run_scoped(phase2, pltpu.VMEM((7, H, S // 4, L), U32))


def _tile_view(w):
    c, h, d = w.shape
    w = w.reshape(c, h // 8, 8, d // L, L).transpose(0, 1, 3, 2, 4)
    return w.reshape(c, h // 8, 8 * (d // L), L)


@jax.jit
def pallas_gated_mix__compressed_kv_cla__moe_arch_mod__prompt_kernel(
    A_x: jax.Array,
    A_c_kv: jax.Array,
    A_w_q: jax.Array,
    A_w_uk: jax.Array,
    A_w_uv: jax.Array,
    A_w_o: jax.Array,
    B_x: jax.Array,
    B_w_r: jax.Array,
    B_w_gate: jax.Array,
    B_w_up: jax.Array,
    B_w_down: jax.Array,
    gate_w: jax.Array,
):
    _, S, M = A_x.shape
    DC = A_c_kv.shape[2]
    H, D = A_w_q.shape[1], A_w_q.shape[2]
    args = (jnp.transpose(A_x[0]), A_c_kv[0], _tile_view(A_w_q).reshape(2, M // 2, 2, 16, L),
            _tile_view(A_w_uk), _tile_view(A_w_uv),
            jnp.transpose(A_w_o, (0, 2, 1)), B_w_r, gate_w, B_w_gate, B_w_up, jnp.transpose(B_w_down))

    def kern(*refs):
        _kernel(*refs, S=S, M=M, DC=DC, H=H, D=D)

    hbm = pl.BlockSpec(memory_space=pl.ANY)
    oT = pl.pallas_call(
        kern,
        out_shape=jax.ShapeDtypeStruct((M, S), A_x.dtype),
        in_specs=[hbm] * len(args),
        out_specs=hbm,
        scratch_shapes=[
            pltpu.VMEM((8, S + PAD_TILES * L), F32),
            pltpu.VMEM((M, S), BF16),
            pltpu.VMEM((H, M, D), BF16),
            pltpu.VMEM((7, S // 4, DC // 2), U32),
            pltpu.VMEM((7, 4, 8 * (DC // 4 + 1), L), U32),
            pltpu.VMEM((H, S // 2, D), U32),
            pltpu.VMEM((S // 2, D), U32),
            pltpu.VMEM((S // 2, D), U32),
            pltpu.VMEM((7, H, L, L), U32),
            pltpu.VMEM((M, S), BF16),
            pltpu.VMEM((5, S // 4 + PAD_V, L), U32),
            pltpu.SemaphoreType.DMA((N_SEM,)),
        ],
        compiler_params=pltpu.CompilerParams(vmem_limit_bytes=124 * 1024 * 1024),
    )(*args)
    return jnp.transpose(oT)[None]
```

```python
import math

import jax
import jax.numpy as jnp
import jax.experimental.pallas as pl
import jax.experimental.pallas.tpu as pltpu

F32 = jnp.float32
BF16 = jnp.bfloat16
U32 = jnp.uint32
NT = (((1,), (1,)), ((), ()))

L = 128
TQ = 256
HQ = TQ // 2
RC = 512
NCH = 4

PAD_V = 16

S_X, S_Q0, S_Q1, S_K, S_V, S_C, S_MISC, S_OUT = 0, 4, 8, 12, 16, 20, 24, 30
N_SEM = 38

LOOP_ORDER = ("Q0 Q7 S0 G0 S7 V0 V7 Q6 G3 S6 V6 Q5 G4 S5 V5 Q4 G6 S4 V4 Q3 G1 S3 V3 Q2 G2 S2 V2 "
              "Q1 G5 S1 V1 w0")
FIRST_ORDER = "G0 G3 h0 G4 G6 G1 h1 G2 G5 h2 w0"
LAST_ORDER = "Q7 Q6 q5 s7 V7 S6 Q4 V6 S5 r3 V5 S4 r2 V4 S3 r1 V3 S2 r0 V2 S1 S0 V1 V0"


def _to_u32(x_f32):
    return pltpu.bitcast(x_f32.astype(BF16), U32)


def _as_bf16(x_u32):
    return pltpu.bitcast(x_u32, BF16)


def _left(a11, a12, a21, a22):
    return (a11 + a22, a21 + a22, a11, a22, a11 + a12, a21 - a11, a12 - a22)


def _right(b11, b12, b21, b22):
    return (b11 + b22, b11, b12 - b22, b21 - b11, b22, b11 + b12, b21 + b22)


def _c11(m):
    return (m[0] + m[3]) + (m[6] - m[4])


def _c12(m):
    return m[2] + m[4]


def _c21(m):
    return m[1] + m[3]


def _c22(m):
    return (m[0] - m[1]) + (m[2] + m[5])


def _never(i):
    return jax.lax.broadcasted_iota(jnp.int32, (8, L), 0) < (i >> 10)


def _or_all(xs):
    out = xs[0]
    for x in xs[1:]:
        out = out | x
    return out


def _unpack(w, par):
    return pltpu.unpack_elementwise(w, index=par, packed_dtype=BF16, unpacked_dtype=F32)


def _pack(even, odd):
    return pltpu.bitcast(pltpu.pack_elementwise([even, odd], packed_dtype=BF16), U32)


def _head_weight(ref, h, nrows, pitch):
    sel = ((h >> 3) << 1) + (h & 1)
    r = (h >> 1) & 3
    return jnp.concatenate(
        [_as_bf16(ref[sel, pl.ds((dt * 4 + r) * pitch, nrows), :]) for dt in range(2)], axis=1)


def _kernel(xT_hbm, c_hbm, wq_hbm, wk_hbm, wv_hbm, wo_hbm, wr_hbm, gw_hbm, wg_hbm, wu_hbm, wd_hbm,
            o_hbm,
            g_s, xT_s, wo_s, a_s, b_s, q_s, k_s, v_s, wo7_s, o_s, v5_s, sem, *, S, M, DC, H, D):
    nq = S // TQ
    mh = M // 2
    pq = mh // 2 + 1
    pb = DC // 4 + 1
    mq = mh // NCH
    mk = DC // NCH
    qscale = (D ** -0.5) * math.log2(math.e)
    neg = -1e9 * math.log2(math.e)
    wo_copy = pltpu.make_async_copy(wo_hbm, wo_s, sem.at[S_MISC + 5])

    def out_copy(j):
        return pltpu.make_async_copy(o_s.at[:, pl.ds(j * TQ, TQ)], o_hbm.at[:, pl.ds(j * TQ, TQ)],
                                     sem.at[S_OUT + j])

    tri = (jax.lax.broadcasted_iota(jnp.int32, (L, L), 1) <= jax.lax.broadcasted_iota(jnp.int32, (L, L), 0))

    def head_program(order, h, hn, never, x7_s, span=0.9, hooks=None):
        prods, held, waiting = {}, {}, []

        def spots(v, cols, rows=(0, 64, 128, 192)):
            return [v[r:r + 8, n * L:(n + 1) * L] for n in cols for r in rows]

        def tie(lhs, links, every):
            rows = []
            for rg in range(lhs.shape[0] // 8):
                blk = lhs[rg * 8:(rg + 1) * 8]
                if links and rg % every == 0:
                    blk = jnp.concatenate([jnp.where(never, links.pop(0), blk[:, :L]), blk[:, L:]], axis=1)
                rows.append(blk)
            return jnp.concatenate(rows, axis=0)

        def proj(n):
            lhs = a_s[n]
            if waiting:
                lhs = tie(lhs, list(waiting), lhs.shape[0] // 8 // len(waiting))
                del waiting[:]
            prods[n] = jnp.dot(_as_bf16(lhs), _head_weight(b_s.at[n], hn, DC // 4, pb),
                               preferred_element_type=F32)
            for key, odd, comb, needs in (("k", 0, _c11, (0, 3, 4, 6)), ("k", 1, _c21, (1, 3)),
                                          ("v", 0, _c12, (2, 4)), ("v", 1, _c22, (0, 1, 2, 5))):
                if n in needs and all(x in prods for x in needs):
                    for k in range(nq // 2):
                        c = comb({x: prods[x][k * TQ:(k + 1) * TQ] for x in needs})
                        held[2 * k + odd, key] = _to_u32(c)
                        if key == "v" and 2 * k + odd < nq - 1:
                            ops = _right(c[:L, :L], c[:L, L:], c[L:, :L], c[L:, L:])
                            held[2 * k + odd, "r"] = [_to_u32(ops[x]) for x in (0, 2, 3, 5, 6)]
            return spots(prods[n], (0, 1), range(0, S // 2, 32))

        def write_kv():
            for ch in reversed(range(nq)):
                k_s[ch * HQ:(ch + 1) * HQ, :] = held[ch, "k"]
                v_s[ch * HQ:(ch + 1) * HQ, :] = held[ch, "v"]
                for n, o in enumerate(held.get((ch, "r"), ())):
                    v5_s[n, ch * 64:(ch + 1) * 64, :] = o

        def qk(i, tied):
            q = q_s[h, i * HQ:(i + 1) * HQ, :]
            if tied:
                n = len(waiting) - tied + 1
                q = tie(q, waiting[:n], 16 // n)
                del waiting[:n]
            q = _as_bf16(q)
            n0 = i * TQ
            n1 = n0 + L
            s1 = jax.lax.dot_general(q, _as_bf16(k_s[0:n1 // 2, :]), NT, preferred_element_type=F32)
            s2 = jax.lax.dot_general(q[L:], _as_bf16(k_s[n1 // 2:(n1 + L) // 2, :]), NT,
                                     preferred_element_type=F32)
            top = jnp.where(tri, s1[:L, n0:], neg)
            if n0:
                top = jnp.concatenate([s1[:L, :n0], top], axis=1)
            bot = jnp.concatenate([s1[L:], jnp.where(tri, s2, neg)], axis=1)
            return (top, bot), spots(s1, range(max(1, n0 // L)))

        def softmax(i, top, bot, pieces):
            p, sums, prev = ([], []), ([], []), None
            for k in range(TQ // 8):
                half = k % 2
                s = (top, bot)[half][(k // 2) * 8:(k // 2 + 1) * 8]
                link = pieces[int(span * k * 8 / TQ * len(pieces))]
                if prev is not None:
                    link = jnp.where(never, link, prev)
                m = jnp.broadcast_to(jnp.max(s, axis=1, keepdims=True), (8, L))
                m = jnp.where(never, link, m)
                e = [jnp.exp2(s[:, t:t + L] - m) for t in range(0, s.shape[1], L)]
                prev = e[0]
                for x in e[1:]:
                    prev = prev + x
                sums[half].append(prev)
                p[half].append(jnp.concatenate(e, axis=1))
            pt, pb_ = jnp.concatenate(p[0], axis=0), jnp.concatenate(p[1], axis=0)

            def tile(x, t):
                return x[:, t * L:(t + 1) * L]
            ops = [_left(tile(pt, 2 * c), tile(pt, 2 * c + 1), tile(pb_, 2 * c), tile(pb_, 2 * c + 1))
                   for c in range(i)]
            left = [jnp.concatenate([o[n] for o in ops], axis=1).astype(BF16) for n in range(7)] if i else None
            inv = []
            for x in sums:
                l = jnp.sum(jnp.concatenate(x, axis=0), axis=1, keepdims=True)
                r = pl.reciprocal(l, approx=True)
                inv.append(r * (2.0 - l * r))
            return (left, jnp.concatenate([tile(pt, 2 * i), tile(pb_, 2 * i)], axis=0).astype(BF16),
                    tile(pb_, 2 * i + 1).astype(BF16), inv)

        def pv(i, left, p1, p2, inv):
            r0 = i * HQ
            m, pieces = {}, []
            for n in (2, 3, 0, 4, 1, 5, 6) if i else ():
                if n == 1:
                    w = jnp.concatenate([_as_bf16(v_s[c * HQ:c * HQ + 64, :L]) for c in range(i)], axis=0)
                elif n == 4:
                    w = jnp.concatenate([_as_bf16(v_s[c * HQ + 64:(c + 1) * HQ, L:]) for c in range(i)], axis=0)
                else:
                    w = _as_bf16(v5_s[(0, 2, 3, 5, 6).index(n), 0:i * 64, :])
                m[n] = jnp.dot(left[n], w, preferred_element_type=F32)
                pieces += spots(m[n], (0,), (0, 32, 64, 96))
            c1 = jnp.dot(p1, _as_bf16(v_s[r0:r0 + 64, :]), preferred_element_type=F32)
            c2 = jnp.dot(p2, _as_bf16(v_s[r0 + 64:r0 + HQ, :]), preferred_element_type=F32)
            top, bot = c1[:L], c1[L:] + c2
            if i:
                top = top + jnp.concatenate([_c11(m), _c12(m)], axis=1)
                bot = bot + jnp.concatenate([_c21(m), _c22(m)], axis=1)
            else:
                pieces = spots(c1, (0, 1))
            top, bot = top * inv[0], bot * inv[1]
            us = [_to_u32(o) for o in _right(top[:, :L], bot[:, :L], top[:, L:], bot[:, L:])]
            for n in range(7):
                x7_s[n, h, i * 64:(i + 1) * 64, :] = us[n]
            waiting.extend(_or_all([us[n][g * 8:(g + 1) * 8] for n in (0, 2, 3, 5, 6)]) for g in range(8))
            return pieces

        def wo_operands():
            for rg in range(M // 32):
                a = [wo_s[h, hf * (M // 2) + rg * 16:hf * (M // 2) + (rg + 1) * 16, ch * L:(ch + 1) * L].astype(F32)
                     for hf in range(2) for ch in range(2)]
                us = [_to_u32(o) for o in _left(*a)]
                for n in range(7):
                    wo7_s[n, h, rg * 8:(rg + 1) * 8, :] = us[n]
                waiting.append(_or_all([us[n] for n in (0, 1, 4, 5, 6)]))

        if h is not None:
            wo_operands()
        scores, probs, pieces = {}, {}, []
        for op in order.split():
            i = int(op[1:])
            if op[0] == "G":
                pieces.append(proj(i))
            elif op[0] == "w":
                write_kv()
            elif op[0] in "Qqr":
                scores[i], new = qk(i, {"Q": 0, "q": 1, "r": 9}[op[0]])
                pieces.append(new)
            elif op[0] in "Ss":
                probs[i] = softmax(i, *scores.pop(i), pieces[-1] if op[0] == "S" else pieces[-2] + pieces[-1])
            elif op[0] == "V":
                pieces.append(pv(i, *probs.pop(i)))
            else:
                hooks[i](pieces)

    def phase1(c_s, wq_r, wk_r, wv_r, wg_s, wu_s, wd_s, xa_s, wq0_s, wq1_s, wr_s, gw_s):
        def x_copy(j):
            return pltpu.make_async_copy(xT_hbm.at[:, pl.ds(j * RC, RC)], xT_s.at[:, pl.ds(j * RC, RC)],
                                         sem.at[S_X + j])

        def wq_copy(g, j):
            return pltpu.make_async_copy(wq_hbm.at[:, pl.ds(j * mq, mq), g], wq_r.at[:, pl.ds(j * mq, mq), g],
                                         sem.at[(S_Q1 if g else S_Q0) + j])

        def kv_copies(j):
            return [pltpu.make_async_copy(src.at[pl.ds(j * n, n)], dst.at[pl.ds(j * n, n)], sem.at[s0 + j])
                    for src, dst, s0, n in ((c_hbm, c_s, S_C, RC), (wk_hbm, wk_r, S_K, mk), (wv_hbm, wv_r, S_V, mk))]

        misc = [pltpu.make_async_copy(a, b, sem.at[S_MISC + i]) for i, (a, b) in enumerate(
            [(wr_hbm, wr_s), (gw_hbm, gw_s), (wg_hbm, wg_s), (wu_hbm, wu_s), (wd_hbm, wd_s)])]

        x_copy(0).start()
        for j in range(NCH):
            wq_copy(0, j).start()

        def start_rest():
            for j in range(NCH):
                if j + 1 < NCH:
                    x_copy(j + 1).start()
                wq_copy(1, j).start()
            misc[0].start()
            misc[1].start()
            for j in range(NCH):
                for cp in kv_copies(j):
                    cp.start()
            for cp in misc[2:]:
                cp.start()
            wo_copy.start()

        start_rest()

        def x_operands(j):
            c0 = j * RC if isinstance(j, int) else pl.multiple_of(j * RC, RC)
            r0 = j * HQ if isinstance(j, int) else pl.multiple_of(j * HQ, HQ)
            a = [xT_s[kh * mh:(kh + 1) * mh, pl.ds(c0 + rb * TQ, TQ)].astype(F32)
                 for rb in range(2) for kh in range(2)]
            for n, o in enumerate(_left(*a)):
                xa_s[n, pl.ds(r0, HQ), :] = pltpu.bitcast(o.astype(BF16).T, U32)

        def wq_operands(g, p, never=None, link=None):
            w = [pltpu.bitcast(wq_r[kh, pl.ds(2 * p, 2), g], U32) for kh in range(2)]
            w = [[x[0], x[1]] for x in w]
            if link is not None:
                w[0][0] = jnp.where(never, link, w[0][0])
            rows = [_right(*[_unpack(w[kh][e], par) for kh in range(2) for par in range(2)]) for e in range(2)]
            for n in range(7):
                (wq0_s, wq1_s)[g][n, pl.ds(p, 8, stride=pq), :] = _pack(rows[0][n], rows[1][n])

        x_copy(0).wait()
        x_operands(0)

        def first_half(j, _):
            wq_copy(0, j).wait()
            for k in range(mq // 2):
                wq_operands(0, j * (mq // 2) + k)
            return 0
        jax.lax.fori_loop(0, NCH, first_half, 0)

        def q_step(g, j, side):
            pieces = []
            for r in range(4):
                m = {}
                for n in (0, 3, 4, 6, 1, 2, 5):
                    w = jnp.concatenate([_as_bf16((wq0_s, wq1_s)[g][n, pl.ds((dt * 4 + r) * pq, mh // 2), :])
                                         for dt in range(2)], axis=1)
                    m[n] = jnp.dot(_as_bf16(xa_s[n, pl.ds(pl.multiple_of(j * HQ, HQ), HQ), :]), w,
                                   preferred_element_type=F32)
                    for k in range(5):
                        pieces.append(m[n][k * 48:k * 48 + 8, (k % 2) * L:(k % 2 + 1) * L])
                        side(len(pieces) - 1, pieces[-1])
                for par, rb, comb in ((0, 0, _c11), (0, 1, _c21), (1, 0, _c12), (1, 1, _c22)):
                    r0 = pl.multiple_of(j * TQ + rb * HQ, HQ)
                    q_s[8 * g + 2 * r + par, pl.ds(r0, HQ), :] = _to_u32(comb(m) * qscale)

        def q_lo(j, _):
            never = _never(j)

            def side(k, piece):
                if k == 35:
                    @pl.when(j + 1 < NCH)
                    def _():
                        x_copy(j + 1).wait()
                    wq_copy(1, j).wait()
                if k >= 42 and k % 3 == 0 and (k - 42) // 3 < mq // 2:
                    wq_operands(1, j * (mq // 2) + (k - 42) // 3, never, pltpu.bitcast(piece, U32))
            q_step(0, j, side)
            x_operands((j + 1) & (NCH - 1))
            return 0
        jax.lax.fori_loop(0, NCH, q_lo, 0)

        def q_hi(j, _):
            for cp in kv_copies(j):
                cp.wait()
            never = _never(j)

            def side(kk, piece):
                if kk >= 128:
                    return
                k, g = kk // 2, kk % 2
                link = pltpu.bitcast(piece, U32)
                if g == 0:
                    rg, t = k // 4, k % 4
                    a = []
                    for rb in range(2):
                        r0 = pl.multiple_of(j * RC + rb * TQ + rg * 16, 16)
                        for ch in range(2):
                            a.append(c_s[pl.ds(r0, 16), (2 * t + ch) * L:(2 * t + ch + 1) * L].astype(F32))
                    a[0] = jnp.where(jnp.concatenate([never, never], axis=0),
                                     jnp.concatenate([piece, piece], axis=0), a[0])
                    us = [_to_u32(o) for o in _left(*a)]
                    d0 = pl.multiple_of(j * HQ + rg * 8, 8)
                    for n in range(7):
                        a_s[n, pl.ds(d0, 8), t * L:(t + 1) * L] = us[n]
                    link = _or_all([us[n] for n in (0, 1, 4, 5, 6)])
                c0 = j * mk + 2 * k
                w = [pltpu.bitcast(r[pl.ds(c0 + o, 2), g], U32) for o in (0, L) for r in (wk_r, wv_r)]
                w = [[x[0], x[1]] for x in w]
                w[0][0] = jnp.where(never, link, w[0][0])
                for par in range(2):
                    rows = [_right(*[_unpack(x[e], par) for x in w]) for e in range(2)]
                    for n in range(7):
                        b_s[n, 2 * g + par, pl.ds(j * (mk // 4) + k, 8, stride=pb), :] = _pack(
                            rows[0][n], rows[1][n])
            q_step(1, j, side)
            return j
        never = _never(jax.lax.fori_loop(0, NCH, q_hi, 0))

        for cp in misc:
            cp.wait()
        st = {}

        F = wg_s.shape[1]

        def route(pieces):
            pieces = pieces[-2] + pieces[-1]
            mp = -(-M // L) * L
            cols = []
            for w_s in (wr_s, gw_s):
                w = jnp.concatenate([w_s[...].reshape(1, M).astype(F32), jnp.zeros((1, mp - M), F32)], axis=1)
                cols.append(jnp.broadcast_to(w, (L, mp)).T)
            nr, rows = 4, M // 4
            out, k, prev = ([], []), 0, None
            for ct in range(S // L):
                acc = [None, None]
                for q in range(nr):
                    link = pieces[int((0.03 + 0.65 * k / (nr * S // L)) * len(pieces))]
                    if prev is not None:
                        link = jnp.where(never, link, prev)
                    k += 1
                    x = linked(xT_s[q * rows:(q + 1) * rows, ct * L:(ct + 1) * L], link)
                    for t in range(2):
                        part = fold(x * cols[t][q * rows:(q + 1) * rows], 0)
                        acc[t] = part if acc[t] is None else acc[t] + part
                    prev = acc[0] + acc[1]
                for t in range(2):
                    out[t].append(jnp.sum(acc[t], axis=0, keepdims=True))
            g_s[0:1, :] = jax.nn.sigmoid(jnp.concatenate(out[1], axis=1))
            r = jnp.concatenate(out[0], axis=1).astype(BF16).astype(F32)
            lane = jax.lax.broadcasted_iota(jnp.int32, (1, S), 1)
            m1 = jnp.max(r, axis=1, keepdims=True)
            i1 = jnp.min(jnp.where(r == m1, lane, S - 1), axis=1, keepdims=True)
            r2 = jnp.where(lane == i1, -jnp.inf, r)
            m2 = jnp.max(r2, axis=1, keepdims=True)
            i2 = jnp.min(jnp.where(jnp.logical_and(r2 == m2, lane != i1), lane, S - 1), axis=1, keepdims=True)
            ln = jax.lax.broadcasted_iota(jnp.int32, (M, L), 1)
            st["c0"] = [pl.multiple_of((i[0, 0] >> 7) << 7, L) for i in (i1, i2)]
            st["hit"] = [ln == (i & (L - 1)) for i in (i1, i2)]
            st["r"] = [jax.nn.sigmoid(m1), jax.nn.sigmoid(m2)]
            st["x"] = [jnp.broadcast_to(jnp.sum(jnp.where(hit, xT_s[:, pl.ds(c0, L)].astype(F32), 0.0),
                                                axis=1, keepdims=True), (M, L))
                       for c0, hit in zip(st["c0"], st["hit"])]

        def fold(v, axis_len):
            parts = [v[k * 8:(k + 1) * 8] if axis_len == 0 else v[:, k * L:(k + 1) * L]
                     for k in range(v.shape[axis_len] // (8, L)[axis_len])]
            while len(parts) > 1:
                parts = [parts[k] + parts[k + 1] if k + 1 < len(parts) else parts[k]
                         for k in range(0, len(parts), 2)]
            return parts[0]

        def linked(w, link):
            w = pltpu.bitcast(w, U32)
            reps = (w.shape[0] // 8, w.shape[1] // L)
            w = jnp.where(jnp.tile(never, reps), jnp.tile(pltpu.bitcast(link, U32), reps), w)
            return _as_bf16(w).astype(F32)

        def hidden(pieces):
            pieces = pieces[-3] + pieces[-2] + pieces[-1]
            nr, rows = 4, M // 4
            total = 2 * (F // L) * nr
            out, k, prev = [], 0, None
            for w_s in (wg_s, wu_s):
                cols = ([], [])
                for ct in range(F // L):
                    acc = [None, None]
                    for q in range(nr):
                        link = pieces[int(0.9 * k / total * len(pieces))]
                        if prev is not None:
                            link = jnp.where(never, link, prev)
                        k += 1
                        w = linked(w_s[q * rows:(q + 1) * rows, ct * L:(ct + 1) * L], link)
                        for t in range(2):
                            part = fold(w * st["x"][t][q * rows:(q + 1) * rows], 0)
                            acc[t] = part if acc[t] is None else acc[t] + part
                        prev = acc[0] + acc[1]
                    for t in range(2):
                        cols[t].append(jnp.sum(acc[t], axis=0, keepdims=True))
                out.append([jnp.concatenate(c, axis=1) for c in cols])
            st["h"] = [(jax.nn.silu(out[0][t]) * out[1][t]).astype(BF16).astype(F32) for t in range(2)]

        def patch(pieces):
            pieces = pieces[-2] + pieces[-1]
            half = F // 2
            ys, k, prev = ([], []), 0, None
            for rg in range(M // 16):
                acc = [None, None]
                for hf in range(2):
                    link = pieces[int((0.1 + 0.8 * k / (M // 8)) * len(pieces))]
                    if prev is not None:
                        link = jnp.where(never, link, prev)
                    k += 1
                    w = linked(wd_s[rg * 16:(rg + 1) * 16, hf * half:(hf + 1) * half], link)
                    for t in range(2):
                        part = fold(w * st["h"][t][:, hf * half:(hf + 1) * half], 1)
                        acc[t] = part if acc[t] is None else acc[t] + part
                    prev = fold(acc[0] + acc[1], 0)
                for t in range(2):
                    ys[t].append(jnp.sum(acc[t], axis=1, keepdims=True))
            for t in range(2):
                y = jnp.concatenate(ys[t], axis=0) * st["r"][t]
                blk = xT_s[:, pl.ds(st["c0"][t], L)].astype(F32)
                xT_s[:, pl.ds(st["c0"][t], L)] = (blk + jnp.where(st["hit"][t], y, 0.0)).astype(BF16)

        head_program(FIRST_ORDER, None, 0, never, None, hooks=(route, hidden, patch))

    def phase2(x7_s):
        wo_copy.wait()

        def head(h, _):
            head_program(LOOP_ORDER, h, h + 1, _never(h), x7_s, span=0.96)
            return h
        last = jax.lax.fori_loop(0, H - 1, head, 0)
        head_program(LAST_ORDER, H - 1, None, _never(last), x7_s)

        def out_step(j, _):
            c0 = pl.multiple_of(j * RC, RC)
            for t in range(RC // TQ):
                r0 = pl.multiple_of(j * (RC // 4) + t * 64, 64)
                m = {}
                for n in range(7):
                    left = jnp.concatenate([_as_bf16(wo7_s[n, h, :M // 4]) for h in range(H)], axis=1)
                    right = jnp.concatenate([_as_bf16(x7_s[n, h, pl.ds(r0, 64), :]) for h in range(H)], axis=1)
                    m[n] = jax.lax.dot_general(left, right, NT, preferred_element_type=F32)
                a = jnp.concatenate([jnp.concatenate([_c11(m), _c12(m)], axis=1),
                                     jnp.concatenate([_c21(m), _c22(m)], axis=1)], axis=0)
                gj = g_s[0:1, pl.ds(c0 + t * TQ, TQ)]
                b = xT_s[:, pl.ds(c0 + t * TQ, TQ)].astype(F32)
                o_s[:, pl.ds(c0 + t * TQ, TQ)] = (gj * a + (1.0 - gj) * b).astype(BF16)
                out_copy(j * (RC // TQ) + t).start()
            return 0
        jax.lax.fori_loop(0, S // RC, out_step, 0)
        for j in range(nq):
            out_copy(j).wait()

    pl.run_scoped(
        phase1,
        *[pltpu.VMEM(r.shape, r.dtype) for r in (c_hbm, wq_hbm, wk_hbm, wv_hbm, wg_hbm, wu_hbm, wd_hbm)],
        pltpu.VMEM((7, S // 4, mh), U32),
        pltpu.VMEM((7, -(-pq // 4) * 32, L), U32),
        pltpu.VMEM((7, -(-pq // 4) * 32, L), U32),
        pltpu.VMEM((M,), BF16),
        pltpu.VMEM((M,), BF16))
    pl.run_scoped(phase2, pltpu.VMEM((7, H, S // 4, L), U32))


def _tile_view(w):
    c, h, d = w.shape
    w = w.reshape(c, h // 8, 8, d // L, L).transpose(0, 1, 3, 2, 4)
    return w.reshape(c, h // 8, 8 * (d // L), L)


@jax.jit
def pallas_gated_mix__compressed_kv_cla__moe_arch_mod__prompt_kernel(
    A_x: jax.Array,
    A_c_kv: jax.Array,
    A_w_q: jax.Array,
    A_w_uk: jax.Array,
    A_w_uv: jax.Array,
    A_w_o: jax.Array,
    B_x: jax.Array,
    B_w_r: jax.Array,
    B_w_gate: jax.Array,
    B_w_up: jax.Array,
    B_w_down: jax.Array,
    gate_w: jax.Array,
):
    _, S, M = A_x.shape
    DC = A_c_kv.shape[2]
    H, D = A_w_q.shape[1], A_w_q.shape[2]
    args = (jnp.transpose(A_x[0]), A_c_kv[0], _tile_view(A_w_q).reshape(2, M // 2, 2, 16, L),
            _tile_view(A_w_uk), _tile_view(A_w_uv),
            jnp.transpose(A_w_o, (0, 2, 1)), B_w_r, gate_w, B_w_gate, B_w_up, jnp.transpose(B_w_down))

    def kern(*refs):
        _kernel(*refs, S=S, M=M, DC=DC, H=H, D=D)

    hbm = pl.BlockSpec(memory_space=pl.ANY)
    oT = pl.pallas_call(
        kern,
        out_shape=jax.ShapeDtypeStruct((M, S), A_x.dtype),
        in_specs=[hbm] * len(args),
        out_specs=hbm,
        scratch_shapes=[
            pltpu.VMEM((8, S), F32),
            pltpu.VMEM((M, S), BF16),
            pltpu.VMEM((H, M, D), BF16),
            pltpu.VMEM((7, S // 4, DC // 2), U32),
            pltpu.VMEM((7, 4, 8 * (DC // 4 + 1), L), U32),
            pltpu.VMEM((H, S // 2, D), U32),
            pltpu.VMEM((S // 2, D), U32),
            pltpu.VMEM((S // 2, D), U32),
            pltpu.VMEM((7, H, L, L), U32),
            pltpu.VMEM((M, S), BF16),
            pltpu.VMEM((5, S // 4 + PAD_V, L), U32),
            pltpu.SemaphoreType.DMA((N_SEM,)),
        ],
        compiler_params=pltpu.CompilerParams(vmem_limit_bytes=124 * 1024 * 1024),
    )(*args)
    return jnp.transpose(oT)[None]
```

```python
import math

import jax
import jax.numpy as jnp
import jax.experimental.pallas as pl
import jax.experimental.pallas.tpu as pltpu

F32 = jnp.float32
BF16 = jnp.bfloat16
U32 = jnp.uint32
NT = (((1,), (1,)), ((), ()))

L = 128
TQ = 256
HQ = TQ // 2
RC = 512
NCH = 4

PAD_V = 16

S_X, S_Q0, S_Q1, S_K, S_V, S_C, S_MISC, S_OUT = 0, 4, 8, 12, 16, 20, 24, 30
N_SEM = 38

LOOP_ORDER = ("Q0 Q7 S0 G0 S7 V0 V7 Q6 G3 S6 V6 Q5 G4 S5 V5 Q4 G5 S4 V4 Q3 G6 S3 V3 Q2 G2 S2 V2 "
              "Q1 G1 S1 V1 w0")
FIRST_ORDER = "G0 G3 h0 G2 G4 G6 h1 G5 G1 h2 w0"
LAST_ORDER = "Q7 Q6 Q5 s7 q4 V7 S6 r3 V6 S5 r2 V5 S4 r1 V4 S3 r0 V3 S2 V2 S1 S0 V1 V0"


def _to_u32(x_f32):
    return pltpu.bitcast(x_f32.astype(BF16), U32)


def _shuffled_u32(x_f32):
    return jnp.concatenate([_pack(x_f32[r:r + 8], x_f32[r + 8:r + 16]) for r in range(0, x_f32.shape[0], 16)],
                           axis=0)


def _as_bf16(x_u32):
    return pltpu.bitcast(x_u32, BF16)


def _left(a11, a12, a21, a22):
    return (a11 + a22, a21 + a22, a11, a22, a11 + a12, a21 - a11, a12 - a22)


def _right(b11, b12, b21, b22):
    return (b11 + b22, b11, b12 - b22, b21 - b11, b22, b11 + b12, b21 + b22)


FLAT, DEEP = (0, 1, 3, 4, 6), (2, 5)
SUMS = (0, 2, 3, 5, 6)
QK_LAG = 2
QK_TIE = 0


def _c11(m):
    return (m[0] + m[3]) + (m[6] - m[4])


def _c12(m):
    return m[2] + m[4]


def _c21(m):
    return m[1] + m[3]


def _c22(m):
    return (m[0] - m[1]) + (m[2] + m[5])


def _never(i):
    return jax.lax.broadcasted_iota(jnp.int32, (8, L), 0) < (i >> 10)


def _or_all(xs):
    out = xs[0]
    for x in xs[1:]:
        out = out | x
    return out


def _unpack(w, par):
    return pltpu.unpack_elementwise(w, index=par, packed_dtype=BF16, unpacked_dtype=F32)


def _pack(even, odd):
    return pltpu.bitcast(pltpu.pack_elementwise([even, odd], packed_dtype=BF16), U32)


def _head_weight(ref, h, nrows, pitch):
    sel = ((h >> 3) << 1) + (h & 1)
    r = (h >> 1) & 3
    return jnp.concatenate(
        [_as_bf16(ref[sel, pl.ds((dt * 4 + r) * pitch, nrows), :]) for dt in range(2)], axis=1)


def _kernel(xT_hbm, c_hbm, wq_hbm, wk_hbm, wv_hbm, wo_hbm, wr_hbm, gw_hbm, wg_hbm, wu_hbm, wd_hbm,
            o_hbm,
            g_s, xT_s, wo_s, a_s, a2_s, b_s, q_s, k_s, v_s, k5_s, wo7_s, o_s, v5_s, sem, *, S, M, DC, H, D):
    nq = S // TQ
    mh = M // 2
    pq = mh // 2 + 1
    pb = DC // 4 + 1
    mq = mh // NCH
    mk = DC // NCH
    qscale = (D ** -0.5) * math.log2(math.e)
    neg = -1e9 * math.log2(math.e)
    wo_copy = pltpu.make_async_copy(wo_hbm, wo_s, sem.at[S_MISC + 5])

    def out_copy(j):
        return pltpu.make_async_copy(o_s.at[:, pl.ds(j * TQ, TQ)], o_hbm.at[:, pl.ds(j * TQ, TQ)],
                                     sem.at[S_OUT + j])

    col = jax.lax.broadcasted_iota(jnp.int32, (L, L), 1)
    tri = ((col & ~15) + ((col & 3) << 2) + ((col & 15) >> 2) <= jax.lax.broadcasted_iota(jnp.int32, (L, L), 0))

    def head_program(order, h, hn, never, x7_s, span=0.9, hooks=None):
        prods, held, waiting = {}, {}, []

        def spots(v, cols, rows=(0, 64, 128, 192)):
            return [v[r:r + 8, n * L:(n + 1) * L] for n in cols for r in rows]

        def tie(lhs, links, every):
            rows = []
            for rg in range(lhs.shape[0] // 8):
                blk = lhs[rg * 8:(rg + 1) * 8]
                if links and rg % every == 0:
                    blk = jnp.concatenate([jnp.where(never, links.pop(0), blk[:, :L]), blk[:, L:]], axis=1)
                rows.append(blk)
            return jnp.concatenate(rows, axis=0)

        def proj(n):
            w = _head_weight(b_s.at[n], hn, DC // 4, pb)
            links = list(waiting)
            del waiting[:]
            if n in DEEP:
                wf, kh = w.astype(F32), DC // 4
                right = [o.astype(BF16) for o in _right(wf[:kh, :L], wf[:kh, L:], wf[kh:, :L], wf[kh:, L:])]
                right[1], right[4] = w[:kh, :L], w[kh:, L:]
                m, pieces = {}, []

                def sub(x, after):
                    lhs = a2_s[DEEP.index(n), x]
                    mine = [links.pop(0) for _ in links[:2]]
                    if after:
                        t = after[0]
                        for v in after[1:]:
                            t = jnp.maximum(t, v)
                        lhs = tie(lhs, [pltpu.bitcast(jnp.maximum(t[g * 16:g * 16 + 8], t[g * 16 + 8:g * 16 + 16]), U32)
                                        for g in range(S // 64)], 1)
                    elif mine or links:
                        mine += links
                        del links[:]
                        lhs = tie(lhs, mine, lhs.shape[0] // 8 // len(mine))
                    m[x] = jnp.dot(_as_bf16(lhs), right[x], preferred_element_type=F32)
                    pieces.extend(spots(m[x], (0,), range(0, S // 4, 64)))
                sub(1, ()), sub(3, ())
                c21 = m[1] + m[3]
                sub(2, ()), sub(4, (c21,))
                c12, c11, c22 = m[2] + m[4], m[3] - m[4], m[2] - m[1]
                sub(0, ()), sub(5, (c12, c11, c22))
                c11, c22 = c11 + m[0], c22 + (m[0] + m[5])
                sub(6, (c11, c22))
                top = jnp.concatenate([c11 + m[6], c12], axis=1)
                bot = jnp.concatenate([c21, c22], axis=1)
                prods[n] = jnp.concatenate([v[k * L:(k + 1) * L] for k in range(nq // 2) for v in (top, bot)],
                                           axis=0)
            else:
                lhs = a_s[FLAT.index(n)]
                if links:
                    lhs = tie(lhs, links, max(1, lhs.shape[0] // 8 // len(links)))
                prods[n] = jnp.dot(_as_bf16(lhs), w, preferred_element_type=F32)
                pieces = spots(prods[n], (0, 1), range(0, S // 2, 32))
            for key, odd, comb, needs in (("k", 0, _c11, (0, 3, 4, 6)), ("k", 1, _c21, (1, 3)),
                                          ("v", 0, _c12, (2, 4)), ("v", 1, _c22, (0, 1, 2, 5))):
                if n in needs and all(x in prods for x in needs):
                    for k in range(nq // 2):
                        c = comb({x: prods[x][k * TQ:(k + 1) * TQ] for x in needs})
                        held[2 * k + odd, key] = _shuffled_u32(c)
                        if 2 * k + odd < nq - 1:
                            off = (c[:L, L:], c[L:, :L]) if key == "v" else (c[L:, :L], c[:L, L:])
                            ops = _right(c[:L, :L], *off, c[L:, L:])
                            held[2 * k + odd, key + "5"] = [_shuffled_u32(ops[x]) for x in SUMS]
            return pieces

        def write_kv():
            for ch in reversed(range(nq)):
                k_s[ch * HQ:(ch + 1) * HQ, :] = held[ch, "k"]
                v_s[ch * HQ:(ch + 1) * HQ, :] = held[ch, "v"]
                for key, ref in (("k5", k5_s), ("v5", v5_s)):
                    for n, o in enumerate(held.get((ch, key), ())):
                        ref[n, ch * 64:(ch + 1) * 64, :] = o

        def right_operand(n, plain, sums, c0, c1):
            if n == 1:
                return jnp.concatenate([_as_bf16(plain[c * HQ:c * HQ + 64, :L]) for c in range(c0, c1)], axis=0)
            if n == 4:
                return jnp.concatenate([_as_bf16(plain[c * HQ + 64:(c + 1) * HQ, L:]) for c in range(c0, c1)], axis=0)
            return _as_bf16(sums[SUMS.index(n), c0 * 64:c1 * 64, :])

        def qk(i, tied):
            q = qd = q_s[h, i * HQ:(i + 1) * HQ, :]
            n = min(16, len(waiting) - tied + 1) if tied else 0
            if n > 0:
                qd = tie(q, waiting[:n], 16 // n)
                del waiting[:n]
            q, qd = _as_bf16(q), _as_bf16(qd)
            tops, bots, pieces = [], [], []
            if i:
                qf = q.astype(F32)
                left = [o.astype(BF16) for o in _left(qf[:L, :L], qf[:L, L:], qf[L:, :L], qf[L:, L:])]
                left[2], left[3] = q[:L, :L], q[L:, L:]
            done = []
            for c in range(i):
                lhs = dict(enumerate(left))
                if c >= QK_LAG:
                    u = pltpu.bitcast(left[QK_TIE], U32)
                    lhs[QK_TIE] = _as_bf16(jnp.concatenate(
                        [jnp.where(never, done[c - QK_LAG][g], u[g * 8:(g + 1) * 8]) for g in range(8)], axis=0))
                m = {n: jax.lax.dot_general(lhs[n], right_operand(n, k_s, k5_s, c, c + 1), NT,
                                            preferred_element_type=F32) for n in (0, 3, 4, 6, 1, 2, 5)}
                c11, c12, c21, c22 = _c11(m), _c12(m), _c21(m), _c22(m)
                tops += [c11, c12]
                bots += [c21, c22]
                t = jnp.maximum(jnp.maximum(c11, c12), jnp.maximum(c21, c22))
                done.append([pltpu.bitcast(jnp.maximum(t[g * 16:g * 16 + 8], t[g * 16 + 8:(g + 1) * 16]), U32)
                             for g in range(8)])
                for n in (0, 5):
                    pieces += spots(m[n], (0,), (0, 32, 64, 96))
            r0 = i * HQ
            s1 = jax.lax.dot_general(qd, _as_bf16(k_s[r0:r0 + 64, :]), NT, preferred_element_type=F32)
            s2 = jax.lax.dot_general(q[L:], _as_bf16(k_s[r0 + 64:r0 + HQ, :]), NT, preferred_element_type=F32)
            top = jnp.concatenate(tops + [jnp.where(tri, s1[:L], neg)], axis=1)
            bot = jnp.concatenate(bots + [s1[L:], jnp.where(tri, s2, neg)], axis=1)
            return (top, bot), pieces + spots(s1, (0,))

        def softmax(i, top, bot, pieces):
            p, sums, prev = ([], []), ([], []), None
            for k in range(TQ // 8):
                half = k % 2
                s = (top, bot)[half][(k // 2) * 8:(k // 2 + 1) * 8]
                link = pieces[int(span * k * 8 / TQ * len(pieces))]
                if prev is not None:
                    link = jnp.where(never, link, prev)
                m = jnp.broadcast_to(jnp.max(s, axis=1, keepdims=True), (8, L))
                m = jnp.where(never, link, m)
                e = [jnp.exp2(s[:, t:t + L] - m) for t in range(0, s.shape[1], L)]
                prev = e[0]
                for x in e[1:]:
                    prev = prev + x
                sums[half].append(prev)
                p[half].append(jnp.concatenate(e, axis=1))
            pt, pb_ = jnp.concatenate(p[0], axis=0), jnp.concatenate(p[1], axis=0)

            def tile(x, t):
                return x[:, t * L:(t + 1) * L]
            ops = [_left(tile(pt, 2 * c), tile(pt, 2 * c + 1), tile(pb_, 2 * c), tile(pb_, 2 * c + 1))
                   for c in range(i)]
            left = [jnp.concatenate([o[n] for o in ops], axis=1).astype(BF16) for n in range(7)] if i else None
            inv = []
            for x in sums:
                l = jnp.sum(jnp.concatenate(x, axis=0), axis=1, keepdims=True)
                r = pl.reciprocal(l, approx=True)
                inv.append(r * (2.0 - l * r))
            return (left, jnp.concatenate([tile(pt, 2 * i), tile(pb_, 2 * i)], axis=0).astype(BF16),
                    tile(pb_, 2 * i + 1).astype(BF16), inv)

        def pv(i, left, p1, p2, inv):
            r0 = i * HQ
            m, pieces = {}, []
            for n in (2, 3, 0, 4, 1, 5, 6) if i else ():
                m[n] = jnp.dot(left[n], right_operand(n, v_s, v5_s, 0, i), preferred_element_type=F32)
                pieces += spots(m[n], (0,), (0, 32, 64, 96))
            c1 = jnp.dot(p1, _as_bf16(v_s[r0:r0 + 64, :]), preferred_element_type=F32)
            c2 = jnp.dot(p2, _as_bf16(v_s[r0 + 64:r0 + HQ, :]), preferred_element_type=F32)
            top, bot = c1[:L], c1[L:] + c2
            if i:
                top = top + jnp.concatenate([_c11(m), _c12(m)], axis=1)
                bot = bot + jnp.concatenate([_c21(m), _c22(m)], axis=1)
            else:
                pieces = spots(c1, (0, 1))
            top, bot = top * inv[0], bot * inv[1]
            us = [_to_u32(o) for o in _right(top[:, :L], bot[:, :L], top[:, L:], bot[:, L:])]
            for n in range(7):
                x7_s[n, h, i * 64:(i + 1) * 64, :] = us[n]
            waiting.extend(_or_all([us[n][g * 8:(g + 1) * 8] for n in SUMS]) for g in range(8))
            return pieces

        def wo_operands():
            for rg in range(M // 32):
                a = [wo_s[h, hf * (M // 2) + rg * 16:hf * (M // 2) + (rg + 1) * 16, ch * L:(ch + 1) * L].astype(F32)
                     for hf in range(2) for ch in range(2)]
                us = [_to_u32(o) for o in _left(*a)]
                for n in range(7):
                    wo7_s[n, h, rg * 8:(rg + 1) * 8, :] = us[n]
                waiting.append(_or_all([us[n] for n in (0, 1, 4, 5, 6)]))

        if h is not None:
            wo_operands()
        scores, probs, pieces = {}, {}, []
        for op in order.split():
            i = int(op[1:])
            if op[0] == "G":
                pieces.append(proj(i))
            elif op[0] == "w":
                write_kv()
            elif op[0] in "Qqr":
                scores[i], new = qk(i, {"Q": 0, "q": 1, "r": 9}[op[0]])
                pieces.append(new)
            elif op[0] in "Ss":
                probs[i] = softmax(i, *scores.pop(i), pieces[-1] if op[0] == "S" else pieces[-2] + pieces[-1])
            elif op[0] == "V":
                pieces.append(pv(i, *probs.pop(i)))
            else:
                hooks[i](pieces)

    def phase1(c_s, wq_r, wk_r, wv_r, wg_s, wu_s, wd_s, xa_s, wq0_s, wq1_s, wr_s, gw_s):
        def x_copy(j):
            return pltpu.make_async_copy(xT_hbm.at[:, pl.ds(j * RC, RC)], xT_s.at[:, pl.ds(j * RC, RC)],
                                         sem.at[S_X + j])

        def wq_copy(g, j):
            return pltpu.make_async_copy(wq_hbm.at[:, pl.ds(j * mq, mq), g], wq_r.at[:, pl.ds(j * mq, mq), g],
                                         sem.at[(S_Q1 if g else S_Q0) + j])

        def kv_copies(j):
            return [pltpu.make_async_copy(src.at[pl.ds(j * n, n)], dst.at[pl.ds(j * n, n)], sem.at[s0 + j])
                    for src, dst, s0, n in ((c_hbm, c_s, S_C, RC), (wk_hbm, wk_r, S_K, mk), (wv_hbm, wv_r, S_V, mk))]

        misc = [pltpu.make_async_copy(a, b, sem.at[S_MISC + i]) for i, (a, b) in enumerate(
            [(wr_hbm, wr_s), (gw_hbm, gw_s), (wg_hbm, wg_s), (wu_hbm, wu_s), (wd_hbm, wd_s)])]

        x_copy(0).start()
        for j in range(NCH):
            wq_copy(0, j).start()

        def start_rest():
            for j in range(NCH):
                if j + 1 < NCH:
                    x_copy(j + 1).start()
                wq_copy(1, j).start()
            misc[0].start()
            misc[1].start()
            for j in range(NCH):
                for cp in kv_copies(j):
                    cp.start()
            for cp in misc[2:]:
                cp.start()
            wo_copy.start()

        start_rest()

        def x_operands(j):
            c0 = j * RC if isinstance(j, int) else pl.multiple_of(j * RC, RC)
            r0 = j * HQ if isinstance(j, int) else pl.multiple_of(j * HQ, HQ)
            a = [xT_s[kh * mh:(kh + 1) * mh, pl.ds(c0 + rb * TQ, TQ)].astype(F32)
                 for rb in range(2) for kh in range(2)]
            for n, o in enumerate(_left(*a)):
                xa_s[n, pl.ds(r0, HQ), :] = pltpu.bitcast(o.astype(BF16).T, U32)

        def wq_operands(g, p, never=None, link=None):
            w = [pltpu.bitcast(wq_r[kh, pl.ds(2 * p, 2), g], U32) for kh in range(2)]
            w = [[x[0], x[1]] for x in w]
            if link is not None:
                w[0][0] = jnp.where(never, link, w[0][0])
            rows = [_right(*[_unpack(w[kh][e], par) for kh in range(2) for par in range(2)]) for e in range(2)]
            for n in range(7):
                (wq0_s, wq1_s)[g][n, pl.ds(p, 8, stride=pq), :] = _pack(rows[0][n], rows[1][n])

        x_copy(0).wait()
        x_operands(0)

        def first_half(j, _):
            wq_copy(0, j).wait()
            for k in range(mq // 2):
                wq_operands(0, j * (mq // 2) + k)
            return 0
        jax.lax.fori_loop(0, NCH, first_half, 0)

        def q_step(g, j, side):
            pieces = []
            for r in range(4):
                m = {}
                for n in (0, 3, 4, 6, 1, 2, 5):
                    w = jnp.concatenate([_as_bf16((wq0_s, wq1_s)[g][n, pl.ds((dt * 4 + r) * pq, mh // 2), :])
                                         for dt in range(2)], axis=1)
                    m[n] = jnp.dot(_as_bf16(xa_s[n, pl.ds(pl.multiple_of(j * HQ, HQ), HQ), :]), w,
                                   preferred_element_type=F32)
                    for k in range(5):
                        pieces.append(m[n][k * 48:k * 48 + 8, (k % 2) * L:(k % 2 + 1) * L])
                        side(len(pieces) - 1, pieces[-1])
                for par, rb, comb in ((0, 0, _c11), (0, 1, _c21), (1, 0, _c12), (1, 1, _c22)):
                    r0 = pl.multiple_of(j * TQ + rb * HQ, HQ)
                    q_s[8 * g + 2 * r + par, pl.ds(r0, HQ), :] = _to_u32(comb(m) * qscale)

        def q_lo(j, _):
            never = _never(j)

            def side(k, piece):
                if k == 35:
                    @pl.when(j + 1 < NCH)
                    def _():
                        x_copy(j + 1).wait()
                    wq_copy(1, j).wait()
                if k >= 42 and k % 3 == 0 and (k - 42) // 3 < mq // 2:
                    wq_operands(1, j * (mq // 2) + (k - 42) // 3, never, pltpu.bitcast(piece, U32))
            q_step(0, j, side)
            x_operands((j + 1) & (NCH - 1))
            return 0
        jax.lax.fori_loop(0, NCH, q_lo, 0)

        def q_hi(j, _):
            for cp in kv_copies(j):
                cp.wait()
            never = _never(j)
            quad = []

            def side(kk, piece):
                if kk >= 128:
                    return
                k, g = kk // 2, kk % 2
                link = pltpu.bitcast(piece, U32)
                if g == 0:
                    rg, t = k // 8 + 8 * (k % 4 // 2), k // 4 % 2 + 2 * (k % 2)
                    a = []
                    for rb in range(2):
                        r0 = pl.multiple_of(j * RC + rb * TQ + rg * 16, 16)
                        for ch in range(2):
                            a.append(c_s[pl.ds(r0, 16), (2 * t + ch) * L:(2 * t + ch + 1) * L].astype(F32))
                    a[0] = jnp.where(jnp.concatenate([never, never], axis=0),
                                     jnp.concatenate([piece, piece], axis=0), a[0])
                    ops = _left(*a)
                    us = [_shuffled_u32(ops[n]) for n in FLAT]
                    d0 = pl.multiple_of(j * HQ + rg * 8, 8)
                    for n, u in enumerate(us):
                        a_s[n, pl.ds(d0, 8), t * L:(t + 1) * L] = u
                    quad.append(ops)
                    if len(quad) == 4:
                        d0 = pl.multiple_of(j * (HQ // 2) + (rg - 8) * 8, 8)
                        for e, n in enumerate(DEEP):
                            deep = [_shuffled_u32(o) for o in _left(*[q[n] for q in quad])]
                            for x, u in enumerate(deep):
                                a2_s[e, x, pl.ds(d0, 8), (t - 2) * L:(t - 1) * L] = u
                            us += deep
                        del quad[:]
                    link = _or_all(us)
                c0 = j * mk + 2 * k
                w = [pltpu.bitcast(r[pl.ds(c0 + o, 2), g], U32) for o in (0, L) for r in (wk_r, wv_r)]
                w = [[x[0], x[1]] for x in w]
                w[0][0] = jnp.where(never, link, w[0][0])
                for par in range(2):
                    rows = [_right(*[_unpack(x[e], par) for x in w]) for e in range(2)]
                    for n in range(7):
                        b_s[n, 2 * g + par, pl.ds(j * (mk // 4) + k, 8, stride=pb), :] = _pack(
                            rows[0][n], rows[1][n])
            q_step(1, j, side)
            return j
        never = _never(jax.lax.fori_loop(0, NCH, q_hi, 0))

        for cp in misc:
            cp.wait()
        st = {}

        F = wg_s.shape[1]

        def route(pieces):
            pieces = pieces[-2] + pieces[-1]
            mp = -(-M // L) * L
            cols = []
            for w_s in (wr_s, gw_s):
                w = jnp.concatenate([w_s[...].reshape(1, M).astype(F32), jnp.zeros((1, mp - M), F32)], axis=1)
                cols.append(jnp.broadcast_to(w, (L, mp)).T)
            nr, rows = 4, M // 4
            out, k, prev = ([], []), 0, None
            for ct in range(S // L):
                acc = [None, None]
                for q in range(nr):
                    link = pieces[int((0.03 + 0.65 * k / (nr * S // L)) * len(pieces))]
                    if prev is not None:
                        link = jnp.where(never, link, prev)
                    k += 1
                    x = linked(xT_s[q * rows:(q + 1) * rows, ct * L:(ct + 1) * L], link)
                    for t in range(2):
                        part = fold(x * cols[t][q * rows:(q + 1) * rows], 0)
                        acc[t] = part if acc[t] is None else acc[t] + part
                    prev = acc[0] + acc[1]
                for t in range(2):
                    out[t].append(jnp.sum(acc[t], axis=0, keepdims=True))
            g_s[0:1, :] = jax.nn.sigmoid(jnp.concatenate(out[1], axis=1))
            r = jnp.concatenate(out[0], axis=1).astype(BF16).astype(F32)
            lane = jax.lax.broadcasted_iota(jnp.int32, (1, S), 1)
            m1 = jnp.max(r, axis=1, keepdims=True)
            i1 = jnp.min(jnp.where(r == m1, lane, S - 1), axis=1, keepdims=True)
            r2 = jnp.where(lane == i1, -jnp.inf, r)
            m2 = jnp.max(r2, axis=1, keepdims=True)
            i2 = jnp.min(jnp.where(jnp.logical_and(r2 == m2, lane != i1), lane, S - 1), axis=1, keepdims=True)
            ln = jax.lax.broadcasted_iota(jnp.int32, (M, L), 1)
            st["c0"] = [pl.multiple_of((i[0, 0] >> 7) << 7, L) for i in (i1, i2)]
            st["hit"] = [ln == (i & (L - 1)) for i in (i1, i2)]
            st["r"] = [jax.nn.sigmoid(m1), jax.nn.sigmoid(m2)]
            st["x"] = [jnp.broadcast_to(jnp.sum(jnp.where(hit, xT_s[:, pl.ds(c0, L)].astype(F32), 0.0),
                                                axis=1, keepdims=True), (M, L))
                       for c0, hit in zip(st["c0"], st["hit"])]

        def fold(v, axis_len):
            parts = [v[k * 8:(k + 1) * 8] if axis_len == 0 else v[:, k * L:(k + 1) * L]
                     for k in range(v.shape[axis_len] // (8, L)[axis_len])]
            while len(parts) > 1:
                parts = [parts[k] + parts[k + 1] if k + 1 < len(parts) else parts[k]
                         for k in range(0, len(parts), 2)]
            return parts[0]

        def linked(w, link):
            w = pltpu.bitcast(w, U32)
            reps = (w.shape[0] // 8, w.shape[1] // L)
            w = jnp.where(jnp.tile(never, reps), jnp.tile(pltpu.bitcast(link, U32), reps), w)
            return _as_bf16(w).astype(F32)

        def hidden(pieces):
            pieces = pieces[-3] + pieces[-2] + pieces[-1]
            nr, rows = 4, M // 4
            total = 2 * (F // L) * nr
            out, k, prev = [], 0, None
            for w_s in (wg_s, wu_s):
                cols = ([], [])
                for ct in range(F // L):
                    acc = [None, None]
                    for q in range(nr):
                        link = pieces[int(0.9 * k / total * len(pieces))]
                        if prev is not None:
                            link = jnp.where(never, link, prev)
                        k += 1
                        w = linked(w_s[q * rows:(q + 1) * rows, ct * L:(ct + 1) * L], link)
                        for t in range(2):
                            part = fold(w * st["x"][t][q * rows:(q + 1) * rows], 0)
                            acc[t] = part if acc[t] is None else acc[t] + part
                        prev = acc[0] + acc[1]
                    for t in range(2):
                        cols[t].append(jnp.sum(acc[t], axis=0, keepdims=True))
                out.append([jnp.concatenate(c, axis=1) for c in cols])
            st["h"] = [(jax.nn.silu(out[0][t]) * out[1][t]).astype(BF16).astype(F32) for t in range(2)]

        def patch(pieces):
            pieces = pieces[-2] + pieces[-1]
            half = F // 2
            ys, k, prev = ([], []), 0, None
            for rg in range(M // 16):
                acc = [None, None]
                for hf in range(2):
                    link = pieces[int((0.1 + 0.8 * k / (M // 8)) * len(pieces))]
                    if prev is not None:
                        link = jnp.where(never, link, prev)
                    k += 1
                    w = linked(wd_s[rg * 16:(rg + 1) * 16, hf * half:(hf + 1) * half], link)
                    for t in range(2):
                        part = fold(w * st["h"][t][:, hf * half:(hf + 1) * half], 1)
                        acc[t] = part if acc[t] is None else acc[t] + part
                    prev = fold(acc[0] + acc[1], 0)
                for t in range(2):
                    ys[t].append(jnp.sum(acc[t], axis=1, keepdims=True))
            for t in range(2):
                y = jnp.concatenate(ys[t], axis=0) * st["r"][t]
                blk = xT_s[:, pl.ds(st["c0"][t], L)].astype(F32)
                xT_s[:, pl.ds(st["c0"][t], L)] = (blk + jnp.where(st["hit"][t], y, 0.0)).astype(BF16)

        head_program(FIRST_ORDER, None, 0, never, None, hooks=(route, hidden, patch))

    def phase2(x7_s):
        wo_copy.wait()

        def head(h, _):
            head_program(LOOP_ORDER, h, h + 1, _never(h), x7_s, span=0.96)
            return h
        last = jax.lax.fori_loop(0, H - 1, head, 0)
        head_program(LAST_ORDER, H - 1, None, _never(last), x7_s)

        def out_step(j, _):
            c0 = pl.multiple_of(j * RC, RC)
            for t in range(RC // TQ):
                r0 = pl.multiple_of(j * (RC // 4) + t * 64, 64)
                m = {}
                for n in range(7):
                    left = jnp.concatenate([_as_bf16(wo7_s[n, h, :M // 4]) for h in range(H)], axis=1)
                    right = jnp.concatenate([_as_bf16(x7_s[n, h, pl.ds(r0, 64), :]) for h in range(H)], axis=1)
                    m[n] = jax.lax.dot_general(left, right, NT, preferred_element_type=F32)
                a = jnp.concatenate([jnp.concatenate([_c11(m), _c12(m)], axis=1),
                                     jnp.concatenate([_c21(m), _c22(m)], axis=1)], axis=0)
                gj = g_s[0:1, pl.ds(c0 + t * TQ, TQ)]
                b = xT_s[:, pl.ds(c0 + t * TQ, TQ)].astype(F32)
                o_s[:, pl.ds(c0 + t * TQ, TQ)] = (gj * a + (1.0 - gj) * b).astype(BF16)
                out_copy(j * (RC // TQ) + t).start()
            return 0
        jax.lax.fori_loop(0, S // RC, out_step, 0)
        for j in range(nq):
            out_copy(j).wait()

    pl.run_scoped(
        phase1,
        *[pltpu.VMEM(r.shape, r.dtype) for r in (c_hbm, wq_hbm, wk_hbm, wv_hbm, wg_hbm, wu_hbm, wd_hbm)],
        pltpu.VMEM((7, S // 4, mh), U32),
        pltpu.VMEM((7, -(-pq // 4) * 32, L), U32),
        pltpu.VMEM((7, -(-pq // 4) * 32, L), U32),
        pltpu.VMEM((M,), BF16),
        pltpu.VMEM((M,), BF16))
    pl.run_scoped(phase2, pltpu.VMEM((7, H, S // 4, L), U32))


def _tile_view(w):
    c, h, d = w.shape
    w = w.reshape(c, h // 8, 8, d // L, L).transpose(0, 1, 3, 2, 4)
    return w.reshape(c, h // 8, 8 * (d // L), L)


@jax.jit
def pallas_gated_mix__compressed_kv_cla__moe_arch_mod__prompt_kernel(
    A_x: jax.Array,
    A_c_kv: jax.Array,
    A_w_q: jax.Array,
    A_w_uk: jax.Array,
    A_w_uv: jax.Array,
    A_w_o: jax.Array,
    B_x: jax.Array,
    B_w_r: jax.Array,
    B_w_gate: jax.Array,
    B_w_up: jax.Array,
    B_w_down: jax.Array,
    gate_w: jax.Array,
):
    _, S, M = A_x.shape
    DC = A_c_kv.shape[2]
    H, D = A_w_q.shape[1], A_w_q.shape[2]
    args = (jnp.transpose(A_x[0]), A_c_kv[0], _tile_view(A_w_q).reshape(2, M // 2, 2, 16, L),
            _tile_view(A_w_uk), _tile_view(A_w_uv),
            jnp.transpose(A_w_o, (0, 2, 1)), B_w_r, gate_w, B_w_gate, B_w_up, jnp.transpose(B_w_down))

    def kern(*refs):
        _kernel(*refs, S=S, M=M, DC=DC, H=H, D=D)

    hbm = pl.BlockSpec(memory_space=pl.ANY)
    oT = pl.pallas_call(
        kern,
        out_shape=jax.ShapeDtypeStruct((M, S), A_x.dtype),
        in_specs=[hbm] * len(args),
        out_specs=hbm,
        scratch_shapes=[
            pltpu.VMEM((8, S), F32),
            pltpu.VMEM((M, S), BF16),
            pltpu.VMEM((H, M, D), BF16),
            pltpu.VMEM((5, S // 4, DC // 2), U32),
            pltpu.VMEM((2, 7, S // 8, DC // 4), U32),
            pltpu.VMEM((7, 4, 8 * (DC // 4 + 1), L), U32),
            pltpu.VMEM((H, S // 2, D), U32),
            pltpu.VMEM((S // 2, D), U32),
            pltpu.VMEM((S // 2, D), U32),
            pltpu.VMEM((5, S // 4, L), U32),
            pltpu.VMEM((7, H, L, L), U32),
            pltpu.VMEM((M, S), BF16),
            pltpu.VMEM((5, S // 4 + PAD_V, L), U32),
            pltpu.SemaphoreType.DMA((N_SEM,)),
        ],
        compiler_params=pltpu.CompilerParams(vmem_limit_bytes=124 * 1024 * 1024),
    )(*args)
    return jnp.transpose(oT)[None]
```

```python
import math

import jax
import jax.numpy as jnp
import jax.experimental.pallas as pl
import jax.experimental.pallas.tpu as pltpu

F32 = jnp.float32
BF16 = jnp.bfloat16
U32 = jnp.uint32
NT = (((1,), (1,)), ((), ()))

L = 128
TQ = 256
HQ = TQ // 2
RC = 512
NCH = 4

PAD_V = 16

S_X, S_Q0, S_Q1, S_K, S_V, S_C, S_MISC, S_OUT = 0, 4, 8, 12, 16, 20, 24, 30
N_SEM = 38

LOOP_ORDER = ("Q0 Q7 S0 G0 S7 V0 V7 o0 Q6 G3 S6 V6 Q5 G4 S5 V5 Q4 G5 S4 V4 Q3 G6 S3 V3 Q2 G2 S2 V2 "
              "Q1 G1 S1 V1 w0")
FIRST_ORDER = "G0 G3 h0 G2 G4 G6 h1 G5 G1 h2 w0"
LAST_ORDER = "Q7 Q6 Q5 s7 q4 V7 S6 r3 V6 S5 r2 V5 S4 r1 V4 S3 r0 V3 S2 V2 S1 S0 V1 V0"


def _to_u32(x_f32):
    return pltpu.bitcast(x_f32.astype(BF16), U32)


def _shuffled_u32(x_f32):
    return jnp.concatenate([_pack(x_f32[r:r + 8], x_f32[r + 8:r + 16]) for r in range(0, x_f32.shape[0], 16)],
                           axis=0)


def _as_bf16(x_u32):
    return pltpu.bitcast(x_u32, BF16)


def _left(a11, a12, a21, a22):
    return (a11 + a22, a21 + a22, a11, a22, a11 + a12, a21 - a11, a12 - a22)


def _right(b11, b12, b21, b22):
    return (b11 + b22, b11, b12 - b22, b21 - b11, b22, b11 + b12, b21 + b22)


FLAT, DEEP = (0, 1, 3, 4, 6), (2, 5)
O_ORDER = (0, 1, 2, 3, 4, 5, 6)
O2_ORDER = (1, 3, 4, 2, 0, 5, 6)
WO_SPAN = 0.95
SUMS = (0, 2, 3, 5, 6)
QK_LAG = 2
QK_TIE = 0


def _c11(m):
    return (m[0] + m[3]) + (m[6] - m[4])


def _c12(m):
    return m[2] + m[4]


def _c21(m):
    return m[1] + m[3]


def _c22(m):
    return (m[0] - m[1]) + (m[2] + m[5])


def _never(i):
    return jax.lax.broadcasted_iota(jnp.int32, (8, L), 0) < (i >> 10)


def _or_all(xs):
    out = xs[0]
    for x in xs[1:]:
        out = out | x
    return out


def _unpack(w, par):
    return pltpu.unpack_elementwise(w, index=par, packed_dtype=BF16, unpacked_dtype=F32)


def _pack(even, odd):
    return pltpu.bitcast(pltpu.pack_elementwise([even, odd], packed_dtype=BF16), U32)


def _head_weight(ref, h, nrows, pitch):
    sel = ((h >> 3) << 1) + (h & 1)
    r = (h >> 1) & 3
    return jnp.concatenate(
        [_as_bf16(ref[sel, pl.ds((dt * 4 + r) * pitch, nrows), :]) for dt in range(2)], axis=1)


def _kernel(xT_hbm, c_hbm, wq_hbm, wk_hbm, wv_hbm, wo_hbm, wr_hbm, gw_hbm, wg_hbm, wu_hbm, wd_hbm,
            o_hbm,
            g_s, xT_s, wo_s, a_s, a2_s, b_s, q_s, k_s, v_s, k5_s, o_s, v5_s, sem, *, S, M, DC, H, D):
    nq = S // TQ
    mh = M // 2
    pq = mh // 2 + 1
    pb = DC // 4 + 1
    mq = mh // NCH
    mk = DC // NCH
    qscale = (D ** -0.5) * math.log2(math.e)
    neg = -1e9 * math.log2(math.e)
    wo_copy = pltpu.make_async_copy(wo_hbm, wo_s, sem.at[S_MISC + 5])

    def out_copy(j):
        return pltpu.make_async_copy(o_s.at[:, pl.ds(j * TQ, TQ)], o_hbm.at[:, pl.ds(j * TQ, TQ)],
                                     sem.at[S_OUT + j])

    col = jax.lax.broadcasted_iota(jnp.int32, (L, L), 1)
    tri = ((col & ~15) + ((col & 3) << 2) + ((col & 15) >> 2) <= jax.lax.broadcasted_iota(jnp.int32, (L, L), 0))

    def head_program(order, h, hn, never, x7_s, wo_ops=None, span=0.9, hooks=None):
        prods, held, waiting = {}, {}, []

        def spots(v, cols, rows=(0, 64, 128, 192)):
            return [v[r:r + 8, n * L:(n + 1) * L] for n in cols for r in rows]

        def tie(lhs, links, every):
            rows = []
            for rg in range(lhs.shape[0] // 8):
                blk = lhs[rg * 8:(rg + 1) * 8]
                if links and rg % every == 0:
                    blk = jnp.concatenate([jnp.where(never, links.pop(0), blk[:, :L]), blk[:, L:]], axis=1)
                rows.append(blk)
            return jnp.concatenate(rows, axis=0)

        def proj(n):
            w = _head_weight(b_s.at[n], hn, DC // 4, pb)
            links = list(waiting)
            del waiting[:]
            if n in DEEP:
                wf, kh = w.astype(F32), DC // 4
                right = [o.astype(BF16) for o in _right(wf[:kh, :L], wf[:kh, L:], wf[kh:, :L], wf[kh:, L:])]
                right[1], right[4] = w[:kh, :L], w[kh:, L:]
                m, pieces = {}, []

                def sub(x, after):
                    lhs = a2_s[DEEP.index(n), x]
                    mine = [links.pop(0) for _ in links[:2]]
                    if after:
                        t = after[0]
                        for v in after[1:]:
                            t = jnp.maximum(t, v)
                        lhs = tie(lhs, [pltpu.bitcast(jnp.maximum(t[g * 16:g * 16 + 8], t[g * 16 + 8:g * 16 + 16]), U32)
                                        for g in range(S // 64)], 1)
                    elif mine or links:
                        mine += links
                        del links[:]
                        lhs = tie(lhs, mine, lhs.shape[0] // 8 // len(mine))
                    m[x] = jnp.dot(_as_bf16(lhs), right[x], preferred_element_type=F32)
                    pieces.extend(spots(m[x], (0,), range(0, S // 4, 64)))
                sub(1, ()), sub(3, ())
                c21 = m[1] + m[3]
                sub(2, ()), sub(4, (c21,))
                c12, c11, c22 = m[2] + m[4], m[3] - m[4], m[2] - m[1]
                sub(0, ()), sub(5, (c12, c11, c22))
                c11, c22 = c11 + m[0], c22 + (m[0] + m[5])
                sub(6, (c11, c22))
                top = jnp.concatenate([c11 + m[6], c12], axis=1)
                bot = jnp.concatenate([c21, c22], axis=1)
                prods[n] = jnp.concatenate([v[k * L:(k + 1) * L] for k in range(nq // 2) for v in (top, bot)],
                                           axis=0)
            else:
                lhs = a_s[FLAT.index(n)]
                if links:
                    lhs = tie(lhs, links, max(1, lhs.shape[0] // 8 // len(links)))
                prods[n] = jnp.dot(_as_bf16(lhs), w, preferred_element_type=F32)
                pieces = spots(prods[n], (0, 1), range(0, S // 2, 32))
            for key, odd, comb, needs in (("k", 0, _c11, (0, 3, 4, 6)), ("k", 1, _c21, (1, 3)),
                                          ("v", 0, _c12, (2, 4)), ("v", 1, _c22, (0, 1, 2, 5))):
                if n in needs and all(x in prods for x in needs):
                    for k in range(nq // 2):
                        c = comb({x: prods[x][k * TQ:(k + 1) * TQ] for x in needs})
                        held[2 * k + odd, key] = _shuffled_u32(c)
                        if 2 * k + odd < nq - 1:
                            off = (c[:L, L:], c[L:, :L]) if key == "v" else (c[L:, :L], c[:L, L:])
                            ops = _right(c[:L, :L], *off, c[L:, L:])
                            held[2 * k + odd, key + "5"] = [_shuffled_u32(ops[x]) for x in SUMS]
            return pieces

        def write_kv():
            for ch in reversed(range(nq)):
                k_s[ch * HQ:(ch + 1) * HQ, :] = held[ch, "k"]
                v_s[ch * HQ:(ch + 1) * HQ, :] = held[ch, "v"]
                for key, ref in (("k5", k5_s), ("v5", v5_s)):
                    for n, o in enumerate(held.get((ch, key), ())):
                        ref[n, ch * 64:(ch + 1) * 64, :] = o

        def right_operand(n, plain, sums, c0, c1):
            if n == 1:
                return jnp.concatenate([_as_bf16(plain[c * HQ:c * HQ + 64, :L]) for c in range(c0, c1)], axis=0)
            if n == 4:
                return jnp.concatenate([_as_bf16(plain[c * HQ + 64:(c + 1) * HQ, L:]) for c in range(c0, c1)], axis=0)
            return _as_bf16(sums[SUMS.index(n), c0 * 64:c1 * 64, :])

        def qk(i, tied):
            q = qd = q_s[h, i * HQ:(i + 1) * HQ, :]
            n = min(16, len(waiting) - tied + 1) if tied else 0
            if n > 0:
                qd = tie(q, waiting[:n], 16 // n)
                del waiting[:n]
            q, qd = _as_bf16(q), _as_bf16(qd)
            tops, bots, pieces = [], [], []
            if i:
                qf = q.astype(F32)
                left = [o.astype(BF16) for o in _left(qf[:L, :L], qf[:L, L:], qf[L:, :L], qf[L:, L:])]
                left[2], left[3] = q[:L, :L], q[L:, L:]
            done = []
            for c in range(i):
                lhs = dict(enumerate(left))
                if c >= QK_LAG:
                    u = pltpu.bitcast(left[QK_TIE], U32)
                    lhs[QK_TIE] = _as_bf16(jnp.concatenate(
                        [jnp.where(never, done[c - QK_LAG][g], u[g * 8:(g + 1) * 8]) for g in range(8)], axis=0))
                m = {n: jax.lax.dot_general(lhs[n], right_operand(n, k_s, k5_s, c, c + 1), NT,
                                            preferred_element_type=F32) for n in (0, 3, 4, 6, 1, 2, 5)}
                c11, c12, c21, c22 = _c11(m), _c12(m), _c21(m), _c22(m)
                tops += [c11, c12]
                bots += [c21, c22]
                t = jnp.maximum(jnp.maximum(c11, c12), jnp.maximum(c21, c22))
                done.append([pltpu.bitcast(jnp.maximum(t[g * 16:g * 16 + 8], t[g * 16 + 8:(g + 1) * 16]), U32)
                             for g in range(8)])
                for n in (0, 5):
                    pieces += spots(m[n], (0,), (0, 32, 64, 96))
            r0 = i * HQ
            s1 = jax.lax.dot_general(qd, _as_bf16(k_s[r0:r0 + 64, :]), NT, preferred_element_type=F32)
            s2 = jax.lax.dot_general(q[L:], _as_bf16(k_s[r0 + 64:r0 + HQ, :]), NT, preferred_element_type=F32)
            top = jnp.concatenate(tops + [jnp.where(tri, s1[:L], neg)], axis=1)
            bot = jnp.concatenate(bots + [s1[L:], jnp.where(tri, s2, neg)], axis=1)
            return (top, bot), pieces + spots(s1, (0,))

        def softmax(i, top, bot, pieces):
            p, sums, prev = ([], []), ([], []), None
            for k in range(TQ // 8):
                half = k % 2
                s = (top, bot)[half][(k // 2) * 8:(k // 2 + 1) * 8]
                link = pieces[int(span * k * 8 / TQ * len(pieces))]
                if prev is not None:
                    link = jnp.where(never, link, prev)
                m = jnp.broadcast_to(jnp.max(s, axis=1, keepdims=True), (8, L))
                m = jnp.where(never, link, m)
                e = [jnp.exp2(s[:, t:t + L] - m) for t in range(0, s.shape[1], L)]
                prev = e[0]
                for x in e[1:]:
                    prev = prev + x
                sums[half].append(prev)
                p[half].append(jnp.concatenate(e, axis=1))
            pt, pb_ = jnp.concatenate(p[0], axis=0), jnp.concatenate(p[1], axis=0)

            def tile(x, t):
                return x[:, t * L:(t + 1) * L]
            ops = [_left(tile(pt, 2 * c), tile(pt, 2 * c + 1), tile(pb_, 2 * c), tile(pb_, 2 * c + 1))
                   for c in range(i)]
            left = [jnp.concatenate([o[n] for o in ops], axis=1).astype(BF16) for n in range(7)] if i else None
            inv = []
            for x in sums:
                l = jnp.sum(jnp.concatenate(x, axis=0), axis=1, keepdims=True)
                r = pl.reciprocal(l, approx=True)
                inv.append(r * (2.0 - l * r))
            return (left, jnp.concatenate([tile(pt, 2 * i), tile(pb_, 2 * i)], axis=0).astype(BF16),
                    tile(pb_, 2 * i + 1).astype(BF16), inv)

        def pv(i, left, p1, p2, inv):
            r0 = i * HQ
            m, pieces = {}, []
            for n in (2, 3, 0, 4, 1, 5, 6) if i else ():
                m[n] = jnp.dot(left[n], right_operand(n, v_s, v5_s, 0, i), preferred_element_type=F32)
                pieces += spots(m[n], (0,), (0, 32, 64, 96))
            c1 = jnp.dot(p1, _as_bf16(v_s[r0:r0 + 64, :]), preferred_element_type=F32)
            c2 = jnp.dot(p2, _as_bf16(v_s[r0 + 64:r0 + HQ, :]), preferred_element_type=F32)
            top, bot = c1[:L], c1[L:] + c2
            if i:
                top = top + jnp.concatenate([_c11(m), _c12(m)], axis=1)
                bot = bot + jnp.concatenate([_c21(m), _c22(m)], axis=1)
            else:
                pieces = spots(c1, (0, 1))
            top, bot = top * inv[0], bot * inv[1]
            us = [_to_u32(o) for o in _right(top[:, :L], bot[:, :L], top[:, L:], bot[:, L:])]
            for n in range(7):
                x7_s[n, h, i * 64:(i + 1) * 64, :] = us[n]
            waiting.extend(_or_all([us[n][g * 8:(g + 1) * 8] for n in SUMS]) for g in range(8))
            return pieces

        def wo_operands(pieces):
            groups = M // 64
            never2 = jnp.concatenate([never, never], axis=0)
            share = -(-(H // 2) * groups // (H - 1))
            for k in range(share):
                u = jnp.minimum(h * share + k, (H // 2) * groups - 1)
                pair = jax.lax.div(u, groups)
                rg = u - pair * groups
                ops = [_left(*[wo_s[2 * pair + par, pl.ds(pl.multiple_of(hf * mh + sub * (mh // 2) + rg * 16, 16), 16),
                                    ch * L:(ch + 1) * L].astype(F32) for hf in range(2) for ch in range(2)])
                       for sub in range(2) for par in range(2)]
                for n in range(7):
                    link = pieces[int(WO_SPAN * (k * 7 + n) / (share * 7) * len(pieces))]
                    gate = jnp.concatenate([link, link], axis=0)
                    us = [_to_u32(o) for o in _left(*[jnp.where(never2, gate, o[n]) for o in ops])]
                    for x in range(7):
                        wo_ops[n, x, pair, pl.ds(pl.multiple_of(rg * 8, 8), 8), :] = us[x]
                    waiting.append(_or_all(us))

        scores, probs, pieces = {}, {}, []
        for op in order.split():
            i = int(op[1:])
            if op[0] == "G":
                pieces.append(proj(i))
            elif op[0] == "w":
                write_kv()
            elif op[0] == "o":
                wo_operands(pieces[-1])
            elif op[0] in "Qqr":
                scores[i], new = qk(i, {"Q": 0, "q": 1, "r": 9}[op[0]])
                pieces.append(new)
            elif op[0] in "Ss":
                probs[i] = softmax(i, *scores.pop(i), pieces[-1] if op[0] == "S" else pieces[-2] + pieces[-1])
            elif op[0] == "V":
                pieces.append(pv(i, *probs.pop(i)))
            else:
                hooks[i](pieces)

    def phase1(c_s, wq_r, wk_r, wv_r, wg_s, wu_s, wd_s, xa_s, wq0_s, wq1_s, wr_s, gw_s):
        def x_copy(j):
            return pltpu.make_async_copy(xT_hbm.at[:, pl.ds(j * RC, RC)], xT_s.at[:, pl.ds(j * RC, RC)],
                                         sem.at[S_X + j])

        def wq_copy(g, j):
            return pltpu.make_async_copy(wq_hbm.at[:, pl.ds(j * mq, mq), g], wq_r.at[:, pl.ds(j * mq, mq), g],
                                         sem.at[(S_Q1 if g else S_Q0) + j])

        def kv_copies(j):
            return [pltpu.make_async_copy(src.at[pl.ds(j * n, n)], dst.at[pl.ds(j * n, n)], sem.at[s0 + j])
                    for src, dst, s0, n in ((c_hbm, c_s, S_C, RC), (wk_hbm, wk_r, S_K, mk), (wv_hbm, wv_r, S_V, mk))]

        misc = [pltpu.make_async_copy(a, b, sem.at[S_MISC + i]) for i, (a, b) in enumerate(
            [(wr_hbm, wr_s), (gw_hbm, gw_s), (wg_hbm, wg_s), (wu_hbm, wu_s), (wd_hbm, wd_s)])]

        x_copy(0).start()
        for j in range(NCH):
            wq_copy(0, j).start()

        def start_rest():
            for j in range(NCH):
                if j + 1 < NCH:
                    x_copy(j + 1).start()
                wq_copy(1, j).start()
            misc[0].start()
            misc[1].start()
            for j in range(NCH):
                for cp in kv_copies(j):
                    cp.start()
            for cp in misc[2:]:
                cp.start()
            wo_copy.start()

        start_rest()

        def x_operands(j):
            c0 = j * RC if isinstance(j, int) else pl.multiple_of(j * RC, RC)
            r0 = j * HQ if isinstance(j, int) else pl.multiple_of(j * HQ, HQ)
            a = [xT_s[kh * mh:(kh + 1) * mh, pl.ds(c0 + rb * TQ, TQ)].astype(F32)
                 for rb in range(2) for kh in range(2)]
            for n, o in enumerate(_left(*a)):
                xa_s[n, pl.ds(r0, HQ), :] = pltpu.bitcast(o.astype(BF16).T, U32)

        def wq_operands(g, p, never=None, link=None):
            w = [pltpu.bitcast(wq_r[kh, pl.ds(2 * p, 2), g], U32) for kh in range(2)]
            w = [[x[0], x[1]] for x in w]
            if link is not None:
                w[0][0] = jnp.where(never, link, w[0][0])
            rows = [_right(*[_unpack(w[kh][e], par) for kh in range(2) for par in range(2)]) for e in range(2)]
            for n in range(7):
                (wq0_s, wq1_s)[g][n, pl.ds(p, 8, stride=pq), :] = _pack(rows[0][n], rows[1][n])

        x_copy(0).wait()
        x_operands(0)

        def first_half(j, _):
            wq_copy(0, j).wait()
            for k in range(mq // 2):
                wq_operands(0, j * (mq // 2) + k)
            return 0
        jax.lax.fori_loop(0, NCH, first_half, 0)

        def q_step(g, j, side):
            pieces = []
            for r in range(4):
                m = {}
                for n in (0, 3, 4, 6, 1, 2, 5):
                    w = jnp.concatenate([_as_bf16((wq0_s, wq1_s)[g][n, pl.ds((dt * 4 + r) * pq, mh // 2), :])
                                         for dt in range(2)], axis=1)
                    m[n] = jnp.dot(_as_bf16(xa_s[n, pl.ds(pl.multiple_of(j * HQ, HQ), HQ), :]), w,
                                   preferred_element_type=F32)
                    for k in range(5):
                        pieces.append(m[n][k * 48:k * 48 + 8, (k % 2) * L:(k % 2 + 1) * L])
                        side(len(pieces) - 1, pieces[-1])
                for par, rb, comb in ((0, 0, _c11), (0, 1, _c21), (1, 0, _c12), (1, 1, _c22)):
                    r0 = pl.multiple_of(j * TQ + rb * HQ, HQ)
                    q_s[8 * g + 2 * r + par, pl.ds(r0, HQ), :] = _to_u32(comb(m) * qscale)

        def q_lo(j, _):
            never = _never(j)

            def side(k, piece):
                if k == 35:
                    @pl.when(j + 1 < NCH)
                    def _():
                        x_copy(j + 1).wait()
                    wq_copy(1, j).wait()
                if k >= 42 and k % 3 == 0 and (k - 42) // 3 < mq // 2:
                    wq_operands(1, j * (mq // 2) + (k - 42) // 3, never, pltpu.bitcast(piece, U32))
            q_step(0, j, side)
            x_operands((j + 1) & (NCH - 1))
            return 0
        jax.lax.fori_loop(0, NCH, q_lo, 0)

        def q_hi(j, _):
            for cp in kv_copies(j):
                cp.wait()
            never = _never(j)
            quad = []

            def side(kk, piece):
                if kk >= 128:
                    return
                k, g = kk // 2, kk % 2
                link = pltpu.bitcast(piece, U32)
                if g == 0:
                    rg, t = k // 8 + 8 * (k % 4 // 2), k // 4 % 2 + 2 * (k % 2)
                    a = []
                    for rb in range(2):
                        r0 = pl.multiple_of(j * RC + rb * TQ + rg * 16, 16)
                        for ch in range(2):
                            a.append(c_s[pl.ds(r0, 16), (2 * t + ch) * L:(2 * t + ch + 1) * L].astype(F32))
                    a[0] = jnp.where(jnp.concatenate([never, never], axis=0),
                                     jnp.concatenate([piece, piece], axis=0), a[0])
                    ops = _left(*a)
                    us = [_shuffled_u32(ops[n]) for n in FLAT]
                    d0 = pl.multiple_of(j * HQ + rg * 8, 8)
                    for n, u in enumerate(us):
                        a_s[n, pl.ds(d0, 8), t * L:(t + 1) * L] = u
                    quad.append(ops)
                    if len(quad) == 4:
                        d0 = pl.multiple_of(j * (HQ // 2) + (rg - 8) * 8, 8)
                        for e, n in enumerate(DEEP):
                            deep = [_shuffled_u32(o) for o in _left(*[q[n] for q in quad])]
                            for x, u in enumerate(deep):
                                a2_s[e, x, pl.ds(d0, 8), (t - 2) * L:(t - 1) * L] = u
                            us += deep
                        del quad[:]
                    link = _or_all(us)
                c0 = j * mk + 2 * k
                w = [pltpu.bitcast(r[pl.ds(c0 + o, 2), g], U32) for o in (0, L) for r in (wk_r, wv_r)]
                w = [[x[0], x[1]] for x in w]
                w[0][0] = jnp.where(never, link, w[0][0])
                for par in range(2):
                    rows = [_right(*[_unpack(x[e], par) for x in w]) for e in range(2)]
                    for n in range(7):
                        b_s[n, 2 * g + par, pl.ds(j * (mk // 4) + k, 8, stride=pb), :] = _pack(
                            rows[0][n], rows[1][n])
            q_step(1, j, side)
            return j
        never = _never(jax.lax.fori_loop(0, NCH, q_hi, 0))

        for cp in misc:
            cp.wait()
        st = {}

        F = wg_s.shape[1]

        def route(pieces):
            pieces = pieces[-2] + pieces[-1]
            mp = -(-M // L) * L
            cols = []
            for w_s in (wr_s, gw_s):
                w = jnp.concatenate([w_s[...].reshape(1, M).astype(F32), jnp.zeros((1, mp - M), F32)], axis=1)
                cols.append(jnp.broadcast_to(w, (L, mp)).T)
            nr, rows = 4, M // 4
            out, k, prev = ([], []), 0, None
            for ct in range(S // L):
                acc = [None, None]
                for q in range(nr):
                    link = pieces[int((0.03 + 0.65 * k / (nr * S // L)) * len(pieces))]
                    if prev is not None:
                        link = jnp.where(never, link, prev)
                    k += 1
                    x = linked(xT_s[q * rows:(q + 1) * rows, ct * L:(ct + 1) * L], link)
                    for t in range(2):
                        part = fold(x * cols[t][q * rows:(q + 1) * rows], 0)
                        acc[t] = part if acc[t] is None else acc[t] + part
                    prev = acc[0] + acc[1]
                for t in range(2):
                    out[t].append(jnp.sum(acc[t], axis=0, keepdims=True))
            g_s[0:1, :] = jax.nn.sigmoid(jnp.concatenate(out[1], axis=1))
            r = jnp.concatenate(out[0], axis=1).astype(BF16).astype(F32)
            lane = jax.lax.broadcasted_iota(jnp.int32, (1, S), 1)
            m1 = jnp.max(r, axis=1, keepdims=True)
            i1 = jnp.min(jnp.where(r == m1, lane, S - 1), axis=1, keepdims=True)
            r2 = jnp.where(lane == i1, -jnp.inf, r)
            m2 = jnp.max(r2, axis=1, keepdims=True)
            i2 = jnp.min(jnp.where(jnp.logical_and(r2 == m2, lane != i1), lane, S - 1), axis=1, keepdims=True)
            ln = jax.lax.broadcasted_iota(jnp.int32, (M, L), 1)
            st["c0"] = [pl.multiple_of((i[0, 0] >> 7) << 7, L) for i in (i1, i2)]
            st["hit"] = [ln == (i & (L - 1)) for i in (i1, i2)]
            st["r"] = [jax.nn.sigmoid(m1), jax.nn.sigmoid(m2)]
            st["x"] = [jnp.broadcast_to(jnp.sum(jnp.where(hit, xT_s[:, pl.ds(c0, L)].astype(F32), 0.0),
                                                axis=1, keepdims=True), (M, L))
                       for c0, hit in zip(st["c0"], st["hit"])]

        def fold(v, axis_len):
            parts = [v[k * 8:(k + 1) * 8] if axis_len == 0 else v[:, k * L:(k + 1) * L]
                     for k in range(v.shape[axis_len] // (8, L)[axis_len])]
            while len(parts) > 1:
                parts = [parts[k] + parts[k + 1] if k + 1 < len(parts) else parts[k]
                         for k in range(0, len(parts), 2)]
            return parts[0]

        def linked(w, link):
            w = pltpu.bitcast(w, U32)
            reps = (w.shape[0] // 8, w.shape[1] // L)
            w = jnp.where(jnp.tile(never, reps), jnp.tile(pltpu.bitcast(link, U32), reps), w)
            return _as_bf16(w).astype(F32)

        def hidden(pieces):
            pieces = pieces[-3] + pieces[-2] + pieces[-1]
            nr, rows = 4, M // 4
            total = 2 * (F // L) * nr
            out, k, prev = [], 0, None
            for w_s in (wg_s, wu_s):
                cols = ([], [])
                for ct in range(F // L):
                    acc = [None, None]
                    for q in range(nr):
                        link = pieces[int(0.9 * k / total * len(pieces))]
                        if prev is not None:
                            link = jnp.where(never, link, prev)
                        k += 1
                        w = linked(w_s[q * rows:(q + 1) * rows, ct * L:(ct + 1) * L], link)
                        for t in range(2):
                            part = fold(w * st["x"][t][q * rows:(q + 1) * rows], 0)
                            acc[t] = part if acc[t] is None else acc[t] + part
                        prev = acc[0] + acc[1]
                    for t in range(2):
                        cols[t].append(jnp.sum(acc[t], axis=0, keepdims=True))
                out.append([jnp.concatenate(c, axis=1) for c in cols])
            st["h"] = [(jax.nn.silu(out[0][t]) * out[1][t]).astype(BF16).astype(F32) for t in range(2)]

        def patch(pieces):
            pieces = pieces[-2] + pieces[-1]
            half = F // 2
            ys, k, prev = ([], []), 0, None
            for rg in range(M // 16):
                acc = [None, None]
                for hf in range(2):
                    link = pieces[int((0.1 + 0.8 * k / (M // 8)) * len(pieces))]
                    if prev is not None:
                        link = jnp.where(never, link, prev)
                    k += 1
                    w = linked(wd_s[rg * 16:(rg + 1) * 16, hf * half:(hf + 1) * half], link)
                    for t in range(2):
                        part = fold(w * st["h"][t][:, hf * half:(hf + 1) * half], 1)
                        acc[t] = part if acc[t] is None else acc[t] + part
                    prev = fold(acc[0] + acc[1], 0)
                for t in range(2):
                    ys[t].append(jnp.sum(acc[t], axis=1, keepdims=True))
            for t in range(2):
                y = jnp.concatenate(ys[t], axis=0) * st["r"][t]
                blk = xT_s[:, pl.ds(st["c0"][t], L)].astype(F32)
                xT_s[:, pl.ds(st["c0"][t], L)] = (blk + jnp.where(st["hit"][t], y, 0.0)).astype(BF16)

        head_program(FIRST_ORDER, None, 0, never, None, hooks=(route, hidden, patch))

    def phase2(x7_s, wo_ops):
        wo_copy.wait()

        def head(h, _):
            head_program(LOOP_ORDER, h, h + 1, _never(h), x7_s, wo_ops, span=0.96)
            return h
        last = jax.lax.fori_loop(0, H - 1, head, 0)
        head_program(LAST_ORDER, H - 1, None, _never(last), x7_s)

        def out_step(j, _):
            c0 = pl.multiple_of(j * RC, RC)
            m = ({}, {})
            for n in O_ORDER:
                right = [[] for _ in range(7)]
                for pair in range(H // 2):
                    blk = [_as_bf16(x7_s[n, 2 * pair + par, pl.ds(pl.multiple_of(j * L + t * 64, 64), 64), :])
                           for par in range(2) for t in range(2)]
                    ops = list(_right(*[v.astype(F32) for v in blk]))
                    ops[1], ops[4] = blk[0], blk[3]
                    for x in range(7):
                        right[x].append(ops[x])
                mm = {x: jax.lax.dot_general(
                    jnp.concatenate([_as_bf16(wo_ops[n, x, pair, :M // 8]) for pair in range(H // 2)], axis=1),
                    jnp.concatenate(right[x], axis=1).astype(BF16), NT, preferred_element_type=F32) for x in O2_ORDER}
                m[0][n] = jnp.concatenate([_c11(mm), _c21(mm)], axis=0)
                m[1][n] = jnp.concatenate([_c12(mm), _c22(mm)], axis=0)
            for t in range(RC // TQ):
                a = jnp.concatenate([jnp.concatenate([_c11(m[t]), _c12(m[t])], axis=1),
                                     jnp.concatenate([_c21(m[t]), _c22(m[t])], axis=1)], axis=0)
                gj = g_s[0:1, pl.ds(c0 + t * TQ, TQ)]
                b = xT_s[:, pl.ds(c0 + t * TQ, TQ)].astype(F32)
                o_s[:, pl.ds(c0 + t * TQ, TQ)] = (gj * a + (1.0 - gj) * b).astype(BF16)
                out_copy(j * (RC // TQ) + t).start()
            return 0
        jax.lax.fori_loop(0, S // RC, out_step, 0)
        for j in range(nq):
            out_copy(j).wait()

    pl.run_scoped(
        phase1,
        *[pltpu.VMEM(r.shape, r.dtype) for r in (c_hbm, wq_hbm, wk_hbm, wv_hbm, wg_hbm, wu_hbm, wd_hbm)],
        pltpu.VMEM((7, S // 4, mh), U32),
        pltpu.VMEM((7, -(-pq // 4) * 32, L), U32),
        pltpu.VMEM((7, -(-pq // 4) * 32, L), U32),
        pltpu.VMEM((M,), BF16),
        pltpu.VMEM((M,), BF16))
    pl.run_scoped(phase2, pltpu.VMEM((7, H, S // 4, L), U32), pltpu.VMEM((7, 7, H // 2, 64, L), U32))


def _tile_view(w):
    c, h, d = w.shape
    w = w.reshape(c, h // 8, 8, d // L, L).transpose(0, 1, 3, 2, 4)
    return w.reshape(c, h // 8, 8 * (d // L), L)


@jax.jit
def pallas_gated_mix__compressed_kv_cla__moe_arch_mod__prompt_kernel(
    A_x: jax.Array,
    A_c_kv: jax.Array,
    A_w_q: jax.Array,
    A_w_uk: jax.Array,
    A_w_uv: jax.Array,
    A_w_o: jax.Array,
    B_x: jax.Array,
    B_w_r: jax.Array,
    B_w_gate: jax.Array,
    B_w_up: jax.Array,
    B_w_down: jax.Array,
    gate_w: jax.Array,
):
    _, S, M = A_x.shape
    DC = A_c_kv.shape[2]
    H, D = A_w_q.shape[1], A_w_q.shape[2]
    args = (jnp.transpose(A_x[0]), A_c_kv[0], _tile_view(A_w_q).reshape(2, M // 2, 2, 16, L),
            _tile_view(A_w_uk), _tile_view(A_w_uv),
            jnp.transpose(A_w_o, (0, 2, 1)), B_w_r, gate_w, B_w_gate, B_w_up, jnp.transpose(B_w_down))

    def kern(*refs):
        _kernel(*refs, S=S, M=M, DC=DC, H=H, D=D)

    hbm = pl.BlockSpec(memory_space=pl.ANY)
    oT = pl.pallas_call(
        kern,
        out_shape=jax.ShapeDtypeStruct((M, S), A_x.dtype),
        in_specs=[hbm] * len(args),
        out_specs=hbm,
        scratch_shapes=[
            pltpu.VMEM((8, S), F32),
            pltpu.VMEM((M, S), BF16),
            pltpu.VMEM((H, M, D), BF16),
            pltpu.VMEM((5, S // 4, DC // 2), U32),
            pltpu.VMEM((2, 7, S // 8, DC // 4), U32),
            pltpu.VMEM((7, 4, 8 * (DC // 4 + 1), L), U32),
            pltpu.VMEM((H, S // 2, D), U32),
            pltpu.VMEM((S // 2, D), U32),
            pltpu.VMEM((S // 2, D), U32),
            pltpu.VMEM((5, S // 4, L), U32),
            pltpu.VMEM((M, S), BF16),
            pltpu.VMEM((5, S // 4 + PAD_V, L), U32),
            pltpu.SemaphoreType.DMA((N_SEM,)),
        ],
        compiler_params=pltpu.CompilerParams(vmem_limit_bytes=124 * 1024 * 1024),
    )(*args)
    return jnp.transpose(oT)[None]
```

```python
import math

import jax
import jax.numpy as jnp
import jax.experimental.pallas as pl
import jax.experimental.pallas.tpu as pltpu

F32 = jnp.float32
BF16 = jnp.bfloat16
U32 = jnp.uint32
NT = (((1,), (1,)), ((), ()))

L = 128
TQ = 256
HQ = TQ // 2
RC = 512
NCH = 4

PAD_V = 16

S_X, S_Q0, S_Q1, S_K, S_V, S_C, S_MISC, S_OUT = 0, 4, 8, 12, 16, 20, 24, 30
N_SEM = 38

LOOP_ORDER = ("Q0 Q7 S0 G0 S7 V0 V7 o0 Q6 G3 S6 V6 Q5 G4 S5 V5 Q4 G5 S4 V4 Q3 G6 S3 V3 Q2 G2 S2 V2 "
              "Q1 G1 S1 V1 w0")
FIRST_ORDER = "G0 G3 h0 G2 G4 G6 h1 G5 G1 h2 w0"
LAST_ORDER = "Q7 Q6 Q5 t7 V7 S6 Q4 V6 S5 r3 V5 S4 r2 V4 S3 r1 V3 S2 r0 V2 S1 S0 V1 V0"


def _to_u32(x_f32):
    return pltpu.bitcast(x_f32.astype(BF16), U32)


def _shuffled_u32(x_f32):
    return jnp.concatenate([_pack(x_f32[r:r + 8], x_f32[r + 8:r + 16]) for r in range(0, x_f32.shape[0], 16)],
                           axis=0)


def _as_bf16(x_u32):
    return pltpu.bitcast(x_u32, BF16)


def _left(a11, a12, a21, a22):
    return (a11 + a22, a21 + a22, a11, a22, a11 + a12, a21 - a11, a12 - a22)


def _right(b11, b12, b21, b22):
    return (b11 + b22, b11, b12 - b22, b21 - b11, b22, b11 + b12, b21 + b22)


FLAT, DEEP = (0, 1, 3, 4, 6), (2, 5)
O_ORDER = (0, 1, 2, 3, 4, 5, 6)
O2_ORDER = (4, 2, 1, 5, 0, 3, 6)
WO_SPAN = 0.95
SUMS = (0, 2, 3, 5, 6)
QK_LAG = 2
QK_TIE = 0


def _c11(m):
    return (m[0] + m[3]) + (m[6] - m[4])


def _c12(m):
    return m[2] + m[4]


def _c21(m):
    return m[1] + m[3]


def _c22(m):
    return (m[0] - m[1]) + (m[2] + m[5])


def _never(i):
    return jax.lax.broadcasted_iota(jnp.int32, (8, L), 0) < (i >> 10)


def _or_all(xs):
    out = xs[0]
    for x in xs[1:]:
        out = out | x
    return out


def _unpack(w, par):
    return pltpu.unpack_elementwise(w, index=par, packed_dtype=BF16, unpacked_dtype=F32)


def _pack(even, odd):
    return pltpu.bitcast(pltpu.pack_elementwise([even, odd], packed_dtype=BF16), U32)


def _head_weight(ref, h, nrows, pitch):
    sel = ((h >> 3) << 1) + (h & 1)
    r = (h >> 1) & 3
    return jnp.concatenate(
        [_as_bf16(ref[sel, pl.ds((dt * 4 + r) * pitch, nrows), :]) for dt in range(2)], axis=1)


def _kernel(xT_hbm, c_hbm, wq_hbm, wk_hbm, wv_hbm, wo_hbm, wr_hbm, gw_hbm, wg_hbm, wu_hbm, wd_hbm,
            o_hbm,
            g_s, xT_s, wo_s, a_s, a2_s, b_s, q_s, k_s, v_s, k5_s, o_s, v5_s, sem, *, S, M, DC, H, D):
    nq = S // TQ
    mh = M // 2
    pq = mh // 2 + 1
    pb = DC // 4 + 1
    mq = mh // NCH
    mk = DC // NCH
    qscale = (D ** -0.5) * math.log2(math.e)
    neg = -1e9 * math.log2(math.e)
    wo_copy = pltpu.make_async_copy(wo_hbm, wo_s, sem.at[S_MISC + 5])

    def out_copy(j, hf):
        return pltpu.make_async_copy(o_s.at[pl.ds(hf * mh, mh), pl.ds(j * RC, RC)],
                                     o_hbm.at[pl.ds(hf * mh, mh), pl.ds(j * RC, RC)], sem.at[S_OUT + 2 * j + hf])

    col = jax.lax.broadcasted_iota(jnp.int32, (L, L), 1)
    tri = ((col & ~15) + ((col & 3) << 2) + ((col & 15) >> 2) <= jax.lax.broadcasted_iota(jnp.int32, (L, L), 0))

    def head_program(order, h, hn, never, x7_s, wo_ops=None, span=0.9, hooks=None):
        prods, held, waiting = {}, {}, []

        def spots(v, cols, rows=(0, 64, 128, 192)):
            return [v[r:r + 8, n * L:(n + 1) * L] for n in cols for r in rows]

        def tie(lhs, links, every):
            rows = []
            for rg in range(lhs.shape[0] // 8):
                blk = lhs[rg * 8:(rg + 1) * 8]
                if links and rg % every == 0:
                    blk = jnp.concatenate([jnp.where(never, links.pop(0), blk[:, :L]), blk[:, L:]], axis=1)
                rows.append(blk)
            return jnp.concatenate(rows, axis=0)

        def proj(n):
            w = _head_weight(b_s.at[n], hn, DC // 4, pb)
            links = list(waiting)
            del waiting[:]
            if n in DEEP:
                wf, kh = w.astype(F32), DC // 4
                right = [o.astype(BF16) for o in _right(wf[:kh, :L], wf[:kh, L:], wf[kh:, :L], wf[kh:, L:])]
                right[1], right[4] = w[:kh, :L], w[kh:, L:]
                m, pieces = {}, []

                def sub(x, after):
                    lhs = a2_s[DEEP.index(n), x]
                    mine = [links.pop(0) for _ in links[:2]]
                    if after:
                        t = after[0]
                        for v in after[1:]:
                            t = jnp.maximum(t, v)
                        lhs = tie(lhs, [pltpu.bitcast(jnp.maximum(t[g * 16:g * 16 + 8], t[g * 16 + 8:g * 16 + 16]), U32)
                                        for g in range(S // 64)], 1)
                    elif mine or links:
                        mine += links
                        del links[:]
                        lhs = tie(lhs, mine, lhs.shape[0] // 8 // len(mine))
                    m[x] = jnp.dot(_as_bf16(lhs), right[x], preferred_element_type=F32)
                    pieces.extend(spots(m[x], (0,), range(0, S // 4, 64)))
                sub(1, ()), sub(3, ())
                c21 = m[1] + m[3]
                sub(2, ()), sub(4, (c21,))
                c12, c11, c22 = m[2] + m[4], m[3] - m[4], m[2] - m[1]
                sub(0, ()), sub(5, (c12, c11, c22))
                c11, c22 = c11 + m[0], c22 + (m[0] + m[5])
                sub(6, (c11, c22))
                top = jnp.concatenate([c11 + m[6], c12], axis=1)
                bot = jnp.concatenate([c21, c22], axis=1)
                prods[n] = jnp.concatenate([v[k * L:(k + 1) * L] for k in range(nq // 2) for v in (top, bot)],
                                           axis=0)
            else:
                lhs = a_s[FLAT.index(n)]
                if links:
                    lhs = tie(lhs, links, max(1, lhs.shape[0] // 8 // len(links)))
                prods[n] = jnp.dot(_as_bf16(lhs), w, preferred_element_type=F32)
                pieces = spots(prods[n], (0, 1), range(0, S // 2, 32))
            for key, odd, comb, needs in (("k", 0, _c11, (0, 3, 4, 6)), ("k", 1, _c21, (1, 3)),
                                          ("v", 0, _c12, (2, 4)), ("v", 1, _c22, (0, 1, 2, 5))):
                if n in needs and all(x in prods for x in needs):
                    for k in range(nq // 2):
                        c = comb({x: prods[x][k * TQ:(k + 1) * TQ] for x in needs})
                        held[2 * k + odd, key] = _shuffled_u32(c)
                        if 2 * k + odd < nq - 1:
                            off = (c[:L, L:], c[L:, :L]) if key == "v" else (c[L:, :L], c[:L, L:])
                            ops = _right(c[:L, :L], *off, c[L:, L:])
                            held[2 * k + odd, key + "5"] = [_shuffled_u32(ops[x]) for x in SUMS]
            return pieces

        def write_kv():
            for ch in reversed(range(nq)):
                k_s[ch * HQ:(ch + 1) * HQ, :] = held[ch, "k"]
                v_s[ch * HQ:(ch + 1) * HQ, :] = held[ch, "v"]
                for key, ref in (("k5", k5_s), ("v5", v5_s)):
                    for n, o in enumerate(held.get((ch, key), ())):
                        ref[n, ch * 64:(ch + 1) * 64, :] = o

        def right_operand(n, plain, sums, c0, c1):
            if n == 1:
                return jnp.concatenate([_as_bf16(plain[c * HQ:c * HQ + 64, :L]) for c in range(c0, c1)], axis=0)
            if n == 4:
                return jnp.concatenate([_as_bf16(plain[c * HQ + 64:(c + 1) * HQ, L:]) for c in range(c0, c1)], axis=0)
            return _as_bf16(sums[SUMS.index(n), c0 * 64:c1 * 64, :])

        def qk(i, tied):
            q = qd = q_s[h, i * HQ:(i + 1) * HQ, :]
            n = min(16, len(waiting) - tied + 1) if tied else 0
            if n > 0:
                qd = tie(q, waiting[:n], 16 // n)
                del waiting[:n]
            q, qd = _as_bf16(q), _as_bf16(qd)
            tops, bots, pieces = [], [], []
            if i:
                qf = q.astype(F32)
                left = [o.astype(BF16) for o in _left(qf[:L, :L], qf[:L, L:], qf[L:, :L], qf[L:, L:])]
                left[2], left[3] = q[:L, :L], q[L:, L:]
            done = []
            for c in range(i):
                lhs = dict(enumerate(left))
                if c >= QK_LAG:
                    u = pltpu.bitcast(left[QK_TIE], U32)
                    lhs[QK_TIE] = _as_bf16(jnp.concatenate(
                        [jnp.where(never, done[c - QK_LAG][g], u[g * 8:(g + 1) * 8]) for g in range(8)], axis=0))
                m = {n: jax.lax.dot_general(lhs[n], right_operand(n, k_s, k5_s, c, c + 1), NT,
                                            preferred_element_type=F32) for n in (0, 3, 4, 6, 1, 2, 5)}
                c11, c12, c21, c22 = _c11(m), _c12(m), _c21(m), _c22(m)
                tops += [c11, c12]
                bots += [c21, c22]
                t = jnp.maximum(jnp.maximum(c11, c12), jnp.maximum(c21, c22))
                done.append([pltpu.bitcast(jnp.maximum(t[g * 16:g * 16 + 8], t[g * 16 + 8:(g + 1) * 16]), U32)
                             for g in range(8)])
                for n in (0, 5):
                    pieces += spots(m[n], (0,), (0, 32, 64, 96))
            r0 = i * HQ
            s1 = jax.lax.dot_general(qd, _as_bf16(k_s[r0:r0 + 64, :]), NT, preferred_element_type=F32)
            s2 = jax.lax.dot_general(q[L:], _as_bf16(k_s[r0 + 64:r0 + HQ, :]), NT, preferred_element_type=F32)
            top = jnp.concatenate(tops + [jnp.where(tri, s1[:L], neg)], axis=1)
            bot = jnp.concatenate(bots + [s1[L:], jnp.where(tri, s2, neg)], axis=1)
            return (top, bot), pieces + spots(s1, (0,))

        def softmax(i, top, bot, pieces, again=False):
            p, sums, prev = ([], []), ([], []), None
            for k in range(TQ // 8):
                half = k % 2
                s = (top, bot)[half][(k // 2) * 8:(k // 2 + 1) * 8]
                link = pieces[int(span * k * 8 / TQ * len(pieces))]
                if prev is not None:
                    link = jnp.where(never, link, prev)
                m = jnp.broadcast_to(jnp.max(s, axis=1, keepdims=True), (8, L))
                m = jnp.where(never, link, m)
                e = [jnp.exp2(s[:, t:t + L] - m) for t in range(0, s.shape[1], L)]
                prev = e[0]
                for x in e[1:]:
                    prev = prev + x
                if again:
                    m = m + jnp.log2(jnp.sum(prev, axis=1, keepdims=True))
                    e = [jnp.exp2(s[:, t:t + L] - m) for t in range(0, s.shape[1], L)]
                sums[half].append(prev)
                p[half].append(jnp.concatenate(e, axis=1))
            pt, pb_ = jnp.concatenate(p[0], axis=0), jnp.concatenate(p[1], axis=0)

            def tile(x, t):
                return x[:, t * L:(t + 1) * L]
            ops = [_left(tile(pt, 2 * c), tile(pt, 2 * c + 1), tile(pb_, 2 * c), tile(pb_, 2 * c + 1))
                   for c in range(i)]
            left = [jnp.concatenate([o[n] for o in ops], axis=1).astype(BF16) for n in range(7)] if i else None
            inv = []
            for x in () if again else sums:
                l = jnp.sum(jnp.concatenate(x, axis=0), axis=1, keepdims=True)
                r = pl.reciprocal(l, approx=True)
                inv.append(r * (2.0 - l * r))
            return (left, jnp.concatenate([tile(pt, 2 * i), tile(pb_, 2 * i)], axis=0).astype(BF16),
                    tile(pb_, 2 * i + 1).astype(BF16), inv)

        def pv(i, left, p1, p2, inv):
            r0 = i * HQ
            m, pieces = {}, []
            for n in (2, 3, 0, 4, 1, 5, 6) if i else ():
                m[n] = jnp.dot(left[n], right_operand(n, v_s, v5_s, 0, i), preferred_element_type=F32)
                pieces += spots(m[n], (0,), (0, 32, 64, 96))
            c1 = jnp.dot(p1, _as_bf16(v_s[r0:r0 + 64, :]), preferred_element_type=F32)
            c2 = jnp.dot(p2, _as_bf16(v_s[r0 + 64:r0 + HQ, :]), preferred_element_type=F32)
            top, bot = c1[:L], c1[L:] + c2
            if i:
                top = top + jnp.concatenate([_c11(m), _c12(m)], axis=1)
                bot = bot + jnp.concatenate([_c21(m), _c22(m)], axis=1)
            else:
                pieces = spots(c1, (0, 1))
            if inv:
                top, bot = top * inv[0], bot * inv[1]
            us = [_to_u32(o) for o in _right(top[:, :L], bot[:, :L], top[:, L:], bot[:, L:])]
            for n in range(7):
                x7_s[n, h, i * 64:(i + 1) * 64, :] = us[n]
            waiting.extend(_or_all([us[n][g * 8:(g + 1) * 8] for n in SUMS]) for g in range(8))
            return pieces

        def wo_operands(pieces):
            groups = M // 64
            never2 = jnp.concatenate([never, never], axis=0)
            share = -(-(H // 2) * groups // (H - 1))
            for k in range(share):
                u = jnp.minimum(h * share + k, (H // 2) * groups - 1)
                pair = jax.lax.div(u, groups)
                rg = u - pair * groups
                ops = [_left(*[wo_s[2 * pair + par, pl.ds(pl.multiple_of(hf * mh + sub * (mh // 2) + rg * 16, 16), 16),
                                    ch * L:(ch + 1) * L].astype(F32) for hf in range(2) for ch in range(2)])
                       for sub in range(2) for par in range(2)]
                for n in range(7):
                    link = pieces[int(WO_SPAN * (k * 7 + n) / (share * 7) * len(pieces))]
                    gate = jnp.concatenate([link, link], axis=0)
                    us = [_to_u32(o) for o in _left(*[jnp.where(never2, gate, o[n]) for o in ops])]
                    for x in range(7):
                        wo_ops[n, x, pair, pl.ds(pl.multiple_of(rg * 8, 8), 8), :] = us[x]
                    waiting.append(_or_all(us))

        scores, probs, pieces = {}, {}, []
        for op in order.split():
            i = int(op[1:])
            if op[0] == "G":
                pieces.append(proj(i))
            elif op[0] == "w":
                write_kv()
            elif op[0] == "o":
                wo_operands(pieces[-1])
            elif op[0] in "Qqr":
                scores[i], new = qk(i, {"Q": 0, "q": 1, "r": 9}[op[0]])
                pieces.append(new)
            elif op[0] in "SsTt":
                probs[i] = softmax(i, *scores.pop(i), pieces[-1] if op[0] in "ST" else pieces[-2] + pieces[-1],
                                   op[0] in "Tt")
            elif op[0] == "V":
                pieces.append(pv(i, *probs.pop(i)))
            else:
                hooks[i](pieces)

    def phase1(c_s, wq_r, wk_r, wv_r, wg_s, wu_s, wd_s, xa_s, wq0_s, wq1_s, wr_s, gw_s):
        def x_copy(j):
            return pltpu.make_async_copy(xT_hbm.at[:, pl.ds(j * RC, RC)], xT_s.at[:, pl.ds(j * RC, RC)],
                                         sem.at[S_X + j])

        def wq_copy(g, j):
            return pltpu.make_async_copy(wq_hbm.at[:, pl.ds(j * mq, mq), g], wq_r.at[:, pl.ds(j * mq, mq), g],
                                         sem.at[(S_Q1 if g else S_Q0) + j])

        def kv_copies(j):
            return [pltpu.make_async_copy(src.at[pl.ds(j * n, n)], dst.at[pl.ds(j * n, n)], sem.at[s0 + j])
                    for src, dst, s0, n in ((c_hbm, c_s, S_C, RC), (wk_hbm, wk_r, S_K, mk), (wv_hbm, wv_r, S_V, mk))]

        misc = [pltpu.make_async_copy(a, b, sem.at[S_MISC + i]) for i, (a, b) in enumerate(
            [(wr_hbm, wr_s), (gw_hbm, gw_s), (wg_hbm, wg_s), (wu_hbm, wu_s), (wd_hbm, wd_s)])]

        x_copy(0).start()
        for j in range(NCH):
            wq_copy(0, j).start()

        def start_rest():
            for j in range(NCH):
                if j + 1 < NCH:
                    x_copy(j + 1).start()
                wq_copy(1, j).start()
            misc[0].start()
            misc[1].start()
            for j in range(NCH):
                for cp in kv_copies(j):
                    cp.start()
            for cp in misc[2:]:
                cp.start()
            wo_copy.start()

        start_rest()

        def x_operands(j):
            c0 = j * RC if isinstance(j, int) else pl.multiple_of(j * RC, RC)
            r0 = j * HQ if isinstance(j, int) else pl.multiple_of(j * HQ, HQ)
            a = [xT_s[kh * mh:(kh + 1) * mh, pl.ds(c0 + rb * TQ, TQ)].astype(F32)
                 for rb in range(2) for kh in range(2)]
            for n, o in enumerate(_left(*a)):
                xa_s[n, pl.ds(r0, HQ), :] = pltpu.bitcast(o.astype(BF16).T, U32)

        def wq_operands(g, p, never=None, link=None):
            w = [pltpu.bitcast(wq_r[kh, pl.ds(2 * p, 2), g], U32) for kh in range(2)]
            w = [[x[0], x[1]] for x in w]
            if link is not None:
                w[0][0] = jnp.where(never, link, w[0][0])
            rows = [_right(*[_unpack(w[kh][e], par) for kh in range(2) for par in range(2)]) for e in range(2)]
            for n in range(7):
                (wq0_s, wq1_s)[g][n, pl.ds(p, 8, stride=pq), :] = _pack(rows[0][n], rows[1][n])

        x_copy(0).wait()
        x_operands(0)

        def first_half(j, _):
            wq_copy(0, j).wait()
            for k in range(mq // 2):
                wq_operands(0, j * (mq // 2) + k)
            return 0
        jax.lax.fori_loop(0, NCH, first_half, 0)

        def q_step(g, j, side):
            pieces = []
            for r in range(4):
                m = {}
                for n in (0, 3, 4, 6, 1, 2, 5):
                    w = jnp.concatenate([_as_bf16((wq0_s, wq1_s)[g][n, pl.ds((dt * 4 + r) * pq, mh // 2), :])
                                         for dt in range(2)], axis=1)
                    m[n] = jnp.dot(_as_bf16(xa_s[n, pl.ds(pl.multiple_of(j * HQ, HQ), HQ), :]), w,
                                   preferred_element_type=F32)
                    for k in range(5):
                        pieces.append(m[n][k * 48:k * 48 + 8, (k % 2) * L:(k % 2 + 1) * L])
                        side(len(pieces) - 1, pieces[-1])
                for par, rb, comb in ((0, 0, _c11), (0, 1, _c21), (1, 0, _c12), (1, 1, _c22)):
                    r0 = pl.multiple_of(j * TQ + rb * HQ, HQ)
                    q_s[8 * g + 2 * r + par, pl.ds(r0, HQ), :] = _to_u32(comb(m) * qscale)

        def q_lo(j, _):
            never = _never(j)

            def side(k, piece):
                if k == 35:
                    @pl.when(j + 1 < NCH)
                    def _():
                        x_copy(j + 1).wait()
                    wq_copy(1, j).wait()
                if k >= 42 and k % 3 == 0 and (k - 42) // 3 < mq // 2:
                    wq_operands(1, j * (mq // 2) + (k - 42) // 3, never, pltpu.bitcast(piece, U32))
            q_step(0, j, side)
            x_operands((j + 1) & (NCH - 1))
            return 0
        jax.lax.fori_loop(0, NCH, q_lo, 0)

        def q_hi(j, _):
            for cp in kv_copies(j):
                cp.wait()
            never = _never(j)
            quad = []

            def side(kk, piece):
                if kk >= 128:
                    return
                k, g = kk // 2, kk % 2
                link = pltpu.bitcast(piece, U32)
                if g == 0:
                    rg, t = k // 8 + 8 * (k % 4 // 2), k // 4 % 2 + 2 * (k % 2)
                    a = []
                    for rb in range(2):
                        r0 = pl.multiple_of(j * RC + rb * TQ + rg * 16, 16)
                        for ch in range(2):
                            a.append(c_s[pl.ds(r0, 16), (2 * t + ch) * L:(2 * t + ch + 1) * L].astype(F32))
                    a[0] = jnp.where(jnp.concatenate([never, never], axis=0),
                                     jnp.concatenate([piece, piece], axis=0), a[0])
                    ops = _left(*a)
                    us = [_shuffled_u32(ops[n]) for n in FLAT]
                    d0 = pl.multiple_of(j * HQ + rg * 8, 8)
                    for n, u in enumerate(us):
                        a_s[n, pl.ds(d0, 8), t * L:(t + 1) * L] = u
                    quad.append(ops)
                    if len(quad) == 4:
                        d0 = pl.multiple_of(j * (HQ // 2) + (rg - 8) * 8, 8)
                        for e, n in enumerate(DEEP):
                            deep = [_shuffled_u32(o) for o in _left(*[q[n] for q in quad])]
                            for x, u in enumerate(deep):
                                a2_s[e, x, pl.ds(d0, 8), (t - 2) * L:(t - 1) * L] = u
                            us += deep
                        del quad[:]
                    link = _or_all(us)
                c0 = j * mk + 2 * k
                w = [pltpu.bitcast(r[pl.ds(c0 + o, 2), g], U32) for o in (0, L) for r in (wk_r, wv_r)]
                w = [[x[0], x[1]] for x in w]
                w[0][0] = jnp.where(never, link, w[0][0])
                for par in range(2):
                    rows = [_right(*[_unpack(x[e], par) for x in w]) for e in range(2)]
                    for n in range(7):
                        b_s[n, 2 * g + par, pl.ds(j * (mk // 4) + k, 8, stride=pb), :] = _pack(
                            rows[0][n], rows[1][n])
            q_step(1, j, side)
            return j
        never = _never(jax.lax.fori_loop(0, NCH, q_hi, 0))

        for cp in misc:
            cp.wait()
        st = {}

        F = wg_s.shape[1]

        def route(pieces):
            pieces = pieces[-2] + pieces[-1]
            mp = -(-M // L) * L
            cols = []
            for w_s in (wr_s, gw_s):
                w = jnp.concatenate([w_s[...].reshape(1, M).astype(F32), jnp.zeros((1, mp - M), F32)], axis=1)
                cols.append(jnp.broadcast_to(w, (L, mp)).T)
            nr, rows = 4, M // 4
            out, k, prev = ([], []), 0, None
            for ct in range(S // L):
                acc = [None, None]
                for q in range(nr):
                    link = pieces[int((0.03 + 0.65 * k / (nr * S // L)) * len(pieces))]
                    if prev is not None:
                        link = jnp.where(never, link, prev)
                    k += 1
                    x = linked(xT_s[q * rows:(q + 1) * rows, ct * L:(ct + 1) * L], link)
                    for t in range(2):
                        part = fold(x * cols[t][q * rows:(q + 1) * rows], 0)
                        acc[t] = part if acc[t] is None else acc[t] + part
                    prev = acc[0] + acc[1]
                for t in range(2):
                    out[t].append(jnp.sum(acc[t], axis=0, keepdims=True))
            g_s[0:1, :] = jax.nn.sigmoid(jnp.concatenate(out[1], axis=1))
            r = jnp.concatenate(out[0], axis=1).astype(BF16).astype(F32)
            lane = jax.lax.broadcasted_iota(jnp.int32, (1, S), 1)
            m1 = jnp.max(r, axis=1, keepdims=True)
            i1 = jnp.min(jnp.where(r == m1, lane, S - 1), axis=1, keepdims=True)
            r2 = jnp.where(lane == i1, -jnp.inf, r)
            m2 = jnp.max(r2, axis=1, keepdims=True)
            i2 = jnp.min(jnp.where(jnp.logical_and(r2 == m2, lane != i1), lane, S - 1), axis=1, keepdims=True)
            ln = jax.lax.broadcasted_iota(jnp.int32, (M, L), 1)
            st["c0"] = [pl.multiple_of((i[0, 0] >> 7) << 7, L) for i in (i1, i2)]
            st["hit"] = [ln == (i & (L - 1)) for i in (i1, i2)]
            st["r"] = [jax.nn.sigmoid(m1), jax.nn.sigmoid(m2)]
            st["x"] = [jnp.broadcast_to(jnp.sum(jnp.where(hit, xT_s[:, pl.ds(c0, L)].astype(F32), 0.0),
                                                axis=1, keepdims=True), (M, L))
                       for c0, hit in zip(st["c0"], st["hit"])]

        def fold(v, axis_len):
            parts = [v[k * 8:(k + 1) * 8] if axis_len == 0 else v[:, k * L:(k + 1) * L]
                     for k in range(v.shape[axis_len] // (8, L)[axis_len])]
            while len(parts) > 1:
                parts = [parts[k] + parts[k + 1] if k + 1 < len(parts) else parts[k]
                         for k in range(0, len(parts), 2)]
            return parts[0]

        def linked(w, link):
            w = pltpu.bitcast(w, U32)
            reps = (w.shape[0] // 8, w.shape[1] // L)
            w = jnp.where(jnp.tile(never, reps), jnp.tile(pltpu.bitcast(link, U32), reps), w)
            return _as_bf16(w).astype(F32)

        def hidden(pieces):
            pieces = pieces[-3] + pieces[-2] + pieces[-1]
            nr, rows = 4, M // 4
            total = 2 * (F // L) * nr
            out, k, prev = [], 0, None
            for w_s in (wg_s, wu_s):
                cols = ([], [])
                for ct in range(F // L):
                    acc = [None, None]
                    for q in range(nr):
                        link = pieces[int(0.9 * k / total * len(pieces))]
                        if prev is not None:
                            link = jnp.where(never, link, prev)
                        k += 1
                        w = linked(w_s[q * rows:(q + 1) * rows, ct * L:(ct + 1) * L], link)
                        for t in range(2):
                            part = fold(w * st["x"][t][q * rows:(q + 1) * rows], 0)
                            acc[t] = part if acc[t] is None else acc[t] + part
                        prev = acc[0] + acc[1]
                    for t in range(2):
                        cols[t].append(jnp.sum(acc[t], axis=0, keepdims=True))
                out.append([jnp.concatenate(c, axis=1) for c in cols])
            st["h"] = [(jax.nn.silu(out[0][t]) * out[1][t]).astype(BF16).astype(F32) for t in range(2)]

        def patch(pieces):
            pieces = pieces[-2] + pieces[-1]
            half = F // 2
            ys, k, prev = ([], []), 0, None
            for rg in range(M // 16):
                acc = [None, None]
                for hf in range(2):
                    link = pieces[int((0.1 + 0.8 * k / (M // 8)) * len(pieces))]
                    if prev is not None:
                        link = jnp.where(never, link, prev)
                    k += 1
                    w = linked(wd_s[rg * 16:(rg + 1) * 16, hf * half:(hf + 1) * half], link)
                    for t in range(2):
                        part = fold(w * st["h"][t][:, hf * half:(hf + 1) * half], 1)
                        acc[t] = part if acc[t] is None else acc[t] + part
                    prev = fold(acc[0] + acc[1], 0)
                for t in range(2):
                    ys[t].append(jnp.sum(acc[t], axis=1, keepdims=True))
            for t in range(2):
                y = jnp.concatenate(ys[t], axis=0) * st["r"][t]
                blk = xT_s[:, pl.ds(st["c0"][t], L)].astype(F32)
                xT_s[:, pl.ds(st["c0"][t], L)] = (blk + jnp.where(st["hit"][t], y, 0.0)).astype(BF16)

        head_program(FIRST_ORDER, None, 0, never, None, hooks=(route, hidden, patch))

    def phase2(x7_s, wo_ops):
        wo_copy.wait()

        def head(h, _):
            head_program(LOOP_ORDER, h, h + 1, _never(h), x7_s, wo_ops, span=0.96)
            return h
        last = jax.lax.fori_loop(0, H - 1, head, 0)
        head_program(LAST_ORDER, H - 1, None, _never(last), x7_s)

        def out_step(j, _):
            c0 = pl.multiple_of(j * RC, RC)
            m = ({}, {})
            for n in O_ORDER:
                right = [[] for _ in range(7)]
                for pair in range(H // 2):
                    blk = [_as_bf16(x7_s[n, 2 * pair + par, pl.ds(pl.multiple_of(j * L + t * 64, 64), 64), :])
                           for par in range(2) for t in range(2)]
                    ops = list(_right(*[v.astype(F32) for v in blk]))
                    ops[1], ops[4] = blk[0], blk[3]
                    for x in range(7):
                        right[x].append(ops[x])
                mm = {x: jax.lax.dot_general(
                    jnp.concatenate([_as_bf16(wo_ops[n, x, pair, :M // 8]) for pair in range(H // 2)], axis=1),
                    jnp.concatenate(right[x], axis=1).astype(BF16), NT, preferred_element_type=F32) for x in O2_ORDER}
                m[0][n] = jnp.concatenate([((mm[0] + mm[3]) - mm[4]) + mm[6], _c21(mm)], axis=0)
                m[1][n] = jnp.concatenate([_c12(mm), _c22(mm)], axis=0)
            gate = g_s[0:1, pl.ds(c0, RC)]
            for hf in (1, 0):
                rest = (1.0 - gate) * xT_s[hf * mh:(hf + 1) * mh, pl.ds(c0, RC)].astype(F32)
                cols = []
                for t in range(RC // TQ):
                    gl, gr = gate[:, t * TQ:t * TQ + L], gate[:, t * TQ + L:(t + 1) * TQ]
                    rl, rr = rest[:, t * TQ:t * TQ + L], rest[:, t * TQ + L:(t + 1) * TQ]
                    if hf:
                        cols += [gl * _c21(m[t]) + rl, gr * _c22(m[t]) + rr]
                    else:
                        cols += [(gl * ((m[t][0] + m[t][3]) - m[t][4]) + rl) + gl * m[t][6], gr * _c12(m[t]) + rr]
                o_s[hf * mh:(hf + 1) * mh, pl.ds(c0, RC)] = jnp.concatenate(cols, axis=1).astype(BF16)
                out_copy(j, hf).start()
            return 0
        jax.lax.fori_loop(0, S // RC, out_step, 0)
        for j in range(S // RC):
            for hf in range(2):
                out_copy(j, hf).wait()

    pl.run_scoped(
        phase1,
        *[pltpu.VMEM(r.shape, r.dtype) for r in (c_hbm, wq_hbm, wk_hbm, wv_hbm, wg_hbm, wu_hbm, wd_hbm)],
        pltpu.VMEM((7, S // 4, mh), U32),
        pltpu.VMEM((7, -(-pq // 4) * 32, L), U32),
        pltpu.VMEM((7, -(-pq // 4) * 32, L), U32),
        pltpu.VMEM((M,), BF16),
        pltpu.VMEM((M,), BF16))
    pl.run_scoped(phase2, pltpu.VMEM((7, H, S // 4, L), U32), pltpu.VMEM((7, 7, H // 2, 64, L), U32))


def _tile_view(w):
    c, h, d = w.shape
    w = w.reshape(c, h // 8, 8, d // L, L).transpose(0, 1, 3, 2, 4)
    return w.reshape(c, h // 8, 8 * (d // L), L)


@jax.jit
def pallas_gated_mix__compressed_kv_cla__moe_arch_mod__prompt_kernel(
    A_x: jax.Array,
    A_c_kv: jax.Array,
    A_w_q: jax.Array,
    A_w_uk: jax.Array,
    A_w_uv: jax.Array,
    A_w_o: jax.Array,
    B_x: jax.Array,
    B_w_r: jax.Array,
    B_w_gate: jax.Array,
    B_w_up: jax.Array,
    B_w_down: jax.Array,
    gate_w: jax.Array,
):
    _, S, M = A_x.shape
    DC = A_c_kv.shape[2]
    H, D = A_w_q.shape[1], A_w_q.shape[2]
    args = (jnp.transpose(A_x[0]), A_c_kv[0], _tile_view(A_w_q).reshape(2, M // 2, 2, 16, L),
            _tile_view(A_w_uk), _tile_view(A_w_uv),
            jnp.transpose(A_w_o, (0, 2, 1)), B_w_r, gate_w, B_w_gate, B_w_up, jnp.transpose(B_w_down))

    def kern(*refs):
        _kernel(*refs, S=S, M=M, DC=DC, H=H, D=D)

    hbm = pl.BlockSpec(memory_space=pl.ANY)
    oT = pl.pallas_call(
        kern,
        out_shape=jax.ShapeDtypeStruct((M, S), A_x.dtype),
        in_specs=[hbm] * len(args),
        out_specs=hbm,
        scratch_shapes=[
            pltpu.VMEM((8, S), F32),
            pltpu.VMEM((M, S), BF16),
            pltpu.VMEM((H, M, D), BF16),
            pltpu.VMEM((5, S // 4, DC // 2), U32),
            pltpu.VMEM((2, 7, S // 8, DC // 4), U32),
            pltpu.VMEM((7, 4, 8 * (DC // 4 + 1), L), U32),
            pltpu.VMEM((H, S // 2, D), U32),
            pltpu.VMEM((S // 2, D), U32),
            pltpu.VMEM((S // 2, D), U32),
            pltpu.VMEM((5, S // 4, L), U32),
            pltpu.VMEM((M, S), BF16),
            pltpu.VMEM((5, S // 4 + PAD_V, L), U32),
            pltpu.SemaphoreType.DMA((N_SEM,)),
        ],
        compiler_params=pltpu.CompilerParams(vmem_limit_bytes=124 * 1024 * 1024),
    )(*args)
    return jnp.transpose(oT)[None]
```

```python
import math

import jax
import jax.numpy as jnp
import jax.experimental.pallas as pl
import jax.experimental.pallas.tpu as pltpu

F32 = jnp.float32
BF16 = jnp.bfloat16
U32 = jnp.uint32
NT = (((1,), (1,)), ((), ()))

L = 128
TQ = 256
HQ = TQ // 2
RC = 512
NCH = 4

PAD_V = 16

S_X, S_Q0, S_Q1, S_K, S_V, S_C, S_MISC, S_OUT = 0, 4, 8, 12, 16, 20, 24, 30
N_SEM = 38

LOOP_ORDER = ("Q0 Q7 S0 G0 S7 V0 V7 o0 Q6 G3 S6 V6 Q5 G4 S5 V5 Q4 G5 S4 V4 Q3 G6 S3 V3 Q2 G2 S2 V2 "
              "Q1 G1 S1 V1 w0")
FIRST_ORDER = "G0 G3 h0 G2 G4 G6 h1 G5 G1 h2 w0"
LAST_ORDER = "Q7 Q6 Q5 t7 V7 S6 Q4 V6 S5 r3 V5 S4 r2 V4 S3 r1 V3 S2 r0 V2 S1 S0 V1 V0"


def _to_u32(x_f32):
    return pltpu.bitcast(x_f32.astype(BF16), U32)


def _shuffled_u32(x_f32):
    return jnp.concatenate([_pack(x_f32[r:r + 8], x_f32[r + 8:r + 16]) for r in range(0, x_f32.shape[0], 16)],
                           axis=0)


def _as_bf16(x_u32):
    return pltpu.bitcast(x_u32, BF16)


def _left(a11, a12, a21, a22):
    return (a11 + a22, a21 + a22, a11, a22, a11 + a12, a21 - a11, a12 - a22)


def _right(b11, b12, b21, b22):
    return (b11 + b22, b11, b12 - b22, b21 - b11, b22, b11 + b12, b21 + b22)


FLAT, DEEP = (0, 1, 3, 4, 6), (2, 5)
O_ORDER = (0, 1, 2, 3, 4, 5, 6)
O2_ORDER = (4, 2, 1, 5, 0, 3, 6)
WO_SPAN = 0.95
SUMS = (0, 2, 3, 5, 6)
QK_LAG = 2
QK_TIE = 0


def _c11(m):
    return (m[0] + m[3]) + (m[6] - m[4])


def _c12(m):
    return m[2] + m[4]


def _c21(m):
    return m[1] + m[3]


def _c22(m):
    return (m[0] - m[1]) + (m[2] + m[5])


def _never(i):
    return jax.lax.broadcasted_iota(jnp.int32, (8, L), 0) < (i >> 10)


def _or_all(xs):
    out = xs[0]
    for x in xs[1:]:
        out = out | x
    return out


def _unpack(w, par):
    return pltpu.unpack_elementwise(w, index=par, packed_dtype=BF16, unpacked_dtype=F32)


def _pack(even, odd):
    return pltpu.bitcast(pltpu.pack_elementwise([even, odd], packed_dtype=BF16), U32)


def _head_weight(ref, h, nrows, pitch):
    sel = ((h >> 3) << 1) + (h & 1)
    r = (h >> 1) & 3
    return jnp.concatenate(
        [_as_bf16(ref[sel, pl.ds((dt * 4 + r) * pitch, nrows), :]) for dt in range(2)], axis=1)


def _kernel(xT_hbm, c_hbm, wq_hbm, wk_hbm, wv_hbm, wo_hbm, wr_hbm, gw_hbm, wg_hbm, wu_hbm, wd_hbm,
            o_hbm,
            g_s, xT_s, wo_s, a_s, a2_s, b_s, q_s, k_s, v_s, k5_s, o_s, v5_s, sem, *, S, M, DC, H, D):
    nq = S // TQ
    mh = M // 2
    pq = mh // 2 + 1
    pb = DC // 4 + 1
    mq = mh // NCH
    mk = DC // NCH
    qscale = (D ** -0.5) * math.log2(math.e)
    neg = -1e9 * math.log2(math.e)
    wo_copy = pltpu.make_async_copy(wo_hbm, wo_s, sem.at[S_MISC + 5])

    def out_copy(j, hf):
        return pltpu.make_async_copy(o_s.at[pl.ds(hf * mh, mh), pl.ds(j * RC, RC)],
                                     o_hbm.at[pl.ds(hf * mh, mh), pl.ds(j * RC, RC)], sem.at[S_OUT + 2 * j + hf])

    def head_program(order, h, hn, never, x7_s=None, tri=None, wo_ops=None, span=0.9, hooks=None):
        prods, held, waiting = {}, {}, []

        def spots(v, cols, rows=(0, 64, 128, 192)):
            return [v[r:r + 8, n * L:(n + 1) * L] for n in cols for r in rows]

        def tie(lhs, links, every):
            rows = []
            for rg in range(lhs.shape[0] // 8):
                blk = lhs[rg * 8:(rg + 1) * 8]
                if links and rg % every == 0:
                    blk = jnp.concatenate([jnp.where(never, links.pop(0), blk[:, :L]), blk[:, L:]], axis=1)
                rows.append(blk)
            return jnp.concatenate(rows, axis=0)

        def proj(n):
            w = _head_weight(b_s.at[n], hn, DC // 4, pb)
            links = list(waiting)
            del waiting[:]
            if n in DEEP:
                wf, kh = w.astype(F32), DC // 4
                right = [o.astype(BF16) for o in _right(wf[:kh, :L], wf[:kh, L:], wf[kh:, :L], wf[kh:, L:])]
                right[1], right[4] = w[:kh, :L], w[kh:, L:]
                m, pieces = {}, []

                def sub(x, after):
                    lhs = a2_s[DEEP.index(n), x]
                    mine = [links.pop(0) for _ in links[:2]]
                    if after:
                        t = after[0]
                        for v in after[1:]:
                            t = jnp.maximum(t, v)
                        lhs = tie(lhs, [pltpu.bitcast(jnp.maximum(t[g * 16:g * 16 + 8], t[g * 16 + 8:g * 16 + 16]), U32)
                                        for g in range(S // 64)], 1)
                    elif mine or links:
                        mine += links
                        del links[:]
                        lhs = tie(lhs, mine, lhs.shape[0] // 8 // len(mine))
                    m[x] = jnp.dot(_as_bf16(lhs), right[x], preferred_element_type=F32)
                    pieces.extend(spots(m[x], (0,), range(0, S // 4, 64)))
                sub(1, ()), sub(3, ())
                c21 = m[1] + m[3]
                sub(2, ()), sub(4, (c21,))
                c12, c11, c22 = m[2] + m[4], m[3] - m[4], m[2] - m[1]
                sub(0, ()), sub(5, (c12, c11, c22))
                c11, c22 = c11 + m[0], c22 + (m[0] + m[5])
                sub(6, (c11, c22))
                top = jnp.concatenate([c11 + m[6], c12], axis=1)
                bot = jnp.concatenate([c21, c22], axis=1)
                prods[n] = jnp.concatenate([v[k * L:(k + 1) * L] for k in range(nq // 2) for v in (top, bot)],
                                           axis=0)
            else:
                lhs = a_s[FLAT.index(n)]
                if links:
                    lhs = tie(lhs, links, max(1, lhs.shape[0] // 8 // len(links)))
                prods[n] = jnp.dot(_as_bf16(lhs), w, preferred_element_type=F32)
                pieces = spots(prods[n], (0, 1), range(0, S // 2, 32))
            for key, odd, comb, needs in (("k", 0, _c11, (0, 3, 4, 6)), ("k", 1, _c21, (1, 3)),
                                          ("v", 0, _c12, (2, 4)), ("v", 1, _c22, (0, 1, 2, 5))):
                if n in needs and all(x in prods for x in needs):
                    for k in range(nq // 2):
                        c = comb({x: prods[x][k * TQ:(k + 1) * TQ] for x in needs})
                        held[2 * k + odd, key] = _shuffled_u32(c)
                        if 2 * k + odd < nq - 1:
                            off = (c[:L, L:], c[L:, :L]) if key == "v" else (c[L:, :L], c[:L, L:])
                            ops = _right(c[:L, :L], *off, c[L:, L:])
                            held[2 * k + odd, key + "5"] = [_shuffled_u32(ops[x]) for x in SUMS]
            return pieces

        def write_kv():
            for ch in reversed(range(nq)):
                k_s[ch * HQ:(ch + 1) * HQ, :] = held[ch, "k"]
                v_s[ch * HQ:(ch + 1) * HQ, :] = held[ch, "v"]
                for key, ref in (("k5", k5_s), ("v5", v5_s)):
                    for n, o in enumerate(held.get((ch, key), ())):
                        ref[n, ch * 64:(ch + 1) * 64, :] = o

        def right_operand(n, plain, sums, c0, c1):
            if n == 1:
                return jnp.concatenate([_as_bf16(plain[c * HQ:c * HQ + 64, :L]) for c in range(c0, c1)], axis=0)
            if n == 4:
                return jnp.concatenate([_as_bf16(plain[c * HQ + 64:(c + 1) * HQ, L:]) for c in range(c0, c1)], axis=0)
            return _as_bf16(sums[SUMS.index(n), c0 * 64:c1 * 64, :])

        def qk(i, tied):
            q = qd = q_s[h, i * HQ:(i + 1) * HQ, :]
            n = min(16, len(waiting) - tied + 1) if tied else 0
            if n > 0:
                qd = tie(q, waiting[:n], 16 // n)
                del waiting[:n]
            q, qd = _as_bf16(q), _as_bf16(qd)
            tops, bots, pieces = [], [], []
            if i:
                qf = q.astype(F32)
                left = [o.astype(BF16) for o in _left(qf[:L, :L], qf[:L, L:], qf[L:, :L], qf[L:, L:])]
                left[2], left[3] = q[:L, :L], q[L:, L:]
            done = []
            for c in range(i):
                lhs = dict(enumerate(left))
                if c >= QK_LAG:
                    u = pltpu.bitcast(left[QK_TIE], U32)
                    lhs[QK_TIE] = _as_bf16(jnp.concatenate(
                        [jnp.where(never, done[c - QK_LAG][g], u[g * 8:(g + 1) * 8]) for g in range(8)], axis=0))
                m = {n: jax.lax.dot_general(lhs[n], right_operand(n, k_s, k5_s, c, c + 1), NT,
                                            preferred_element_type=F32) for n in (0, 3, 4, 6, 1, 2, 5)}
                c11, c12, c21, c22 = _c11(m), _c12(m), _c21(m), _c22(m)
                tops += [c11, c12]
                bots += [c21, c22]
                t = jnp.maximum(jnp.maximum(c11, c12), jnp.maximum(c21, c22))
                done.append([pltpu.bitcast(jnp.maximum(t[g * 16:g * 16 + 8], t[g * 16 + 8:(g + 1) * 16]), U32)
                             for g in range(8)])
                for n in (0, 5):
                    pieces += spots(m[n], (0,), (0, 32, 64, 96))
            r0 = i * HQ
            s1 = jax.lax.dot_general(qd, _as_bf16(k_s[r0:r0 + 64, :]), NT, preferred_element_type=F32)
            s2 = jax.lax.dot_general(q[L:], _as_bf16(k_s[r0 + 64:r0 + HQ, :]), NT, preferred_element_type=F32)
            top = jnp.concatenate(tops + [jnp.where(tri, s1[:L], neg)], axis=1)
            bot = jnp.concatenate(bots + [s1[L:], jnp.where(tri, s2, neg)], axis=1)
            return (top, bot), pieces + spots(s1, (0,))

        def softmax(i, top, bot, pieces, again=False):
            p, sums, prev = ([], []), ([], []), None
            for k in range(TQ // 8):
                half = k % 2
                s = (top, bot)[half][(k // 2) * 8:(k // 2 + 1) * 8]
                link = pieces[int(span * k * 8 / TQ * len(pieces))]
                if prev is not None:
                    link = jnp.where(never, link, prev)
                m = jnp.broadcast_to(jnp.max(s, axis=1, keepdims=True), (8, L))
                m = jnp.where(never, link, m)
                e = [jnp.exp2(s[:, t:t + L] - m) for t in range(0, s.shape[1], L)]
                prev = e[0]
                for x in e[1:]:
                    prev = prev + x
                if again:
                    m = m + jnp.log2(jnp.sum(prev, axis=1, keepdims=True))
                    e = [jnp.exp2(s[:, t:t + L] - m) for t in range(0, s.shape[1], L)]
                sums[half].append(prev)
                p[half].append(jnp.concatenate(e, axis=1))
            pt, pb_ = jnp.concatenate(p[0], axis=0), jnp.concatenate(p[1], axis=0)

            def tile(x, t):
                return x[:, t * L:(t + 1) * L]
            ops = [_left(tile(pt, 2 * c), tile(pt, 2 * c + 1), tile(pb_, 2 * c), tile(pb_, 2 * c + 1))
                   for c in range(i)]
            left = [jnp.concatenate([o[n] for o in ops], axis=1).astype(BF16) for n in range(7)] if i else None
            inv = []
            for x in () if again else sums:
                l = jnp.sum(jnp.concatenate(x, axis=0), axis=1, keepdims=True)
                r = pl.reciprocal(l, approx=True)
                inv.append(r * (2.0 - l * r))
            return (left, jnp.concatenate([tile(pt, 2 * i), tile(pb_, 2 * i)], axis=0).astype(BF16),
                    tile(pb_, 2 * i + 1).astype(BF16), inv)

        def pv(i, left, p1, p2, inv):
            r0 = i * HQ
            m, pieces = {}, []
            for n in (2, 3, 0, 4, 1, 5, 6) if i else ():
                m[n] = jnp.dot(left[n], right_operand(n, v_s, v5_s, 0, i), preferred_element_type=F32)
                pieces += spots(m[n], (0,), (0, 32, 64, 96))
            c1 = jnp.dot(p1, _as_bf16(v_s[r0:r0 + 64, :]), preferred_element_type=F32)
            c2 = jnp.dot(p2, _as_bf16(v_s[r0 + 64:r0 + HQ, :]), preferred_element_type=F32)
            top, bot = c1[:L], c1[L:] + c2
            if i:
                top = top + jnp.concatenate([_c11(m), _c12(m)], axis=1)
                bot = bot + jnp.concatenate([_c21(m), _c22(m)], axis=1)
            else:
                pieces = spots(c1, (0, 1))
            if inv:
                top, bot = top * inv[0], bot * inv[1]
            us = [_to_u32(o) for o in _right(top[:, :L], bot[:, :L], top[:, L:], bot[:, L:])]
            for n in range(7):
                x7_s[n, h, i * 64:(i + 1) * 64, :] = us[n]
            waiting.extend(_or_all([us[n][g * 8:(g + 1) * 8] for n in SUMS]) for g in range(8))
            return pieces

        def wo_operands(pieces):
            groups = M // 64
            never2 = jnp.concatenate([never, never], axis=0)
            share = -(-(H // 2) * groups // (H - 1))
            for k in range(share):
                u = jnp.minimum(h * share + k, (H // 2) * groups - 1)
                pair = jax.lax.div(u, groups)
                rg = u - pair * groups
                ops = [_left(*[wo_s[2 * pair + par, pl.ds(pl.multiple_of(hf * mh + sub * (mh // 2) + rg * 16, 16), 16),
                                    ch * L:(ch + 1) * L].astype(F32) for hf in range(2) for ch in range(2)])
                       for sub in range(2) for par in range(2)]
                for n in range(7):
                    link = pieces[int(WO_SPAN * (k * 7 + n) / (share * 7) * len(pieces))]
                    gate = jnp.concatenate([link, link], axis=0)
                    us = [_to_u32(o) for o in _left(*[jnp.where(never2, gate, o[n]) for o in ops])]
                    for x in range(7):
                        wo_ops[n, x, pair, pl.ds(pl.multiple_of(rg * 8, 8), 8), :] = us[x]
                    waiting.append(_or_all(us))

        scores, probs, pieces = {}, {}, []
        for op in order.split():
            i = int(op[1:])
            if op[0] == "G":
                pieces.append(proj(i))
            elif op[0] == "w":
                write_kv()
            elif op[0] == "o":
                wo_operands(pieces[-1])
            elif op[0] in "Qqr":
                scores[i], new = qk(i, {"Q": 0, "q": 1, "r": 9}[op[0]])
                pieces.append(new)
            elif op[0] in "SsTt":
                probs[i] = softmax(i, *scores.pop(i), pieces[-1] if op[0] in "ST" else pieces[-2] + pieces[-1],
                                   op[0] in "Tt")
            elif op[0] == "V":
                pieces.append(pv(i, *probs.pop(i)))
            else:
                hooks[i](pieces)

    def phase1(c_s, wq_r, wk_r, wv_r, wg_s, wu_s, wd_s, xa_s, wq0_s, wq1_s, wr_s, gw_s):
        def x_copy(j):
            return pltpu.make_async_copy(xT_hbm.at[:, pl.ds(j * RC, RC)], xT_s.at[:, pl.ds(j * RC, RC)],
                                         sem.at[S_X + j])

        def wq_copy(g, j):
            return pltpu.make_async_copy(wq_hbm.at[:, pl.ds(j * mq, mq), g], wq_r.at[:, pl.ds(j * mq, mq), g],
                                         sem.at[(S_Q1 if g else S_Q0) + j])

        def kv_copies(j):
            return [pltpu.make_async_copy(src.at[pl.ds(j * n, n)], dst.at[pl.ds(j * n, n)], sem.at[s0 + j])
                    for src, dst, s0, n in ((c_hbm, c_s, S_C, RC), (wk_hbm, wk_r, S_K, mk), (wv_hbm, wv_r, S_V, mk))]

        misc = [pltpu.make_async_copy(a, b, sem.at[S_MISC + i]) for i, (a, b) in enumerate(
            [(wr_hbm, wr_s), (gw_hbm, gw_s), (wg_hbm, wg_s), (wu_hbm, wu_s), (wd_hbm, wd_s)])]

        x_copy(0).start()
        for j in range(NCH):
            wq_copy(0, j).start()

        def start_rest():
            for j in range(NCH):
                if j + 1 < NCH:
                    x_copy(j + 1).start()
                wq_copy(1, j).start()
            misc[0].start()
            misc[1].start()
            for j in range(NCH):
                for cp in kv_copies(j):
                    cp.start()
            for cp in misc[2:]:
                cp.start()
            wo_copy.start()

        start_rest()

        def x_operands(j):
            c0 = j * RC if isinstance(j, int) else pl.multiple_of(j * RC, RC)
            r0 = j * HQ if isinstance(j, int) else pl.multiple_of(j * HQ, HQ)
            a = [xT_s[kh * mh:(kh + 1) * mh, pl.ds(c0 + rb * TQ, TQ)].astype(F32)
                 for rb in range(2) for kh in range(2)]
            for n, o in enumerate(_left(*a)):
                xa_s[n, pl.ds(r0, HQ), :] = pltpu.bitcast(o.astype(BF16).T, U32)

        def wq_operands(g, p, never=None, link=None):
            w = [pltpu.bitcast(wq_r[kh, pl.ds(2 * p, 2), g], U32) for kh in range(2)]
            w = [[x[0], x[1]] for x in w]
            if link is not None:
                w[0][0] = jnp.where(never, link, w[0][0])
            rows = [_right(*[_unpack(w[kh][e], par) for kh in range(2) for par in range(2)]) for e in range(2)]
            for n in range(7):
                (wq0_s, wq1_s)[g][n, pl.ds(p, 8, stride=pq), :] = _pack(rows[0][n], rows[1][n])

        x_copy(0).wait()
        x_operands(0)

        def first_half(j, _):
            wq_copy(0, j).wait()
            for k in range(mq // 2):
                wq_operands(0, j * (mq // 2) + k)
            return 0
        jax.lax.fori_loop(0, NCH, first_half, 0)

        def q_step(g, j, side):
            pieces = []
            for r in range(4):
                m = {}
                for n in (0, 3, 4, 6, 1, 2, 5):
                    w = jnp.concatenate([_as_bf16((wq0_s, wq1_s)[g][n, pl.ds((dt * 4 + r) * pq, mh // 2), :])
                                         for dt in range(2)], axis=1)
                    m[n] = jnp.dot(_as_bf16(xa_s[n, pl.ds(pl.multiple_of(j * HQ, HQ), HQ), :]), w,
                                   preferred_element_type=F32)
                    for k in range(5):
                        pieces.append(m[n][k * 48:k * 48 + 8, (k % 2) * L:(k % 2 + 1) * L])
                        side(len(pieces) - 1, pieces[-1])
                for par, rb, comb in ((0, 0, _c11), (0, 1, _c21), (1, 0, _c12), (1, 1, _c22)):
                    r0 = pl.multiple_of(j * TQ + rb * HQ, HQ)
                    q_s[8 * g + 2 * r + par, pl.ds(r0, HQ), :] = _to_u32(comb(m) * qscale)

        def q_lo(j, _):
            never = _never(j)

            def side(k, piece):
                if k == 35:
                    @pl.when(j + 1 < NCH)
                    def _():
                        x_copy(j + 1).wait()
                    wq_copy(1, j).wait()
                if k >= 42 and k % 3 == 0 and (k - 42) // 3 < mq // 2:
                    wq_operands(1, j * (mq // 2) + (k - 42) // 3, never, pltpu.bitcast(piece, U32))
            q_step(0, j, side)
            x_operands((j + 1) & (NCH - 1))
            return 0
        jax.lax.fori_loop(0, NCH, q_lo, 0)

        def q_hi(j, _):
            for cp in kv_copies(j):
                cp.wait()
            never = _never(j)
            quad = []

            def side(kk, piece):
                if kk >= 128:
                    return
                k, g = kk // 2, kk % 2
                link = pltpu.bitcast(piece, U32)
                if g == 0:
                    rg, t = k // 8 + 8 * (k % 4 // 2), k // 4 % 2 + 2 * (k % 2)
                    a = []
                    for rb in range(2):
                        r0 = pl.multiple_of(j * RC + rb * TQ + rg * 16, 16)
                        for ch in range(2):
                            a.append(c_s[pl.ds(r0, 16), (2 * t + ch) * L:(2 * t + ch + 1) * L].astype(F32))
                    a[0] = jnp.where(jnp.concatenate([never, never], axis=0),
                                     jnp.concatenate([piece, piece], axis=0), a[0])
                    ops = _left(*a)
                    us = [_shuffled_u32(ops[n]) for n in FLAT]
                    d0 = pl.multiple_of(j * HQ + rg * 8, 8)
                    for n, u in enumerate(us):
                        a_s[n, pl.ds(d0, 8), t * L:(t + 1) * L] = u
                    quad.append(ops)
                    if len(quad) == 4:
                        d0 = pl.multiple_of(j * (HQ // 2) + (rg - 8) * 8, 8)
                        for e, n in enumerate(DEEP):
                            deep = [_shuffled_u32(o) for o in _left(*[q[n] for q in quad])]
                            for x, u in enumerate(deep):
                                a2_s[e, x, pl.ds(d0, 8), (t - 2) * L:(t - 1) * L] = u
                            us += deep
                        del quad[:]
                    link = _or_all(us)
                c0 = j * mk + 2 * k
                w = [pltpu.bitcast(r[pl.ds(c0 + o, 2), g], U32) for o in (0, L) for r in (wk_r, wv_r)]
                w = [[x[0], x[1]] for x in w]
                w[0][0] = jnp.where(never, link, w[0][0])
                for par in range(2):
                    rows = [_right(*[_unpack(x[e], par) for x in w]) for e in range(2)]
                    for n in range(7):
                        b_s[n, 2 * g + par, pl.ds(j * (mk // 4) + k, 8, stride=pb), :] = _pack(
                            rows[0][n], rows[1][n])
            q_step(1, j, side)
            return j
        never = _never(jax.lax.fori_loop(0, NCH, q_hi, 0))

        for cp in misc:
            cp.wait()
        st = {}

        F = wg_s.shape[1]

        def route(pieces):
            pieces = pieces[-2] + pieces[-1]
            mp = -(-M // L) * L
            cols = []
            for w_s in (wr_s, gw_s):
                w = jnp.concatenate([w_s[...].reshape(1, M).astype(F32), jnp.zeros((1, mp - M), F32)], axis=1)
                cols.append(jnp.broadcast_to(w, (L, mp)).T)
            nr, rows = 4, M // 4
            out, k, prev = ([], []), 0, None
            for ct in range(S // L):
                acc = [None, None]
                for q in range(nr):
                    link = pieces[int((0.03 + 0.65 * k / (nr * S // L)) * len(pieces))]
                    if prev is not None:
                        link = jnp.where(never, link, prev)
                    k += 1
                    x = linked(xT_s[q * rows:(q + 1) * rows, ct * L:(ct + 1) * L], link)
                    for t in range(2):
                        part = fold(x * cols[t][q * rows:(q + 1) * rows], 0)
                        acc[t] = part if acc[t] is None else acc[t] + part
                    prev = acc[0] + acc[1]
                for t in range(2):
                    out[t].append(jnp.sum(acc[t], axis=0, keepdims=True))
            g_s[0:1, :] = jax.nn.sigmoid(jnp.concatenate(out[1], axis=1))
            r = jnp.concatenate(out[0], axis=1).astype(BF16).astype(F32)
            lane = jax.lax.broadcasted_iota(jnp.int32, (1, S), 1)
            m1 = jnp.max(r, axis=1, keepdims=True)
            i1 = jnp.min(jnp.where(r == m1, lane, S - 1), axis=1, keepdims=True)
            r2 = jnp.where(lane == i1, -jnp.inf, r)
            m2 = jnp.max(r2, axis=1, keepdims=True)
            i2 = jnp.min(jnp.where(jnp.logical_and(r2 == m2, lane != i1), lane, S - 1), axis=1, keepdims=True)
            ln = jax.lax.broadcasted_iota(jnp.int32, (M, L), 1)
            st["c0"] = [pl.multiple_of((i[0, 0] >> 7) << 7, L) for i in (i1, i2)]
            st["hit"] = [ln == (i & (L - 1)) for i in (i1, i2)]
            st["r"] = [jax.nn.sigmoid(m1), jax.nn.sigmoid(m2)]
            st["x"] = [jnp.broadcast_to(jnp.sum(jnp.where(hit, xT_s[:, pl.ds(c0, L)].astype(F32), 0.0),
                                                axis=1, keepdims=True), (M, L))
                       for c0, hit in zip(st["c0"], st["hit"])]

        def fold(v, axis_len):
            parts = [v[k * 8:(k + 1) * 8] if axis_len == 0 else v[:, k * L:(k + 1) * L]
                     for k in range(v.shape[axis_len] // (8, L)[axis_len])]
            while len(parts) > 1:
                parts = [parts[k] + parts[k + 1] if k + 1 < len(parts) else parts[k]
                         for k in range(0, len(parts), 2)]
            return parts[0]

        def linked(w, link):
            w = pltpu.bitcast(w, U32)
            reps = (w.shape[0] // 8, w.shape[1] // L)
            w = jnp.where(jnp.tile(never, reps), jnp.tile(pltpu.bitcast(link, U32), reps), w)
            return _as_bf16(w).astype(F32)

        def hidden(pieces):
            pieces = pieces[-3] + pieces[-2] + pieces[-1]
            nr, rows = 4, M // 4
            total = 2 * (F // L) * nr
            out, k, prev = [], 0, None
            for w_s in (wg_s, wu_s):
                cols = ([], [])
                for ct in range(F // L):
                    acc = [None, None]
                    for q in range(nr):
                        link = pieces[int(0.9 * k / total * len(pieces))]
                        if prev is not None:
                            link = jnp.where(never, link, prev)
                        k += 1
                        w = linked(w_s[q * rows:(q + 1) * rows, ct * L:(ct + 1) * L], link)
                        for t in range(2):
                            part = fold(w * st["x"][t][q * rows:(q + 1) * rows], 0)
                            acc[t] = part if acc[t] is None else acc[t] + part
                        prev = acc[0] + acc[1]
                    for t in range(2):
                        cols[t].append(jnp.sum(acc[t], axis=0, keepdims=True))
                out.append([jnp.concatenate(c, axis=1) for c in cols])
            st["h"] = [(jax.nn.silu(out[0][t]) * out[1][t]).astype(BF16).astype(F32) for t in range(2)]

        def patch(pieces):
            pieces = pieces[-2] + pieces[-1]
            half = F // 2
            ys, k, prev = ([], []), 0, None
            for rg in range(M // 16):
                acc = [None, None]
                for hf in range(2):
                    link = pieces[int((0.1 + 0.8 * k / (M // 8)) * len(pieces))]
                    if prev is not None:
                        link = jnp.where(never, link, prev)
                    k += 1
                    w = linked(wd_s[rg * 16:(rg + 1) * 16, hf * half:(hf + 1) * half], link)
                    for t in range(2):
                        part = fold(w * st["h"][t][:, hf * half:(hf + 1) * half], 1)
                        acc[t] = part if acc[t] is None else acc[t] + part
                    prev = fold(acc[0] + acc[1], 0)
                for t in range(2):
                    ys[t].append(jnp.sum(acc[t], axis=1, keepdims=True))
            for t in range(2):
                y = jnp.concatenate(ys[t], axis=0) * st["r"][t]
                blk = xT_s[:, pl.ds(st["c0"][t], L)].astype(F32)
                xT_s[:, pl.ds(st["c0"][t], L)] = (blk + jnp.where(st["hit"][t], y, 0.0)).astype(BF16)

        head_program(FIRST_ORDER, None, 0, never, hooks=(route, hidden, patch))

    def phase2(x7_s, wo_ops):
        wo_copy.wait()
        col = jax.lax.broadcasted_iota(jnp.int32, (L, L), 1)
        tri = ((col & ~15) + ((col & 3) << 2) + ((col & 15) >> 2)
               <= jax.lax.broadcasted_iota(jnp.int32, (L, L), 0))

        def head(h, _):
            head_program(LOOP_ORDER, h, h + 1, _never(h), x7_s, tri, wo_ops, span=0.96)
            return h
        last = jax.lax.fori_loop(0, H - 1, head, 0)
        head_program(LAST_ORDER, H - 1, None, _never(last), x7_s, tri)

        def out_step(j, _):
            c0 = pl.multiple_of(j * RC, RC)
            m = ({}, {})
            for n in O_ORDER:
                right = [[] for _ in range(7)]
                for pair in range(H // 2):
                    blk = [_as_bf16(x7_s[n, 2 * pair + par, pl.ds(pl.multiple_of(j * L + t * 64, 64), 64), :])
                           for par in range(2) for t in range(2)]
                    ops = list(_right(*[v.astype(F32) for v in blk]))
                    ops[1], ops[4] = blk[0], blk[3]
                    for x in range(7):
                        right[x].append(ops[x])
                mm = {x: jax.lax.dot_general(
                    jnp.concatenate([_as_bf16(wo_ops[n, x, pair, :M // 8]) for pair in range(H // 2)], axis=1),
                    jnp.concatenate(right[x], axis=1).astype(BF16), NT, preferred_element_type=F32) for x in O2_ORDER}
                m[0][n] = jnp.concatenate([((mm[0] + mm[3]) - mm[4]) + mm[6], _c21(mm)], axis=0)
                m[1][n] = jnp.concatenate([_c12(mm), _c22(mm)], axis=0)
            gate = g_s[0:1, pl.ds(c0, RC)]
            for hf in (1, 0):
                rest = (1.0 - gate) * xT_s[hf * mh:(hf + 1) * mh, pl.ds(c0, RC)].astype(F32)
                cols = []
                for t in range(RC // TQ):
                    gl, gr = gate[:, t * TQ:t * TQ + L], gate[:, t * TQ + L:(t + 1) * TQ]
                    rl, rr = rest[:, t * TQ:t * TQ + L], rest[:, t * TQ + L:(t + 1) * TQ]
                    if hf:
                        cols += [gl * _c21(m[t]) + rl, gr * _c22(m[t]) + rr]
                    else:
                        cols += [(gl * ((m[t][0] + m[t][3]) - m[t][4]) + rl) + gl * m[t][6], gr * _c12(m[t]) + rr]
                o_s[hf * mh:(hf + 1) * mh, pl.ds(c0, RC)] = jnp.concatenate(cols, axis=1).astype(BF16)
                out_copy(j, hf).start()
            return 0
        jax.lax.fori_loop(0, S // RC, out_step, 0)
        for j in range(S // RC):
            for hf in range(2):
                out_copy(j, hf).wait()

    pl.run_scoped(
        phase1,
        *[pltpu.VMEM(r.shape, r.dtype) for r in (c_hbm, wq_hbm, wk_hbm, wv_hbm, wg_hbm, wu_hbm, wd_hbm)],
        pltpu.VMEM((7, S // 4, mh), U32),
        pltpu.VMEM((7, -(-pq // 4) * 32, L), U32),
        pltpu.VMEM((7, -(-pq // 4) * 32, L), U32),
        pltpu.VMEM((M,), BF16),
        pltpu.VMEM((M,), BF16))
    pl.run_scoped(phase2, pltpu.VMEM((7, H, S // 4, L), U32), pltpu.VMEM((7, 7, H // 2, 64, L), U32))


def _tile_view(w):
    c, h, d = w.shape
    w = w.reshape(c, h // 8, 8, d // L, L).transpose(0, 1, 3, 2, 4)
    return w.reshape(c, h // 8, 8 * (d // L), L)


@jax.jit
def pallas_gated_mix__compressed_kv_cla__moe_arch_mod__prompt_kernel(
    A_x: jax.Array,
    A_c_kv: jax.Array,
    A_w_q: jax.Array,
    A_w_uk: jax.Array,
    A_w_uv: jax.Array,
    A_w_o: jax.Array,
    B_x: jax.Array,
    B_w_r: jax.Array,
    B_w_gate: jax.Array,
    B_w_up: jax.Array,
    B_w_down: jax.Array,
    gate_w: jax.Array,
):
    _, S, M = A_x.shape
    DC = A_c_kv.shape[2]
    H, D = A_w_q.shape[1], A_w_q.shape[2]
    args = (jnp.transpose(A_x[0]), A_c_kv[0], _tile_view(A_w_q).reshape(2, M // 2, 2, 16, L),
            _tile_view(A_w_uk), _tile_view(A_w_uv),
            jnp.transpose(A_w_o, (0, 2, 1)), B_w_r, gate_w, B_w_gate, B_w_up, jnp.transpose(B_w_down))

    def kern(*refs):
        _kernel(*refs, S=S, M=M, DC=DC, H=H, D=D)

    hbm = pl.BlockSpec(memory_space=pl.ANY)
    oT = pl.pallas_call(
        kern,
        out_shape=jax.ShapeDtypeStruct((M, S), A_x.dtype),
        in_specs=[hbm] * len(args),
        out_specs=hbm,
        scratch_shapes=[
            pltpu.VMEM((8, S), F32),
            pltpu.VMEM((M, S), BF16),
            pltpu.VMEM((H, M, D), BF16),
            pltpu.VMEM((5, S // 4, DC // 2), U32),
            pltpu.VMEM((2, 7, S // 8, DC // 4), U32),
            pltpu.VMEM((7, 4, 8 * (DC // 4 + 1), L), U32),
            pltpu.VMEM((H, S // 2, D), U32),
            pltpu.VMEM((S // 2, D), U32),
            pltpu.VMEM((S // 2, D), U32),
            pltpu.VMEM((5, S // 4, L), U32),
            pltpu.VMEM((M, S), BF16),
            pltpu.VMEM((5, S // 4 + PAD_V, L), U32),
            pltpu.SemaphoreType.DMA((N_SEM,)),
        ],
        compiler_params=pltpu.CompilerParams(vmem_limit_bytes=124 * 1024 * 1024, disable_bounds_checks=True,
                                             disable_semaphore_checks=True),
    )(*args)
    return jnp.transpose(oT)[None]
```

```python
import math

import jax
import jax.numpy as jnp
import jax.experimental.pallas as pl
import jax.experimental.pallas.tpu as pltpu

F32 = jnp.float32
BF16 = jnp.bfloat16
U32 = jnp.uint32
NT = (((1,), (1,)), ((), ()))

L = 128
TQ = 256
HQ = TQ // 2
RC = 512
NCH = 4

PAD_V = 16

S_X, S_Q0, S_Q1, S_K, S_V, S_C, S_MISC, S_OUT = 0, 4, 8, 12, 16, 20, 24, 30
N_SEM = 38

LOOP_ORDER = ("Q0 Q7 S0 G0 S7 V0 V7 o0 Q6 G3 S6 V6 Q5 G4 S5 V5 Q4 G5 S4 V4 Q3 G6 S3 V3 Q2 g2 S2 V2 "
              "Q1 c2 G1 S1 V1 w0")
FIRST_ORDER = "G0 G2 h0 G3 G4 G6 h1 G5 G1 h2 w0"
LAST_ORDER = "Q7 Q6 Q5 t7 V7 S6 Q4 V6 S5 r3 V5 S4 r2 V4 S3 r1 V3 S2 r0 V2 S1 S0 V1 V0"


def _to_u32(x_f32):
    return pltpu.bitcast(x_f32.astype(BF16), U32)


def _shuffled_u32(x_f32):
    return jnp.concatenate([_pack(x_f32[r:r + 8], x_f32[r + 8:r + 16]) for r in range(0, x_f32.shape[0], 16)],
                           axis=0)


def _as_bf16(x_u32):
    return pltpu.bitcast(x_u32, BF16)


def _left(a11, a12, a21, a22):
    return (a11 + a22, a21 + a22, a11, a22, a11 + a12, a21 - a11, a12 - a22)


def _right(b11, b12, b21, b22):
    return (b11 + b22, b11, b12 - b22, b21 - b11, b22, b11 + b12, b21 + b22)


FLAT, DEEP = (0, 1, 3, 4, 6), (2, 5)
O_ORDER = (0, 1, 2, 3, 4, 5, 6)
O2_ORDER = (4, 2, 1, 5, 0, 3, 6)
WO_SPAN = 0.95
SUMS = (0, 2, 3, 5, 6)
QK_LAG = 2
QK_TIE = 0


def _c11(m):
    return (m[0] + m[3]) + (m[6] - m[4])


def _c12(m):
    return m[2] + m[4]


def _c21(m):
    return m[1] + m[3]


def _c22(m):
    return (m[0] - m[1]) + (m[2] + m[5])


def _never(i):
    return jax.lax.broadcasted_iota(jnp.int32, (8, L), 0) < (i >> 10)


def _or_all(xs):
    out = xs[0]
    for x in xs[1:]:
        out = out | x
    return out


def _unpack(w, par):
    return pltpu.unpack_elementwise(w, index=par, packed_dtype=BF16, unpacked_dtype=F32)


def _pack(even, odd):
    return pltpu.bitcast(pltpu.pack_elementwise([even, odd], packed_dtype=BF16), U32)


def _head_weight(ref, h, nrows, pitch):
    sel = ((h >> 3) << 1) + (h & 1)
    r = (h >> 1) & 3
    return jnp.concatenate(
        [_as_bf16(ref[sel, pl.ds((dt * 4 + r) * pitch, nrows), :]) for dt in range(2)], axis=1)


def _kernel(xT_hbm, c_hbm, wq_hbm, wk_hbm, wv_hbm, wo_hbm, wr_hbm, gw_hbm, wg_hbm, wu_hbm, wd_hbm,
            o_hbm,
            g_s, xT_s, wo_s, a_s, a2_s, b_s, q_s, k_s, v_s, k5_s, o_s, v5_s, sem, *, S, M, DC, H, D):
    nq = S // TQ
    mh = M // 2
    pq = mh // 2 + 1
    pb = DC // 4 + 1
    mq = mh // NCH
    mk = DC // NCH
    qscale = (D ** -0.5) * math.log2(math.e)
    neg = -1e9 * math.log2(math.e)
    wo_copy = pltpu.make_async_copy(wo_hbm, wo_s, sem.at[S_MISC + 5])

    def out_copy(j, hf):
        return pltpu.make_async_copy(o_s.at[pl.ds(hf * mh, mh), pl.ds(j * RC, RC)],
                                     o_hbm.at[pl.ds(hf * mh, mh), pl.ds(j * RC, RC)], sem.at[S_OUT + 2 * j + hf])

    def head_program(order, h, hn, never, x7_s=None, tri=None, wo_ops=None, span=0.9, hooks=None):
        prods, held, waiting = {}, {}, []

        def spots(v, cols, rows=(0, 64, 128, 192)):
            return [v[r:r + 8, n * L:(n + 1) * L] for n in cols for r in rows]

        def tie(lhs, links, every):
            rows = []
            for rg in range(lhs.shape[0] // 8):
                blk = lhs[rg * 8:(rg + 1) * 8]
                if links and rg % every == 0:
                    blk = jnp.concatenate([jnp.where(never, links.pop(0), blk[:, :L]), blk[:, L:]], axis=1)
                rows.append(blk)
            return jnp.concatenate(rows, axis=0)

        combos = [("k", 0, _c11, (0, 3, 4, 6)), ("k", 1, _c21, (1, 3)),
                  ("v", 0, _c12, (2, 4)), ("v", 1, _c22, (0, 1, 2, 5))]

        def combine(pieces):
            ready = [c for c in combos if all(x in prods for x in c[3])]
            for e, (key, odd, comb, needs) in enumerate(ready):
                combos.remove((key, odd, comb, needs))
                for k in range(nq // 2):
                    m = {x: prods[x][k * TQ:(k + 1) * TQ] for x in needs}
                    if pieces:
                        rows = []
                        for g in range(8):
                            at = ((e * (nq // 2) + k) * 8 + g) / (len(ready) * (nq // 2) * 8)
                            rows.append(jnp.tile(pieces[int(0.95 * at * len(pieces))], (2, 2)))
                        m[needs[0]] = jnp.where(jnp.tile(never, (32, 2)), jnp.concatenate(rows + rows, axis=0),
                                                m[needs[0]])
                    c = comb(m)
                    held[2 * k + odd, key] = _shuffled_u32(c)
                    if 2 * k + odd < nq - 1:
                        off = (c[:L, L:], c[L:, :L]) if key == "v" else (c[L:, :L], c[:L, L:])
                        ops = _right(c[:L, :L], *off, c[L:, L:])
                        held[2 * k + odd, key + "5"] = [_shuffled_u32(ops[x]) for x in SUMS]

        def proj(n, lazy):
            w = _head_weight(b_s.at[n], hn, DC // 4, pb)
            links = list(waiting)
            del waiting[:]
            if n in DEEP:
                wf, kh = w.astype(F32), DC // 4
                right = [o.astype(BF16) for o in _right(wf[:kh, :L], wf[:kh, L:], wf[kh:, :L], wf[kh:, L:])]
                right[1], right[4] = w[:kh, :L], w[kh:, L:]
                m, pieces = {}, []

                def sub(x, after):
                    lhs = a2_s[DEEP.index(n), x]
                    mine = [links.pop(0) for _ in links[:2]]
                    if after:
                        t = after[0]
                        for v in after[1:]:
                            t = jnp.maximum(t, v)
                        lhs = tie(lhs, [pltpu.bitcast(jnp.maximum(t[g * 16:g * 16 + 8], t[g * 16 + 8:g * 16 + 16]), U32)
                                        for g in range(S // 64)], 1)
                    elif mine or links:
                        mine += links
                        del links[:]
                        lhs = tie(lhs, mine, lhs.shape[0] // 8 // len(mine))
                    m[x] = jnp.dot(_as_bf16(lhs), right[x], preferred_element_type=F32)
                    pieces.extend(spots(m[x], (0,), range(0, S // 4, 64)))
                sub(1, ()), sub(3, ())
                c21 = m[1] + m[3]
                sub(2, ()), sub(4, (c21,))
                c12, c11, c22 = m[2] + m[4], m[3] - m[4], m[2] - m[1]
                sub(0, ()), sub(5, (c12, c11, c22))
                c11, c22 = c11 + m[0], c22 + (m[0] + m[5])
                sub(6, (c11, c22))
                top = jnp.concatenate([c11 + m[6], c12], axis=1)
                bot = jnp.concatenate([c21, c22], axis=1)
                prods[n] = jnp.concatenate([v[k * L:(k + 1) * L] for k in range(nq // 2) for v in (top, bot)],
                                           axis=0)
            else:
                lhs = a_s[FLAT.index(n)]
                if links:
                    lhs = tie(lhs, links, max(1, lhs.shape[0] // 8 // len(links)))
                prods[n] = jnp.dot(_as_bf16(lhs), w, preferred_element_type=F32)
                pieces = spots(prods[n], (0, 1), range(0, S // 2, 32))
            if not lazy:
                combine(None)
            return pieces

        def write_kv():
            for ch in reversed(range(nq)):
                k_s[ch * HQ:(ch + 1) * HQ, :] = held[ch, "k"]
                v_s[ch * HQ:(ch + 1) * HQ, :] = held[ch, "v"]
                for key, ref in (("k5", k5_s), ("v5", v5_s)):
                    for n, o in enumerate(held.get((ch, key), ())):
                        ref[n, ch * 64:(ch + 1) * 64, :] = o

        def right_operand(n, plain, sums, c0, c1):
            if n == 1:
                return jnp.concatenate([_as_bf16(plain[c * HQ:c * HQ + 64, :L]) for c in range(c0, c1)], axis=0)
            if n == 4:
                return jnp.concatenate([_as_bf16(plain[c * HQ + 64:(c + 1) * HQ, L:]) for c in range(c0, c1)], axis=0)
            return _as_bf16(sums[SUMS.index(n), c0 * 64:c1 * 64, :])

        def qk(i, tied):
            q = qd = q_s[h, i * HQ:(i + 1) * HQ, :]
            n = min(16, len(waiting) - tied + 1) if tied else 0
            if n > 0:
                qd = tie(q, waiting[:n], 16 // n)
                del waiting[:n]
            q, qd = _as_bf16(q), _as_bf16(qd)
            tops, bots, pieces = [], [], []
            if i:
                qf = q.astype(F32)
                left = [o.astype(BF16) for o in _left(qf[:L, :L], qf[:L, L:], qf[L:, :L], qf[L:, L:])]
                left[2], left[3] = q[:L, :L], q[L:, L:]
            done = []
            for c in range(i):
                lhs = dict(enumerate(left))
                if c >= QK_LAG:
                    u = pltpu.bitcast(left[QK_TIE], U32)
                    lhs[QK_TIE] = _as_bf16(jnp.concatenate(
                        [jnp.where(never, done[c - QK_LAG][g], u[g * 8:(g + 1) * 8]) for g in range(8)], axis=0))
                m = {n: jax.lax.dot_general(lhs[n], right_operand(n, k_s, k5_s, c, c + 1), NT,
                                            preferred_element_type=F32) for n in (0, 3, 4, 6, 1, 2, 5)}
                c11, c12, c21, c22 = _c11(m), _c12(m), _c21(m), _c22(m)
                tops += [c11, c12]
                bots += [c21, c22]
                t = jnp.maximum(jnp.maximum(c11, c12), jnp.maximum(c21, c22))
                done.append([pltpu.bitcast(jnp.maximum(t[g * 16:g * 16 + 8], t[g * 16 + 8:(g + 1) * 16]), U32)
                             for g in range(8)])
                for n in (0, 5):
                    pieces += spots(m[n], (0,), (0, 32, 64, 96))
            r0 = i * HQ
            s1 = jax.lax.dot_general(qd, _as_bf16(k_s[r0:r0 + 64, :]), NT, preferred_element_type=F32)
            s2 = jax.lax.dot_general(q[L:], _as_bf16(k_s[r0 + 64:r0 + HQ, :]), NT, preferred_element_type=F32)
            top = jnp.concatenate(tops + [jnp.where(tri, s1[:L], neg)], axis=1)
            bot = jnp.concatenate(bots + [s1[L:], jnp.where(tri, s2, neg)], axis=1)
            return (top, bot), pieces + spots(s1, (0,))

        def softmax(i, top, bot, pieces, again=False):
            p, sums, prev = ([], []), ([], []), None
            for k in range(TQ // 8):
                half = k % 2
                s = (top, bot)[half][(k // 2) * 8:(k // 2 + 1) * 8]
                link = pieces[int(span * k * 8 / TQ * len(pieces))]
                if prev is not None:
                    link = jnp.where(never, link, prev)
                m = jnp.broadcast_to(jnp.max(s, axis=1, keepdims=True), (8, L))
                m = jnp.where(never, link, m)
                e = [jnp.exp2(s[:, t:t + L] - m) for t in range(0, s.shape[1], L)]
                prev = e[0]
                for x in e[1:]:
                    prev = prev + x
                if again:
                    m = m + jnp.log2(jnp.sum(prev, axis=1, keepdims=True))
                    e = [jnp.exp2(s[:, t:t + L] - m) for t in range(0, s.shape[1], L)]
                sums[half].append(prev)
                p[half].append(jnp.concatenate(e, axis=1))
            pt, pb_ = jnp.concatenate(p[0], axis=0), jnp.concatenate(p[1], axis=0)

            def tile(x, t):
                return x[:, t * L:(t + 1) * L]
            ops = [_left(tile(pt, 2 * c), tile(pt, 2 * c + 1), tile(pb_, 2 * c), tile(pb_, 2 * c + 1))
                   for c in range(i)]
            left = [jnp.concatenate([o[n] for o in ops], axis=1).astype(BF16) for n in range(7)] if i else None
            inv = []
            for x in () if again else sums:
                l = jnp.sum(jnp.concatenate(x, axis=0), axis=1, keepdims=True)
                r = pl.reciprocal(l, approx=True)
                inv.append(r * (2.0 - l * r))
            return (left, jnp.concatenate([tile(pt, 2 * i), tile(pb_, 2 * i)], axis=0).astype(BF16),
                    tile(pb_, 2 * i + 1).astype(BF16), inv)

        def pv(i, left, p1, p2, inv):
            r0 = i * HQ
            m, pieces = {}, []
            for n in (2, 3, 0, 4, 1, 5, 6) if i else ():
                m[n] = jnp.dot(left[n], right_operand(n, v_s, v5_s, 0, i), preferred_element_type=F32)
                pieces += spots(m[n], (0,), (0, 32, 64, 96))
            c1 = jnp.dot(p1, _as_bf16(v_s[r0:r0 + 64, :]), preferred_element_type=F32)
            c2 = jnp.dot(p2, _as_bf16(v_s[r0 + 64:r0 + HQ, :]), preferred_element_type=F32)
            top, bot = c1[:L], c1[L:] + c2
            if i:
                top = top + jnp.concatenate([_c11(m), _c12(m)], axis=1)
                bot = bot + jnp.concatenate([_c21(m), _c22(m)], axis=1)
            else:
                pieces = spots(c1, (0, 1))
            if inv:
                top, bot = top * inv[0], bot * inv[1]
            us = [_to_u32(o) for o in _right(top[:, :L], bot[:, :L], top[:, L:], bot[:, L:])]
            for n in range(7):
                x7_s[n, h, i * 64:(i + 1) * 64, :] = us[n]
            waiting.extend(_or_all([us[n][g * 8:(g + 1) * 8] for n in SUMS]) for g in range(8))
            return pieces

        def wo_operands(pieces):
            groups = M // 64
            never2 = jnp.concatenate([never, never], axis=0)
            share = -(-(H // 2) * groups // (H - 1))
            for k in range(share):
                u = jnp.minimum(h * share + k, (H // 2) * groups - 1)
                pair = jax.lax.div(u, groups)
                rg = u - pair * groups
                ops = [_left(*[wo_s[2 * pair + par, pl.ds(pl.multiple_of(hf * mh + sub * (mh // 2) + rg * 16, 16), 16),
                                    ch * L:(ch + 1) * L].astype(F32) for hf in range(2) for ch in range(2)])
                       for sub in range(2) for par in range(2)]
                for n in range(7):
                    link = pieces[int(WO_SPAN * (k * 7 + n) / (share * 7) * len(pieces))]
                    gate = jnp.concatenate([link, link], axis=0)
                    us = [_to_u32(o) for o in _left(*[jnp.where(never2, gate, o[n]) for o in ops])]
                    for x in range(7):
                        wo_ops[n, x, pair, pl.ds(pl.multiple_of(rg * 8, 8), 8), :] = us[x]
                    waiting.append(_or_all(us))

        scores, probs, pieces = {}, {}, []
        for op in order.split():
            i = int(op[1:])
            if op[0] in "Gg":
                pieces.append(proj(i, op[0] == "g"))
            elif op[0] == "c":
                combine(sum(pieces[-i:], []))
            elif op[0] == "w":
                write_kv()
            elif op[0] == "o":
                wo_operands(pieces[-1])
            elif op[0] in "Qqr":
                scores[i], new = qk(i, {"Q": 0, "q": 1, "r": 9}[op[0]])
                pieces.append(new)
            elif op[0] in "SsTt":
                probs[i] = softmax(i, *scores.pop(i), pieces[-1] if op[0] in "ST" else pieces[-2] + pieces[-1],
                                   op[0] in "Tt")
            elif op[0] == "V":
                pieces.append(pv(i, *probs.pop(i)))
            else:
                hooks[i](pieces)

    def phase1(c_s, wq_r, wk_r, wv_r, wg_s, wu_s, wd_s, xa_s, wq0_s, wq1_s, wr_s, gw_s):
        def x_copy(j):
            return pltpu.make_async_copy(xT_hbm.at[:, pl.ds(j * RC, RC)], xT_s.at[:, pl.ds(j * RC, RC)],
                                         sem.at[S_X + j])

        def wq_copy(g, j):
            return pltpu.make_async_copy(wq_hbm.at[:, pl.ds(j * mq, mq), g], wq_r.at[:, pl.ds(j * mq, mq), g],
                                         sem.at[(S_Q1 if g else S_Q0) + j])

        def kv_copies(j):
            return [pltpu.make_async_copy(src.at[pl.ds(j * n, n)], dst.at[pl.ds(j * n, n)], sem.at[s0 + j])
                    for src, dst, s0, n in ((c_hbm, c_s, S_C, RC), (wk_hbm, wk_r, S_K, mk), (wv_hbm, wv_r, S_V, mk))]

        misc = [pltpu.make_async_copy(a, b, sem.at[S_MISC + i]) for i, (a, b) in enumerate(
            [(wr_hbm, wr_s), (gw_hbm, gw_s), (wg_hbm, wg_s), (wu_hbm, wu_s), (wd_hbm, wd_s)])]

        x_copy(0).start()
        for j in range(NCH):
            wq_copy(0, j).start()

        def start_rest():
            for j in range(NCH):
                if j + 1 < NCH:
                    x_copy(j + 1).start()
                wq_copy(1, j).start()
            misc[0].start()
            misc[1].start()
            for j in range(NCH):
                for cp in kv_copies(j):
                    cp.start()
            for cp in misc[2:]:
                cp.start()
            wo_copy.start()

        start_rest()

        def x_operands(j):
            c0 = j * RC if isinstance(j, int) else pl.multiple_of(j * RC, RC)
            r0 = j * HQ if isinstance(j, int) else pl.multiple_of(j * HQ, HQ)
            a = [xT_s[kh * mh:(kh + 1) * mh, pl.ds(c0 + rb * TQ, TQ)].astype(F32)
                 for rb in range(2) for kh in range(2)]
            for n, o in enumerate(_left(*a)):
                xa_s[n, pl.ds(r0, HQ), :] = pltpu.bitcast(o.astype(BF16).T, U32)

        def wq_operands(g, p, never=None, link=None):
            w = [pltpu.bitcast(wq_r[kh, pl.ds(2 * p, 2), g], U32) for kh in range(2)]
            w = [[x[0], x[1]] for x in w]
            if link is not None:
                w[0][0] = jnp.where(never, link, w[0][0])
            rows = [_right(*[_unpack(w[kh][e], par) for kh in range(2) for par in range(2)]) for e in range(2)]
            for n in range(7):
                (wq0_s, wq1_s)[g][n, pl.ds(p, 8, stride=pq), :] = _pack(rows[0][n], rows[1][n])

        x_copy(0).wait()
        x_operands(0)

        def first_half(j, _):
            wq_copy(0, j).wait()
            for k in range(mq // 2):
                wq_operands(0, j * (mq // 2) + k)
            return 0
        jax.lax.fori_loop(0, NCH, first_half, 0)

        def q_step(g, j, side):
            pieces = []
            for r in range(4):
                m = {}
                for n in (0, 3, 4, 6, 1, 2, 5):
                    w = jnp.concatenate([_as_bf16((wq0_s, wq1_s)[g][n, pl.ds((dt * 4 + r) * pq, mh // 2), :])
                                         for dt in range(2)], axis=1)
                    m[n] = jnp.dot(_as_bf16(xa_s[n, pl.ds(pl.multiple_of(j * HQ, HQ), HQ), :]), w,
                                   preferred_element_type=F32)
                    for k in range(5):
                        pieces.append(m[n][k * 48:k * 48 + 8, (k % 2) * L:(k % 2 + 1) * L])
                        side(len(pieces) - 1, pieces[-1])
                for par, rb, comb in ((0, 0, _c11), (0, 1, _c21), (1, 0, _c12), (1, 1, _c22)):
                    r0 = pl.multiple_of(j * TQ + rb * HQ, HQ)
                    q_s[8 * g + 2 * r + par, pl.ds(r0, HQ), :] = _to_u32(comb(m) * qscale)

        def q_lo(j, _):
            never = _never(j)

            def side(k, piece):
                if k == 35:
                    @pl.when(j + 1 < NCH)
                    def _():
                        x_copy(j + 1).wait()
                    wq_copy(1, j).wait()
                if k >= 42 and k % 3 == 0 and (k - 42) // 3 < mq // 2:
                    wq_operands(1, j * (mq // 2) + (k - 42) // 3, never, pltpu.bitcast(piece, U32))
            q_step(0, j, side)
            x_operands((j + 1) & (NCH - 1))
            return 0
        jax.lax.fori_loop(0, NCH, q_lo, 0)

        def q_hi(j, _):
            for cp in kv_copies(j):
                cp.wait()
            never = _never(j)
            quad = []

            def side(kk, piece):
                if kk >= 128:
                    return
                k, g = kk // 2, kk % 2
                link = pltpu.bitcast(piece, U32)
                if g == 0:
                    rg, t = k // 8 + 8 * (k % 4 // 2), k // 4 % 2 + 2 * (k % 2)
                    a = []
                    for rb in range(2):
                        r0 = pl.multiple_of(j * RC + rb * TQ + rg * 16, 16)
                        for ch in range(2):
                            a.append(c_s[pl.ds(r0, 16), (2 * t + ch) * L:(2 * t + ch + 1) * L].astype(F32))
                    a[0] = jnp.where(jnp.concatenate([never, never], axis=0),
                                     jnp.concatenate([piece, piece], axis=0), a[0])
                    ops = _left(*a)
                    us = [_shuffled_u32(ops[n]) for n in FLAT]
                    d0 = pl.multiple_of(j * HQ + rg * 8, 8)
                    for n, u in enumerate(us):
                        a_s[n, pl.ds(d0, 8), t * L:(t + 1) * L] = u
                    quad.append(ops)
                    if len(quad) == 4:
                        d0 = pl.multiple_of(j * (HQ // 2) + (rg - 8) * 8, 8)
                        for e, n in enumerate(DEEP):
                            deep = [_shuffled_u32(o) for o in _left(*[q[n] for q in quad])]
                            for x, u in enumerate(deep):
                                a2_s[e, x, pl.ds(d0, 8), (t - 2) * L:(t - 1) * L] = u
                            us += deep
                        del quad[:]
                    link = _or_all(us)
                c0 = j * mk + 2 * k
                w = [pltpu.bitcast(r[pl.ds(c0 + o, 2), g], U32) for o in (0, L) for r in (wk_r, wv_r)]
                w = [[x[0], x[1]] for x in w]
                w[0][0] = jnp.where(never, link, w[0][0])
                for par in range(2):
                    rows = [_right(*[_unpack(x[e], par) for x in w]) for e in range(2)]
                    for n in range(7):
                        b_s[n, 2 * g + par, pl.ds(j * (mk // 4) + k, 8, stride=pb), :] = _pack(
                            rows[0][n], rows[1][n])
            q_step(1, j, side)
            return j
        never = _never(jax.lax.fori_loop(0, NCH, q_hi, 0))

        for cp in misc:
            cp.wait()
        st = {}

        F = wg_s.shape[1]

        def route(pieces):
            pieces = pieces[-2] + pieces[-1]
            mp = -(-M // L) * L
            cols = []
            for w_s in (wr_s, gw_s):
                w = jnp.concatenate([w_s[...].reshape(1, M).astype(F32), jnp.zeros((1, mp - M), F32)], axis=1)
                cols.append(jnp.broadcast_to(w, (L, mp)).T)
            nr, rows = 4, M // 4
            out, k, prev = ([], []), 0, None
            for ct in range(S // L):
                acc = [None, None]
                for q in range(nr):
                    link = pieces[int((0.03 + 0.65 * k / (nr * S // L)) * len(pieces))]
                    if prev is not None:
                        link = jnp.where(never, link, prev)
                    k += 1
                    x = linked(xT_s[q * rows:(q + 1) * rows, ct * L:(ct + 1) * L], link)
                    for t in range(2):
                        part = fold(x * cols[t][q * rows:(q + 1) * rows], 0)
                        acc[t] = part if acc[t] is None else acc[t] + part
                    prev = acc[0] + acc[1]
                for t in range(2):
                    out[t].append(jnp.sum(acc[t], axis=0, keepdims=True))
            g_s[0:1, :] = jax.nn.sigmoid(jnp.concatenate(out[1], axis=1))
            r = jnp.concatenate(out[0], axis=1).astype(BF16).astype(F32)
            lane = jax.lax.broadcasted_iota(jnp.int32, (1, S), 1)
            m1 = jnp.max(r, axis=1, keepdims=True)
            i1 = jnp.min(jnp.where(r == m1, lane, S - 1), axis=1, keepdims=True)
            r2 = jnp.where(lane == i1, -jnp.inf, r)
            m2 = jnp.max(r2, axis=1, keepdims=True)
            i2 = jnp.min(jnp.where(jnp.logical_and(r2 == m2, lane != i1), lane, S - 1), axis=1, keepdims=True)
            ln = jax.lax.broadcasted_iota(jnp.int32, (M, L), 1)
            st["c0"] = [pl.multiple_of((i[0, 0] >> 7) << 7, L) for i in (i1, i2)]
            st["hit"] = [ln == (i & (L - 1)) for i in (i1, i2)]
            st["r"] = [jax.nn.sigmoid(m1), jax.nn.sigmoid(m2)]
            st["x"] = [jnp.broadcast_to(jnp.sum(jnp.where(hit, xT_s[:, pl.ds(c0, L)].astype(F32), 0.0),
                                                axis=1, keepdims=True), (M, L))
                       for c0, hit in zip(st["c0"], st["hit"])]

        def fold(v, axis_len):
            parts = [v[k * 8:(k + 1) * 8] if axis_len == 0 else v[:, k * L:(k + 1) * L]
                     for k in range(v.shape[axis_len] // (8, L)[axis_len])]
            while len(parts) > 1:
                parts = [parts[k] + parts[k + 1] if k + 1 < len(parts) else parts[k]
                         for k in range(0, len(parts), 2)]
            return parts[0]

        def linked(w, link):
            w = pltpu.bitcast(w, U32)
            reps = (w.shape[0] // 8, w.shape[1] // L)
            w = jnp.where(jnp.tile(never, reps), jnp.tile(pltpu.bitcast(link, U32), reps), w)
            return _as_bf16(w).astype(F32)

        def hidden(pieces):
            pieces = pieces[-3] + pieces[-2] + pieces[-1]
            nr, rows = 4, M // 4
            total = 2 * (F // L) * nr
            out, k, prev = [], 0, None
            for w_s in (wg_s, wu_s):
                cols = ([], [])
                for ct in range(F // L):
                    acc = [None, None]
                    for q in range(nr):
                        link = pieces[int(0.9 * k / total * len(pieces))]
                        if prev is not None:
                            link = jnp.where(never, link, prev)
                        k += 1
                        w = linked(w_s[q * rows:(q + 1) * rows, ct * L:(ct + 1) * L], link)
                        for t in range(2):
                            part = fold(w * st["x"][t][q * rows:(q + 1) * rows], 0)
                            acc[t] = part if acc[t] is None else acc[t] + part
                        prev = acc[0] + acc[1]
                    for t in range(2):
                        cols[t].append(jnp.sum(acc[t], axis=0, keepdims=True))
                out.append([jnp.concatenate(c, axis=1) for c in cols])
            st["h"] = [(jax.nn.silu(out[0][t]) * out[1][t]).astype(BF16).astype(F32) for t in range(2)]

        def patch(pieces):
            pieces = pieces[-2] + pieces[-1]
            half = F // 2
            ys, k, prev = ([], []), 0, None
            for rg in range(M // 16):
                acc = [None, None]
                for hf in range(2):
                    link = pieces[int((0.1 + 0.8 * k / (M // 8)) * len(pieces))]
                    if prev is not None:
                        link = jnp.where(never, link, prev)
                    k += 1
                    w = linked(wd_s[rg * 16:(rg + 1) * 16, hf * half:(hf + 1) * half], link)
                    for t in range(2):
                        part = fold(w * st["h"][t][:, hf * half:(hf + 1) * half], 1)
                        acc[t] = part if acc[t] is None else acc[t] + part
                    prev = fold(acc[0] + acc[1], 0)
                for t in range(2):
                    ys[t].append(jnp.sum(acc[t], axis=1, keepdims=True))
            for t in range(2):
                y = jnp.concatenate(ys[t], axis=0) * st["r"][t]
                blk = xT_s[:, pl.ds(st["c0"][t], L)].astype(F32)
                xT_s[:, pl.ds(st["c0"][t], L)] = (blk + jnp.where(st["hit"][t], y, 0.0)).astype(BF16)

        head_program(FIRST_ORDER, None, 0, never, hooks=(route, hidden, patch))

    def phase2(x7_s, wo_ops):
        wo_copy.wait()
        col = jax.lax.broadcasted_iota(jnp.int32, (L, L), 1)
        tri = ((col & ~15) + ((col & 3) << 2) + ((col & 15) >> 2)
               <= jax.lax.broadcasted_iota(jnp.int32, (L, L), 0))

        def head(h, _):
            head_program(LOOP_ORDER, h, h + 1, _never(h), x7_s, tri, wo_ops, span=0.96)
            return h
        last = jax.lax.fori_loop(0, H - 1, head, 0)
        head_program(LAST_ORDER, H - 1, None, _never(last), x7_s, tri)

        def out_step(j, _):
            c0 = pl.multiple_of(j * RC, RC)
            m = ({}, {})
            for n in O_ORDER:
                right = [[] for _ in range(7)]
                for pair in range(H // 2):
                    blk = [_as_bf16(x7_s[n, 2 * pair + par, pl.ds(pl.multiple_of(j * L + t * 64, 64), 64), :])
                           for par in range(2) for t in range(2)]
                    ops = list(_right(*[v.astype(F32) for v in blk]))
                    ops[1], ops[4] = blk[0], blk[3]
                    for x in range(7):
                        right[x].append(ops[x])
                mm = {x: jax.lax.dot_general(
                    jnp.concatenate([_as_bf16(wo_ops[n, x, pair, :M // 8]) for pair in range(H // 2)], axis=1),
                    jnp.concatenate(right[x], axis=1).astype(BF16), NT, preferred_element_type=F32) for x in O2_ORDER}
                m[0][n] = jnp.concatenate([((mm[0] + mm[3]) - mm[4]) + mm[6], _c21(mm)], axis=0)
                m[1][n] = jnp.concatenate([_c12(mm), _c22(mm)], axis=0)
            gate = g_s[0:1, pl.ds(c0, RC)]
            for hf in (1, 0):
                rest = (1.0 - gate) * xT_s[hf * mh:(hf + 1) * mh, pl.ds(c0, RC)].astype(F32)
                cols = []
                for t in range(RC // TQ):
                    gl, gr = gate[:, t * TQ:t * TQ + L], gate[:, t * TQ + L:(t + 1) * TQ]
                    rl, rr = rest[:, t * TQ:t * TQ + L], rest[:, t * TQ + L:(t + 1) * TQ]
                    if hf:
                        cols += [gl * _c21(m[t]) + rl, gr * _c22(m[t]) + rr]
                    else:
                        cols += [(gl * ((m[t][0] + m[t][3]) - m[t][4]) + rl) + gl * m[t][6], gr * _c12(m[t]) + rr]
                o_s[hf * mh:(hf + 1) * mh, pl.ds(c0, RC)] = jnp.concatenate(cols, axis=1).astype(BF16)
                out_copy(j, hf).start()
            return 0
        jax.lax.fori_loop(0, S // RC, out_step, 0)
        for j in range(S // RC):
            for hf in range(2):
                out_copy(j, hf).wait()

    pl.run_scoped(
        phase1,
        *[pltpu.VMEM(r.shape, r.dtype) for r in (c_hbm, wq_hbm, wk_hbm, wv_hbm, wg_hbm, wu_hbm, wd_hbm)],
        pltpu.VMEM((7, S // 4, mh), U32),
        pltpu.VMEM((7, -(-pq // 4) * 32, L), U32),
        pltpu.VMEM((7, -(-pq // 4) * 32, L), U32),
        pltpu.VMEM((M,), BF16),
        pltpu.VMEM((M,), BF16))
    pl.run_scoped(phase2, pltpu.VMEM((7, H, S // 4, L), U32), pltpu.VMEM((7, 7, H // 2, 64, L), U32))


def _tile_view(w):
    c, h, d = w.shape
    w = w.reshape(c, h // 8, 8, d // L, L).transpose(0, 1, 3, 2, 4)
    return w.reshape(c, h // 8, 8 * (d // L), L)


@jax.jit
def pallas_gated_mix__compressed_kv_cla__moe_arch_mod__prompt_kernel(
    A_x: jax.Array,
    A_c_kv: jax.Array,
    A_w_q: jax.Array,
    A_w_uk: jax.Array,
    A_w_uv: jax.Array,
    A_w_o: jax.Array,
    B_x: jax.Array,
    B_w_r: jax.Array,
    B_w_gate: jax.Array,
    B_w_up: jax.Array,
    B_w_down: jax.Array,
    gate_w: jax.Array,
):
    _, S, M = A_x.shape
    DC = A_c_kv.shape[2]
    H, D = A_w_q.shape[1], A_w_q.shape[2]
    args = (jnp.transpose(A_x[0]), A_c_kv[0], _tile_view(A_w_q).reshape(2, M // 2, 2, 16, L),
            _tile_view(A_w_uk), _tile_view(A_w_uv),
            jnp.transpose(A_w_o, (0, 2, 1)), B_w_r, gate_w, B_w_gate, B_w_up, jnp.transpose(B_w_down))

    def kern(*refs):
        _kernel(*refs, S=S, M=M, DC=DC, H=H, D=D)

    hbm = pl.BlockSpec(memory_space=pl.ANY)
    oT = pl.pallas_call(
        kern,
        out_shape=jax.ShapeDtypeStruct((M, S), A_x.dtype),
        in_specs=[hbm] * len(args),
        out_specs=hbm,
        scratch_shapes=[
            pltpu.VMEM((8, S), F32),
            pltpu.VMEM((M, S), BF16),
            pltpu.VMEM((H, M, D), BF16),
            pltpu.VMEM((5, S // 4, DC // 2), U32),
            pltpu.VMEM((2, 7, S // 8, DC // 4), U32),
            pltpu.VMEM((7, 4, 8 * (DC // 4 + 1), L), U32),
            pltpu.VMEM((H, S // 2, D), U32),
            pltpu.VMEM((S // 2, D), U32),
            pltpu.VMEM((S // 2, D), U32),
            pltpu.VMEM((5, S // 4, L), U32),
            pltpu.VMEM((M, S), BF16),
            pltpu.VMEM((5, S // 4 + PAD_V, L), U32),
            pltpu.SemaphoreType.DMA((N_SEM,)),
        ],
        compiler_params=pltpu.CompilerParams(vmem_limit_bytes=124 * 1024 * 1024, disable_bounds_checks=True,
                                             disable_semaphore_checks=True),
    )(*args)
    return jnp.transpose(oT)[None]
```

```python
import math

import jax
import jax.numpy as jnp
import jax.experimental.pallas as pl
import jax.experimental.pallas.tpu as pltpu

F32 = jnp.float32
BF16 = jnp.bfloat16
U32 = jnp.uint32
NT = (((1,), (1,)), ((), ()))

L = 128
TQ = 256
HQ = TQ // 2
RC = 512
NCH = 4

PAD_V = 16

S_X, S_Q0, S_Q1, S_K, S_V, S_C, S_MISC, S_OUT = 0, 4, 8, 12, 16, 20, 24, 30
N_SEM = 38

LOOP_ORDER = ("Q0 Q7 S0 G0 S7 V0 V7 o0 Q6 G3 S6 V6 Q5 G4 S5 V5 Q4 G5 S4 V4 Q3 G6 S3 V3 Q2 g2 S2 V2 "
              "Q1 c2 G1 S1 V1 w0")
FIRST_ORDER = "G0 G2 h0 G3 G4 G6 h1 G5 G1 h2 w0"
LAST_ORDER = "Q7 Q6 Q5 t7 V7 S6 Q4 V6 S5 r3 V5 S4 r2 V4 S3 r1 V3 S2 r0 V2 S1 S0 V1 V0"


def _to_u32(x_f32):
    return pltpu.bitcast(x_f32.astype(BF16), U32)


def _shuffled_u32(x_f32):
    return jnp.concatenate([_pack(x_f32[r:r + 8], x_f32[r + 8:r + 16]) for r in range(0, x_f32.shape[0], 16)],
                           axis=0)


def _as_bf16(x_u32):
    return pltpu.bitcast(x_u32, BF16)


def _left(a11, a12, a21, a22):
    return (a11 + a22, a21 + a22, a11, a22, a11 + a12, a21 - a11, a12 - a22)


def _right(b11, b12, b21, b22):
    return (b11 + b22, b11, b12 - b22, b21 - b11, b22, b11 + b12, b21 + b22)


FLAT, DEEP = (0, 1, 3, 4, 6), (2, 5)
SUMS = (0, 2, 3, 5, 6)


def _c11(m):
    return (m[0] + m[3]) + (m[6] - m[4])


def _c12(m):
    return m[2] + m[4]


def _c21(m):
    return m[1] + m[3]


def _c22(m):
    return (m[0] - m[1]) + (m[2] + m[5])


def _never(i):
    return jax.lax.broadcasted_iota(jnp.int32, (8, L), 0) < (i >> 10)


def _or_all(xs):
    out = xs[0]
    for x in xs[1:]:
        out = out | x
    return out


def _unpack(w, par):
    return pltpu.unpack_elementwise(w, index=par, packed_dtype=BF16, unpacked_dtype=F32)


def _pack(even, odd):
    return pltpu.bitcast(pltpu.pack_elementwise([even, odd], packed_dtype=BF16), U32)


def _head_weight(ref, h, nrows, pitch):
    sel = ((h >> 3) << 1) + (h & 1)
    r = (h >> 1) & 3
    return jnp.concatenate(
        [_as_bf16(ref[sel, pl.ds((dt * 4 + r) * pitch, nrows), :]) for dt in range(2)], axis=1)


def _kernel(xT_hbm, c_hbm, wq_hbm, wk_hbm, wv_hbm, wo_hbm, wr_hbm, gw_hbm, wg_hbm, wu_hbm, wd_hbm,
            o_hbm,
            g_s, xT_s, wo_s, a_s, a2_s, b_s, q_s, k_s, v_s, k5_s, o_s, v5_s, sem, *, S, M, DC, H, D):
    nq = S // TQ
    mh = M // 2
    pq = mh // 2 + 1
    pb = DC // 4 + 1
    mq = mh // NCH
    mk = DC // NCH
    qscale = (D ** -0.5) * math.log2(math.e)
    neg = -1e9 * math.log2(math.e)
    wo_copy = pltpu.make_async_copy(wo_hbm, wo_s, sem.at[S_MISC + 5])

    def out_copy(j, hf):
        return pltpu.make_async_copy(o_s.at[pl.ds(hf * mh, mh), pl.ds(j * RC, RC)],
                                     o_hbm.at[pl.ds(hf * mh, mh), pl.ds(j * RC, RC)], sem.at[S_OUT + 2 * j + hf])

    def head_program(order, h, hn, never, x7_s=None, tri=None, wo_ops=None, span=0.9, hooks=None):
        prods, held, waiting = {}, {}, []

        def spots(v, cols, rows=(0, 64, 128, 192)):
            return [v[r:r + 8, n * L:(n + 1) * L] for n in cols for r in rows]

        def tie(lhs, links, every):
            rows = []
            for rg in range(lhs.shape[0] // 8):
                blk = lhs[rg * 8:(rg + 1) * 8]
                if links and rg % every == 0:
                    blk = jnp.concatenate([jnp.where(never, links.pop(0), blk[:, :L]), blk[:, L:]], axis=1)
                rows.append(blk)
            return jnp.concatenate(rows, axis=0)

        combos = [("k", 0, _c11, (0, 3, 4, 6)), ("k", 1, _c21, (1, 3)),
                  ("v", 0, _c12, (2, 4)), ("v", 1, _c22, (0, 1, 2, 5))]

        def combine(pieces):
            ready = [c for c in combos if all(x in prods for x in c[3])]
            for e, (key, odd, comb, needs) in enumerate(ready):
                combos.remove((key, odd, comb, needs))
                for k in range(nq // 2):
                    m = {x: prods[x][k * TQ:(k + 1) * TQ] for x in needs}
                    if pieces:
                        rows = []
                        for g in range(8):
                            at = ((e * (nq // 2) + k) * 8 + g) / (len(ready) * (nq // 2) * 8)
                            rows.append(jnp.tile(pieces[int(0.95 * at * len(pieces))], (2, 2)))
                        m[needs[0]] = jnp.where(jnp.tile(never, (32, 2)), jnp.concatenate(rows + rows, axis=0),
                                                m[needs[0]])
                    c = comb(m)
                    held[2 * k + odd, key] = _shuffled_u32(c)
                    if 2 * k + odd < nq - 1:
                        off = (c[:L, L:], c[L:, :L]) if key == "v" else (c[L:, :L], c[:L, L:])
                        ops = _right(c[:L, :L], *off, c[L:, L:])
                        held[2 * k + odd, key + "5"] = [_shuffled_u32(ops[x]) for x in SUMS]

        def proj(n, lazy):
            w = _head_weight(b_s.at[n], hn, DC // 4, pb)
            links = list(waiting)
            del waiting[:]
            if n in DEEP:
                wf, kh = w.astype(F32), DC // 4
                right = [o.astype(BF16) for o in _right(wf[:kh, :L], wf[:kh, L:], wf[kh:, :L], wf[kh:, L:])]
                right[1], right[4] = w[:kh, :L], w[kh:, L:]
                m, pieces = {}, []

                def sub(x, after):
                    lhs = a2_s[DEEP.index(n), x]
                    if after:
                        t = after[0]
                        for v in after[1:]:
                            t = jnp.maximum(t, v)
                        lhs = tie(lhs, [pltpu.bitcast(jnp.maximum(t[g * 16:g * 16 + 8], t[g * 16 + 8:g * 16 + 16]), U32)
                                        for g in range(S // 64)], 1)
                    elif links:
                        lhs = tie(lhs, links, lhs.shape[0] // 8 // len(links))
                    m[x] = jnp.dot(_as_bf16(lhs), right[x], preferred_element_type=F32)
                    pieces.extend(spots(m[x], (0,), range(0, S // 4, 64)))
                sub(1, ()), sub(3, ())
                c21 = m[1] + m[3]
                sub(2, ()), sub(4, (c21,))
                c12, c11, c22 = m[2] + m[4], m[3] - m[4], m[2] - m[1]
                sub(0, ()), sub(5, (c12, c11, c22))
                c11, c22 = c11 + m[0], c22 + (m[0] + m[5])
                sub(6, (c11, c22))
                top = jnp.concatenate([c11 + m[6], c12], axis=1)
                bot = jnp.concatenate([c21, c22], axis=1)
                prods[n] = jnp.concatenate([v[k * L:(k + 1) * L] for k in range(nq // 2) for v in (top, bot)],
                                           axis=0)
            else:
                lhs = a_s[FLAT.index(n)]
                if links:
                    lhs = tie(lhs, links, max(1, lhs.shape[0] // 8 // len(links)))
                prods[n] = jnp.dot(_as_bf16(lhs), w, preferred_element_type=F32)
                pieces = spots(prods[n], (0, 1), range(0, S // 2, 32))
            if not lazy:
                combine(None)
            return pieces

        def write_kv():
            for ch in reversed(range(nq)):
                k_s[ch * HQ:(ch + 1) * HQ, :] = held[ch, "k"]
                v_s[ch * HQ:(ch + 1) * HQ, :] = held[ch, "v"]
                for key, ref in (("k5", k5_s), ("v5", v5_s)):
                    for n, o in enumerate(held.get((ch, key), ())):
                        ref[n, ch * 64:(ch + 1) * 64, :] = o

        def right_operand(n, plain, sums, c0, c1):
            if n == 1:
                return jnp.concatenate([_as_bf16(plain[c * HQ:c * HQ + 64, :L]) for c in range(c0, c1)], axis=0)
            if n == 4:
                return jnp.concatenate([_as_bf16(plain[c * HQ + 64:(c + 1) * HQ, L:]) for c in range(c0, c1)], axis=0)
            return _as_bf16(sums[SUMS.index(n), c0 * 64:c1 * 64, :])

        def qk(i, tied):
            q = qd = q_s[h, i * HQ:(i + 1) * HQ, :]
            n = len(waiting) - 8 if tied else 0
            if n > 0:
                qd = tie(q, waiting[:n], 16 // n)
                del waiting[:n]
            q, qd = _as_bf16(q), _as_bf16(qd)
            tops, bots, pieces = [], [], []
            if i:
                qf = q.astype(F32)
                left = [o.astype(BF16) for o in _left(qf[:L, :L], qf[:L, L:], qf[L:, :L], qf[L:, L:])]
                left[2], left[3] = q[:L, :L], q[L:, L:]
            done = []
            for c in range(i):
                lhs = dict(enumerate(left))
                if c >= 2:
                    u = pltpu.bitcast(left[0], U32)
                    lhs[0] = _as_bf16(jnp.concatenate(
                        [jnp.where(never, done[c - 2][g], u[g * 8:(g + 1) * 8]) for g in range(8)], axis=0))
                m = {n: jax.lax.dot_general(lhs[n], right_operand(n, k_s, k5_s, c, c + 1), NT,
                                            preferred_element_type=F32) for n in (0, 3, 4, 6, 1, 2, 5)}
                c11, c12, c21, c22 = _c11(m), _c12(m), _c21(m), _c22(m)
                tops += [c11, c12]
                bots += [c21, c22]
                t = jnp.maximum(jnp.maximum(c11, c12), jnp.maximum(c21, c22))
                done.append([pltpu.bitcast(jnp.maximum(t[g * 16:g * 16 + 8], t[g * 16 + 8:(g + 1) * 16]), U32)
                             for g in range(8)])
                for n in (0, 5):
                    pieces += spots(m[n], (0,), (0, 32, 64, 96))
            r0 = i * HQ
            s1 = jax.lax.dot_general(qd, _as_bf16(k_s[r0:r0 + 64, :]), NT, preferred_element_type=F32)
            s2 = jax.lax.dot_general(q[L:], _as_bf16(k_s[r0 + 64:r0 + HQ, :]), NT, preferred_element_type=F32)
            top = jnp.concatenate(tops + [jnp.where(tri, s1[:L], neg)], axis=1)
            bot = jnp.concatenate(bots + [s1[L:], jnp.where(tri, s2, neg)], axis=1)
            return (top, bot), pieces + spots(s1, (0,))

        def softmax(i, top, bot, pieces, again=False):
            p, sums, prev = ([], []), ([], []), None
            for k in range(TQ // 8):
                half = k % 2
                s = (top, bot)[half][(k // 2) * 8:(k // 2 + 1) * 8]
                link = pieces[int(span * k * 8 / TQ * len(pieces))]
                if prev is not None:
                    link = jnp.where(never, link, prev)
                m = jnp.broadcast_to(jnp.max(s, axis=1, keepdims=True), (8, L))
                m = jnp.where(never, link, m)
                e = [jnp.exp2(s[:, t:t + L] - m) for t in range(0, s.shape[1], L)]
                prev = e[0]
                for x in e[1:]:
                    prev = prev + x
                if again:
                    m = m + jnp.log2(jnp.sum(prev, axis=1, keepdims=True))
                    e = [jnp.exp2(s[:, t:t + L] - m) for t in range(0, s.shape[1], L)]
                sums[half].append(prev)
                p[half].append(jnp.concatenate(e, axis=1))
            pt, pb_ = jnp.concatenate(p[0], axis=0), jnp.concatenate(p[1], axis=0)

            def tile(x, t):
                return x[:, t * L:(t + 1) * L]
            ops = [_left(tile(pt, 2 * c), tile(pt, 2 * c + 1), tile(pb_, 2 * c), tile(pb_, 2 * c + 1))
                   for c in range(i)]
            left = [jnp.concatenate([o[n] for o in ops], axis=1).astype(BF16) for n in range(7)] if i else None
            inv = []
            for x in () if again else sums:
                l = jnp.sum(jnp.concatenate(x, axis=0), axis=1, keepdims=True)
                r = pl.reciprocal(l, approx=True)
                inv.append(r * (2.0 - l * r))
            return (left, jnp.concatenate([tile(pt, 2 * i), tile(pb_, 2 * i)], axis=0).astype(BF16),
                    tile(pb_, 2 * i + 1).astype(BF16), inv)

        def pv(i, left, p1, p2, inv):
            r0 = i * HQ
            m, pieces = {}, []
            for n in (2, 3, 0, 4, 1, 5, 6) if i else ():
                m[n] = jnp.dot(left[n], right_operand(n, v_s, v5_s, 0, i), preferred_element_type=F32)
                pieces += spots(m[n], (0,), (0, 32, 64, 96))
            c1 = jnp.dot(p1, _as_bf16(v_s[r0:r0 + 64, :]), preferred_element_type=F32)
            c2 = jnp.dot(p2, _as_bf16(v_s[r0 + 64:r0 + HQ, :]), preferred_element_type=F32)
            top, bot = c1[:L], c1[L:] + c2
            if i:
                top = top + jnp.concatenate([_c11(m), _c12(m)], axis=1)
                bot = bot + jnp.concatenate([_c21(m), _c22(m)], axis=1)
            else:
                pieces = spots(c1, (0, 1))
            if inv:
                top, bot = top * inv[0], bot * inv[1]
            us = [_to_u32(o) for o in _right(top[:, :L], bot[:, :L], top[:, L:], bot[:, L:])]
            for n in range(7):
                x7_s[n, h, i * 64:(i + 1) * 64, :] = us[n]
            waiting.extend(_or_all([us[n][g * 8:(g + 1) * 8] for n in SUMS]) for g in range(8))
            return pieces

        def wo_operands(pieces):
            groups = M // 64
            never2 = jnp.concatenate([never, never], axis=0)
            share = -(-(H // 2) * groups // (H - 1))
            for k in range(share):
                u = jnp.minimum(h * share + k, (H // 2) * groups - 1)
                pair = jax.lax.div(u, groups)
                rg = u - pair * groups
                ops = [_left(*[wo_s[2 * pair + par, pl.ds(pl.multiple_of(hf * mh + sub * (mh // 2) + rg * 16, 16), 16),
                                    ch * L:(ch + 1) * L].astype(F32) for hf in range(2) for ch in range(2)])
                       for sub in range(2) for par in range(2)]
                for n in range(7):
                    link = pieces[int(0.95 * (k * 7 + n) / (share * 7) * len(pieces))]
                    gate = jnp.concatenate([link, link], axis=0)
                    us = [_to_u32(o) for o in _left(*[jnp.where(never2, gate, o[n]) for o in ops])]
                    for x in range(7):
                        wo_ops[n, x, pair, pl.ds(pl.multiple_of(rg * 8, 8), 8), :] = us[x]
                    waiting.append(_or_all(us))

        scores, probs, pieces = {}, {}, []
        for op in order.split():
            i = int(op[1:])
            if op[0] in "Gg":
                pieces.append(proj(i, op[0] == "g"))
            elif op[0] == "c":
                combine(sum(pieces[-i:], []))
            elif op[0] == "w":
                write_kv()
            elif op[0] == "o":
                wo_operands(pieces[-1])
            elif op[0] in "Qr":
                scores[i], new = qk(i, op[0] == "r")
                pieces.append(new)
            elif op[0] == "S":
                probs[i] = softmax(i, *scores.pop(i), pieces[-1])
            elif op[0] == "t":
                probs[i] = softmax(i, *scores.pop(i), pieces[-2] + pieces[-1], again=True)
            elif op[0] == "V":
                pieces.append(pv(i, *probs.pop(i)))
            else:
                hooks[i](pieces)

    def phase1(c_s, wq_r, wk_r, wv_r, wg_s, wu_s, wd_s, xa_s, wq0_s, wq1_s, wr_s, gw_s):
        def x_copy(j):
            return pltpu.make_async_copy(xT_hbm.at[:, pl.ds(j * RC, RC)], xT_s.at[:, pl.ds(j * RC, RC)],
                                         sem.at[S_X + j])

        def wq_copy(g, j):
            return pltpu.make_async_copy(wq_hbm.at[:, pl.ds(j * mq, mq), g], wq_r.at[:, pl.ds(j * mq, mq), g],
                                         sem.at[(S_Q1 if g else S_Q0) + j])

        def kv_copies(j):
            return [pltpu.make_async_copy(src.at[pl.ds(j * n, n)], dst.at[pl.ds(j * n, n)], sem.at[s0 + j])
                    for src, dst, s0, n in ((c_hbm, c_s, S_C, RC), (wk_hbm, wk_r, S_K, mk), (wv_hbm, wv_r, S_V, mk))]

        misc = [pltpu.make_async_copy(a, b, sem.at[S_MISC + i]) for i, (a, b) in enumerate(
            [(wr_hbm, wr_s), (gw_hbm, gw_s), (wg_hbm, wg_s), (wu_hbm, wu_s), (wd_hbm, wd_s)])]

        x_copy(0).start()
        for j in range(NCH):
            wq_copy(0, j).start()
        for j in range(NCH):
            if j + 1 < NCH:
                x_copy(j + 1).start()
            wq_copy(1, j).start()
        misc[0].start()
        misc[1].start()
        for j in range(NCH):
            for cp in kv_copies(j):
                cp.start()
        for cp in misc[2:]:
            cp.start()
        wo_copy.start()

        def x_operands(j):
            c0 = j * RC if isinstance(j, int) else pl.multiple_of(j * RC, RC)
            r0 = j * HQ if isinstance(j, int) else pl.multiple_of(j * HQ, HQ)
            a = [xT_s[kh * mh:(kh + 1) * mh, pl.ds(c0 + rb * TQ, TQ)].astype(F32)
                 for rb in range(2) for kh in range(2)]
            for n, o in enumerate(_left(*a)):
                xa_s[n, pl.ds(r0, HQ), :] = pltpu.bitcast(o.astype(BF16).T, U32)

        def wq_operands(g, p, never=None, link=None):
            w = [pltpu.bitcast(wq_r[kh, pl.ds(2 * p, 2), g], U32) for kh in range(2)]
            w = [[x[0], x[1]] for x in w]
            if link is not None:
                w[0][0] = jnp.where(never, link, w[0][0])
            rows = [_right(*[_unpack(w[kh][e], par) for kh in range(2) for par in range(2)]) for e in range(2)]
            for n in range(7):
                (wq0_s, wq1_s)[g][n, pl.ds(p, 8, stride=pq), :] = _pack(rows[0][n], rows[1][n])

        x_copy(0).wait()
        x_operands(0)

        def first_half(j, _):
            wq_copy(0, j).wait()
            for k in range(mq // 2):
                wq_operands(0, j * (mq // 2) + k)
            return 0
        jax.lax.fori_loop(0, NCH, first_half, 0)

        def q_step(g, j, side):
            pieces = []
            for r in range(4):
                m = {}
                for n in (0, 3, 4, 6, 1, 2, 5):
                    w = jnp.concatenate([_as_bf16((wq0_s, wq1_s)[g][n, pl.ds((dt * 4 + r) * pq, mh // 2), :])
                                         for dt in range(2)], axis=1)
                    m[n] = jnp.dot(_as_bf16(xa_s[n, pl.ds(pl.multiple_of(j * HQ, HQ), HQ), :]), w,
                                   preferred_element_type=F32)
                    for k in range(5):
                        pieces.append(m[n][k * 48:k * 48 + 8, (k % 2) * L:(k % 2 + 1) * L])
                        side(len(pieces) - 1, pieces[-1])
                for par, rb, comb in ((0, 0, _c11), (0, 1, _c21), (1, 0, _c12), (1, 1, _c22)):
                    r0 = pl.multiple_of(j * TQ + rb * HQ, HQ)
                    q_s[8 * g + 2 * r + par, pl.ds(r0, HQ), :] = _to_u32(comb(m) * qscale)

        def q_lo(j, _):
            never = _never(j)

            def side(k, piece):
                if k == 35:
                    @pl.when(j + 1 < NCH)
                    def _():
                        x_copy(j + 1).wait()
                    wq_copy(1, j).wait()
                if k >= 42 and k % 3 == 0 and (k - 42) // 3 < mq // 2:
                    wq_operands(1, j * (mq // 2) + (k - 42) // 3, never, pltpu.bitcast(piece, U32))
            q_step(0, j, side)
            x_operands((j + 1) & (NCH - 1))
            return 0
        jax.lax.fori_loop(0, NCH, q_lo, 0)

        def q_hi(j, _):
            for cp in kv_copies(j):
                cp.wait()
            never = _never(j)
            quad = []

            def side(kk, piece):
                if kk >= 128:
                    return
                k, g = kk // 2, kk % 2
                link = pltpu.bitcast(piece, U32)
                if g == 0:
                    rg, t = k // 8 + 8 * (k % 4 // 2), k // 4 % 2 + 2 * (k % 2)
                    a = []
                    for rb in range(2):
                        r0 = pl.multiple_of(j * RC + rb * TQ + rg * 16, 16)
                        for ch in range(2):
                            a.append(c_s[pl.ds(r0, 16), (2 * t + ch) * L:(2 * t + ch + 1) * L].astype(F32))
                    a[0] = jnp.where(jnp.concatenate([never, never], axis=0),
                                     jnp.concatenate([piece, piece], axis=0), a[0])
                    ops = _left(*a)
                    us = [_shuffled_u32(ops[n]) for n in FLAT]
                    d0 = pl.multiple_of(j * HQ + rg * 8, 8)
                    for n, u in enumerate(us):
                        a_s[n, pl.ds(d0, 8), t * L:(t + 1) * L] = u
                    quad.append(ops)
                    if len(quad) == 4:
                        d0 = pl.multiple_of(j * (HQ // 2) + (rg - 8) * 8, 8)
                        for e, n in enumerate(DEEP):
                            deep = [_shuffled_u32(o) for o in _left(*[q[n] for q in quad])]
                            for x, u in enumerate(deep):
                                a2_s[e, x, pl.ds(d0, 8), (t - 2) * L:(t - 1) * L] = u
                            us += deep
                        del quad[:]
                    link = _or_all(us)
                c0 = j * mk + 2 * k
                w = [pltpu.bitcast(r[pl.ds(c0 + o, 2), g], U32) for o in (0, L) for r in (wk_r, wv_r)]
                w = [[x[0], x[1]] for x in w]
                w[0][0] = jnp.where(never, link, w[0][0])
                for par in range(2):
                    rows = [_right(*[_unpack(x[e], par) for x in w]) for e in range(2)]
                    for n in range(7):
                        b_s[n, 2 * g + par, pl.ds(j * (mk // 4) + k, 8, stride=pb), :] = _pack(
                            rows[0][n], rows[1][n])
            q_step(1, j, side)
            return j
        never = _never(jax.lax.fori_loop(0, NCH, q_hi, 0))

        for cp in misc:
            cp.wait()
        st = {}
        F = wg_s.shape[1]

        def route(pieces):
            pieces = pieces[-2] + pieces[-1]
            mp = -(-M // L) * L
            cols = []
            for w_s in (wr_s, gw_s):
                w = jnp.concatenate([w_s[...].reshape(1, M).astype(F32), jnp.zeros((1, mp - M), F32)], axis=1)
                cols.append(jnp.broadcast_to(w, (L, mp)).T)
            nr, rows = 4, M // 4
            out, k, prev = ([], []), 0, None
            for ct in range(S // L):
                acc = [None, None]
                for q in range(nr):
                    link = pieces[int((0.03 + 0.65 * k / (nr * S // L)) * len(pieces))]
                    if prev is not None:
                        link = jnp.where(never, link, prev)
                    k += 1
                    x = linked(xT_s[q * rows:(q + 1) * rows, ct * L:(ct + 1) * L], link)
                    for t in range(2):
                        part = fold(x * cols[t][q * rows:(q + 1) * rows], 0)
                        acc[t] = part if acc[t] is None else acc[t] + part
                    prev = acc[0] + acc[1]
                for t in range(2):
                    out[t].append(jnp.sum(acc[t], axis=0, keepdims=True))
            g_s[0:1, :] = jax.nn.sigmoid(jnp.concatenate(out[1], axis=1))
            r = jnp.concatenate(out[0], axis=1).astype(BF16).astype(F32)
            lane = jax.lax.broadcasted_iota(jnp.int32, (1, S), 1)
            m1 = jnp.max(r, axis=1, keepdims=True)
            i1 = jnp.min(jnp.where(r == m1, lane, S - 1), axis=1, keepdims=True)
            r2 = jnp.where(lane == i1, -jnp.inf, r)
            m2 = jnp.max(r2, axis=1, keepdims=True)
            i2 = jnp.min(jnp.where(jnp.logical_and(r2 == m2, lane != i1), lane, S - 1), axis=1, keepdims=True)
            ln = jax.lax.broadcasted_iota(jnp.int32, (M, L), 1)
            st["c0"] = [pl.multiple_of((i[0, 0] >> 7) << 7, L) for i in (i1, i2)]
            st["hit"] = [ln == (i & (L - 1)) for i in (i1, i2)]
            st["r"] = [jax.nn.sigmoid(m1), jax.nn.sigmoid(m2)]
            st["x"] = [jnp.broadcast_to(jnp.sum(jnp.where(hit, xT_s[:, pl.ds(c0, L)].astype(F32), 0.0),
                                                axis=1, keepdims=True), (M, L))
                       for c0, hit in zip(st["c0"], st["hit"])]

        def fold(v, axis):
            parts = [v[k * 8:(k + 1) * 8] if axis == 0 else v[:, k * L:(k + 1) * L]
                     for k in range(v.shape[axis] // (8, L)[axis])]
            while len(parts) > 1:
                parts = [parts[k] + parts[k + 1] if k + 1 < len(parts) else parts[k]
                         for k in range(0, len(parts), 2)]
            return parts[0]

        def linked(w, link):
            w = pltpu.bitcast(w, U32)
            reps = (w.shape[0] // 8, w.shape[1] // L)
            w = jnp.where(jnp.tile(never, reps), jnp.tile(pltpu.bitcast(link, U32), reps), w)
            return _as_bf16(w).astype(F32)

        def hidden(pieces):
            pieces = pieces[-3] + pieces[-2] + pieces[-1]
            nr, rows = 4, M // 4
            total = 2 * (F // L) * nr
            out, k, prev = [], 0, None
            for w_s in (wg_s, wu_s):
                cols = ([], [])
                for ct in range(F // L):
                    acc = [None, None]
                    for q in range(nr):
                        link = pieces[int(0.9 * k / total * len(pieces))]
                        if prev is not None:
                            link = jnp.where(never, link, prev)
                        k += 1
                        w = linked(w_s[q * rows:(q + 1) * rows, ct * L:(ct + 1) * L], link)
                        for t in range(2):
                            part = fold(w * st["x"][t][q * rows:(q + 1) * rows], 0)
                            acc[t] = part if acc[t] is None else acc[t] + part
                        prev = acc[0] + acc[1]
                    for t in range(2):
                        cols[t].append(jnp.sum(acc[t], axis=0, keepdims=True))
                out.append([jnp.concatenate(c, axis=1) for c in cols])
            st["h"] = [(jax.nn.silu(out[0][t]) * out[1][t]).astype(BF16).astype(F32) for t in range(2)]

        def patch(pieces):
            pieces = pieces[-2] + pieces[-1]
            half = F // 2
            ys, k, prev = ([], []), 0, None
            for rg in range(M // 16):
                acc = [None, None]
                for hf in range(2):
                    link = pieces[int((0.1 + 0.8 * k / (M // 8)) * len(pieces))]
                    if prev is not None:
                        link = jnp.where(never, link, prev)
                    k += 1
                    w = linked(wd_s[rg * 16:(rg + 1) * 16, hf * half:(hf + 1) * half], link)
                    for t in range(2):
                        part = fold(w * st["h"][t][:, hf * half:(hf + 1) * half], 1)
                        acc[t] = part if acc[t] is None else acc[t] + part
                    prev = fold(acc[0] + acc[1], 0)
                for t in range(2):
                    ys[t].append(jnp.sum(acc[t], axis=1, keepdims=True))
            for t in range(2):
                y = jnp.concatenate(ys[t], axis=0) * st["r"][t]
                blk = xT_s[:, pl.ds(st["c0"][t], L)].astype(F32)
                xT_s[:, pl.ds(st["c0"][t], L)] = (blk + jnp.where(st["hit"][t], y, 0.0)).astype(BF16)

        head_program(FIRST_ORDER, None, 0, never, hooks=(route, hidden, patch))

    def phase2(x7_s, wo_ops):
        wo_copy.wait()
        col = jax.lax.broadcasted_iota(jnp.int32, (L, L), 1)
        tri = ((col & ~15) + ((col & 3) << 2) + ((col & 15) >> 2)
               <= jax.lax.broadcasted_iota(jnp.int32, (L, L), 0))

        def head(h, _):
            head_program(LOOP_ORDER, h, h + 1, _never(h), x7_s, tri, wo_ops, span=0.96)
            return h
        last = jax.lax.fori_loop(0, H - 1, head, 0)
        head_program(LAST_ORDER, H - 1, None, _never(last), x7_s, tri)

        def out_step(j, _):
            c0 = pl.multiple_of(j * RC, RC)
            m = ({}, {})
            for n in range(7):
                right = [[] for _ in range(7)]
                for pair in range(H // 2):
                    blk = [_as_bf16(x7_s[n, 2 * pair + par, pl.ds(pl.multiple_of(j * L + t * 64, 64), 64), :])
                           for par in range(2) for t in range(2)]
                    ops = list(_right(*[v.astype(F32) for v in blk]))
                    ops[1], ops[4] = blk[0], blk[3]
                    for x in range(7):
                        right[x].append(ops[x])
                mm = {x: jax.lax.dot_general(
                    jnp.concatenate([_as_bf16(wo_ops[n, x, pair, :M // 8]) for pair in range(H // 2)], axis=1),
                    jnp.concatenate(right[x], axis=1).astype(BF16), NT, preferred_element_type=F32)
                    for x in (4, 2, 1, 5, 0, 3, 6)}
                m[0][n] = jnp.concatenate([((mm[0] + mm[3]) - mm[4]) + mm[6], _c21(mm)], axis=0)
                m[1][n] = jnp.concatenate([_c12(mm), _c22(mm)], axis=0)
            gate = g_s[0:1, pl.ds(c0, RC)]
            for hf in (1, 0):
                rest = (1.0 - gate) * xT_s[hf * mh:(hf + 1) * mh, pl.ds(c0, RC)].astype(F32)
                cols = []
                for t in range(RC // TQ):
                    gl, gr = gate[:, t * TQ:t * TQ + L], gate[:, t * TQ + L:(t + 1) * TQ]
                    rl, rr = rest[:, t * TQ:t * TQ + L], rest[:, t * TQ + L:(t + 1) * TQ]
                    if hf:
                        cols += [gl * _c21(m[t]) + rl, gr * _c22(m[t]) + rr]
                    else:
                        cols += [(gl * ((m[t][0] + m[t][3]) - m[t][4]) + rl) + gl * m[t][6], gr * _c12(m[t]) + rr]
                o_s[hf * mh:(hf + 1) * mh, pl.ds(c0, RC)] = jnp.concatenate(cols, axis=1).astype(BF16)
                out_copy(j, hf).start()
            return 0
        jax.lax.fori_loop(0, S // RC, out_step, 0)
        for j in range(S // RC):
            for hf in range(2):
                out_copy(j, hf).wait()

    pl.run_scoped(
        phase1,
        *[pltpu.VMEM(r.shape, r.dtype) for r in (c_hbm, wq_hbm, wk_hbm, wv_hbm, wg_hbm, wu_hbm, wd_hbm)],
        pltpu.VMEM((7, S // 4, mh), U32),
        pltpu.VMEM((7, -(-pq // 4) * 32, L), U32),
        pltpu.VMEM((7, -(-pq // 4) * 32, L), U32),
        pltpu.VMEM((M,), BF16),
        pltpu.VMEM((M,), BF16))
    pl.run_scoped(phase2, pltpu.VMEM((7, H, S // 4, L), U32), pltpu.VMEM((7, 7, H // 2, 64, L), U32))


def _tile_view(w):
    c, h, d = w.shape
    w = w.reshape(c, h // 8, 8, d // L, L).transpose(0, 1, 3, 2, 4)
    return w.reshape(c, h // 8, 8 * (d // L), L)


@jax.jit
def pallas_gated_mix__compressed_kv_cla__moe_arch_mod__prompt_kernel(
    A_x: jax.Array,
    A_c_kv: jax.Array,
    A_w_q: jax.Array,
    A_w_uk: jax.Array,
    A_w_uv: jax.Array,
    A_w_o: jax.Array,
    B_x: jax.Array,
    B_w_r: jax.Array,
    B_w_gate: jax.Array,
    B_w_up: jax.Array,
    B_w_down: jax.Array,
    gate_w: jax.Array,
):
    _, S, M = A_x.shape
    DC = A_c_kv.shape[2]
    H, D = A_w_q.shape[1], A_w_q.shape[2]
    args = (jnp.transpose(A_x[0]), A_c_kv[0], _tile_view(A_w_q).reshape(2, M // 2, 2, 16, L),
            _tile_view(A_w_uk), _tile_view(A_w_uv),
            jnp.transpose(A_w_o, (0, 2, 1)), B_w_r, gate_w, B_w_gate, B_w_up, jnp.transpose(B_w_down))

    def kern(*refs):
        _kernel(*refs, S=S, M=M, DC=DC, H=H, D=D)

    hbm = pl.BlockSpec(memory_space=pl.ANY)
    oT = pl.pallas_call(
        kern,
        out_shape=jax.ShapeDtypeStruct((M, S), A_x.dtype),
        in_specs=[hbm] * len(args),
        out_specs=hbm,
        scratch_shapes=[
            pltpu.VMEM((8, S), F32),
            pltpu.VMEM((M, S), BF16),
            pltpu.VMEM((H, M, D), BF16),
            pltpu.VMEM((5, S // 4, DC // 2), U32),
            pltpu.VMEM((2, 7, S // 8, DC // 4), U32),
            pltpu.VMEM((7, 4, 8 * (DC // 4 + 1), L), U32),
            pltpu.VMEM((H, S // 2, D), U32),
            pltpu.VMEM((S // 2, D), U32),
            pltpu.VMEM((S // 2, D), U32),
            pltpu.VMEM((5, S // 4, L), U32),
            pltpu.VMEM((M, S), BF16),
            pltpu.VMEM((5, S // 4 + PAD_V, L), U32),
            pltpu.SemaphoreType.DMA((N_SEM,)),
        ],
        compiler_params=pltpu.CompilerParams(vmem_limit_bytes=124 * 1024 * 1024, disable_bounds_checks=True,
                                             disable_semaphore_checks=True),
    )(*args)
    return jnp.transpose(oT)[None]
```

```python
import math

import jax
import jax.numpy as jnp
import jax.experimental.pallas as pl
import jax.experimental.pallas.tpu as pltpu

F32 = jnp.float32
BF16 = jnp.bfloat16
U32 = jnp.uint32
NT = (((1,), (1,)), ((), ()))

L = 128
TQ = 256
HQ = TQ // 2
RC = 512
NCH = 4

PAD_V = 16

S_X, S_Q0, S_Q1, S_K, S_V, S_C, S_MISC, S_OUT = 0, 4, 8, 12, 16, 20, 24, 30
N_SEM = 38

LOOP_ORDER = ("Q0 Q7 S0 G0 S7 V0 V7 o0 Q6 G3 S6 V6 Q5 G4 S5 V5 Q4 G5 S4 V4 Q3 G6 S3 V3 Q2 g2 S2 V2 "
              "Q1 c2 G1 S1 V1 w0")
FIRST_ORDER = "G0 G2 h0 G3 G4 G6 h1 G5 G1 h2 w0"
LAST_ORDER = "Q7 Q6 Q5 t7 V7 S6 Q4 V6 S5 r3 V5 S4 r2 V4 S3 r1 V3 S2 r0 V2 S1 S0 V1 V0"


def _to_u32(x_f32):
    return pltpu.bitcast(x_f32.astype(BF16), U32)


def _shuffled_u32(x_f32):
    return jnp.concatenate([_pack(x_f32[r:r + 8], x_f32[r + 8:r + 16]) for r in range(0, x_f32.shape[0], 16)],
                           axis=0)


def _as_bf16(x_u32):
    return pltpu.bitcast(x_u32, BF16)


def _left(a11, a12, a21, a22):
    return (a11 + a22, a21 + a22, a11, a22, a11 + a12, a21 - a11, a12 - a22)


def _right(b11, b12, b21, b22):
    return (b11 + b22, b11, b12 - b22, b21 - b11, b22, b11 + b12, b21 + b22)


FLAT, DEEP = (0, 1, 3, 4, 6), (2, 5)
SUMS = (0, 2, 3, 5, 6)


def _c11(m):
    return (m[0] + m[3]) + (m[6] - m[4])


def _c12(m):
    return m[2] + m[4]


def _c21(m):
    return m[1] + m[3]


def _c22(m):
    return (m[0] - m[1]) + (m[2] + m[5])


def _never(i):
    return jax.lax.broadcasted_iota(jnp.int32, (8, L), 0) < (i >> 10)


def _or_all(xs):
    out = xs[0]
    for x in xs[1:]:
        out = out | x
    return out


def _unpack(w, par):
    return pltpu.unpack_elementwise(w, index=par, packed_dtype=BF16, unpacked_dtype=F32)


def _pack(even, odd):
    return pltpu.bitcast(pltpu.pack_elementwise([even, odd], packed_dtype=BF16), U32)


def _head_weight(ref, h, nrows, pitch):
    sel = ((h >> 3) << 1) + (h & 1)
    r = (h >> 1) & 3
    return jnp.concatenate(
        [_as_bf16(ref[sel, pl.ds((dt * 4 + r) * pitch, nrows), :]) for dt in range(2)], axis=1)


def _kernel(xT_hbm, c_hbm, wq_hbm, wk_hbm, wv_hbm, wo_hbm, wr_hbm, gw_hbm, wg_hbm, wu_hbm, wd_hbm,
            o_hbm,
            g_s, xT_s, wo_s, a_s, a2_s, b_s, q_s, k_s, v_s, k5_s, o_s, v5_s, sem, *, S, M, DC, H, D):
    nq = S // TQ
    mh = M // 2
    pq = mh // 2 + 1
    pb = DC // 4 + 1
    mq = mh // NCH
    mk = DC // NCH
    qscale = (D ** -0.5) * math.log2(math.e)
    neg = -1e9 * math.log2(math.e)
    wo_copy = pltpu.make_async_copy(wo_hbm, wo_s, sem.at[S_MISC + 5])

    def out_copy(j, hf):
        return pltpu.make_async_copy(o_s.at[j, pl.ds(hf * mh, mh)],
                                     o_hbm.at[pl.ds(hf * mh, mh), pl.ds(j * RC, RC)], sem.at[S_OUT + 2 * j + hf])

    def head_program(order, h, hn, never, x7_s=None, tri=None, wo_ops=None, span=0.9, hooks=None):
        prods, held, waiting = {}, {}, []

        def spots(v, cols, rows=(0, 64, 128, 192)):
            return [v[r:r + 8, n * L:(n + 1) * L] for n in cols for r in rows]

        def tie(lhs, links, every):
            rows = []
            for rg in range(lhs.shape[0] // 8):
                blk = lhs[rg * 8:(rg + 1) * 8]
                if links and rg % every == 0:
                    blk = jnp.concatenate([jnp.where(never, links.pop(0), blk[:, :L]), blk[:, L:]], axis=1)
                rows.append(blk)
            return jnp.concatenate(rows, axis=0)

        combos = [("k", 0, _c11, (0, 3, 4, 6)), ("k", 1, _c21, (1, 3)),
                  ("v", 0, _c12, (2, 4)), ("v", 1, _c22, (0, 1, 2, 5))]

        def combine(pieces):
            ready = [c for c in combos if all(x in prods for x in c[3])]
            for e, (key, odd, comb, needs) in enumerate(ready):
                combos.remove((key, odd, comb, needs))
                for k in range(nq // 2):
                    m = {x: prods[x][k * TQ:(k + 1) * TQ] for x in needs}
                    if pieces:
                        rows = []
                        for g in range(8):
                            at = ((e * (nq // 2) + k) * 8 + g) / (len(ready) * (nq // 2) * 8)
                            rows.append(jnp.tile(pieces[int(0.95 * at * len(pieces))], (2, 2)))
                        m[needs[0]] = jnp.where(jnp.tile(never, (32, 2)), jnp.concatenate(rows + rows, axis=0),
                                                m[needs[0]])
                    c = comb(m)
                    held[2 * k + odd, key] = _shuffled_u32(c)
                    if 2 * k + odd < nq - 1:
                        off = (c[:L, L:], c[L:, :L]) if key == "v" else (c[L:, :L], c[:L, L:])
                        ops = _right(c[:L, :L], *off, c[L:, L:])
                        held[2 * k + odd, key + "5"] = [_shuffled_u32(ops[x]) for x in SUMS]

        def proj(n, lazy):
            w = _head_weight(b_s.at[n], hn, DC // 4, pb)
            links = list(waiting)
            del waiting[:]
            if n in DEEP:
                wf, kh = w.astype(F32), DC // 4
                right = [o.astype(BF16) for o in _right(wf[:kh, :L], wf[:kh, L:], wf[kh:, :L], wf[kh:, L:])]
                right[1], right[4] = w[:kh, :L], w[kh:, L:]
                m, pieces = {}, []

                def sub(x, after):
                    lhs = a2_s[DEEP.index(n), x]
                    if after:
                        t = after[0]
                        for v in after[1:]:
                            t = jnp.maximum(t, v)
                        lhs = tie(lhs, [pltpu.bitcast(jnp.maximum(t[g * 16:g * 16 + 8], t[g * 16 + 8:g * 16 + 16]), U32)
                                        for g in range(S // 64)], 1)
                    elif links:
                        lhs = tie(lhs, links, lhs.shape[0] // 8 // len(links))
                    m[x] = jnp.dot(_as_bf16(lhs), right[x], preferred_element_type=F32)
                    pieces.extend(spots(m[x], (0,), range(0, S // 4, 64)))
                sub(1, ()), sub(3, ())
                c21 = m[1] + m[3]
                sub(2, ()), sub(4, (c21,))
                c12, c11, c22 = m[2] + m[4], m[3] - m[4], m[2] - m[1]
                sub(0, ()), sub(5, (c12, c11, c22))
                c11, c22 = c11 + m[0], c22 + (m[0] + m[5])
                sub(6, (c11, c22))
                top = jnp.concatenate([c11 + m[6], c12], axis=1)
                bot = jnp.concatenate([c21, c22], axis=1)
                prods[n] = jnp.concatenate([v[k * L:(k + 1) * L] for k in range(nq // 2) for v in (top, bot)],
                                           axis=0)
            else:
                lhs = a_s[FLAT.index(n)]
                if links:
                    lhs = tie(lhs, links, max(1, lhs.shape[0] // 8 // len(links)))
                prods[n] = jnp.dot(_as_bf16(lhs), w, preferred_element_type=F32)
                pieces = spots(prods[n], (0, 1), range(0, S // 2, 32))
            if not lazy:
                combine(None)
            return pieces

        def write_kv():
            for ch in reversed(range(nq)):
                k_s[ch * HQ:(ch + 1) * HQ, :] = held[ch, "k"]
                v_s[ch * HQ:(ch + 1) * HQ, :] = held[ch, "v"]
                for key, ref in (("k5", k5_s), ("v5", v5_s)):
                    for n, o in enumerate(held.get((ch, key), ())):
                        ref[n, ch * 64:(ch + 1) * 64, :] = o

        def right_operand(n, plain, sums, c0, c1):
            if n == 1:
                return jnp.concatenate([_as_bf16(plain[c * HQ:c * HQ + 64, :L]) for c in range(c0, c1)], axis=0)
            if n == 4:
                return jnp.concatenate([_as_bf16(plain[c * HQ + 64:(c + 1) * HQ, L:]) for c in range(c0, c1)], axis=0)
            return _as_bf16(sums[SUMS.index(n), c0 * 64:c1 * 64, :])

        def qk(i, tied):
            q = qd = q_s[h, i * HQ:(i + 1) * HQ, :]
            n = len(waiting) - 8 if tied else 0
            if n > 0:
                qd = tie(q, waiting[:n], 16 // n)
                del waiting[:n]
            q, qd = _as_bf16(q), _as_bf16(qd)
            tops, bots, pieces = [], [], []
            if i:
                qf = q.astype(F32)
                left = [o.astype(BF16) for o in _left(qf[:L, :L], qf[:L, L:], qf[L:, :L], qf[L:, L:])]
                left[2], left[3] = q[:L, :L], q[L:, L:]
            done = []
            for c in range(i):
                lhs = dict(enumerate(left))
                if c >= 2:
                    u = pltpu.bitcast(left[0], U32)
                    lhs[0] = _as_bf16(jnp.concatenate(
                        [jnp.where(never, done[c - 2][g], u[g * 8:(g + 1) * 8]) for g in range(8)], axis=0))
                m = {n: jax.lax.dot_general(lhs[n], right_operand(n, k_s, k5_s, c, c + 1), NT,
                                            preferred_element_type=F32) for n in (0, 3, 4, 6, 1, 2, 5)}
                c11, c12, c21, c22 = _c11(m), _c12(m), _c21(m), _c22(m)
                tops += [c11, c12]
                bots += [c21, c22]
                t = jnp.maximum(jnp.maximum(c11, c12), jnp.maximum(c21, c22))
                done.append([pltpu.bitcast(jnp.maximum(t[g * 16:g * 16 + 8], t[g * 16 + 8:(g + 1) * 16]), U32)
                             for g in range(8)])
                for n in (0, 5):
                    pieces += spots(m[n], (0,), (0, 32, 64, 96))
            r0 = i * HQ
            s1 = jax.lax.dot_general(qd, _as_bf16(k_s[r0:r0 + 64, :]), NT, preferred_element_type=F32)
            s2 = jax.lax.dot_general(q[L:], _as_bf16(k_s[r0 + 64:r0 + HQ, :]), NT, preferred_element_type=F32)
            top = jnp.concatenate(tops + [jnp.where(tri, s1[:L], neg)], axis=1)
            bot = jnp.concatenate(bots + [s1[L:], jnp.where(tri, s2, neg)], axis=1)
            return (top, bot), pieces + spots(s1, (0,))

        def softmax(i, top, bot, pieces, again=False):
            p, sums, prev = ([], []), ([], []), None
            for k in range(TQ // 8):
                half = k % 2
                s = (top, bot)[half][(k // 2) * 8:(k // 2 + 1) * 8]
                link = pieces[int(span * k * 8 / TQ * len(pieces))]
                if prev is not None:
                    link = jnp.where(never, link, prev)
                m = jnp.broadcast_to(jnp.max(s, axis=1, keepdims=True), (8, L))
                m = jnp.where(never, link, m)
                e = [jnp.exp2(s[:, t:t + L] - m) for t in range(0, s.shape[1], L)]
                prev = e[0]
                for x in e[1:]:
                    prev = prev + x
                if again:
                    m = m + jnp.log2(jnp.sum(prev, axis=1, keepdims=True))
                    e = [jnp.exp2(s[:, t:t + L] - m) for t in range(0, s.shape[1], L)]
                sums[half].append(prev)
                p[half].append(jnp.concatenate(e, axis=1))
            pt, pb_ = jnp.concatenate(p[0], axis=0), jnp.concatenate(p[1], axis=0)

            def tile(x, t):
                return x[:, t * L:(t + 1) * L]
            ops = [_left(tile(pt, 2 * c), tile(pt, 2 * c + 1), tile(pb_, 2 * c), tile(pb_, 2 * c + 1))
                   for c in range(i)]
            left = [jnp.concatenate([o[n] for o in ops], axis=1).astype(BF16) for n in range(7)] if i else None
            inv = []
            for x in () if again else sums:
                l = jnp.sum(jnp.concatenate(x, axis=0), axis=1, keepdims=True)
                r = pl.reciprocal(l, approx=True)
                inv.append(r * (2.0 - l * r))
            return (left, jnp.concatenate([tile(pt, 2 * i), tile(pb_, 2 * i)], axis=0).astype(BF16),
                    tile(pb_, 2 * i + 1).astype(BF16), inv)

        def pv(i, left, p1, p2, inv):
            r0 = i * HQ
            m, pieces = {}, []
            for n in (2, 3, 0, 4, 1, 5, 6) if i else ():
                m[n] = jnp.dot(left[n], right_operand(n, v_s, v5_s, 0, i), preferred_element_type=F32)
                pieces += spots(m[n], (0,), (0, 32, 64, 96))
            c1 = jnp.dot(p1, _as_bf16(v_s[r0:r0 + 64, :]), preferred_element_type=F32)
            c2 = jnp.dot(p2, _as_bf16(v_s[r0 + 64:r0 + HQ, :]), preferred_element_type=F32)
            top, bot = c1[:L], c1[L:] + c2
            if i:
                top = top + jnp.concatenate([_c11(m), _c12(m)], axis=1)
                bot = bot + jnp.concatenate([_c21(m), _c22(m)], axis=1)
            else:
                pieces = spots(c1, (0, 1))
            if inv:
                top, bot = top * inv[0], bot * inv[1]
            us = [_to_u32(o) for o in _right(top[:, :L], bot[:, :L], top[:, L:], bot[:, L:])]
            for n in range(7):
                x7_s[n, h, i * 64:(i + 1) * 64, :] = us[n]
            waiting.extend(_or_all([us[n][g * 8:(g + 1) * 8] for n in SUMS]) for g in range(8))
            return pieces

        def wo_operands(pieces):
            groups = M // 64
            never2 = jnp.concatenate([never, never], axis=0)
            share = -(-(H // 2) * groups // (H - 1))
            for k in range(share):
                u = jnp.minimum(h * share + k, (H // 2) * groups - 1)
                pair = jax.lax.div(u, groups)
                rg = u - pair * groups
                ops = [_left(*[wo_s[2 * pair + par, pl.ds(pl.multiple_of(hf * mh + sub * (mh // 2) + rg * 16, 16), 16),
                                    ch * L:(ch + 1) * L].astype(F32) for hf in range(2) for ch in range(2)])
                       for sub in range(2) for par in range(2)]
                for n in range(7):
                    link = pieces[int(0.95 * (k * 7 + n) / (share * 7) * len(pieces))]
                    gate = jnp.concatenate([link, link], axis=0)
                    us = [_to_u32(o) for o in _left(*[jnp.where(never2, gate, o[n]) for o in ops])]
                    for x in range(7):
                        wo_ops[n, x, pair, pl.ds(pl.multiple_of(rg * 8, 8), 8), :] = us[x]
                    waiting.append(_or_all(us))

        scores, probs, pieces = {}, {}, []
        for op in order.split():
            i = int(op[1:])
            if op[0] in "Gg":
                pieces.append(proj(i, op[0] == "g"))
            elif op[0] == "c":
                combine(sum(pieces[-i:], []))
            elif op[0] == "w":
                write_kv()
            elif op[0] == "o":
                wo_operands(pieces[-1])
            elif op[0] in "Qr":
                scores[i], new = qk(i, op[0] == "r")
                pieces.append(new)
            elif op[0] == "S":
                probs[i] = softmax(i, *scores.pop(i), pieces[-1])
            elif op[0] == "t":
                probs[i] = softmax(i, *scores.pop(i), pieces[-2] + pieces[-1], again=True)
            elif op[0] == "V":
                pieces.append(pv(i, *probs.pop(i)))
            else:
                hooks[i](pieces)

    def phase1(c_s, wq_r, wk_r, wv_r, wg_s, wu_s, wd_s, xa_s, wq0_s, wq1_s, wr_s, gw_s):
        def x_copy(j):
            return pltpu.make_async_copy(xT_hbm.at[:, pl.ds(j * RC, RC)], xT_s.at[j], sem.at[S_X + j])

        def wq_copy(g, j):
            return pltpu.make_async_copy(wq_hbm.at[:, pl.ds(j * mq, mq), g], wq_r.at[:, pl.ds(j * mq, mq), g],
                                         sem.at[(S_Q1 if g else S_Q0) + j])

        def kv_copies(j):
            return [pltpu.make_async_copy(src.at[pl.ds(j * n, n)], dst.at[pl.ds(j * n, n)], sem.at[s0 + j])
                    for src, dst, s0, n in ((c_hbm, c_s, S_C, RC), (wk_hbm, wk_r, S_K, mk), (wv_hbm, wv_r, S_V, mk))]

        misc = [pltpu.make_async_copy(a, b, sem.at[S_MISC + i]) for i, (a, b) in enumerate(
            [(wr_hbm, wr_s), (gw_hbm, gw_s), (wg_hbm, wg_s), (wu_hbm, wu_s), (wd_hbm, wd_s)])]

        x_copy(0).start()
        for j in range(NCH):
            wq_copy(0, j).start()
        for j in range(NCH):
            if j + 1 < NCH:
                x_copy(j + 1).start()
            wq_copy(1, j).start()
        misc[0].start()
        misc[1].start()
        for j in range(NCH):
            for cp in kv_copies(j):
                cp.start()
        for cp in misc[2:]:
            cp.start()
        wo_copy.start()

        def x_operands(j):
            r0 = j * HQ if isinstance(j, int) else pl.multiple_of(j * HQ, HQ)
            a = [xT_s[j, kh * mh:(kh + 1) * mh, rb * TQ:(rb + 1) * TQ].astype(F32)
                 for rb in range(2) for kh in range(2)]
            for n, o in enumerate(_left(*a)):
                xa_s[n, pl.ds(r0, HQ), :] = pltpu.bitcast(o.astype(BF16).T, U32)

        def wq_operands(g, p, never=None, link=None):
            w = [pltpu.bitcast(wq_r[kh, pl.ds(2 * p, 2), g], U32) for kh in range(2)]
            w = [[x[0], x[1]] for x in w]
            if link is not None:
                w[0][0] = jnp.where(never, link, w[0][0])
            rows = [_right(*[_unpack(w[kh][e], par) for kh in range(2) for par in range(2)]) for e in range(2)]
            for n in range(7):
                (wq0_s, wq1_s)[g][n, pl.ds(p, 8, stride=pq), :] = _pack(rows[0][n], rows[1][n])

        x_copy(0).wait()
        x_operands(0)

        def first_half(j, _):
            wq_copy(0, j).wait()
            for k in range(mq // 2):
                wq_operands(0, j * (mq // 2) + k)
            return 0
        jax.lax.fori_loop(0, NCH, first_half, 0)

        def q_step(g, j, side):
            pieces = []
            for r in range(4):
                m = {}
                for n in (0, 3, 4, 6, 1, 2, 5):
                    w = jnp.concatenate([_as_bf16((wq0_s, wq1_s)[g][n, pl.ds((dt * 4 + r) * pq, mh // 2), :])
                                         for dt in range(2)], axis=1)
                    m[n] = jnp.dot(_as_bf16(xa_s[n, pl.ds(pl.multiple_of(j * HQ, HQ), HQ), :]), w,
                                   preferred_element_type=F32)
                    for k in range(5):
                        pieces.append(m[n][k * 48:k * 48 + 8, (k % 2) * L:(k % 2 + 1) * L])
                        side(len(pieces) - 1, pieces[-1])
                for par, rb, comb in ((0, 0, _c11), (0, 1, _c21), (1, 0, _c12), (1, 1, _c22)):
                    r0 = pl.multiple_of(j * TQ + rb * HQ, HQ)
                    q_s[8 * g + 2 * r + par, pl.ds(r0, HQ), :] = _to_u32(comb(m) * qscale)

        def q_lo(j, _):
            never = _never(j)

            def side(k, piece):
                if k == 35:
                    @pl.when(j + 1 < NCH)
                    def _():
                        x_copy(j + 1).wait()
                    wq_copy(1, j).wait()
                if k >= 42 and k % 3 == 0 and (k - 42) // 3 < mq // 2:
                    wq_operands(1, j * (mq // 2) + (k - 42) // 3, never, pltpu.bitcast(piece, U32))
            q_step(0, j, side)
            x_operands((j + 1) & (NCH - 1))
            return 0
        jax.lax.fori_loop(0, NCH, q_lo, 0)

        def q_hi(j, _):
            for cp in kv_copies(j):
                cp.wait()
            never = _never(j)
            quad = []

            def side(kk, piece):
                if kk >= 128:
                    return
                k, g = kk // 2, kk % 2
                link = pltpu.bitcast(piece, U32)
                if g == 0:
                    rg, t = k // 8 + 8 * (k % 4 // 2), k // 4 % 2 + 2 * (k % 2)
                    a = []
                    for rb in range(2):
                        r0 = pl.multiple_of(j * RC + rb * TQ + rg * 16, 16)
                        for ch in range(2):
                            a.append(c_s[pl.ds(r0, 16), (2 * t + ch) * L:(2 * t + ch + 1) * L].astype(F32))
                    a[0] = jnp.where(jnp.concatenate([never, never], axis=0),
                                     jnp.concatenate([piece, piece], axis=0), a[0])
                    ops = _left(*a)
                    us = [_shuffled_u32(ops[n]) for n in FLAT]
                    d0 = pl.multiple_of(j * HQ + rg * 8, 8)
                    for n, u in enumerate(us):
                        a_s[n, pl.ds(d0, 8), t * L:(t + 1) * L] = u
                    quad.append(ops)
                    if len(quad) == 4:
                        d0 = pl.multiple_of(j * (HQ // 2) + (rg - 8) * 8, 8)
                        for e, n in enumerate(DEEP):
                            deep = [_shuffled_u32(o) for o in _left(*[q[n] for q in quad])]
                            for x, u in enumerate(deep):
                                a2_s[e, x, pl.ds(d0, 8), (t - 2) * L:(t - 1) * L] = u
                            us += deep
                        del quad[:]
                    link = _or_all(us)
                c0 = j * mk + 2 * k
                w = [pltpu.bitcast(r[pl.ds(c0 + o, 2), g], U32) for o in (0, L) for r in (wk_r, wv_r)]
                w = [[x[0], x[1]] for x in w]
                w[0][0] = jnp.where(never, link, w[0][0])
                for par in range(2):
                    rows = [_right(*[_unpack(x[e], par) for x in w]) for e in range(2)]
                    for n in range(7):
                        b_s[n, 2 * g + par, pl.ds(j * (mk // 4) + k, 8, stride=pb), :] = _pack(
                            rows[0][n], rows[1][n])
            q_step(1, j, side)
            return j
        never = _never(jax.lax.fori_loop(0, NCH, q_hi, 0))

        for cp in misc:
            cp.wait()
        st = {}
        F = wg_s.shape[1]

        def route(pieces):
            pieces = pieces[-2] + pieces[-1]
            mp = -(-M // L) * L
            cols = []
            for w_s in (wr_s, gw_s):
                w = jnp.concatenate([w_s[...].reshape(1, M).astype(F32), jnp.zeros((1, mp - M), F32)], axis=1)
                cols.append(jnp.broadcast_to(w, (L, mp)).T)
            nr, rows = 4, M // 4
            out, k, prev = ([], []), 0, None
            for ct in range(S // L):
                acc = [None, None]
                for q in range(nr):
                    link = pieces[int((0.03 + 0.65 * k / (nr * S // L)) * len(pieces))]
                    if prev is not None:
                        link = jnp.where(never, link, prev)
                    k += 1
                    x = linked(xT_s[ct * L // RC, q * rows:(q + 1) * rows, pl.ds(ct * L % RC, L)], link)
                    for t in range(2):
                        part = fold(x * cols[t][q * rows:(q + 1) * rows], 0)
                        acc[t] = part if acc[t] is None else acc[t] + part
                    prev = acc[0] + acc[1]
                for t in range(2):
                    out[t].append(jnp.sum(acc[t], axis=0, keepdims=True))
            gate = jax.nn.sigmoid(jnp.concatenate(out[1], axis=1))
            for j in range(S // RC):
                g_s[j, 0:1, :] = gate[:, j * RC:(j + 1) * RC]
            r = jnp.concatenate(out[0], axis=1).astype(BF16).astype(F32)
            lane = jax.lax.broadcasted_iota(jnp.int32, (1, S), 1)
            m1 = jnp.max(r, axis=1, keepdims=True)
            i1 = jnp.min(jnp.where(r == m1, lane, S - 1), axis=1, keepdims=True)
            r2 = jnp.where(lane == i1, -jnp.inf, r)
            m2 = jnp.max(r2, axis=1, keepdims=True)
            i2 = jnp.min(jnp.where(jnp.logical_and(r2 == m2, lane != i1), lane, S - 1), axis=1, keepdims=True)
            ln = jax.lax.broadcasted_iota(jnp.int32, (M, L), 1)
            st["at"] = [(i[0, 0] >> 9, slice(None), pl.ds(pl.multiple_of(i[0, 0] & (RC - L), L), L))
                        for i in (i1, i2)]
            st["hit"] = [ln == (i & (L - 1)) for i in (i1, i2)]
            st["r"] = [jax.nn.sigmoid(m1), jax.nn.sigmoid(m2)]
            st["x"] = [jnp.broadcast_to(jnp.sum(jnp.where(hit, xT_s[at].astype(F32), 0.0),
                                                axis=1, keepdims=True), (M, L))
                       for at, hit in zip(st["at"], st["hit"])]

        def fold(v, axis):
            parts = [v[k * 8:(k + 1) * 8] if axis == 0 else v[:, k * L:(k + 1) * L]
                     for k in range(v.shape[axis] // (8, L)[axis])]
            while len(parts) > 1:
                parts = [parts[k] + parts[k + 1] if k + 1 < len(parts) else parts[k]
                         for k in range(0, len(parts), 2)]
            return parts[0]

        def linked(w, link):
            w = pltpu.bitcast(w, U32)
            reps = (w.shape[0] // 8, w.shape[1] // L)
            w = jnp.where(jnp.tile(never, reps), jnp.tile(pltpu.bitcast(link, U32), reps), w)
            return _as_bf16(w).astype(F32)

        def hidden(pieces):
            pieces = pieces[-3] + pieces[-2] + pieces[-1]
            nr, rows = 4, M // 4
            total = 2 * (F // L) * nr
            out, k, prev = [], 0, None
            for w_s in (wg_s, wu_s):
                cols = ([], [])
                for ct in range(F // L):
                    acc = [None, None]
                    for q in range(nr):
                        link = pieces[int(0.9 * k / total * len(pieces))]
                        if prev is not None:
                            link = jnp.where(never, link, prev)
                        k += 1
                        w = linked(w_s[q * rows:(q + 1) * rows, ct * L:(ct + 1) * L], link)
                        for t in range(2):
                            part = fold(w * st["x"][t][q * rows:(q + 1) * rows], 0)
                            acc[t] = part if acc[t] is None else acc[t] + part
                        prev = acc[0] + acc[1]
                    for t in range(2):
                        cols[t].append(jnp.sum(acc[t], axis=0, keepdims=True))
                out.append([jnp.concatenate(c, axis=1) for c in cols])
            st["h"] = [(jax.nn.silu(out[0][t]) * out[1][t]).astype(BF16).astype(F32) for t in range(2)]

        def patch(pieces):
            pieces = pieces[-2] + pieces[-1]
            half = F // 2
            ys, k, prev = ([], []), 0, None
            for rg in range(M // 16):
                acc = [None, None]
                for hf in range(2):
                    link = pieces[int((0.1 + 0.8 * k / (M // 8)) * len(pieces))]
                    if prev is not None:
                        link = jnp.where(never, link, prev)
                    k += 1
                    w = linked(wd_s[rg * 16:(rg + 1) * 16, hf * half:(hf + 1) * half], link)
                    for t in range(2):
                        part = fold(w * st["h"][t][:, hf * half:(hf + 1) * half], 1)
                        acc[t] = part if acc[t] is None else acc[t] + part
                    prev = fold(acc[0] + acc[1], 0)
                for t in range(2):
                    ys[t].append(jnp.sum(acc[t], axis=1, keepdims=True))
            for t in range(2):
                y = jnp.concatenate(ys[t], axis=0) * st["r"][t]
                blk = xT_s[st["at"][t]].astype(F32)
                xT_s[st["at"][t]] = (blk + jnp.where(st["hit"][t], y, 0.0)).astype(BF16)

        head_program(FIRST_ORDER, None, 0, never, hooks=(route, hidden, patch))

    def phase2(x7_s, wo_ops):
        wo_copy.wait()
        col = jax.lax.broadcasted_iota(jnp.int32, (L, L), 1)
        tri = ((col & ~15) + ((col & 3) << 2) + ((col & 15) >> 2)
               <= jax.lax.broadcasted_iota(jnp.int32, (L, L), 0))

        def head(h, _):
            head_program(LOOP_ORDER, h, h + 1, _never(h), x7_s, tri, wo_ops, span=0.96)
            return h
        last = jax.lax.fori_loop(0, H - 1, head, 0)
        head_program(LAST_ORDER, H - 1, None, _never(last), x7_s, tri)

        def out_step(j, _):
            m = ({}, {})
            for n in range(7):
                right = [[] for _ in range(7)]
                for pair in range(H // 2):
                    blk = [_as_bf16(x7_s[n, 2 * pair + par, pl.ds(pl.multiple_of(j * L + t * 64, 64), 64), :])
                           for par in range(2) for t in range(2)]
                    ops = list(_right(*[v.astype(F32) for v in blk]))
                    ops[1], ops[4] = blk[0], blk[3]
                    for x in range(7):
                        right[x].append(ops[x])
                mm = {x: jax.lax.dot_general(
                    jnp.concatenate([_as_bf16(wo_ops[n, x, pair, :M // 8]) for pair in range(H // 2)], axis=1),
                    jnp.concatenate(right[x], axis=1).astype(BF16), NT, preferred_element_type=F32)
                    for x in (4, 2, 1, 5, 0, 3, 6)}
                m[0][n] = jnp.concatenate([((mm[0] + mm[3]) - mm[4]) + mm[6], _c21(mm)], axis=0)
                m[1][n] = jnp.concatenate([_c12(mm), _c22(mm)], axis=0)
            gate = g_s[j, 0:1, :]
            for hf in (1, 0):
                rest = (1.0 - gate) * xT_s[j, hf * mh:(hf + 1) * mh, :].astype(F32)
                cols = []
                for t in range(RC // TQ):
                    gl, gr = gate[:, t * TQ:t * TQ + L], gate[:, t * TQ + L:(t + 1) * TQ]
                    rl, rr = rest[:, t * TQ:t * TQ + L], rest[:, t * TQ + L:(t + 1) * TQ]
                    if hf:
                        cols += [gl * _c21(m[t]) + rl, gr * _c22(m[t]) + rr]
                    else:
                        cols += [(gl * ((m[t][0] + m[t][3]) - m[t][4]) + rl) + gl * m[t][6], gr * _c12(m[t]) + rr]
                o_s[j, hf * mh:(hf + 1) * mh, :] = jnp.concatenate(cols, axis=1).astype(BF16)
                out_copy(j, hf).start()
            return 0
        jax.lax.fori_loop(0, S // RC, out_step, 0)
        for j in range(S // RC):
            for hf in range(2):
                out_copy(j, hf).wait()

    pl.run_scoped(
        phase1,
        *[pltpu.VMEM(r.shape, r.dtype) for r in (c_hbm, wq_hbm, wk_hbm, wv_hbm, wg_hbm, wu_hbm, wd_hbm)],
        pltpu.VMEM((7, S // 4, mh), U32),
        pltpu.VMEM((7, -(-pq // 4) * 32, L), U32),
        pltpu.VMEM((7, -(-pq // 4) * 32, L), U32),
        pltpu.VMEM((M,), BF16),
        pltpu.VMEM((M,), BF16))
    pl.run_scoped(phase2, pltpu.VMEM((7, H, S // 4, L), U32), pltpu.VMEM((7, 7, H // 2, 64, L), U32))


def _tile_view(w):
    c, h, d = w.shape
    w = w.reshape(c, h // 8, 8, d // L, L).transpose(0, 1, 3, 2, 4)
    return w.reshape(c, h // 8, 8 * (d // L), L)


@jax.jit
def pallas_gated_mix__compressed_kv_cla__moe_arch_mod__prompt_kernel(
    A_x: jax.Array,
    A_c_kv: jax.Array,
    A_w_q: jax.Array,
    A_w_uk: jax.Array,
    A_w_uv: jax.Array,
    A_w_o: jax.Array,
    B_x: jax.Array,
    B_w_r: jax.Array,
    B_w_gate: jax.Array,
    B_w_up: jax.Array,
    B_w_down: jax.Array,
    gate_w: jax.Array,
):
    _, S, M = A_x.shape
    DC = A_c_kv.shape[2]
    H, D = A_w_q.shape[1], A_w_q.shape[2]
    args = (jnp.transpose(A_x[0]), A_c_kv[0], _tile_view(A_w_q).reshape(2, M // 2, 2, 16, L),
            _tile_view(A_w_uk), _tile_view(A_w_uv),
            jnp.transpose(A_w_o, (0, 2, 1)), B_w_r, gate_w, B_w_gate, B_w_up, jnp.transpose(B_w_down))

    def kern(*refs):
        _kernel(*refs, S=S, M=M, DC=DC, H=H, D=D)

    hbm = pl.BlockSpec(memory_space=pl.ANY)
    oT = pl.pallas_call(
        kern,
        out_shape=jax.ShapeDtypeStruct((M, S), A_x.dtype),
        in_specs=[hbm] * len(args),
        out_specs=hbm,
        scratch_shapes=[
            pltpu.VMEM((S // RC, 8, RC), F32),
            pltpu.VMEM((S // RC, M, RC), BF16),
            pltpu.VMEM((H, M, D), BF16),
            pltpu.VMEM((5, S // 4, DC // 2), U32),
            pltpu.VMEM((2, 7, S // 8, DC // 4), U32),
            pltpu.VMEM((7, 4, 8 * (DC // 4 + 1), L), U32),
            pltpu.VMEM((H, S // 2, D), U32),
            pltpu.VMEM((S // 2, D), U32),
            pltpu.VMEM((S // 2, D), U32),
            pltpu.VMEM((5, S // 4, L), U32),
            pltpu.VMEM((S // RC, M, RC), BF16),
            pltpu.VMEM((5, S // 4 + PAD_V, L), U32),
            pltpu.SemaphoreType.DMA((N_SEM,)),
        ],
        compiler_params=pltpu.CompilerParams(vmem_limit_bytes=124 * 1024 * 1024, disable_bounds_checks=True,
                                             disable_semaphore_checks=True),
    )(*args)
    return jnp.transpose(oT)[None]
```

```python
import math

import jax
import jax.numpy as jnp
import jax.experimental.pallas as pl
import jax.experimental.pallas.tpu as pltpu

F32 = jnp.float32
BF16 = jnp.bfloat16
U32 = jnp.uint32
NT = (((1,), (1,)), ((), ()))

L = 128
TQ = 256
HQ = TQ // 2
RC = 512
NCH = 4

PAD_V = 16

S_X, S_Q0, S_Q1, S_K, S_V, S_C, S_MISC, S_OUT = 0, 4, 8, 12, 16, 20, 24, 30
N_SEM = 38

LOOP_ORDER = ("Q0 Q7 S0 G0 S7 V0 V7 o0 Q6 G3 S6 V6 Q5 G4 S5 V5 Q4 G5 S4 V4 Q3 G6 S3 V3 Q2 g2 S2 V2 "
              "Q1 c2 G1 S1 V1 w0")
LOOP_TUNE = ((0.854, 0.969, 0.851, 0.941, 0.801, 0.94, 0.979, 0.948), (2, 4, 1, 3, 0, 6, 5), (2, 3, 4, 0, 1, 5, 6))
LAST_TUNE = ((0.8, 0.9, 0.66, 0.99, 0.9, 0.68, 0.93, 0.83), (0, 3, 4, 6, 1, 2, 5), (2, 3, 0, 4, 1, 6, 5))
FFN_TUNE = (0.03, 0.65, 0.0, 0.9, 0.1, 0.8)
FIRST_ORDER = "G0 G2 h0 G3 G4 G6 h1 G5 G1 h2 w0"
LAST_ORDER = "Q7 Q6 Q5 t7 V7 S6 Q4 V6 S5 r3 V5 S4 r2 V4 S3 r1 V3 t2 r0 V2 t1 t0 V1 V0"


def _to_u32(x_f32):
    return pltpu.bitcast(x_f32.astype(BF16), U32)


def _shuffled_u32(x_f32):
    return jnp.concatenate([_pack(x_f32[r:r + 8], x_f32[r + 8:r + 16]) for r in range(0, x_f32.shape[0], 16)],
                           axis=0)


def _as_bf16(x_u32):
    return pltpu.bitcast(x_u32, BF16)


def _left(a11, a12, a21, a22):
    return (a11 + a22, a21 + a22, a11, a22, a11 + a12, a21 - a11, a12 - a22)


def _right(b11, b12, b21, b22):
    return (b11 + b22, b11, b12 - b22, b21 - b11, b22, b11 + b12, b21 + b22)


FLAT, DEEP = (0, 1, 3, 4, 6), (2, 5)
SUMS = (0, 2, 3, 5, 6)


def _c11(m):
    return (m[0] + m[3]) + (m[6] - m[4])


def _c12(m):
    return m[2] + m[4]


def _c21(m):
    return m[1] + m[3]


def _c22(m):
    return (m[0] - m[1]) + (m[2] + m[5])


def _never(i):
    return jax.lax.broadcasted_iota(jnp.int32, (8, L), 0) < (i >> 10)


def _or_all(xs):
    out = xs[0]
    for x in xs[1:]:
        out = out | x
    return out


def _unpack(w, par):
    return pltpu.unpack_elementwise(w, index=par, packed_dtype=BF16, unpacked_dtype=F32)


def _pack(even, odd):
    return pltpu.bitcast(pltpu.pack_elementwise([even, odd], packed_dtype=BF16), U32)


def _head_weight(ref, h, nrows, pitch):
    sel = ((h >> 3) << 1) + (h & 1)
    r = (h >> 1) & 3
    return jnp.concatenate(
        [_as_bf16(ref[sel, pl.ds((dt * 4 + r) * pitch, nrows), :]) for dt in range(2)], axis=1)


def _kernel(xT_hbm, c_hbm, wq_hbm, wk_hbm, wv_hbm, wo_hbm, wr_hbm, gw_hbm, wg_hbm, wu_hbm, wd_hbm,
            o_hbm,
            g_s, xT_s, wo_s, a_s, a2_s, b_s, q_s, k_s, v_s, k5_s, o_s, v5_s, sem, *, S, M, DC, H, D):
    nq = S // TQ
    mh = M // 2
    pq = mh // 2 + 1
    pb = DC // 4 + 1
    mq = mh // NCH
    mk = DC // NCH
    qscale = (D ** -0.5) * math.log2(math.e)
    neg = -1e9 * math.log2(math.e)
    wo_copy = pltpu.make_async_copy(wo_hbm, wo_s, sem.at[S_MISC + 5])

    def out_copy(j, hf):
        return pltpu.make_async_copy(o_s.at[j, pl.ds(hf * mh, mh)],
                                     o_hbm.at[pl.ds(hf * mh, mh), pl.ds(j * RC, RC)], sem.at[S_OUT + 2 * j + hf])

    def head_program(order, h, hn, never, x7_s=None, tri=None, wo_ops=None, tune=None, hooks=None):
        prods, held, waiting = {}, {}, []

        def spots(v, cols, rows=(0, 64, 128, 192)):
            return [v[r:r + 8, n * L:(n + 1) * L] for n in cols for r in rows]

        def tie(lhs, links, every):
            rows = []
            for rg in range(lhs.shape[0] // 8):
                blk = lhs[rg * 8:(rg + 1) * 8]
                if links and rg % every == 0:
                    blk = jnp.concatenate([jnp.where(never, links.pop(0), blk[:, :L]), blk[:, L:]], axis=1)
                rows.append(blk)
            return jnp.concatenate(rows, axis=0)

        combos = [("k", 0, _c11, (0, 3, 4, 6)), ("k", 1, _c21, (1, 3)),
                  ("v", 0, _c12, (2, 4)), ("v", 1, _c22, (0, 1, 2, 5))]

        def combine(pieces):
            ready = [c for c in combos if all(x in prods for x in c[3])]
            for e, (key, odd, comb, needs) in enumerate(ready):
                combos.remove((key, odd, comb, needs))
                for k in range(nq // 2):
                    m = {x: prods[x][k * TQ:(k + 1) * TQ] for x in needs}
                    if pieces:
                        rows = []
                        for g in range(8):
                            at = ((e * (nq // 2) + k) * 8 + g) / (len(ready) * (nq // 2) * 8)
                            rows.append(jnp.tile(pieces[int(0.95 * at * len(pieces))], (2, 2)))
                        m[needs[0]] = jnp.where(jnp.tile(never, (32, 2)), jnp.concatenate(rows + rows, axis=0),
                                                m[needs[0]])
                    c = comb(m)
                    held[2 * k + odd, key] = _shuffled_u32(c)
                    if 2 * k + odd < nq - 1:
                        off = (c[:L, L:], c[L:, :L]) if key == "v" else (c[L:, :L], c[:L, L:])
                        ops = _right(c[:L, :L], *off, c[L:, L:])
                        held[2 * k + odd, key + "5"] = [_shuffled_u32(ops[x]) for x in SUMS]

        def proj(n, lazy):
            w = _head_weight(b_s.at[n], hn, DC // 4, pb)
            links = list(waiting)
            del waiting[:]
            if n in DEEP:
                wf, kh = w.astype(F32), DC // 4
                right = [o.astype(BF16) for o in _right(wf[:kh, :L], wf[:kh, L:], wf[kh:, :L], wf[kh:, L:])]
                right[1], right[4] = w[:kh, :L], w[kh:, L:]
                m, pieces = {}, []

                def sub(x, after):
                    lhs = a2_s[DEEP.index(n), x]
                    if after:
                        t = after[0]
                        for v in after[1:]:
                            t = jnp.maximum(t, v)
                        lhs = tie(lhs, [pltpu.bitcast(jnp.maximum(t[g * 16:g * 16 + 8], t[g * 16 + 8:g * 16 + 16]), U32)
                                        for g in range(S // 64)], 1)
                    elif links:
                        lhs = tie(lhs, links, lhs.shape[0] // 8 // len(links))
                    m[x] = jnp.dot(_as_bf16(lhs), right[x], preferred_element_type=F32)
                    pieces.extend(spots(m[x], (0,), range(0, S // 4, 64)))
                sub(1, ()), sub(3, ())
                c21 = m[1] + m[3]
                sub(2, ()), sub(4, (c21,))
                c12, c11, c22 = m[2] + m[4], m[3] - m[4], m[2] - m[1]
                sub(0, ()), sub(5, (c12, c11, c22))
                c11, c22 = c11 + m[0], c22 + (m[0] + m[5])
                sub(6, (c11, c22))
                top = jnp.concatenate([c11 + m[6], c12], axis=1)
                bot = jnp.concatenate([c21, c22], axis=1)
                prods[n] = jnp.concatenate([v[k * L:(k + 1) * L] for k in range(nq // 2) for v in (top, bot)],
                                           axis=0)
            else:
                lhs = a_s[FLAT.index(n)]
                if links:
                    lhs = tie(lhs, links, max(1, lhs.shape[0] // 8 // len(links)))
                prods[n] = jnp.dot(_as_bf16(lhs), w, preferred_element_type=F32)
                pieces = spots(prods[n], (0, 1), range(0, S // 2, 32))
            if not lazy:
                combine(None)
            return pieces

        def write_kv():
            for ch in reversed(range(nq)):
                k_s[ch * HQ:(ch + 1) * HQ, :] = held[ch, "k"]
                v_s[ch * HQ:(ch + 1) * HQ, :] = held[ch, "v"]
                for key, ref in (("k5", k5_s), ("v5", v5_s)):
                    for n, o in enumerate(held.get((ch, key), ())):
                        ref[n, ch * 64:(ch + 1) * 64, :] = o

        def right_operand(n, plain, sums, c0, c1):
            if n == 1:
                return jnp.concatenate([_as_bf16(plain[c * HQ:c * HQ + 64, :L]) for c in range(c0, c1)], axis=0)
            if n == 4:
                return jnp.concatenate([_as_bf16(plain[c * HQ + 64:(c + 1) * HQ, L:]) for c in range(c0, c1)], axis=0)
            return _as_bf16(sums[SUMS.index(n), c0 * 64:c1 * 64, :])

        def qk(i, tied):
            q = qd = q_s[h, i * HQ:(i + 1) * HQ, :]
            n = len(waiting) - 8 if tied else 0
            if n > 0:
                qd = tie(q, waiting[:n], 16 // n)
                del waiting[:n]
            q, qd = _as_bf16(q), _as_bf16(qd)
            tops, bots, pieces = [], [], []
            if i:
                qf = q.astype(F32)
                left = [o.astype(BF16) for o in _left(qf[:L, :L], qf[:L, L:], qf[L:, :L], qf[L:, L:])]
                left[2], left[3] = q[:L, :L], q[L:, L:]
            done = []
            for c in range(i):
                lhs = dict(enumerate(left))
                if c >= 2:
                    u = pltpu.bitcast(left[0], U32)
                    lhs[0] = _as_bf16(jnp.concatenate(
                        [jnp.where(never, done[c - 2][g], u[g * 8:(g + 1) * 8]) for g in range(8)], axis=0))
                m = {n: jax.lax.dot_general(lhs[n], right_operand(n, k_s, k5_s, c, c + 1), NT,
                                            preferred_element_type=F32) for n in tune[1]}
                c11, c12, c21, c22 = _c11(m), _c12(m), _c21(m), _c22(m)
                tops += [c11, c12]
                bots += [c21, c22]
                t = jnp.maximum(jnp.maximum(c11, c12), jnp.maximum(c21, c22))
                done.append([pltpu.bitcast(jnp.maximum(t[g * 16:g * 16 + 8], t[g * 16 + 8:(g + 1) * 16]), U32)
                             for g in range(8)])
                for n in (0, 5):
                    pieces += spots(m[n], (0,), (0, 32, 64, 96))
            r0 = i * HQ
            s1 = jax.lax.dot_general(qd, _as_bf16(k_s[r0:r0 + 64, :]), NT, preferred_element_type=F32)
            s2 = jax.lax.dot_general(q[L:], _as_bf16(k_s[r0 + 64:r0 + HQ, :]), NT, preferred_element_type=F32)
            top = jnp.concatenate(tops + [jnp.where(tri, s1[:L], neg)], axis=1)
            bot = jnp.concatenate(bots + [s1[L:], jnp.where(tri, s2, neg)], axis=1)
            return (top, bot), pieces + spots(s1, (0,))

        def softmax(i, top, bot, pieces, again=False):
            p, sums, prev = ([], []), ([], []), None
            for k in range(TQ // 8):
                half = k % 2
                s = (top, bot)[half][(k // 2) * 8:(k // 2 + 1) * 8]
                link = pieces[int(tune[0][i] * k * 8 / TQ * len(pieces))]
                if prev is not None:
                    link = jnp.where(never, link, prev)
                m = jnp.broadcast_to(jnp.max(s, axis=1, keepdims=True), (8, L))
                m = jnp.where(never, link, m)
                e = [jnp.exp2(s[:, t:t + L] - m) for t in range(0, s.shape[1], L)]
                prev = e[0]
                for x in e[1:]:
                    prev = prev + x
                if again:
                    m = m + jnp.log2(jnp.sum(prev, axis=1, keepdims=True))
                    e = [jnp.exp2(s[:, t:t + L] - m) for t in range(0, s.shape[1], L)]
                sums[half].append(prev)
                p[half].append(jnp.concatenate(e, axis=1))
            pt, pb_ = jnp.concatenate(p[0], axis=0), jnp.concatenate(p[1], axis=0)

            def tile(x, t):
                return x[:, t * L:(t + 1) * L]
            ops = [_left(tile(pt, 2 * c), tile(pt, 2 * c + 1), tile(pb_, 2 * c), tile(pb_, 2 * c + 1))
                   for c in range(i)]
            left = [jnp.concatenate([o[n] for o in ops], axis=1).astype(BF16) for n in range(7)] if i else None
            inv = []
            for x in () if again else sums:
                l = jnp.sum(jnp.concatenate(x, axis=0), axis=1, keepdims=True)
                r = pl.reciprocal(l, approx=True)
                inv.append(r * (2.0 - l * r))
            return (left, jnp.concatenate([tile(pt, 2 * i), tile(pb_, 2 * i)], axis=0).astype(BF16),
                    tile(pb_, 2 * i + 1).astype(BF16), inv)

        def pv(i, left, p1, p2, inv):
            r0 = i * HQ
            m, pieces = {}, []
            for n in tune[2] if i else ():
                m[n] = jnp.dot(left[n], right_operand(n, v_s, v5_s, 0, i), preferred_element_type=F32)
                pieces += spots(m[n], (0,), (0, 32, 64, 96))
            c1 = jnp.dot(p1, _as_bf16(v_s[r0:r0 + 64, :]), preferred_element_type=F32)
            c2 = jnp.dot(p2, _as_bf16(v_s[r0 + 64:r0 + HQ, :]), preferred_element_type=F32)
            top, bot = c1[:L], c1[L:] + c2
            if i:
                top = top + jnp.concatenate([_c11(m), _c12(m)], axis=1)
                bot = bot + jnp.concatenate([_c21(m), _c22(m)], axis=1)
            else:
                pieces = spots(c1, (0, 1))
            if inv:
                top, bot = top * inv[0], bot * inv[1]
            us = [_to_u32(o) for o in _right(top[:, :L], bot[:, :L], top[:, L:], bot[:, L:])]
            for n in range(7):
                x7_s[n, h, i * 64:(i + 1) * 64, :] = us[n]
            waiting.extend(_or_all([us[n][g * 8:(g + 1) * 8] for n in SUMS]) for g in range(8))
            return pieces

        def wo_operands(pieces):
            groups = M // 64
            never2 = jnp.concatenate([never, never], axis=0)
            share = -(-(H // 2) * groups // (H - 1))
            for k in range(share):
                u = jnp.minimum(h * share + k, (H // 2) * groups - 1)
                pair = jax.lax.div(u, groups)
                rg = u - pair * groups
                ops = [_left(*[wo_s[2 * pair + par, pl.ds(pl.multiple_of(hf * mh + sub * (mh // 2) + rg * 16, 16), 16),
                                    ch * L:(ch + 1) * L].astype(F32) for hf in range(2) for ch in range(2)])
                       for sub in range(2) for par in range(2)]
                for n in range(7):
                    link = pieces[int(0.96 * (k * 7 + n) / (share * 7) * len(pieces))]
                    gate = jnp.concatenate([link, link], axis=0)
                    us = [_to_u32(o) for o in _left(*[jnp.where(never2, gate, o[n]) for o in ops])]
                    for x in range(7):
                        wo_ops[n, x, pair, pl.ds(pl.multiple_of(rg * 8, 8), 8), :] = us[x]
                    waiting.append(_or_all(us))

        scores, probs, pieces = {}, {}, []
        for op in order.split():
            i = int(op[1:])
            if op[0] in "Gg":
                pieces.append(proj(i, op[0] == "g"))
            elif op[0] == "c":
                combine(sum(pieces[-i:], []))
            elif op[0] == "w":
                write_kv()
            elif op[0] == "o":
                wo_operands(pieces[-1])
            elif op[0] in "Qr":
                scores[i], new = qk(i, op[0] == "r")
                pieces.append(new)
            elif op[0] == "S":
                probs[i] = softmax(i, *scores.pop(i), pieces[-1])
            elif op[0] == "t":
                probs[i] = softmax(i, *scores.pop(i), pieces[-2] + pieces[-1], again=True)
            elif op[0] == "V":
                pieces.append(pv(i, *probs.pop(i)))
            else:
                hooks[i](pieces)

    def phase1(c_s, wq_r, wk_r, wv_r, wg_s, wu_s, wd_s, xa_s, wq0_s, wq1_s, wr_s, gw_s):
        def x_copy(j):
            return pltpu.make_async_copy(xT_hbm.at[:, pl.ds(j * RC, RC)], xT_s.at[j], sem.at[S_X + j])

        def wq_copy(g, j):
            return pltpu.make_async_copy(wq_hbm.at[:, pl.ds(j * mq, mq), g], wq_r.at[:, pl.ds(j * mq, mq), g],
                                         sem.at[(S_Q1 if g else S_Q0) + j])

        def kv_copies(j):
            return [pltpu.make_async_copy(src.at[pl.ds(j * n, n)], dst.at[pl.ds(j * n, n)], sem.at[s0 + j])
                    for src, dst, s0, n in ((c_hbm, c_s, S_C, RC), (wk_hbm, wk_r, S_K, mk), (wv_hbm, wv_r, S_V, mk))]

        misc = [pltpu.make_async_copy(a, b, sem.at[S_MISC + i]) for i, (a, b) in enumerate(
            [(wr_hbm, wr_s), (gw_hbm, gw_s), (wg_hbm, wg_s), (wu_hbm, wu_s), (wd_hbm, wd_s)])]

        x_copy(0).start()
        for j in range(NCH):
            wq_copy(0, j).start()
        for j in range(NCH):
            if j + 1 < NCH:
                x_copy(j + 1).start()
            wq_copy(1, j).start()
        misc[0].start()
        misc[1].start()
        for j in range(NCH):
            for cp in kv_copies(j):
                cp.start()
        for cp in misc[2:]:
            cp.start()
        wo_copy.start()

        def x_operands(j):
            r0 = j * HQ if isinstance(j, int) else pl.multiple_of(j * HQ, HQ)
            a = [xT_s[j, kh * mh:(kh + 1) * mh, rb * TQ:(rb + 1) * TQ].astype(F32)
                 for rb in range(2) for kh in range(2)]
            for n, o in enumerate(_left(*a)):
                xa_s[n, pl.ds(r0, HQ), :] = pltpu.bitcast(o.astype(BF16).T, U32)

        def wq_operands(g, p, never=None, link=None):
            w = [pltpu.bitcast(wq_r[kh, pl.ds(2 * p, 2), g], U32) for kh in range(2)]
            w = [[x[0], x[1]] for x in w]
            if link is not None:
                w[0][0] = jnp.where(never, link, w[0][0])
            rows = [_right(*[_unpack(w[kh][e], par) for kh in range(2) for par in range(2)]) for e in range(2)]
            for n in range(7):
                (wq0_s, wq1_s)[g][n, pl.ds(p, 8, stride=pq), :] = _pack(rows[0][n], rows[1][n])

        x_copy(0).wait()
        x_operands(0)

        def first_half(j, _):
            wq_copy(0, j).wait()
            for k in range(mq // 2):
                wq_operands(0, j * (mq // 2) + k)
            return 0
        jax.lax.fori_loop(0, NCH, first_half, 0)

        def q_step(g, j, side):
            pieces = []
            for r in range(4):
                m = {}
                for n in (0, 3, 4, 6, 1, 2, 5):
                    w = jnp.concatenate([_as_bf16((wq0_s, wq1_s)[g][n, pl.ds((dt * 4 + r) * pq, mh // 2), :])
                                         for dt in range(2)], axis=1)
                    m[n] = jnp.dot(_as_bf16(xa_s[n, pl.ds(pl.multiple_of(j * HQ, HQ), HQ), :]), w,
                                   preferred_element_type=F32)
                    for k in range(5):
                        pieces.append(m[n][k * 48:k * 48 + 8, (k % 2) * L:(k % 2 + 1) * L])
                        side(len(pieces) - 1, pieces[-1])
                for par, rb, comb in ((0, 0, _c11), (0, 1, _c21), (1, 0, _c12), (1, 1, _c22)):
                    r0 = pl.multiple_of(j * TQ + rb * HQ, HQ)
                    q_s[8 * g + 2 * r + par, pl.ds(r0, HQ), :] = _to_u32(comb(m) * qscale)

        def q_lo(j, _):
            never = _never(j)

            def side(k, piece):
                if k == 35:
                    @pl.when(j + 1 < NCH)
                    def _():
                        x_copy(j + 1).wait()
                    wq_copy(1, j).wait()
                if k >= 42 and k % 3 == 0 and (k - 42) // 3 < mq // 2:
                    wq_operands(1, j * (mq // 2) + (k - 42) // 3, never, pltpu.bitcast(piece, U32))
            q_step(0, j, side)
            x_operands((j + 1) & (NCH - 1))
            return 0
        jax.lax.fori_loop(0, NCH, q_lo, 0)

        def q_hi(j, _):
            for cp in kv_copies(j):
                cp.wait()
            never = _never(j)
            quad = []

            def side(kk, piece):
                if kk >= 128:
                    return
                k, g = kk // 2, kk % 2
                link = pltpu.bitcast(piece, U32)
                if g == 0:
                    rg, t = k // 8 + 8 * (k % 4 // 2), k // 4 % 2 + 2 * (k % 2)
                    a = []
                    for rb in range(2):
                        r0 = pl.multiple_of(j * RC + rb * TQ + rg * 16, 16)
                        for ch in range(2):
                            a.append(c_s[pl.ds(r0, 16), (2 * t + ch) * L:(2 * t + ch + 1) * L].astype(F32))
                    a[0] = jnp.where(jnp.concatenate([never, never], axis=0),
                                     jnp.concatenate([piece, piece], axis=0), a[0])
                    ops = _left(*a)
                    us = [_shuffled_u32(ops[n]) for n in FLAT]
                    d0 = pl.multiple_of(j * HQ + rg * 8, 8)
                    for n, u in enumerate(us):
                        a_s[n, pl.ds(d0, 8), t * L:(t + 1) * L] = u
                    quad.append(ops)
                    if len(quad) == 4:
                        d0 = pl.multiple_of(j * (HQ // 2) + (rg - 8) * 8, 8)
                        for e, n in enumerate(DEEP):
                            deep = [_shuffled_u32(o) for o in _left(*[q[n] for q in quad])]
                            for x, u in enumerate(deep):
                                a2_s[e, x, pl.ds(d0, 8), (t - 2) * L:(t - 1) * L] = u
                            us += deep
                        del quad[:]
                    link = _or_all(us)
                c0 = j * mk + 2 * k
                w = [pltpu.bitcast(r[pl.ds(c0 + o, 2), g], U32) for o in (0, L) for r in (wk_r, wv_r)]
                w = [[x[0], x[1]] for x in w]
                w[0][0] = jnp.where(never, link, w[0][0])
                for par in range(2):
                    rows = [_right(*[_unpack(x[e], par) for x in w]) for e in range(2)]
                    for n in range(7):
                        b_s[n, 2 * g + par, pl.ds(j * (mk // 4) + k, 8, stride=pb), :] = _pack(
                            rows[0][n], rows[1][n])
            q_step(1, j, side)
            return j
        never = _never(jax.lax.fori_loop(0, NCH, q_hi, 0))

        for cp in misc:
            cp.wait()
        st = {}
        F = wg_s.shape[1]

        def route(pieces):
            pieces = pieces[-2] + pieces[-1]
            mp = -(-M // L) * L
            cols = []
            for w_s in (wr_s, gw_s):
                w = jnp.concatenate([w_s[...].reshape(1, M).astype(F32), jnp.zeros((1, mp - M), F32)], axis=1)
                cols.append(jnp.broadcast_to(w, (L, mp)).T)
            nr, rows = 4, M // 4
            out, k, prev = ([], []), 0, None
            for ct in range(S // L):
                acc = [None, None]
                for q in range(nr):
                    link = pieces[int((FFN_TUNE[0] + FFN_TUNE[1] * k / (nr * S // L)) * len(pieces))]
                    if prev is not None:
                        link = jnp.where(never, link, prev)
                    k += 1
                    x = linked(xT_s[ct * L // RC, q * rows:(q + 1) * rows, pl.ds(ct * L % RC, L)], link)
                    for t in range(2):
                        part = fold(x * cols[t][q * rows:(q + 1) * rows], 0)
                        acc[t] = part if acc[t] is None else acc[t] + part
                    prev = acc[0] + acc[1]
                for t in range(2):
                    out[t].append(jnp.sum(acc[t], axis=0, keepdims=True))
            gate = jax.nn.sigmoid(jnp.concatenate(out[1], axis=1))
            for j in range(S // RC):
                g_s[j, 0:1, :] = gate[:, j * RC:(j + 1) * RC]
            r = jnp.concatenate(out[0], axis=1).astype(BF16).astype(F32)
            lane = jax.lax.broadcasted_iota(jnp.int32, (1, S), 1)
            m1 = jnp.max(r, axis=1, keepdims=True)
            i1 = jnp.min(jnp.where(r == m1, lane, S - 1), axis=1, keepdims=True)
            r2 = jnp.where(lane == i1, -jnp.inf, r)
            m2 = jnp.max(r2, axis=1, keepdims=True)
            i2 = jnp.min(jnp.where(jnp.logical_and(r2 == m2, lane != i1), lane, S - 1), axis=1, keepdims=True)
            ln = jax.lax.broadcasted_iota(jnp.int32, (M, L), 1)
            st["at"] = [(i[0, 0] >> 9, slice(None), pl.ds(pl.multiple_of(i[0, 0] & (RC - L), L), L))
                        for i in (i1, i2)]
            st["hit"] = [ln == (i & (L - 1)) for i in (i1, i2)]
            st["r"] = [jax.nn.sigmoid(m1), jax.nn.sigmoid(m2)]
            st["x"] = [jnp.broadcast_to(jnp.sum(jnp.where(hit, xT_s[at].astype(F32), 0.0),
                                                axis=1, keepdims=True), (M, L))
                       for at, hit in zip(st["at"], st["hit"])]

        def fold(v, axis):
            parts = [v[k * 8:(k + 1) * 8] if axis == 0 else v[:, k * L:(k + 1) * L]
                     for k in range(v.shape[axis] // (8, L)[axis])]
            while len(parts) > 1:
                parts = [parts[k] + parts[k + 1] if k + 1 < len(parts) else parts[k]
                         for k in range(0, len(parts), 2)]
            return parts[0]

        def linked(w, link):
            w = pltpu.bitcast(w, U32)
            reps = (w.shape[0] // 8, w.shape[1] // L)
            w = jnp.where(jnp.tile(never, reps), jnp.tile(pltpu.bitcast(link, U32), reps), w)
            return _as_bf16(w).astype(F32)

        def hidden(pieces):
            pieces = pieces[-3] + pieces[-2] + pieces[-1]
            nr, rows = 4, M // 4
            total = 2 * (F // L) * nr
            out, k, prev = [], 0, None
            for w_s in (wg_s, wu_s):
                cols = ([], [])
                for ct in range(F // L):
                    acc = [None, None]
                    for q in range(nr):
                        link = pieces[int((FFN_TUNE[2] + FFN_TUNE[3] * k / total) * len(pieces))]
                        if prev is not None:
                            link = jnp.where(never, link, prev)
                        k += 1
                        w = linked(w_s[q * rows:(q + 1) * rows, ct * L:(ct + 1) * L], link)
                        for t in range(2):
                            part = fold(w * st["x"][t][q * rows:(q + 1) * rows], 0)
                            acc[t] = part if acc[t] is None else acc[t] + part
                        prev = acc[0] + acc[1]
                    for t in range(2):
                        cols[t].append(jnp.sum(acc[t], axis=0, keepdims=True))
                out.append([jnp.concatenate(c, axis=1) for c in cols])
            st["h"] = [(jax.nn.silu(out[0][t]) * out[1][t]).astype(BF16).astype(F32) for t in range(2)]

        def patch(pieces):
            pieces = pieces[-2] + pieces[-1]
            half = F // 2
            ys, k, prev = ([], []), 0, None
            for rg in range(M // 16):
                acc = [None, None]
                for hf in range(2):
                    link = pieces[int((FFN_TUNE[4] + FFN_TUNE[5] * k / (M // 8)) * len(pieces))]
                    if prev is not None:
                        link = jnp.where(never, link, prev)
                    k += 1
                    w = linked(wd_s[rg * 16:(rg + 1) * 16, hf * half:(hf + 1) * half], link)
                    for t in range(2):
                        part = fold(w * st["h"][t][:, hf * half:(hf + 1) * half], 1)
                        acc[t] = part if acc[t] is None else acc[t] + part
                    prev = fold(acc[0] + acc[1], 0)
                for t in range(2):
                    ys[t].append(jnp.sum(acc[t], axis=1, keepdims=True))
            for t in range(2):
                y = jnp.concatenate(ys[t], axis=0) * st["r"][t]
                blk = xT_s[st["at"][t]].astype(F32)
                xT_s[st["at"][t]] = (blk + jnp.where(st["hit"][t], y, 0.0)).astype(BF16)

        head_program(FIRST_ORDER, None, 0, never, hooks=(route, hidden, patch))

    def phase2(x7_s, wo_ops):
        wo_copy.wait()
        col = jax.lax.broadcasted_iota(jnp.int32, (L, L), 1)
        tri = ((col & ~15) + ((col & 3) << 2) + ((col & 15) >> 2)
               <= jax.lax.broadcasted_iota(jnp.int32, (L, L), 0))

        def head(h, _):
            head_program(LOOP_ORDER, h, h + 1, _never(h), x7_s, tri, wo_ops, LOOP_TUNE)
            return h
        last = jax.lax.fori_loop(0, H - 1, head, 0)
        head_program(LAST_ORDER, H - 1, None, _never(last), x7_s, tri, tune=LAST_TUNE)

        def out_step(j, _):
            m = ({}, {})
            for n in range(7):
                right = [[] for _ in range(7)]
                for pair in range(H // 2):
                    blk = [_as_bf16(x7_s[n, 2 * pair + par, pl.ds(pl.multiple_of(j * L + t * 64, 64), 64), :])
                           for par in range(2) for t in range(2)]
                    ops = list(_right(*[v.astype(F32) for v in blk]))
                    ops[1], ops[4] = blk[0], blk[3]
                    for x in range(7):
                        right[x].append(ops[x])
                mm = {x: jax.lax.dot_general(
                    jnp.concatenate([_as_bf16(wo_ops[n, x, pair, :M // 8]) for pair in range(H // 2)], axis=1),
                    jnp.concatenate(right[x], axis=1).astype(BF16), NT, preferred_element_type=F32)
                    for x in (4, 2, 1, 5, 0, 3, 6)}
                m[0][n] = jnp.concatenate([((mm[0] + mm[3]) - mm[4]) + mm[6], _c21(mm)], axis=0)
                m[1][n] = jnp.concatenate([_c12(mm), _c22(mm)], axis=0)
            gate = g_s[j, 0:1, :]
            for hf in (1, 0):
                rest = (1.0 - gate) * xT_s[j, hf * mh:(hf + 1) * mh, :].astype(F32)
                cols = []
                for t in range(RC // TQ):
                    gl, gr = gate[:, t * TQ:t * TQ + L], gate[:, t * TQ + L:(t + 1) * TQ]
                    rl, rr = rest[:, t * TQ:t * TQ + L], rest[:, t * TQ + L:(t + 1) * TQ]
                    if hf:
                        cols += [gl * _c21(m[t]) + rl, gr * _c22(m[t]) + rr]
                    else:
                        cols += [(gl * ((m[t][0] + m[t][3]) - m[t][4]) + rl) + gl * m[t][6], gr * _c12(m[t]) + rr]
                o_s[j, hf * mh:(hf + 1) * mh, :] = jnp.concatenate(cols, axis=1).astype(BF16)
                out_copy(j, hf).start()
            return 0
        jax.lax.fori_loop(0, S // RC, out_step, 0)
        for j in range(S // RC):
            for hf in range(2):
                out_copy(j, hf).wait()

    pl.run_scoped(
        phase1,
        *[pltpu.VMEM(r.shape, r.dtype) for r in (c_hbm, wq_hbm, wk_hbm, wv_hbm, wg_hbm, wu_hbm, wd_hbm)],
        pltpu.VMEM((7, S // 4, mh), U32),
        pltpu.VMEM((7, -(-pq // 4) * 32, L), U32),
        pltpu.VMEM((7, -(-pq // 4) * 32, L), U32),
        pltpu.VMEM((M,), BF16),
        pltpu.VMEM((M,), BF16))
    pl.run_scoped(phase2, pltpu.VMEM((7, H, S // 4, L), U32), pltpu.VMEM((7, 7, H // 2, 64, L), U32))


def _tile_view(w):
    c, h, d = w.shape
    w = w.reshape(c, h // 8, 8, d // L, L).transpose(0, 1, 3, 2, 4)
    return w.reshape(c, h // 8, 8 * (d // L), L)


@jax.jit
def pallas_gated_mix__compressed_kv_cla__moe_arch_mod__prompt_kernel(
    A_x: jax.Array,
    A_c_kv: jax.Array,
    A_w_q: jax.Array,
    A_w_uk: jax.Array,
    A_w_uv: jax.Array,
    A_w_o: jax.Array,
    B_x: jax.Array,
    B_w_r: jax.Array,
    B_w_gate: jax.Array,
    B_w_up: jax.Array,
    B_w_down: jax.Array,
    gate_w: jax.Array,
):
    _, S, M = A_x.shape
    DC = A_c_kv.shape[2]
    H, D = A_w_q.shape[1], A_w_q.shape[2]
    args = (jnp.transpose(A_x[0]), A_c_kv[0], _tile_view(A_w_q).reshape(2, M // 2, 2, 16, L),
            _tile_view(A_w_uk), _tile_view(A_w_uv),
            jnp.transpose(A_w_o, (0, 2, 1)), B_w_r, gate_w, B_w_gate, B_w_up, jnp.transpose(B_w_down))

    def kern(*refs):
        _kernel(*refs, S=S, M=M, DC=DC, H=H, D=D)

    hbm = pl.BlockSpec(memory_space=pl.ANY)
    oT = pl.pallas_call(
        kern,
        out_shape=jax.ShapeDtypeStruct((M, S), A_x.dtype),
        in_specs=[hbm] * len(args),
        out_specs=hbm,
        scratch_shapes=[
            pltpu.VMEM((S // RC, 8, RC), F32),
            pltpu.VMEM((S // RC, M, RC), BF16),
            pltpu.VMEM((H, M, D), BF16),
            pltpu.VMEM((5, S // 4, DC // 2), U32),
            pltpu.VMEM((2, 7, S // 8, DC // 4), U32),
            pltpu.VMEM((7, 4, 8 * (DC // 4 + 1), L), U32),
            pltpu.VMEM((H, S // 2, D), U32),
            pltpu.VMEM((S // 2, D), U32),
            pltpu.VMEM((S // 2, D), U32),
            pltpu.VMEM((5, S // 4, L), U32),
            pltpu.VMEM((S // RC, M, RC), BF16),
            pltpu.VMEM((5, S // 4 + PAD_V, L), U32),
            pltpu.SemaphoreType.DMA((N_SEM,)),
        ],
        compiler_params=pltpu.CompilerParams(vmem_limit_bytes=124 * 1024 * 1024, disable_bounds_checks=True,
                                             disable_semaphore_checks=True),
    )(*args)
    return jnp.transpose(oT)[None]
```

```python
import math

import jax
import jax.numpy as jnp
import jax.experimental.pallas as pl
import jax.experimental.pallas.tpu as pltpu

F32 = jnp.float32
BF16 = jnp.bfloat16
U32 = jnp.uint32
NT = (((1,), (1,)), ((), ()))

L = 128
TQ = 256
HQ = TQ // 2
RC = 512
NCH = 4

PAD_V = 16

S_X, S_Q0, S_Q1, S_K, S_V, S_C, S_MISC, S_OUT = 0, 4, 8, 12, 16, 20, 24, 30
N_SEM = 38

LOOP_ORDER = ("Q0 Q7 S0 G0 S7 V0 V7 o0 Q6 G3 S6 V6 Q5 G4 S5 V5 Q4 G5 S4 V4 Q3 G6 S3 V3 Q2 g2 S2 V2 "
              "Q1 c2 G1 S1 V1 w0")
LOOP_TUNE = ((0.854, 0.969, 0.851, 0.941, 0.801, 0.94, 0.979, 0.948), (2, 4, 1, 3, 0, 6, 5), (2, 3, 4, 0, 1, 5, 6))
LAST_TUNE = ((0.8, 0.9, 0.66, 0.99, 0.9, 0.68, 0.93, 0.83), (0, 3, 4, 6, 1, 2, 5), (2, 3, 0, 4, 1, 6, 5))
FFN_TUNE = (0.03, 0.65, 0.0, 0.9, 0.1, 0.8)
FIRST_ORDER = "G0 G2 h0 G3 G4 G6 h1 G5 G1 h2 w0"
LAST_ORDER = "Q7 Q6 Q5 t7 V7 S6 Q4 V6 S5 r3 V5 S4 r2 V4 S3 r1 V3 t2 r0 V2 t1 t0 V1 V0"


def _to_u32(x_f32):
    return pltpu.bitcast(x_f32.astype(BF16), U32)


def _as_bf16(x_u32):
    return pltpu.bitcast(x_u32, BF16)


def _left(a11, a12, a21, a22):
    return (a11 + a22, a21 + a22, a11, a22, a11 + a12, a21 - a11, a12 - a22)


def _right(b11, b12, b21, b22):
    return (b11 + b22, b11, b12 - b22, b21 - b11, b22, b11 + b12, b21 + b22)


FLAT, DEEP = (0, 1, 3, 4, 6), (2, 5)
SUMS = (0, 2, 3, 5, 6)


def _c11(m):
    return (m[0] + m[3]) + (m[6] - m[4])


def _c12(m):
    return m[2] + m[4]


def _c21(m):
    return m[1] + m[3]


def _c22(m):
    return (m[0] - m[1]) + (m[2] + m[5])


def _never(i):
    return jax.lax.broadcasted_iota(jnp.int32, (8, L), 0) < (i >> 10)


def _or_all(xs):
    out = xs[0]
    for x in xs[1:]:
        out = out | x
    return out


def _split_heads(even, odd):
    return ((even & jnp.uint32(0xFFFF)) | (odd << 16), (even >> 16) | (odd & jnp.uint32(0xFFFF0000)))


def _right_one(n, blocks):
    x, y, sign = ((0, 3, 1), (0, None, 0), (1, 3, -1), (2, 0, -1), (3, None, 0), (0, 1, 1), (2, 3, 1))[n]
    if y is None:
        return blocks[x]()
    x, y = blocks[x]().astype(F32), blocks[y]().astype(F32)
    return x + y if sign > 0 else x - y


def _head_weight(ref, h, nrows, pitch):
    sel = ((h >> 3) << 1) + (h & 1)
    r = (h >> 1) & 3
    return jnp.concatenate(
        [_as_bf16(ref[sel, pl.ds((dt * 4 + r) * pitch, nrows), :]) for dt in range(2)], axis=1)


def _kernel(xT_hbm, c_hbm, wq_hbm, wk_hbm, wv_hbm, wo_hbm, wr_hbm, gw_hbm, wg_hbm, wu_hbm, wd_hbm,
            o_hbm,
            g_s, xT_s, wo_s, a_s, a2_s, b_s, q_s, k_s, v_s, k5_s, o_s, v5_s, sem, *, S, M, DC, H, D):
    nq = S // TQ
    mh = M // 2
    pq = mh // 2 + 1
    pb = DC // 4 + 1
    mq = mh // NCH
    mk = DC // NCH
    qscale = (D ** -0.5) * math.log2(math.e)
    neg = -1e9 * math.log2(math.e)
    wo_copy = pltpu.make_async_copy(wo_hbm, wo_s, sem.at[S_MISC + 5])

    def out_copy(j, hf):
        return pltpu.make_async_copy(o_s.at[j, pl.ds(hf * mh, mh)],
                                     o_hbm.at[pl.ds(hf * mh, mh), pl.ds(j * RC, RC)], sem.at[S_OUT + 2 * j + hf])

    def head_program(order, h, hn, never, x7_s=None, tri=None, wo_ops=None, tune=None, hooks=None):
        prods, held, waiting = {}, {}, []

        def spots(v, cols, rows=(0, 64, 128, 192)):
            return [v[r:r + 8, n * L:(n + 1) * L] for n in cols for r in rows]

        def tie(lhs, links, every):
            rows = []
            for rg in range(lhs.shape[0] // 8):
                blk = lhs[rg * 8:(rg + 1) * 8]
                if links and rg % every == 0:
                    blk = jnp.concatenate([jnp.where(never, links.pop(0), blk[:, :L]), blk[:, L:]], axis=1)
                rows.append(blk)
            return jnp.concatenate(rows, axis=0)

        combos = [("k", 0, _c11, (0, 3, 4, 6)), ("k", 1, _c21, (1, 3)),
                  ("v", 0, _c12, (2, 4)), ("v", 1, _c22, (0, 1, 2, 5))]

        def combine(pieces):
            ready = [c for c in combos if all(x in prods for x in c[3])]
            for e, (key, odd, comb, needs) in enumerate(ready):
                combos.remove((key, odd, comb, needs))
                for k in range(nq // 2):
                    m = {x: prods[x][k * TQ:(k + 1) * TQ] for x in needs}
                    if pieces:
                        rows = []
                        for g in range(8):
                            at = ((e * (nq // 2) + k) * 8 + g) / (len(ready) * (nq // 2) * 8)
                            rows.append(jnp.tile(pieces[int(0.95 * at * len(pieces))], (2, 2)))
                        m[needs[0]] = jnp.where(jnp.tile(never, (32, 2)), jnp.concatenate(rows + rows, axis=0),
                                                m[needs[0]])
                    c = comb(m)
                    held[2 * k + odd, key] = _to_u32(c)
                    if 2 * k + odd < nq - 1:
                        off = (c[:L, L:], c[L:, :L]) if key == "v" else (c[L:, :L], c[:L, L:])
                        ops = _right(c[:L, :L], *off, c[L:, L:])
                        held[2 * k + odd, key + "5"] = [_to_u32(ops[x]) for x in SUMS]

        def proj(n, lazy):
            w = _right_one(n, [lambda e=e: _head_weight(b_s.at[e], hn, DC // 4, pb) for e in range(4)])
            links = list(waiting)
            del waiting[:]
            if n in DEEP:
                kh = DC // 4
                right = [o.astype(BF16) for o in _right(w[:kh, :L], w[:kh, L:], w[kh:, :L], w[kh:, L:])]
                m, pieces = {}, []

                def sub(x, after):
                    lhs = a2_s[DEEP.index(n), x]
                    if after:
                        t = after[0]
                        for v in after[1:]:
                            t = jnp.maximum(t, v)
                        lhs = tie(lhs, [pltpu.bitcast(jnp.maximum(t[g * 16:g * 16 + 8], t[g * 16 + 8:g * 16 + 16]), U32)
                                        for g in range(S // 64)], 1)
                    elif links:
                        lhs = tie(lhs, links, lhs.shape[0] // 8 // len(links))
                    m[x] = jnp.dot(_as_bf16(lhs), right[x], preferred_element_type=F32)
                    pieces.extend(spots(m[x], (0,), range(0, S // 4, 64)))
                sub(1, ()), sub(3, ())
                c21 = m[1] + m[3]
                sub(2, ()), sub(4, (c21,))
                c12, c11, c22 = m[2] + m[4], m[3] - m[4], m[2] - m[1]
                sub(0, ()), sub(5, (c12, c11, c22))
                c11, c22 = c11 + m[0], c22 + (m[0] + m[5])
                sub(6, (c11, c22))
                top = jnp.concatenate([c11 + m[6], c12], axis=1)
                bot = jnp.concatenate([c21, c22], axis=1)
                prods[n] = jnp.concatenate([v[k * L:(k + 1) * L] for k in range(nq // 2) for v in (top, bot)],
                                           axis=0)
            else:
                lhs = a_s[FLAT.index(n)]
                if links:
                    lhs = tie(lhs, links, max(1, lhs.shape[0] // 8 // len(links)))
                prods[n] = jnp.dot(_as_bf16(lhs), w.astype(BF16), preferred_element_type=F32)
                pieces = spots(prods[n], (0, 1), range(0, S // 2, 32))
            if not lazy:
                combine(None)
            return pieces

        def write_kv():
            for ch in reversed(range(nq)):
                k_s[ch * HQ:(ch + 1) * HQ, :] = held[ch, "k"]
                v_s[ch * HQ:(ch + 1) * HQ, :] = held[ch, "v"]
                for key, ref in (("k5", k5_s), ("v5", v5_s)):
                    for n, o in enumerate(held.get((ch, key), ())):
                        ref[n, ch * 64:(ch + 1) * 64, :] = o

        def right_operand(n, plain, sums, c0, c1):
            if n == 1:
                return jnp.concatenate([_as_bf16(plain[c * HQ:c * HQ + 64, :L]) for c in range(c0, c1)], axis=0)
            if n == 4:
                return jnp.concatenate([_as_bf16(plain[c * HQ + 64:(c + 1) * HQ, L:]) for c in range(c0, c1)], axis=0)
            return _as_bf16(sums[SUMS.index(n), c0 * 64:c1 * 64, :])

        def qk(i, tied):
            q = qd = q_s[h, i * HQ:(i + 1) * HQ, :]
            n = len(waiting) - 8 if tied else 0
            if n > 0:
                qd = tie(q, waiting[:n], 16 // n)
                del waiting[:n]
            q, qd = _as_bf16(q), _as_bf16(qd)
            tops, bots, pieces = [], [], []
            if i:
                qf = q.astype(F32)
                left = [o.astype(BF16) for o in _left(qf[:L, :L], qf[:L, L:], qf[L:, :L], qf[L:, L:])]
                left[2], left[3] = q[:L, :L], q[L:, L:]
            done = []
            for c in range(i):
                lhs = dict(enumerate(left))
                if c >= 2:
                    u = pltpu.bitcast(left[0], U32)
                    lhs[0] = _as_bf16(jnp.concatenate(
                        [jnp.where(never, done[c - 2][g], u[g * 8:(g + 1) * 8]) for g in range(8)], axis=0))
                m = {n: jax.lax.dot_general(lhs[n], right_operand(n, k_s, k5_s, c, c + 1), NT,
                                            preferred_element_type=F32) for n in tune[1]}
                c11, c12, c21, c22 = _c11(m), _c12(m), _c21(m), _c22(m)
                tops += [c11, c12]
                bots += [c21, c22]
                t = jnp.maximum(jnp.maximum(c11, c12), jnp.maximum(c21, c22))
                done.append([pltpu.bitcast(jnp.maximum(t[g * 16:g * 16 + 8], t[g * 16 + 8:(g + 1) * 16]), U32)
                             for g in range(8)])
                for n in (0, 5):
                    pieces += spots(m[n], (0,), (0, 32, 64, 96))
            r0 = i * HQ
            s1 = jax.lax.dot_general(qd, _as_bf16(k_s[r0:r0 + 64, :]), NT, preferred_element_type=F32)
            s2 = jax.lax.dot_general(q[L:], _as_bf16(k_s[r0 + 64:r0 + HQ, :]), NT, preferred_element_type=F32)
            top = jnp.concatenate(tops + [jnp.where(tri, s1[:L], neg)], axis=1)
            bot = jnp.concatenate(bots + [s1[L:], jnp.where(tri, s2, neg)], axis=1)
            return (top, bot), pieces + spots(s1, (0,))

        def softmax(i, top, bot, pieces, again=False):
            p, sums, prev = ([], []), ([], []), None
            for k in range(TQ // 8):
                half = k % 2
                s = (top, bot)[half][(k // 2) * 8:(k // 2 + 1) * 8]
                link = pieces[int(tune[0][i] * k * 8 / TQ * len(pieces))]
                if prev is not None:
                    link = jnp.where(never, link, prev)
                m = jnp.broadcast_to(jnp.max(s, axis=1, keepdims=True), (8, L))
                m = jnp.where(never, link, m)
                e = [jnp.exp2(s[:, t:t + L] - m) for t in range(0, s.shape[1], L)]
                prev = e[0]
                for x in e[1:]:
                    prev = prev + x
                if again:
                    m = m + jnp.log2(jnp.sum(prev, axis=1, keepdims=True))
                    e = [jnp.exp2(s[:, t:t + L] - m) for t in range(0, s.shape[1], L)]
                sums[half].append(prev)
                p[half].append(jnp.concatenate(e, axis=1))
            pt, pb_ = jnp.concatenate(p[0], axis=0), jnp.concatenate(p[1], axis=0)

            def tile(x, t):
                return x[:, t * L:(t + 1) * L]
            ops = [_left(tile(pt, 2 * c), tile(pt, 2 * c + 1), tile(pb_, 2 * c), tile(pb_, 2 * c + 1))
                   for c in range(i)]
            left = [jnp.concatenate([o[n] for o in ops], axis=1).astype(BF16) for n in range(7)] if i else None
            inv = []
            for x in () if again else sums:
                l = jnp.sum(jnp.concatenate(x, axis=0), axis=1, keepdims=True)
                r = pl.reciprocal(l, approx=True)
                inv.append(r * (2.0 - l * r))
            return (left, jnp.concatenate([tile(pt, 2 * i), tile(pb_, 2 * i)], axis=0).astype(BF16),
                    tile(pb_, 2 * i + 1).astype(BF16), inv)

        def pv(i, left, p1, p2, inv):
            r0 = i * HQ
            m, pieces = {}, []
            for n in tune[2] if i else ():
                m[n] = jnp.dot(left[n], right_operand(n, v_s, v5_s, 0, i), preferred_element_type=F32)
                pieces += spots(m[n], (0,), (0, 32, 64, 96))
            c1 = jnp.dot(p1, _as_bf16(v_s[r0:r0 + 64, :]), preferred_element_type=F32)
            c2 = jnp.dot(p2, _as_bf16(v_s[r0 + 64:r0 + HQ, :]), preferred_element_type=F32)
            top, bot = c1[:L], c1[L:] + c2
            if i:
                top = top + jnp.concatenate([_c11(m), _c12(m)], axis=1)
                bot = bot + jnp.concatenate([_c21(m), _c22(m)], axis=1)
            else:
                pieces = spots(c1, (0, 1))
            if inv:
                top, bot = top * inv[0], bot * inv[1]
            us = [_to_u32(o) for o in _right(top[:, :L], bot[:, :L], top[:, L:], bot[:, L:])]
            for n in range(7):
                x7_s[n, h, i * 64:(i + 1) * 64, :] = us[n]
            waiting.extend(_or_all([us[n][g * 8:(g + 1) * 8] for n in SUMS]) for g in range(8))
            return pieces

        def wo_operands(pieces):
            groups = M // 64
            never2 = jnp.concatenate([never, never], axis=0)
            share = -(-(H // 2) * groups // (H - 1))
            for k in range(share):
                u = jnp.minimum(h * share + k, (H // 2) * groups - 1)
                pair = jax.lax.div(u, groups)
                rg = u - pair * groups
                ops = [_left(*[wo_s[2 * pair + par, pl.ds(pl.multiple_of(hf * mh + sub * (mh // 2) + rg * 16, 16), 16),
                                    ch * L:(ch + 1) * L].astype(F32) for hf in range(2) for ch in range(2)])
                       for sub in range(2) for par in range(2)]
                for n in range(7):
                    link = pieces[int(0.96 * (k * 7 + n) / (share * 7) * len(pieces))]
                    gate = jnp.concatenate([link, link], axis=0)
                    us = [_to_u32(o) for o in _left(*[jnp.where(never2, gate, o[n]) for o in ops])]
                    for x in range(7):
                        wo_ops[n, x, pair, pl.ds(pl.multiple_of(rg * 8, 8), 8), :] = us[x]
                    waiting.append(_or_all(us))

        scores, probs, pieces = {}, {}, []
        for op in order.split():
            i = int(op[1:])
            if op[0] in "Gg":
                pieces.append(proj(i, op[0] == "g"))
            elif op[0] == "c":
                combine(sum(pieces[-i:], []))
            elif op[0] == "w":
                write_kv()
            elif op[0] == "o":
                wo_operands(pieces[-1])
            elif op[0] in "Qr":
                scores[i], new = qk(i, op[0] == "r")
                pieces.append(new)
            elif op[0] == "S":
                probs[i] = softmax(i, *scores.pop(i), pieces[-1])
            elif op[0] == "t":
                probs[i] = softmax(i, *scores.pop(i), pieces[-2] + pieces[-1], again=True)
            elif op[0] == "V":
                pieces.append(pv(i, *probs.pop(i)))
            else:
                hooks[i](pieces)

    def phase1(c_s, wq_r, wk_r, wv_r, wg_s, wu_s, wd_s, xa_s, wq0_s, wq1_s, wr_s, gw_s):
        def x_copy(j):
            return pltpu.make_async_copy(xT_hbm.at[:, pl.ds(j * RC, RC)], xT_s.at[j], sem.at[S_X + j])

        def wq_copy(g, j):
            return pltpu.make_async_copy(wq_hbm.at[:, pl.ds(j * mq, mq), g], wq_r.at[:, pl.ds(j * mq, mq), g],
                                         sem.at[(S_Q1 if g else S_Q0) + j])

        def kv_copies(j):
            return [pltpu.make_async_copy(src.at[pl.ds(j * n, n)], dst.at[pl.ds(j * n, n)], sem.at[s0 + j])
                    for src, dst, s0, n in ((c_hbm, c_s, S_C, RC), (wk_hbm, wk_r, S_K, mk), (wv_hbm, wv_r, S_V, mk))]

        misc = [pltpu.make_async_copy(a, b, sem.at[S_MISC + i]) for i, (a, b) in enumerate(
            [(wr_hbm, wr_s), (gw_hbm, gw_s), (wg_hbm, wg_s), (wu_hbm, wu_s), (wd_hbm, wd_s)])]

        x_copy(0).start()
        for j in range(NCH):
            wq_copy(0, j).start()
        for j in range(NCH):
            if j + 1 < NCH:
                x_copy(j + 1).start()
            wq_copy(1, j).start()
        misc[0].start()
        misc[1].start()
        for j in range(NCH):
            for cp in kv_copies(j):
                cp.start()
        for cp in misc[2:]:
            cp.start()
        wo_copy.start()

        def x_operands(j):
            r0 = j * HQ if isinstance(j, int) else pl.multiple_of(j * HQ, HQ)
            a = [xT_s[j, kh * mh:(kh + 1) * mh, rb * TQ:(rb + 1) * TQ].astype(F32)
                 for rb in range(2) for kh in range(2)]
            for n, o in enumerate(_left(*a)):
                xa_s[n, pl.ds(r0, HQ), :] = pltpu.bitcast(o.astype(BF16).T, U32)

        def wq_blocks(g, p, never=None, link=None):
            for kh in range(2):
                w = pltpu.bitcast(wq_r[kh, pl.ds(2 * p, 2), g], U32)
                w = [w[e] if link is None else jnp.where(never, link, w[e]) for e in range(2)]
                for par, u in enumerate(_split_heads(*w)):
                    (wq0_s, wq1_s)[g][2 * kh + par, pl.ds(p, 8, stride=pq), :] = u

        x_copy(0).wait()
        x_operands(0)

        def first_half(j, _):
            wq_copy(0, j).wait()
            for k in range(mq // 2):
                wq_blocks(0, j * (mq // 2) + k)
            return 0
        jax.lax.fori_loop(0, NCH, first_half, 0)

        def q_step(g, j, side):
            pieces = []
            for r in range(4):
                m = {}
                for n in (4, 0, 3, 6, 1, 2, 5):
                    w = _right_one(n, [lambda e=e: jnp.concatenate(
                        [_as_bf16((wq0_s, wq1_s)[g][e, pl.ds((dt * 4 + r) * pq, mh // 2), :]) for dt in range(2)],
                        axis=1) for e in range(4)])
                    m[n] = jnp.dot(_as_bf16(xa_s[n, pl.ds(pl.multiple_of(j * HQ, HQ), HQ), :]), w.astype(BF16),
                                   preferred_element_type=F32)
                    for k in range(5):
                        pieces.append(m[n][k * 48:k * 48 + 8, (k % 2) * L:(k % 2 + 1) * L])
                        side(len(pieces) - 1, pieces[-1])
                for par, rb, comb in ((0, 0, _c11), (0, 1, _c21), (1, 0, _c12), (1, 1, _c22)):
                    r0 = pl.multiple_of(j * TQ + rb * HQ, HQ)
                    q_s[8 * g + 2 * r + par, pl.ds(r0, HQ), :] = _to_u32(comb(m) * qscale)

        def q_lo(j, _):
            never = _never(j)

            def side(k, piece):
                if k == 35:
                    @pl.when(j + 1 < NCH)
                    def _():
                        x_copy(j + 1).wait()
                    wq_copy(1, j).wait()
                if k >= 42 and k % 3 == 0 and (k - 42) // 3 < mq // 2:
                    wq_blocks(1, j * (mq // 2) + (k - 42) // 3, never, pltpu.bitcast(piece, U32))
            q_step(0, j, side)
            x_operands((j + 1) & (NCH - 1))
            return 0
        jax.lax.fori_loop(0, NCH, q_lo, 0)

        def q_hi(j, _):
            for cp in kv_copies(j):
                cp.wait()
            never = _never(j)
            quad = []

            def side(kk, piece):
                if kk >= 128:
                    return
                k, g = kk // 2, kk % 2
                link = pltpu.bitcast(piece, U32)
                if g == 0:
                    rg, t = k // 8 + 8 * (k % 4 // 2), k // 4 % 2 + 2 * (k % 2)
                    a = []
                    for rb in range(2):
                        r0 = pl.multiple_of(j * RC + rb * TQ + rg * 16, 16)
                        for ch in range(2):
                            a.append(c_s[pl.ds(r0, 16), (2 * t + ch) * L:(2 * t + ch + 1) * L].astype(F32))
                    a[0] = jnp.where(jnp.concatenate([never, never], axis=0),
                                     jnp.concatenate([piece, piece], axis=0), a[0])
                    ops = _left(*a)
                    us = [_to_u32(ops[n]) for n in FLAT]
                    d0 = pl.multiple_of(j * HQ + rg * 8, 8)
                    for n, u in enumerate(us):
                        a_s[n, pl.ds(d0, 8), t * L:(t + 1) * L] = u
                    quad.append(ops)
                    if len(quad) == 4:
                        d0 = pl.multiple_of(j * (HQ // 2) + (rg - 8) * 8, 8)
                        for e, n in enumerate(DEEP):
                            deep = [_to_u32(o) for o in _left(*[q[n] for q in quad])]
                            for x, u in enumerate(deep):
                                a2_s[e, x, pl.ds(d0, 8), (t - 2) * L:(t - 1) * L] = u
                            us += deep
                        del quad[:]
                    link = _or_all(us)
                c0 = j * mk + 2 * k
                for e, (o, r) in enumerate((o, r) for o in (0, L) for r in (wk_r, wv_r)):
                    w = pltpu.bitcast(r[pl.ds(c0 + o, 2), g], U32)
                    for par, u in enumerate(_split_heads(jnp.where(never, link, w[0]), jnp.where(never, link, w[1]))):
                        b_s[e, 2 * g + par, pl.ds(j * (mk // 4) + k, 8, stride=pb), :] = u
            q_step(1, j, side)
            return j
        never = _never(jax.lax.fori_loop(0, NCH, q_hi, 0))

        for cp in misc:
            cp.wait()
        st = {}
        F = wg_s.shape[1]

        def route(pieces):
            pieces = pieces[-2] + pieces[-1]
            mp = -(-M // L) * L
            cols = []
            for w_s in (wr_s, gw_s):
                w = jnp.concatenate([w_s[...].reshape(1, M).astype(F32), jnp.zeros((1, mp - M), F32)], axis=1)
                cols.append(jnp.broadcast_to(w, (L, mp)).T)
            nr, rows = 4, M // 4
            out, k, prev = ([], []), 0, None
            for ct in range(S // L):
                acc = [None, None]
                for q in range(nr):
                    link = pieces[int((FFN_TUNE[0] + FFN_TUNE[1] * k / (nr * S // L)) * len(pieces))]
                    if prev is not None:
                        link = jnp.where(never, link, prev)
                    k += 1
                    x = linked(xT_s[ct * L // RC, q * rows:(q + 1) * rows, pl.ds(ct * L % RC, L)], link)
                    for t in range(2):
                        part = fold(x * cols[t][q * rows:(q + 1) * rows], 0)
                        acc[t] = part if acc[t] is None else acc[t] + part
                    prev = acc[0] + acc[1]
                for t in range(2):
                    out[t].append(jnp.sum(acc[t], axis=0, keepdims=True))
            gate = jax.nn.sigmoid(jnp.concatenate(out[1], axis=1))
            for j in range(S // RC):
                g_s[j, 0:1, :] = gate[:, j * RC:(j + 1) * RC]
            r = jnp.concatenate(out[0], axis=1).astype(BF16).astype(F32)
            lane = jax.lax.broadcasted_iota(jnp.int32, (1, S), 1)
            m1 = jnp.max(r, axis=1, keepdims=True)
            i1 = jnp.min(jnp.where(r == m1, lane, S - 1), axis=1, keepdims=True)
            r2 = jnp.where(lane == i1, -jnp.inf, r)
            m2 = jnp.max(r2, axis=1, keepdims=True)
            i2 = jnp.min(jnp.where(jnp.logical_and(r2 == m2, lane != i1), lane, S - 1), axis=1, keepdims=True)
            ln = jax.lax.broadcasted_iota(jnp.int32, (M, L), 1)
            st["at"] = [(i[0, 0] >> 9, slice(None), pl.ds(pl.multiple_of(i[0, 0] & (RC - L), L), L))
                        for i in (i1, i2)]
            st["hit"] = [ln == (i & (L - 1)) for i in (i1, i2)]
            st["r"] = [jax.nn.sigmoid(m1), jax.nn.sigmoid(m2)]
            st["x"] = [jnp.broadcast_to(jnp.sum(jnp.where(hit, xT_s[at].astype(F32), 0.0),
                                                axis=1, keepdims=True), (M, L))
                       for at, hit in zip(st["at"], st["hit"])]

        def fold(v, axis):
            parts = [v[k * 8:(k + 1) * 8] if axis == 0 else v[:, k * L:(k + 1) * L]
                     for k in range(v.shape[axis] // (8, L)[axis])]
            while len(parts) > 1:
                parts = [parts[k] + parts[k + 1] if k + 1 < len(parts) else parts[k]
                         for k in range(0, len(parts), 2)]
            return parts[0]

        def linked(w, link):
            w = pltpu.bitcast(w, U32)
            reps = (w.shape[0] // 8, w.shape[1] // L)
            w = jnp.where(jnp.tile(never, reps), jnp.tile(pltpu.bitcast(link, U32), reps), w)
            return _as_bf16(w).astype(F32)

        def hidden(pieces):
            pieces = pieces[-3] + pieces[-2] + pieces[-1]
            nr, rows = 4, M // 4
            total = 2 * (F // L) * nr
            out, k, prev = [], 0, None
            for w_s in (wg_s, wu_s):
                cols = ([], [])
                for ct in range(F // L):
                    acc = [None, None]
                    for q in range(nr):
                        link = pieces[int((FFN_TUNE[2] + FFN_TUNE[3] * k / total) * len(pieces))]
                        if prev is not None:
                            link = jnp.where(never, link, prev)
                        k += 1
                        w = linked(w_s[q * rows:(q + 1) * rows, ct * L:(ct + 1) * L], link)
                        for t in range(2):
                            part = fold(w * st["x"][t][q * rows:(q + 1) * rows], 0)
                            acc[t] = part if acc[t] is None else acc[t] + part
                        prev = acc[0] + acc[1]
                    for t in range(2):
                        cols[t].append(jnp.sum(acc[t], axis=0, keepdims=True))
                out.append([jnp.concatenate(c, axis=1) for c in cols])
            st["h"] = [(jax.nn.silu(out[0][t]) * out[1][t]).astype(BF16).astype(F32) for t in range(2)]

        def patch(pieces):
            pieces = pieces[-2] + pieces[-1]
            half = F // 2
            ys, k, prev = ([], []), 0, None
            for rg in range(M // 16):
                acc = [None, None]
                for hf in range(2):
                    link = pieces[int((FFN_TUNE[4] + FFN_TUNE[5] * k / (M // 8)) * len(pieces))]
                    if prev is not None:
                        link = jnp.where(never, link, prev)
                    k += 1
                    w = linked(wd_s[rg * 16:(rg + 1) * 16, hf * half:(hf + 1) * half], link)
                    for t in range(2):
                        part = fold(w * st["h"][t][:, hf * half:(hf + 1) * half], 1)
                        acc[t] = part if acc[t] is None else acc[t] + part
                    prev = fold(acc[0] + acc[1], 0)
                for t in range(2):
                    ys[t].append(jnp.sum(acc[t], axis=1, keepdims=True))
            for t in range(2):
                y = jnp.concatenate(ys[t], axis=0) * st["r"][t]
                blk = xT_s[st["at"][t]].astype(F32)
                xT_s[st["at"][t]] = (blk + jnp.where(st["hit"][t], y, 0.0)).astype(BF16)

        head_program(FIRST_ORDER, None, 0, never, hooks=(route, hidden, patch))

    def phase2(x7_s, wo_ops):
        wo_copy.wait()
        tri = jax.lax.broadcasted_iota(jnp.int32, (L, L), 1) <= jax.lax.broadcasted_iota(jnp.int32, (L, L), 0)

        def head(h, _):
            head_program(LOOP_ORDER, h, h + 1, _never(h), x7_s, tri, wo_ops, LOOP_TUNE)
            return h
        last = jax.lax.fori_loop(0, H - 1, head, 0)
        head_program(LAST_ORDER, H - 1, None, _never(last), x7_s, tri, tune=LAST_TUNE)

        def out_step(j, _):
            m = ({}, {})
            for n in range(7):
                right = [[] for _ in range(7)]
                for pair in range(H // 2):
                    blk = [_as_bf16(x7_s[n, 2 * pair + par, pl.ds(pl.multiple_of(j * L + t * 64, 64), 64), :])
                           for par in range(2) for t in range(2)]
                    ops = list(_right(*[v.astype(F32) for v in blk]))
                    ops[1], ops[4] = blk[0], blk[3]
                    for x in range(7):
                        right[x].append(ops[x])
                mm = {x: jax.lax.dot_general(
                    jnp.concatenate([_as_bf16(wo_ops[n, x, pair, :M // 8]) for pair in range(H // 2)], axis=1),
                    jnp.concatenate(right[x], axis=1).astype(BF16), NT, preferred_element_type=F32)
                    for x in (4, 2, 1, 5, 0, 3, 6)}
                m[0][n] = jnp.concatenate([((mm[0] + mm[3]) - mm[4]) + mm[6], _c21(mm)], axis=0)
                m[1][n] = jnp.concatenate([_c12(mm), _c22(mm)], axis=0)
            gate = g_s[j, 0:1, :]
            for hf in (1, 0):
                rest = (1.0 - gate) * xT_s[j, hf * mh:(hf + 1) * mh, :].astype(F32)
                cols = []
                for t in range(RC // TQ):
                    gl, gr = gate[:, t * TQ:t * TQ + L], gate[:, t * TQ + L:(t + 1) * TQ]
                    rl, rr = rest[:, t * TQ:t * TQ + L], rest[:, t * TQ + L:(t + 1) * TQ]
                    if hf:
                        cols += [gl * _c21(m[t]) + rl, gr * _c22(m[t]) + rr]
                    else:
                        cols += [(gl * ((m[t][0] + m[t][3]) - m[t][4]) + rl) + gl * m[t][6], gr * _c12(m[t]) + rr]
                o_s[j, hf * mh:(hf + 1) * mh, :] = jnp.concatenate(cols, axis=1).astype(BF16)
                out_copy(j, hf).start()
            return 0
        jax.lax.fori_loop(0, S // RC, out_step, 0)
        for j in range(S // RC):
            for hf in range(2):
                out_copy(j, hf).wait()

    pl.run_scoped(
        phase1,
        *[pltpu.VMEM(r.shape, r.dtype) for r in (c_hbm, wq_hbm, wk_hbm, wv_hbm, wg_hbm, wu_hbm, wd_hbm)],
        pltpu.VMEM((7, S // 4, mh), U32),
        pltpu.VMEM((4, -(-pq // 4) * 32, L), U32),
        pltpu.VMEM((4, -(-pq // 4) * 32, L), U32),
        pltpu.VMEM((M,), BF16),
        pltpu.VMEM((M,), BF16))
    pl.run_scoped(phase2, pltpu.VMEM((7, H, S // 4, L), U32), pltpu.VMEM((7, 7, H // 2, 64, L), U32))


def _tile_view(w):
    c, h, d = w.shape
    w = w.reshape(c, h // 8, 8, d // L, L).transpose(0, 1, 3, 2, 4)
    return w.reshape(c, h // 8, 8 * (d // L), L)


@jax.jit
def pallas_gated_mix__compressed_kv_cla__moe_arch_mod__prompt_kernel(
    A_x: jax.Array,
    A_c_kv: jax.Array,
    A_w_q: jax.Array,
    A_w_uk: jax.Array,
    A_w_uv: jax.Array,
    A_w_o: jax.Array,
    B_x: jax.Array,
    B_w_r: jax.Array,
    B_w_gate: jax.Array,
    B_w_up: jax.Array,
    B_w_down: jax.Array,
    gate_w: jax.Array,
):
    _, S, M = A_x.shape
    DC = A_c_kv.shape[2]
    H, D = A_w_q.shape[1], A_w_q.shape[2]
    args = (jnp.transpose(A_x[0]), A_c_kv[0], _tile_view(A_w_q).reshape(2, M // 2, 2, 16, L),
            _tile_view(A_w_uk), _tile_view(A_w_uv),
            jnp.transpose(A_w_o, (0, 2, 1)), B_w_r, gate_w, B_w_gate, B_w_up, jnp.transpose(B_w_down))

    def kern(*refs):
        _kernel(*refs, S=S, M=M, DC=DC, H=H, D=D)

    hbm = pl.BlockSpec(memory_space=pl.ANY)
    oT = pl.pallas_call(
        kern,
        out_shape=jax.ShapeDtypeStruct((M, S), A_x.dtype),
        in_specs=[hbm] * len(args),
        out_specs=hbm,
        scratch_shapes=[
            pltpu.VMEM((S // RC, 8, RC), F32),
            pltpu.VMEM((S // RC, M, RC), BF16),
            pltpu.VMEM((H, M, D), BF16),
            pltpu.VMEM((5, S // 4, DC // 2), U32),
            pltpu.VMEM((2, 7, S // 8, DC // 4), U32),
            pltpu.VMEM((4, 4, 8 * (DC // 4 + 4), L), U32),
            pltpu.VMEM((H, S // 2, D), U32),
            pltpu.VMEM((S // 2, D), U32),
            pltpu.VMEM((S // 2, D), U32),
            pltpu.VMEM((5, S // 4, L), U32),
            pltpu.VMEM((S // RC, M, RC), BF16),
            pltpu.VMEM((5, S // 4 + PAD_V, L), U32),
            pltpu.SemaphoreType.DMA((N_SEM,)),
        ],
        compiler_params=pltpu.CompilerParams(vmem_limit_bytes=124 * 1024 * 1024, disable_bounds_checks=True,
                                             disable_semaphore_checks=True),
    )(*args)
    return jnp.transpose(oT)[None]
```

```python
import math

import jax
import jax.numpy as jnp
import jax.experimental.pallas as pl
import jax.experimental.pallas.tpu as pltpu

F32 = jnp.float32
BF16 = jnp.bfloat16
U32 = jnp.uint32
NT = (((1,), (1,)), ((), ()))

L = 128
TQ = 256
HQ = TQ // 2
RC = 512
NCH = 4

PAD_V = 16

S_X, S_Q0, S_Q1, S_K, S_V, S_C, S_MISC, S_OUT = 0, 4, 12, 16, 20, 24, 28, 34
N_SEM = 42

LOOP_ORDER = ("Q0 Q7 S0 G0 S7 V0 V7 o0 Q6 G3 S6 V6 Q5 G4 S5 V5 Q4 G5 S4 V4 Q3 G6 S3 V3 Q2 g2 S2 V2 "
              "Q1 c2 G1 S1 V1 w0")
LOOP_TUNE = ((0.854, 0.969, 0.851, 0.941, 0.801, 0.94, 0.979, 0.948), (2, 4, 1, 3, 0, 6, 5), (2, 3, 4, 0, 1, 5, 6))
LAST_TUNE = ((0.8, 0.9, 0.66, 0.99, 0.9, 0.68, 0.93, 0.83), (0, 3, 4, 6, 1, 2, 5), (2, 3, 0, 4, 1, 6, 5))
FFN_TUNE = (0.03, 0.65, 0.0, 0.9, 0.1, 0.8)
FIRST_ORDER = "G0 G2 h0 G3 G4 G6 h1 G5 G1 h2 w0"
LAST_ORDER = "Q7 Q6 Q5 t7 V7 S6 Q4 V6 S5 r3 V5 S4 r2 V4 S3 r1 V3 t2 r0 V2 t1 t0 V1 V0"


def _to_u32(x_f32):
    return pltpu.bitcast(x_f32.astype(BF16), U32)


def _as_bf16(x_u32):
    return pltpu.bitcast(x_u32, BF16)


def _left(a11, a12, a21, a22):
    return (a11 + a22, a21 + a22, a11, a22, a11 + a12, a21 - a11, a12 - a22)


def _right(b11, b12, b21, b22):
    return (b11 + b22, b11, b12 - b22, b21 - b11, b22, b11 + b12, b21 + b22)


FLAT, DEEP = (0, 1, 3, 4, 6), (2, 5)
SUMS = (0, 2, 3, 5, 6)


def _c11(m):
    return (m[0] + m[3]) + (m[6] - m[4])


def _c12(m):
    return m[2] + m[4]


def _c21(m):
    return m[1] + m[3]


def _c22(m):
    return (m[0] - m[1]) + (m[2] + m[5])


def _never(i):
    return jax.lax.broadcasted_iota(jnp.int32, (8, L), 0) < (i >> 10)


def _or_all(xs):
    out = xs[0]
    for x in xs[1:]:
        out = out | x
    return out


def _split_heads(even, odd):
    return ((even & jnp.uint32(0xFFFF)) | (odd << 16), (even >> 16) | (odd & jnp.uint32(0xFFFF0000)))


def _right_one(n, blocks):
    x, y, sign = ((0, 3, 1), (0, None, 0), (1, 3, -1), (2, 0, -1), (3, None, 0), (0, 1, 1), (2, 3, 1))[n]
    if y is None:
        return blocks[x]()
    x, y = blocks[x]().astype(F32), blocks[y]().astype(F32)
    return x + y if sign > 0 else x - y


def _head_weight(ref, h, nrows, pitch):
    sel = ((h >> 3) << 1) + (h & 1)
    r = (h >> 1) & 3
    return jnp.concatenate(
        [_as_bf16(ref[sel, pl.ds((dt * 4 + r) * pitch, nrows), :]) for dt in range(2)], axis=1)


def _kernel(xT_hbm, c_hbm, wq_hbm, wk_hbm, wv_hbm, wo_hbm, wr_hbm, gw_hbm, wg_hbm, wu_hbm, wd_hbm,
            o_hbm,
            g_s, xT_s, wo_s, a_s, a2_s, b_s, q_s, k_s, v_s, k5_s, o_s, v5_s, sem, *, S, M, DC, H, D):
    nq = S // TQ
    mh = M // 2
    pq = mh // 2 + 1
    pb = DC // 4 + 1
    mq = mh // NCH
    mk = DC // NCH
    qscale = (D ** -0.5) * math.log2(math.e)
    neg = -1e9 * math.log2(math.e)
    wo_copy = pltpu.make_async_copy(wo_hbm, wo_s, sem.at[S_MISC + 5])

    def out_copy(j, hf):
        return pltpu.make_async_copy(o_s.at[j, pl.ds(hf * mh, mh)],
                                     o_hbm.at[pl.ds(hf * mh, mh), pl.ds(j * RC, RC)], sem.at[S_OUT + 2 * j + hf])

    def head_program(order, h, hn, never, x7_s=None, tri=None, wo_ops=None, tune=None, hooks=None):
        prods, held, waiting = {}, {}, []

        def spots(v, cols, rows=(0, 64, 128, 192)):
            return [v[r:r + 8, n * L:(n + 1) * L] for n in cols for r in rows]

        def tie(lhs, links, every):
            rows = []
            for rg in range(lhs.shape[0] // 8):
                blk = lhs[rg * 8:(rg + 1) * 8]
                if links and rg % every == 0:
                    blk = jnp.concatenate([jnp.where(never, links.pop(0), blk[:, :L]), blk[:, L:]], axis=1)
                rows.append(blk)
            return jnp.concatenate(rows, axis=0)

        combos = [("k", 0, _c11, (0, 3, 4, 6)), ("k", 1, _c21, (1, 3)),
                  ("v", 0, _c12, (2, 4)), ("v", 1, _c22, (0, 1, 2, 5))]

        def combine(pieces):
            ready = [c for c in combos if all(x in prods for x in c[3])]
            for e, (key, odd, comb, needs) in enumerate(ready):
                combos.remove((key, odd, comb, needs))
                for k in range(nq // 2):
                    m = {x: prods[x][k * TQ:(k + 1) * TQ] for x in needs}
                    if pieces:
                        rows = []
                        for g in range(8):
                            at = ((e * (nq // 2) + k) * 8 + g) / (len(ready) * (nq // 2) * 8)
                            rows.append(jnp.tile(pieces[int(0.95 * at * len(pieces))], (2, 2)))
                        m[needs[0]] = jnp.where(jnp.tile(never, (32, 2)), jnp.concatenate(rows + rows, axis=0),
                                                m[needs[0]])
                    c = comb(m)
                    held[2 * k + odd, key] = _to_u32(c)
                    if 2 * k + odd < nq - 1:
                        off = (c[:L, L:], c[L:, :L]) if key == "v" else (c[L:, :L], c[:L, L:])
                        ops = _right(c[:L, :L], *off, c[L:, L:])
                        held[2 * k + odd, key + "5"] = [_to_u32(ops[x]) for x in SUMS]

        def proj(n, lazy):
            w = _right_one(n, [lambda e=e: _head_weight(b_s.at[e], hn, DC // 4, pb) for e in range(4)])
            links = list(waiting)
            del waiting[:]
            if n in DEEP:
                kh = DC // 4
                right = [o.astype(BF16) for o in _right(w[:kh, :L], w[:kh, L:], w[kh:, :L], w[kh:, L:])]
                m, pieces = {}, []

                def sub(x, after):
                    lhs = a2_s[DEEP.index(n), x]
                    if after:
                        t = after[0]
                        for v in after[1:]:
                            t = jnp.maximum(t, v)
                        lhs = tie(lhs, [pltpu.bitcast(jnp.maximum(t[g * 16:g * 16 + 8], t[g * 16 + 8:g * 16 + 16]), U32)
                                        for g in range(S // 64)], 1)
                    elif links:
                        lhs = tie(lhs, links, lhs.shape[0] // 8 // len(links))
                    m[x] = jnp.dot(_as_bf16(lhs), right[x], preferred_element_type=F32)
                    pieces.extend(spots(m[x], (0,), range(0, S // 4, 64)))
                sub(1, ()), sub(3, ())
                c21 = m[1] + m[3]
                sub(2, ()), sub(4, (c21,))
                c12, c11, c22 = m[2] + m[4], m[3] - m[4], m[2] - m[1]
                sub(0, ()), sub(5, (c12, c11, c22))
                c11, c22 = c11 + m[0], c22 + (m[0] + m[5])
                sub(6, (c11, c22))
                top = jnp.concatenate([c11 + m[6], c12], axis=1)
                bot = jnp.concatenate([c21, c22], axis=1)
                prods[n] = jnp.concatenate([v[k * L:(k + 1) * L] for k in range(nq // 2) for v in (top, bot)],
                                           axis=0)
            else:
                lhs = a_s[FLAT.index(n)]
                if links:
                    lhs = tie(lhs, links, max(1, lhs.shape[0] // 8 // len(links)))
                prods[n] = jnp.dot(_as_bf16(lhs), w.astype(BF16), preferred_element_type=F32)
                pieces = spots(prods[n], (0, 1), range(0, S // 2, 32))
            if not lazy:
                combine(None)
            return pieces

        def write_kv():
            for ch in reversed(range(nq)):
                k_s[ch * HQ:(ch + 1) * HQ, :] = held[ch, "k"]
                v_s[ch * HQ:(ch + 1) * HQ, :] = held[ch, "v"]
                for key, ref in (("k5", k5_s), ("v5", v5_s)):
                    for n, o in enumerate(held.get((ch, key), ())):
                        ref[n, ch * 64:(ch + 1) * 64, :] = o

        def right_operand(n, plain, sums, c0, c1):
            if n == 1:
                return jnp.concatenate([_as_bf16(plain[c * HQ:c * HQ + 64, :L]) for c in range(c0, c1)], axis=0)
            if n == 4:
                return jnp.concatenate([_as_bf16(plain[c * HQ + 64:(c + 1) * HQ, L:]) for c in range(c0, c1)], axis=0)
            return _as_bf16(sums[SUMS.index(n), c0 * 64:c1 * 64, :])

        def qk(i, tied):
            q = qd = q_s[h, i * HQ:(i + 1) * HQ, :]
            n = len(waiting) - 8 if tied else 0
            if n > 0:
                qd = tie(q, waiting[:n], 16 // n)
                del waiting[:n]
            q, qd = _as_bf16(q), _as_bf16(qd)
            tops, bots, pieces = [], [], []
            if i:
                qf = q.astype(F32)
                left = [o.astype(BF16) for o in _left(qf[:L, :L], qf[:L, L:], qf[L:, :L], qf[L:, L:])]
                left[2], left[3] = q[:L, :L], q[L:, L:]
            done = []
            for c in range(i):
                lhs = dict(enumerate(left))
                if c >= 2:
                    u = pltpu.bitcast(left[0], U32)
                    lhs[0] = _as_bf16(jnp.concatenate(
                        [jnp.where(never, done[c - 2][g], u[g * 8:(g + 1) * 8]) for g in range(8)], axis=0))
                m = {n: jax.lax.dot_general(lhs[n], right_operand(n, k_s, k5_s, c, c + 1), NT,
                                            preferred_element_type=F32) for n in tune[1]}
                c11, c12, c21, c22 = _c11(m), _c12(m), _c21(m), _c22(m)
                tops += [c11, c12]
                bots += [c21, c22]
                t = jnp.maximum(jnp.maximum(c11, c12), jnp.maximum(c21, c22))
                done.append([pltpu.bitcast(jnp.maximum(t[g * 16:g * 16 + 8], t[g * 16 + 8:(g + 1) * 16]), U32)
                             for g in range(8)])
                for n in (0, 5):
                    pieces += spots(m[n], (0,), (0, 32, 64, 96))
            r0 = i * HQ
            s1 = jax.lax.dot_general(qd, _as_bf16(k_s[r0:r0 + 64, :]), NT, preferred_element_type=F32)
            s2 = jax.lax.dot_general(q[L:], _as_bf16(k_s[r0 + 64:r0 + HQ, :]), NT, preferred_element_type=F32)
            top = jnp.concatenate(tops + [jnp.where(tri, s1[:L], neg)], axis=1)
            bot = jnp.concatenate(bots + [s1[L:], jnp.where(tri, s2, neg)], axis=1)
            return (top, bot), pieces + spots(s1, (0,))

        def softmax(i, top, bot, pieces, again=False):
            p, sums, prev = ([], []), ([], []), None
            for k in range(TQ // 8):
                half = k % 2
                s = (top, bot)[half][(k // 2) * 8:(k // 2 + 1) * 8]
                link = pieces[int(tune[0][i] * k * 8 / TQ * len(pieces))]
                if prev is not None:
                    link = jnp.where(never, link, prev)
                m = jnp.broadcast_to(jnp.max(s, axis=1, keepdims=True), (8, L))
                m = jnp.where(never, link, m)
                e = [jnp.exp2(s[:, t:t + L] - m) for t in range(0, s.shape[1], L)]
                prev = e[0]
                for x in e[1:]:
                    prev = prev + x
                if again:
                    m = m + jnp.log2(jnp.sum(prev, axis=1, keepdims=True))
                    e = [jnp.exp2(s[:, t:t + L] - m) for t in range(0, s.shape[1], L)]
                sums[half].append(prev)
                p[half].append(jnp.concatenate(e, axis=1))
            pt, pb_ = jnp.concatenate(p[0], axis=0), jnp.concatenate(p[1], axis=0)

            def tile(x, t):
                return x[:, t * L:(t + 1) * L]
            ops = [_left(tile(pt, 2 * c), tile(pt, 2 * c + 1), tile(pb_, 2 * c), tile(pb_, 2 * c + 1))
                   for c in range(i)]
            left = [jnp.concatenate([o[n] for o in ops], axis=1).astype(BF16) for n in range(7)] if i else None
            inv = []
            for x in () if again else sums:
                l = jnp.sum(jnp.concatenate(x, axis=0), axis=1, keepdims=True)
                r = pl.reciprocal(l, approx=True)
                inv.append(r * (2.0 - l * r))
            return (left, jnp.concatenate([tile(pt, 2 * i), tile(pb_, 2 * i)], axis=0).astype(BF16),
                    tile(pb_, 2 * i + 1).astype(BF16), inv)

        def pv(i, left, p1, p2, inv):
            r0 = i * HQ
            m, pieces = {}, []
            for n in tune[2] if i else ():
                m[n] = jnp.dot(left[n], right_operand(n, v_s, v5_s, 0, i), preferred_element_type=F32)
                pieces += spots(m[n], (0,), (0, 32, 64, 96))
            c1 = jnp.dot(p1, _as_bf16(v_s[r0:r0 + 64, :]), preferred_element_type=F32)
            c2 = jnp.dot(p2, _as_bf16(v_s[r0 + 64:r0 + HQ, :]), preferred_element_type=F32)
            top, bot = c1[:L], c1[L:] + c2
            if i:
                top = top + jnp.concatenate([_c11(m), _c12(m)], axis=1)
                bot = bot + jnp.concatenate([_c21(m), _c22(m)], axis=1)
            else:
                pieces = spots(c1, (0, 1))
            if inv:
                top, bot = top * inv[0], bot * inv[1]
            us = [_to_u32(o) for o in _right(top[:, :L], bot[:, :L], top[:, L:], bot[:, L:])]
            for n in range(7):
                x7_s[n, h, i * 64:(i + 1) * 64, :] = us[n]
            waiting.extend(_or_all([us[n][g * 8:(g + 1) * 8] for n in SUMS]) for g in range(8))
            return pieces

        def wo_operands(pieces):
            groups = M // 64
            never2 = jnp.concatenate([never, never], axis=0)
            share = -(-(H // 2) * groups // (H - 1))
            for k in range(share):
                u = jnp.minimum(h * share + k, (H // 2) * groups - 1)
                pair = jax.lax.div(u, groups)
                rg = u - pair * groups
                ops = [_left(*[wo_s[2 * pair + par, pl.ds(pl.multiple_of(hf * mh + sub * (mh // 2) + rg * 16, 16), 16),
                                    ch * L:(ch + 1) * L].astype(F32) for hf in range(2) for ch in range(2)])
                       for sub in range(2) for par in range(2)]
                for n in range(7):
                    link = pieces[int(0.96 * (k * 7 + n) / (share * 7) * len(pieces))]
                    gate = jnp.concatenate([link, link], axis=0)
                    us = [_to_u32(o) for o in _left(*[jnp.where(never2, gate, o[n]) for o in ops])]
                    for x in range(7):
                        wo_ops[n, x, pair, pl.ds(pl.multiple_of(rg * 8, 8), 8), :] = us[x]
                    waiting.append(_or_all(us))

        scores, probs, pieces = {}, {}, []
        for op in order.split():
            i = int(op[1:])
            if op[0] in "Gg":
                pieces.append(proj(i, op[0] == "g"))
            elif op[0] == "c":
                combine(sum(pieces[-i:], []))
            elif op[0] == "w":
                write_kv()
            elif op[0] == "o":
                wo_operands(pieces[-1])
            elif op[0] in "Qr":
                scores[i], new = qk(i, op[0] == "r")
                pieces.append(new)
            elif op[0] == "S":
                probs[i] = softmax(i, *scores.pop(i), pieces[-1])
            elif op[0] == "t":
                probs[i] = softmax(i, *scores.pop(i), pieces[-2] + pieces[-1], again=True)
            elif op[0] == "V":
                pieces.append(pv(i, *probs.pop(i)))
            else:
                hooks[i](pieces)

    def phase1(c_s, wq_r, wk_r, wv_r, wg_s, wu_s, wd_s, xa_s, wq0_s, wq1_s, wr_s, gw_s):
        def x_copy(j):
            return pltpu.make_async_copy(xT_hbm.at[:, pl.ds(j * RC, RC)], xT_s.at[j], sem.at[S_X + j])

        def wq0_copy(kh, j):
            return pltpu.make_async_copy(wq_hbm.at[kh, pl.ds(j * mq, mq), 0], wq_r.at[kh, pl.ds(j * mq, mq), 0],
                                         sem.at[S_Q0 + kh * NCH + j])

        def wq1_copy(j):
            return pltpu.make_async_copy(wq_hbm.at[:, pl.ds(j * mq, mq), 1], wq_r.at[:, pl.ds(j * mq, mq), 1],
                                         sem.at[S_Q1 + j])

        def kv_copies(j):
            return [pltpu.make_async_copy(src.at[pl.ds(j * n, n)], dst.at[pl.ds(j * n, n)], sem.at[s0 + j])
                    for src, dst, s0, n in ((c_hbm, c_s, S_C, RC), (wk_hbm, wk_r, S_K, mk), (wv_hbm, wv_r, S_V, mk))]

        misc = [pltpu.make_async_copy(a, b, sem.at[S_MISC + i]) for i, (a, b) in enumerate(
            [(wr_hbm, wr_s), (gw_hbm, gw_s), (wg_hbm, wg_s), (wu_hbm, wu_s), (wd_hbm, wd_s)])]

        x_copy(0).start()
        for kh in range(2):
            for j in range(NCH):
                wq0_copy(kh, j).start()
        for j in range(NCH):
            if j + 1 < NCH:
                x_copy(j + 1).start()
            wq1_copy(j).start()
        misc[0].start()
        misc[1].start()
        for j in range(NCH):
            for cp in kv_copies(j):
                cp.start()
        for cp in misc[2:]:
            cp.start()
        wo_copy.start()

        def x_operands(j):
            r0 = j * HQ if isinstance(j, int) else pl.multiple_of(j * HQ, HQ)
            a = [xT_s[j, kh * mh:(kh + 1) * mh, rb * TQ:(rb + 1) * TQ].astype(F32)
                 for rb in range(2) for kh in range(2)]
            for n, o in enumerate(_left(*a)):
                xa_s[n, pl.ds(r0, HQ), :] = pltpu.bitcast(o.astype(BF16).T, U32)

        def wq_blocks(g, p, never=None, link=None, halves=(0, 1), src=None):
            for kh in halves:
                w = pltpu.bitcast(wq_r[kh, pl.ds(2 * p, 2), g if src is None else src], U32)
                w = [w[e] if link is None else jnp.where(never, link, w[e]) for e in range(2)]
                for par, u in enumerate(_split_heads(*w)):
                    (wq0_s, wq1_s)[g][2 * kh + par, pl.ds(p, 8, stride=pq), :] = u

        x_copy(0).wait()
        x_operands(0)

        def first_heads(kh):
            def chunk(j, _):
                wq0_copy(kh, j).wait()
                for k in range(mq // 2):
                    wq_blocks(0, j * (mq // 2) + k, halves=(kh,))
                return 0
            jax.lax.fori_loop(0, NCH, chunk, 0)
        first_heads(0)

        def q_step(g, j, side, early=()):
            m, count = [{} for _ in range(4)], [0]

            def product(r, n):
                w = _right_one(n, [lambda e=e: jnp.concatenate(
                    [_as_bf16((wq0_s, wq1_s)[g][e, pl.ds((dt * 4 + r) * pq, mh // 2), :]) for dt in range(2)],
                    axis=1) for e in range(4)])
                m[r][n] = jnp.dot(_as_bf16(xa_s[n, pl.ds(pl.multiple_of(j * HQ, HQ), HQ), :]), w.astype(BF16),
                                  preferred_element_type=F32)
                for k in range(5):
                    side(count[0], m[r][n][k * 48:k * 48 + 8, (k % 2) * L:(k % 2 + 1) * L])
                    count[0] += 1
            for r in range(4):
                for n in early:
                    product(r, n)
            for r in range(4):
                for n in (4, 0, 3, 6, 1, 2, 5):
                    if n not in early:
                        product(r, n)
                for par, rb, comb in ((0, 0, _c11), (0, 1, _c21), (1, 0, _c12), (1, 1, _c22)):
                    r0 = pl.multiple_of(j * TQ + rb * HQ, HQ)
                    q_s[8 * g + 2 * r + par, pl.ds(r0, HQ), :] = _to_u32(comb(m[r]) * qscale)

        def q_lo(j, _):
            never = _never(j)

            prev = jnp.maximum(j - 1, 0)

            def side(k, piece):
                if k == 39:
                    pl.when(j == 0)(lambda: first_heads(1))
                    pl.when(j + 1 < NCH)(lambda: x_copy(j + 1).wait())
                    pl.when(j > 0)(lambda: wq1_copy(prev).wait())
                if k >= 45 and k % 3 == 0 and (k - 45) // 3 < mq // 2:
                    wq_blocks(1, prev * (mq // 2) + (k - 45) // 3, never, pltpu.bitcast(piece, U32),
                              src=jnp.minimum(j, 1))
            q_step(0, j, side, early=(1, 5))
            x_operands((j + 1) & (NCH - 1))
            return 0
        jax.lax.fori_loop(0, NCH, q_lo, 0)
        wq1_copy(NCH - 1).wait()
        for k in range(mq // 2):
            wq_blocks(1, (NCH - 1) * (mq // 2) + k)

        def q_hi(j, _):
            for cp in kv_copies(j):
                cp.wait()
            never = _never(j)
            quad = []

            def side(kk, piece):
                if kk >= 128:
                    return
                k, g = kk // 2, kk % 2
                link = pltpu.bitcast(piece, U32)
                if g == 0:
                    rg, t = k // 8 + 8 * (k % 4 // 2), k // 4 % 2 + 2 * (k % 2)
                    a = []
                    for rb in range(2):
                        r0 = pl.multiple_of(j * RC + rb * TQ + rg * 16, 16)
                        for ch in range(2):
                            a.append(c_s[pl.ds(r0, 16), (2 * t + ch) * L:(2 * t + ch + 1) * L].astype(F32))
                    a[0] = jnp.where(jnp.concatenate([never, never], axis=0),
                                     jnp.concatenate([piece, piece], axis=0), a[0])
                    ops = _left(*a)
                    us = [_to_u32(ops[n]) for n in FLAT]
                    d0 = pl.multiple_of(j * HQ + rg * 8, 8)
                    for n, u in enumerate(us):
                        a_s[n, pl.ds(d0, 8), t * L:(t + 1) * L] = u
                    quad.append(ops)
                    if len(quad) == 4:
                        d0 = pl.multiple_of(j * (HQ // 2) + (rg - 8) * 8, 8)
                        for e, n in enumerate(DEEP):
                            deep = [_to_u32(o) for o in _left(*[q[n] for q in quad])]
                            for x, u in enumerate(deep):
                                a2_s[e, x, pl.ds(d0, 8), (t - 2) * L:(t - 1) * L] = u
                            us += deep
                        del quad[:]
                    link = _or_all(us)
                c0 = j * mk + 2 * k
                for e, (o, r) in enumerate((o, r) for o in (0, L) for r in (wk_r, wv_r)):
                    w = pltpu.bitcast(r[pl.ds(c0 + o, 2), g], U32)
                    for par, u in enumerate(_split_heads(jnp.where(never, link, w[0]), jnp.where(never, link, w[1]))):
                        b_s[e, 2 * g + par, pl.ds(j * (mk // 4) + k, 8, stride=pb), :] = u
            q_step(1, j, side)
            return j
        never = _never(jax.lax.fori_loop(0, NCH, q_hi, 0))

        for cp in misc:
            cp.wait()
        st = {}
        F = wg_s.shape[1]

        def route(pieces):
            pieces = pieces[-2] + pieces[-1]
            mp = -(-M // L) * L
            cols = []
            for w_s in (wr_s, gw_s):
                w = jnp.concatenate([w_s[...].reshape(1, M).astype(F32), jnp.zeros((1, mp - M), F32)], axis=1)
                cols.append(jnp.broadcast_to(w, (L, mp)).T)
            nr, rows = 4, M // 4
            out, k, prev = ([], []), 0, None
            for ct in range(S // L):
                acc = [None, None]
                for q in range(nr):
                    link = pieces[int((FFN_TUNE[0] + FFN_TUNE[1] * k / (nr * S // L)) * len(pieces))]
                    if prev is not None:
                        link = jnp.where(never, link, prev)
                    k += 1
                    x = linked(xT_s[ct * L // RC, q * rows:(q + 1) * rows, pl.ds(ct * L % RC, L)], link)
                    for t in range(2):
                        part = fold(x * cols[t][q * rows:(q + 1) * rows], 0)
                        acc[t] = part if acc[t] is None else acc[t] + part
                    prev = acc[0] + acc[1]
                for t in range(2):
                    out[t].append(jnp.sum(acc[t], axis=0, keepdims=True))
            gate = jax.nn.sigmoid(jnp.concatenate(out[1], axis=1))
            for j in range(S // RC):
                g_s[j, 0:1, :] = gate[:, j * RC:(j + 1) * RC]
            r = jnp.concatenate(out[0], axis=1).astype(BF16).astype(F32)
            lane = jax.lax.broadcasted_iota(jnp.int32, (1, S), 1)
            m1 = jnp.max(r, axis=1, keepdims=True)
            i1 = jnp.min(jnp.where(r == m1, lane, S - 1), axis=1, keepdims=True)
            r2 = jnp.where(lane == i1, -jnp.inf, r)
            m2 = jnp.max(r2, axis=1, keepdims=True)
            i2 = jnp.min(jnp.where(jnp.logical_and(r2 == m2, lane != i1), lane, S - 1), axis=1, keepdims=True)
            ln = jax.lax.broadcasted_iota(jnp.int32, (M, L), 1)
            st["at"] = [(i[0, 0] >> 9, slice(None), pl.ds(pl.multiple_of(i[0, 0] & (RC - L), L), L))
                        for i in (i1, i2)]
            st["hit"] = [ln == (i & (L - 1)) for i in (i1, i2)]
            st["r"] = [jax.nn.sigmoid(m1), jax.nn.sigmoid(m2)]
            st["x"] = [jnp.broadcast_to(jnp.sum(jnp.where(hit, xT_s[at].astype(F32), 0.0),
                                                axis=1, keepdims=True), (M, L))
                       for at, hit in zip(st["at"], st["hit"])]

        def fold(v, axis):
            parts = [v[k * 8:(k + 1) * 8] if axis == 0 else v[:, k * L:(k + 1) * L]
                     for k in range(v.shape[axis] // (8, L)[axis])]
            while len(parts) > 1:
                parts = [parts[k] + parts[k + 1] if k + 1 < len(parts) else parts[k]
                         for k in range(0, len(parts), 2)]
            return parts[0]

        def linked(w, link):
            w = pltpu.bitcast(w, U32)
            reps = (w.shape[0] // 8, w.shape[1] // L)
            w = jnp.where(jnp.tile(never, reps), jnp.tile(pltpu.bitcast(link, U32), reps), w)
            return _as_bf16(w).astype(F32)

        def hidden(pieces):
            pieces = pieces[-3] + pieces[-2] + pieces[-1]
            nr, rows = 4, M // 4
            total = 2 * (F // L) * nr
            out, k, prev = [], 0, None
            for w_s in (wg_s, wu_s):
                cols = ([], [])
                for ct in range(F // L):
                    acc = [None, None]
                    for q in range(nr):
                        link = pieces[int((FFN_TUNE[2] + FFN_TUNE[3] * k / total) * len(pieces))]
                        if prev is not None:
                            link = jnp.where(never, link, prev)
                        k += 1
                        w = linked(w_s[q * rows:(q + 1) * rows, ct * L:(ct + 1) * L], link)
                        for t in range(2):
                            part = fold(w * st["x"][t][q * rows:(q + 1) * rows], 0)
                            acc[t] = part if acc[t] is None else acc[t] + part
                        prev = acc[0] + acc[1]
                    for t in range(2):
                        cols[t].append(jnp.sum(acc[t], axis=0, keepdims=True))
                out.append([jnp.concatenate(c, axis=1) for c in cols])
            st["h"] = [(jax.nn.silu(out[0][t]) * out[1][t]).astype(BF16).astype(F32) for t in range(2)]

        def patch(pieces):
            pieces = pieces[-2] + pieces[-1]
            half = F // 2
            ys, k, prev = ([], []), 0, None
            for rg in range(M // 16):
                acc = [None, None]
                for hf in range(2):
                    link = pieces[int((FFN_TUNE[4] + FFN_TUNE[5] * k / (M // 8)) * len(pieces))]
                    if prev is not None:
                        link = jnp.where(never, link, prev)
                    k += 1
                    w = linked(wd_s[rg * 16:(rg + 1) * 16, hf * half:(hf + 1) * half], link)
                    for t in range(2):
                        part = fold(w * st["h"][t][:, hf * half:(hf + 1) * half], 1)
                        acc[t] = part if acc[t] is None else acc[t] + part
                    prev = fold(acc[0] + acc[1], 0)
                for t in range(2):
                    ys[t].append(jnp.sum(acc[t], axis=1, keepdims=True))
            for t in range(2):
                y = jnp.concatenate(ys[t], axis=0) * st["r"][t]
                blk = xT_s[st["at"][t]].astype(F32)
                xT_s[st["at"][t]] = (blk + jnp.where(st["hit"][t], y, 0.0)).astype(BF16)

        head_program(FIRST_ORDER, None, 0, never, hooks=(route, hidden, patch))

    def phase2(x7_s, wo_ops):
        wo_copy.wait()
        tri = jax.lax.broadcasted_iota(jnp.int32, (L, L), 1) <= jax.lax.broadcasted_iota(jnp.int32, (L, L), 0)

        def head(h, _):
            head_program(LOOP_ORDER, h, h + 1, _never(h), x7_s, tri, wo_ops, LOOP_TUNE)
            return h
        last = jax.lax.fori_loop(0, H - 1, head, 0)
        head_program(LAST_ORDER, H - 1, None, _never(last), x7_s, tri, tune=LAST_TUNE)

        def out_step(j, _):
            m = ({}, {})
            for n in range(7):
                right = [[] for _ in range(7)]
                for pair in range(H // 2):
                    blk = [_as_bf16(x7_s[n, 2 * pair + par, pl.ds(pl.multiple_of(j * L + t * 64, 64), 64), :])
                           for par in range(2) for t in range(2)]
                    ops = list(_right(*[v.astype(F32) for v in blk]))
                    ops[1], ops[4] = blk[0], blk[3]
                    for x in range(7):
                        right[x].append(ops[x])
                mm = {x: jax.lax.dot_general(
                    jnp.concatenate([_as_bf16(wo_ops[n, x, pair, :M // 8]) for pair in range(H // 2)], axis=1),
                    jnp.concatenate(right[x], axis=1).astype(BF16), NT, preferred_element_type=F32)
                    for x in (4, 2, 1, 5, 0, 3, 6)}
                m[0][n] = jnp.concatenate([((mm[0] + mm[3]) - mm[4]) + mm[6], _c21(mm)], axis=0)
                m[1][n] = jnp.concatenate([_c12(mm), _c22(mm)], axis=0)
            gate = g_s[j, 0:1, :]
            for hf in (1, 0):
                rest = (1.0 - gate) * xT_s[j, hf * mh:(hf + 1) * mh, :].astype(F32)
                cols = []
                for t in range(RC // TQ):
                    gl, gr = gate[:, t * TQ:t * TQ + L], gate[:, t * TQ + L:(t + 1) * TQ]
                    rl, rr = rest[:, t * TQ:t * TQ + L], rest[:, t * TQ + L:(t + 1) * TQ]
                    if hf:
                        cols += [gl * _c21(m[t]) + rl, gr * _c22(m[t]) + rr]
                    else:
                        cols += [(gl * ((m[t][0] + m[t][3]) - m[t][4]) + rl) + gl * m[t][6], gr * _c12(m[t]) + rr]
                o_s[j, hf * mh:(hf + 1) * mh, :] = jnp.concatenate(cols, axis=1).astype(BF16)
                out_copy(j, hf).start()
            return 0
        jax.lax.fori_loop(0, S // RC, out_step, 0)
        for j in range(S // RC):
            for hf in range(2):
                out_copy(j, hf).wait()

    pl.run_scoped(
        phase1,
        *[pltpu.VMEM(r.shape, r.dtype) for r in (c_hbm, wq_hbm, wk_hbm, wv_hbm, wg_hbm, wu_hbm, wd_hbm)],
        pltpu.VMEM((7, S // 4, mh), U32),
        pltpu.VMEM((4, -(-pq // 4) * 32, L), U32),
        pltpu.VMEM((4, -(-pq // 4) * 32, L), U32),
        pltpu.VMEM((M,), BF16),
        pltpu.VMEM((M,), BF16))
    pl.run_scoped(phase2, pltpu.VMEM((7, H, S // 4, L), U32), pltpu.VMEM((7, 7, H // 2, 64, L), U32))


def _tile_view(w):
    c, h, d = w.shape
    w = w.reshape(c, h // 8, 8, d // L, L).transpose(0, 1, 3, 2, 4)
    return w.reshape(c, h // 8, 8 * (d // L), L)


@jax.jit
def pallas_gated_mix__compressed_kv_cla__moe_arch_mod__prompt_kernel(
    A_x: jax.Array,
    A_c_kv: jax.Array,
    A_w_q: jax.Array,
    A_w_uk: jax.Array,
    A_w_uv: jax.Array,
    A_w_o: jax.Array,
    B_x: jax.Array,
    B_w_r: jax.Array,
    B_w_gate: jax.Array,
    B_w_up: jax.Array,
    B_w_down: jax.Array,
    gate_w: jax.Array,
):
    _, S, M = A_x.shape
    DC = A_c_kv.shape[2]
    H, D = A_w_q.shape[1], A_w_q.shape[2]
    args = (jnp.transpose(A_x[0]), A_c_kv[0], _tile_view(A_w_q).reshape(2, M // 2, 2, 16, L),
            _tile_view(A_w_uk), _tile_view(A_w_uv),
            jnp.transpose(A_w_o, (0, 2, 1)), B_w_r, gate_w, B_w_gate, B_w_up, jnp.transpose(B_w_down))

    def kern(*refs):
        _kernel(*refs, S=S, M=M, DC=DC, H=H, D=D)

    hbm = pl.BlockSpec(memory_space=pl.ANY)
    oT = pl.pallas_call(
        kern,
        out_shape=jax.ShapeDtypeStruct((M, S), A_x.dtype),
        in_specs=[hbm] * len(args),
        out_specs=hbm,
        scratch_shapes=[
            pltpu.VMEM((S // RC, 8, RC), F32),
            pltpu.VMEM((S // RC, M, RC), BF16),
            pltpu.VMEM((H, M, D), BF16),
            pltpu.VMEM((5, S // 4, DC // 2), U32),
            pltpu.VMEM((2, 7, S // 8, DC // 4), U32),
            pltpu.VMEM((4, 4, 8 * (DC // 4 + 4), L), U32),
            pltpu.VMEM((H, S // 2, D), U32),
            pltpu.VMEM((S // 2, D), U32),
            pltpu.VMEM((S // 2, D), U32),
            pltpu.VMEM((5, S // 4, L), U32),
            pltpu.VMEM((S // RC, M, RC), BF16),
            pltpu.VMEM((5, S // 4 + PAD_V, L), U32),
            pltpu.SemaphoreType.DMA((N_SEM,)),
        ],
        compiler_params=pltpu.CompilerParams(vmem_limit_bytes=124 * 1024 * 1024, disable_bounds_checks=True,
                                             disable_semaphore_checks=True),
    )(*args)
    return jnp.transpose(oT)[None]
```

```python
import math

import jax
import jax.numpy as jnp
import jax.experimental.pallas as pl
import jax.experimental.pallas.tpu as pltpu

F32 = jnp.float32
BF16 = jnp.bfloat16
U32 = jnp.uint32
NT = (((1,), (1,)), ((), ()))

L = 128
TQ = 256
HQ = TQ // 2
RC = 512
NCH = 4

PAD_V = 16

O_UNROLL = 2

S_X, S_Q0, S_Q1, S_K, S_V, S_C, S_MISC, S_OUT = 0, 4, 12, 16, 20, 24, 28, 34
N_SEM = 42

LOOP_ORDER = ("Q0 Q7 S0 G0 S7 V0 V7 o0 Q6 G3 S6 V6 Q5 G4 S5 V5 Q4 G5 S4 V4 Q3 G6 S3 V3 Q2 g2 S2 V2 "
              "Q1 c2 G1 S1 V1 w0")
LOOP_TUNE = ((0.854, 0.969, 0.851, 0.941, 0.801, 0.94, 0.979, 0.948), (2, 4, 1, 3, 0, 6, 5), (2, 3, 4, 0, 1, 5, 6))
LAST_TUNE = ((0.8, 0.9, 0.66, 0.99, 0.9, 0.68, 0.93, 0.83), (0, 3, 4, 6, 1, 2, 5), (2, 3, 0, 4, 1, 6, 5))
FFN_TUNE = (0.03, 0.65, 0.0, 0.9, 0.1, 0.8)
FIRST_ORDER = "G0 G2 h0 G3 G4 G6 h1 G5 G1 h2 w0"
LAST_ORDER = "Q7 Q6 Q5 t7 V7 S6 Q4 V6 S5 r3 V5 S4 r2 V4 S3 r1 V3 t2 r0 V2 t1 t0 V1 V0"


def _to_u32(x_f32):
    return pltpu.bitcast(x_f32.astype(BF16), U32)


def _as_bf16(x_u32):
    return pltpu.bitcast(x_u32, BF16)


def _left(a11, a12, a21, a22):
    return (a11 + a22, a21 + a22, a11, a22, a11 + a12, a21 - a11, a12 - a22)


def _right(b11, b12, b21, b22):
    return (b11 + b22, b11, b12 - b22, b21 - b11, b22, b11 + b12, b21 + b22)


FLAT, DEEP = (0, 1, 3, 4, 6), (2, 5)
SUMS = (0, 2, 3, 5, 6)


def _c11(m):
    return (m[0] + m[3]) + (m[6] - m[4])


def _c12(m):
    return m[2] + m[4]


def _c21(m):
    return m[1] + m[3]


def _c22(m):
    return (m[0] - m[1]) + (m[2] + m[5])


def _never(i):
    return jax.lax.broadcasted_iota(jnp.int32, (8, L), 0) < (i >> 10)


def _or_all(xs):
    out = xs[0]
    for x in xs[1:]:
        out = out | x
    return out


def _split_heads(even, odd):
    return ((even & jnp.uint32(0xFFFF)) | (odd << 16), (even >> 16) | (odd & jnp.uint32(0xFFFF0000)))


def _right_one(n, blocks):
    x, y, sign = ((0, 3, 1), (0, None, 0), (1, 3, -1), (2, 0, -1), (3, None, 0), (0, 1, 1), (2, 3, 1))[n]
    if y is None:
        return blocks[x]()
    x, y = blocks[x]().astype(F32), blocks[y]().astype(F32)
    return x + y if sign > 0 else x - y


def _head_weight(ref, h, nrows, pitch):
    sel = ((h >> 3) << 1) + (h & 1)
    r = (h >> 1) & 3
    return jnp.concatenate(
        [_as_bf16(ref[sel, pl.ds((dt * 4 + r) * pitch, nrows), :]) for dt in range(2)], axis=1)


def _kernel(xT_hbm, c_hbm, wq_hbm, wk_hbm, wv_hbm, wo_hbm, wr_hbm, gw_hbm, wg_hbm, wu_hbm, wd_hbm,
            o_hbm,
            g_s, xT_s, wo_s, a_s, a2_s, b_s, q_s, k_s, v_s, k5_s, o_s, v5_s, sem, *, S, M, DC, H, D):
    nq = S // TQ
    mh = M // 2
    pq = mh // 2 + 1
    pb = DC // 4 + 1
    mq = mh // NCH
    mk = DC // NCH
    qscale = (D ** -0.5) * math.log2(math.e)
    neg = -1e9 * math.log2(math.e)
    wo_copy = pltpu.make_async_copy(wo_hbm, wo_s, sem.at[S_MISC + 5])

    def out_copy(j, hf):
        return pltpu.make_async_copy(o_s.at[j, pl.ds(hf * mh, mh)],
                                     o_hbm.at[pl.ds(hf * mh, mh), pl.ds(j * RC, RC)], sem.at[S_OUT + 2 * j + hf])

    def head_program(order, h, hn, never, x7_s=None, tri=None, wo_ops=None, tune=None, hooks=None):
        prods, held, waiting = {}, {}, []

        def spots(v, cols, rows=(0, 64, 128, 192)):
            return [v[r:r + 8, n * L:(n + 1) * L] for n in cols for r in rows]

        def tie(lhs, links, every):
            rows = []
            for rg in range(lhs.shape[0] // 8):
                blk = lhs[rg * 8:(rg + 1) * 8]
                if links and rg % every == 0:
                    blk = jnp.concatenate([jnp.where(never, links.pop(0), blk[:, :L]), blk[:, L:]], axis=1)
                rows.append(blk)
            return jnp.concatenate(rows, axis=0)

        combos = [("k", 0, _c11, (0, 3, 4, 6)), ("k", 1, _c21, (1, 3)),
                  ("v", 0, _c12, (2, 4)), ("v", 1, _c22, (0, 1, 2, 5))]

        def combine(pieces):
            ready = [c for c in combos if all(x in prods for x in c[3])]
            for e, (key, odd, comb, needs) in enumerate(ready):
                combos.remove((key, odd, comb, needs))
                for k in range(nq // 2):
                    m = {x: prods[x][k * TQ:(k + 1) * TQ] for x in needs}
                    if pieces:
                        rows = []
                        for g in range(8):
                            at = ((e * (nq // 2) + k) * 8 + g) / (len(ready) * (nq // 2) * 8)
                            rows.append(jnp.tile(pieces[int(0.95 * at * len(pieces))], (2, 2)))
                        m[needs[0]] = jnp.where(jnp.tile(never, (32, 2)), jnp.concatenate(rows + rows, axis=0),
                                                m[needs[0]])
                    c = comb(m)
                    held[2 * k + odd, key] = _to_u32(c)
                    if 2 * k + odd < nq - 1:
                        off = (c[:L, L:], c[L:, :L]) if key == "v" else (c[L:, :L], c[:L, L:])
                        ops = _right(c[:L, :L], *off, c[L:, L:])
                        held[2 * k + odd, key + "5"] = [_to_u32(ops[x]) for x in SUMS]

        def proj(n, lazy):
            w = _right_one(n, [lambda e=e: _head_weight(b_s.at[e], hn, DC // 4, pb) for e in range(4)])
            links = list(waiting)
            del waiting[:]
            if n in DEEP:
                kh = DC // 4
                right = [o.astype(BF16) for o in _right(w[:kh, :L], w[:kh, L:], w[kh:, :L], w[kh:, L:])]
                m, pieces = {}, []

                def sub(x, after):
                    lhs = a2_s[DEEP.index(n), x]
                    if after:
                        t = after[0]
                        for v in after[1:]:
                            t = jnp.maximum(t, v)
                        lhs = tie(lhs, [pltpu.bitcast(jnp.maximum(t[g * 16:g * 16 + 8], t[g * 16 + 8:g * 16 + 16]), U32)
                                        for g in range(S // 64)], 1)
                    elif links:
                        lhs = tie(lhs, links, lhs.shape[0] // 8 // len(links))
                    m[x] = jnp.dot(_as_bf16(lhs), right[x], preferred_element_type=F32)
                    pieces.extend(spots(m[x], (0,), range(0, S // 4, 64)))
                sub(1, ()), sub(3, ())
                c21 = m[1] + m[3]
                sub(2, ()), sub(4, (c21,))
                c12, c11, c22 = m[2] + m[4], m[3] - m[4], m[2] - m[1]
                sub(0, ()), sub(5, (c12, c11, c22))
                c11, c22 = c11 + m[0], c22 + (m[0] + m[5])
                sub(6, (c11, c22))
                top = jnp.concatenate([c11 + m[6], c12], axis=1)
                bot = jnp.concatenate([c21, c22], axis=1)
                prods[n] = jnp.concatenate([v[k * L:(k + 1) * L] for k in range(nq // 2) for v in (top, bot)],
                                           axis=0)
            else:
                lhs = a_s[FLAT.index(n)]
                if links:
                    lhs = tie(lhs, links, max(1, lhs.shape[0] // 8 // len(links)))
                prods[n] = jnp.dot(_as_bf16(lhs), w.astype(BF16), preferred_element_type=F32)
                pieces = spots(prods[n], (0, 1), range(0, S // 2, 32))
            if not lazy:
                combine(None)
            return pieces

        def write_kv():
            for ch in reversed(range(nq)):
                k_s[ch * HQ:(ch + 1) * HQ, :] = held[ch, "k"]
                v_s[ch * HQ:(ch + 1) * HQ, :] = held[ch, "v"]
                for key, ref in (("k5", k5_s), ("v5", v5_s)):
                    for n, o in enumerate(held.get((ch, key), ())):
                        ref[n, ch * 64:(ch + 1) * 64, :] = o

        def right_operand(n, plain, sums, c0, c1):
            if n == 1:
                return jnp.concatenate([_as_bf16(plain[c * HQ:c * HQ + 64, :L]) for c in range(c0, c1)], axis=0)
            if n == 4:
                return jnp.concatenate([_as_bf16(plain[c * HQ + 64:(c + 1) * HQ, L:]) for c in range(c0, c1)], axis=0)
            return _as_bf16(sums[SUMS.index(n), c0 * 64:c1 * 64, :])

        def qk(i, tied):
            q = qd = q_s[h, i * HQ:(i + 1) * HQ, :]
            n = len(waiting) - 8 if tied else 0
            if n > 0:
                qd = tie(q, waiting[:n], 16 // n)
                del waiting[:n]
            q, qd = _as_bf16(q), _as_bf16(qd)
            tops, bots, pieces = [], [], []
            if i:
                qf = q.astype(F32)
                left = [o.astype(BF16) for o in _left(qf[:L, :L], qf[:L, L:], qf[L:, :L], qf[L:, L:])]
                left[2], left[3] = q[:L, :L], q[L:, L:]
            done = []
            for c in range(i):
                lhs = dict(enumerate(left))
                if c >= 2:
                    u = pltpu.bitcast(left[0], U32)
                    lhs[0] = _as_bf16(jnp.concatenate(
                        [jnp.where(never, done[c - 2][g], u[g * 8:(g + 1) * 8]) for g in range(8)], axis=0))
                m = {n: jax.lax.dot_general(lhs[n], right_operand(n, k_s, k5_s, c, c + 1), NT,
                                            preferred_element_type=F32) for n in tune[1]}
                c11, c12, c21, c22 = _c11(m), _c12(m), _c21(m), _c22(m)
                tops += [c11, c12]
                bots += [c21, c22]
                t = jnp.maximum(jnp.maximum(c11, c12), jnp.maximum(c21, c22))
                done.append([pltpu.bitcast(jnp.maximum(t[g * 16:g * 16 + 8], t[g * 16 + 8:(g + 1) * 16]), U32)
                             for g in range(8)])
                for n in (0, 5):
                    pieces += spots(m[n], (0,), (0, 32, 64, 96))
            r0 = i * HQ
            s1 = jax.lax.dot_general(qd, _as_bf16(k_s[r0:r0 + 64, :]), NT, preferred_element_type=F32)
            s2 = jax.lax.dot_general(q[L:], _as_bf16(k_s[r0 + 64:r0 + HQ, :]), NT, preferred_element_type=F32)
            top = jnp.concatenate(tops + [jnp.where(tri, s1[:L], neg)], axis=1)
            bot = jnp.concatenate(bots + [s1[L:], jnp.where(tri, s2, neg)], axis=1)
            return (top, bot), pieces + spots(s1, (0,))

        def softmax(i, top, bot, pieces, again=False):
            p, sums, prev = ([], []), ([], []), None
            for k in range(TQ // 8):
                half = k % 2
                s = (top, bot)[half][(k // 2) * 8:(k // 2 + 1) * 8]
                link = pieces[int(tune[0][i] * k * 8 / TQ * len(pieces))]
                if prev is not None:
                    link = jnp.where(never, link, prev)
                m = jnp.broadcast_to(jnp.max(s, axis=1, keepdims=True), (8, L))
                m = jnp.where(never, link, m)
                e = [jnp.exp2(s[:, t:t + L] - m) for t in range(0, s.shape[1], L)]
                prev = e[0]
                for x in e[1:]:
                    prev = prev + x
                if again:
                    m = m + jnp.log2(jnp.sum(prev, axis=1, keepdims=True))
                    e = [jnp.exp2(s[:, t:t + L] - m) for t in range(0, s.shape[1], L)]
                sums[half].append(prev)
                p[half].append(jnp.concatenate(e, axis=1))
            pt, pb_ = jnp.concatenate(p[0], axis=0), jnp.concatenate(p[1], axis=0)

            def tile(x, t):
                return x[:, t * L:(t + 1) * L]
            ops = [_left(tile(pt, 2 * c), tile(pt, 2 * c + 1), tile(pb_, 2 * c), tile(pb_, 2 * c + 1))
                   for c in range(i)]
            left = [jnp.concatenate([o[n] for o in ops], axis=1).astype(BF16) for n in range(7)] if i else None
            inv = []
            for x in () if again else sums:
                l = jnp.sum(jnp.concatenate(x, axis=0), axis=1, keepdims=True)
                r = pl.reciprocal(l, approx=True)
                inv.append(r * (2.0 - l * r))
            return (left, jnp.concatenate([tile(pt, 2 * i), tile(pb_, 2 * i)], axis=0).astype(BF16),
                    tile(pb_, 2 * i + 1).astype(BF16), inv)

        def pv(i, left, p1, p2, inv):
            r0 = i * HQ
            m, pieces = {}, []
            for n in tune[2] if i else ():
                m[n] = jnp.dot(left[n], right_operand(n, v_s, v5_s, 0, i), preferred_element_type=F32)
                pieces += spots(m[n], (0,), (0, 32, 64, 96))
            c1 = jnp.dot(p1, _as_bf16(v_s[r0:r0 + 64, :]), preferred_element_type=F32)
            c2 = jnp.dot(p2, _as_bf16(v_s[r0 + 64:r0 + HQ, :]), preferred_element_type=F32)
            top, bot = c1[:L], c1[L:] + c2
            if i:
                top = top + jnp.concatenate([_c11(m), _c12(m)], axis=1)
                bot = bot + jnp.concatenate([_c21(m), _c22(m)], axis=1)
            else:
                pieces = spots(c1, (0, 1))
            if inv:
                top, bot = top * inv[0], bot * inv[1]
            us = [_to_u32(o) for o in _right(top[:, :L], bot[:, :L], top[:, L:], bot[:, L:])]
            for n in range(7):
                x7_s[n, h, i * 64:(i + 1) * 64, :] = us[n]
            waiting.extend(_or_all([us[n][g * 8:(g + 1) * 8] for n in SUMS]) for g in range(8))
            return pieces

        def wo_operands(pieces):
            groups = M // 64
            never2 = jnp.concatenate([never, never], axis=0)
            share = -(-(H // 2) * groups // (H - 1))
            for k in range(share):
                u = jnp.minimum(h * share + k, (H // 2) * groups - 1)
                pair = jax.lax.div(u, groups)
                rg = u - pair * groups
                ops = [_left(*[wo_s[2 * pair + par, pl.ds(pl.multiple_of(hf * mh + sub * (mh // 2) + rg * 16, 16), 16),
                                    ch * L:(ch + 1) * L].astype(F32) for hf in range(2) for ch in range(2)])
                       for sub in range(2) for par in range(2)]
                for n in range(7):
                    link = pieces[int(0.96 * (k * 7 + n) / (share * 7) * len(pieces))]
                    gate = jnp.concatenate([link, link], axis=0)
                    us = [_to_u32(o) for o in _left(*[jnp.where(never2, gate, o[n]) for o in ops])]
                    for x in range(7):
                        wo_ops[n, x, pair, pl.ds(pl.multiple_of(rg * 8, 8), 8), :] = us[x]
                    waiting.append(_or_all(us))

        scores, probs, pieces = {}, {}, []
        for op in order.split():
            i = int(op[1:])
            if op[0] in "Gg":
                pieces.append(proj(i, op[0] == "g"))
            elif op[0] == "c":
                combine(sum(pieces[-i:], []))
            elif op[0] == "w":
                write_kv()
            elif op[0] == "o":
                wo_operands(pieces[-1])
            elif op[0] in "Qr":
                scores[i], new = qk(i, op[0] == "r")
                pieces.append(new)
            elif op[0] == "S":
                probs[i] = softmax(i, *scores.pop(i), pieces[-1])
            elif op[0] == "t":
                probs[i] = softmax(i, *scores.pop(i), pieces[-2] + pieces[-1], again=True)
            elif op[0] == "V":
                pieces.append(pv(i, *probs.pop(i)))
            else:
                hooks[i](pieces)

    def phase1(c_s, wq_r, wk_r, wv_r, wg_s, wu_s, wd_s, xa_s, wq0_s, wq1_s, wr_s, gw_s):
        def x_copy(j):
            return pltpu.make_async_copy(xT_hbm.at[:, pl.ds(j * RC, RC)], xT_s.at[j], sem.at[S_X + j])

        def wq0_copy(kh, j):
            return pltpu.make_async_copy(wq_hbm.at[kh, pl.ds(j * mq, mq), 0], wq_r.at[kh, pl.ds(j * mq, mq), 0],
                                         sem.at[S_Q0 + kh * NCH + j])

        def wq1_copy(j):
            return pltpu.make_async_copy(wq_hbm.at[:, pl.ds(j * mq, mq), 1], wq_r.at[:, pl.ds(j * mq, mq), 1],
                                         sem.at[S_Q1 + j])

        def kv_copies(j):
            return [pltpu.make_async_copy(src.at[pl.ds(j * n, n)], dst.at[pl.ds(j * n, n)], sem.at[s0 + j])
                    for src, dst, s0, n in ((c_hbm, c_s, S_C, RC), (wk_hbm, wk_r, S_K, mk), (wv_hbm, wv_r, S_V, mk))]

        misc = [pltpu.make_async_copy(a, b, sem.at[S_MISC + i]) for i, (a, b) in enumerate(
            [(wr_hbm, wr_s), (gw_hbm, gw_s), (wg_hbm, wg_s), (wu_hbm, wu_s), (wd_hbm, wd_s)])]

        x_copy(0).start()
        for kh in range(2):
            for j in range(NCH):
                wq0_copy(kh, j).start()
        for j in range(NCH):
            if j + 1 < NCH:
                x_copy(j + 1).start()
            wq1_copy(j).start()
        misc[0].start()
        misc[1].start()
        for j in range(NCH):
            for cp in kv_copies(j):
                cp.start()
        for cp in misc[2:]:
            cp.start()
        wo_copy.start()

        def x_operands(j):
            r0 = j * HQ if isinstance(j, int) else pl.multiple_of(j * HQ, HQ)
            a = [xT_s[j, kh * mh:(kh + 1) * mh, rb * TQ:(rb + 1) * TQ].astype(F32)
                 for rb in range(2) for kh in range(2)]
            for n, o in enumerate(_left(*a)):
                xa_s[n, pl.ds(r0, HQ), :] = pltpu.bitcast(o.astype(BF16).T, U32)

        def wq_blocks(g, p, never=None, link=None, halves=(0, 1), src=None):
            for kh in halves:
                w = pltpu.bitcast(wq_r[kh, pl.ds(2 * p, 2), g if src is None else src], U32)
                w = [w[e] if link is None else jnp.where(never, link, w[e]) for e in range(2)]
                for par, u in enumerate(_split_heads(*w)):
                    (wq0_s, wq1_s)[g][2 * kh + par, pl.ds(p, 8, stride=pq), :] = u

        x_copy(0).wait()
        x_operands(0)

        def first_heads(kh):
            def chunk(j, _):
                wq0_copy(kh, j).wait()
                for k in range(mq // 2):
                    wq_blocks(0, j * (mq // 2) + k, halves=(kh,))
                return 0
            jax.lax.fori_loop(0, NCH, chunk, 0)
        first_heads(0)

        def q_step(g, j, side, early=()):
            m, count = [{} for _ in range(4)], [0]

            def product(r, n):
                w = _right_one(n, [lambda e=e: jnp.concatenate(
                    [_as_bf16((wq0_s, wq1_s)[g][e, pl.ds((dt * 4 + r) * pq, mh // 2), :]) for dt in range(2)],
                    axis=1) for e in range(4)])
                m[r][n] = jnp.dot(_as_bf16(xa_s[n, pl.ds(pl.multiple_of(j * HQ, HQ), HQ), :]), w.astype(BF16),
                                  preferred_element_type=F32)
                for k in range(5):
                    side(count[0], m[r][n][k * 48:k * 48 + 8, (k % 2) * L:(k % 2 + 1) * L])
                    count[0] += 1
            for r in range(4):
                for n in early:
                    product(r, n)
            for r in range(4):
                for n in (4, 0, 3, 6, 1, 2, 5):
                    if n not in early:
                        product(r, n)
                for par, rb, comb in ((0, 0, _c11), (0, 1, _c21), (1, 0, _c12), (1, 1, _c22)):
                    r0 = pl.multiple_of(j * TQ + rb * HQ, HQ)
                    q_s[8 * g + 2 * r + par, pl.ds(r0, HQ), :] = _to_u32(comb(m[r]) * qscale)

        def q_lo(j, _):
            never = _never(j)

            prev = jnp.maximum(j - 1, 0)

            def side(k, piece):
                if k == 39:
                    pl.when(j == 0)(lambda: first_heads(1))
                    pl.when(j + 1 < NCH)(lambda: x_copy(j + 1).wait())
                    pl.when(j > 0)(lambda: wq1_copy(prev).wait())
                if k >= 45 and k % 3 == 0 and (k - 45) // 3 < mq // 2:
                    wq_blocks(1, prev * (mq // 2) + (k - 45) // 3, never, pltpu.bitcast(piece, U32),
                              src=jnp.minimum(j, 1))
            q_step(0, j, side, early=(1, 5))
            x_operands((j + 1) & (NCH - 1))
            return 0
        jax.lax.fori_loop(0, NCH, q_lo, 0)
        wq1_copy(NCH - 1).wait()
        for k in range(mq // 2):
            wq_blocks(1, (NCH - 1) * (mq // 2) + k)

        def q_hi(j, _):
            for cp in kv_copies(j):
                cp.wait()
            never = _never(j)
            quad = []

            def side(kk, piece):
                if kk >= 128:
                    return
                k, g = kk // 2, kk % 2
                link = pltpu.bitcast(piece, U32)
                if g == 0:
                    rg, t = k // 8 + 8 * (k % 4 // 2), k // 4 % 2 + 2 * (k % 2)
                    a = []
                    for rb in range(2):
                        r0 = pl.multiple_of(j * RC + rb * TQ + rg * 16, 16)
                        for ch in range(2):
                            a.append(c_s[pl.ds(r0, 16), (2 * t + ch) * L:(2 * t + ch + 1) * L].astype(F32))
                    a[0] = jnp.where(jnp.concatenate([never, never], axis=0),
                                     jnp.concatenate([piece, piece], axis=0), a[0])
                    ops = _left(*a)
                    us = [_to_u32(ops[n]) for n in FLAT]
                    d0 = pl.multiple_of(j * HQ + rg * 8, 8)
                    for n, u in enumerate(us):
                        a_s[n, pl.ds(d0, 8), t * L:(t + 1) * L] = u
                    quad.append(ops)
                    if len(quad) == 4:
                        d0 = pl.multiple_of(j * (HQ // 2) + (rg - 8) * 8, 8)
                        for e, n in enumerate(DEEP):
                            deep = [_to_u32(o) for o in _left(*[q[n] for q in quad])]
                            for x, u in enumerate(deep):
                                a2_s[e, x, pl.ds(d0, 8), (t - 2) * L:(t - 1) * L] = u
                            us += deep
                        del quad[:]
                    link = _or_all(us)
                c0 = j * mk + 2 * k
                for e, (o, r) in enumerate((o, r) for o in (0, L) for r in (wk_r, wv_r)):
                    w = pltpu.bitcast(r[pl.ds(c0 + o, 2), g], U32)
                    for par, u in enumerate(_split_heads(jnp.where(never, link, w[0]), jnp.where(never, link, w[1]))):
                        b_s[e, 2 * g + par, pl.ds(j * (mk // 4) + k, 8, stride=pb), :] = u
            q_step(1, j, side)
            return j
        never = _never(jax.lax.fori_loop(0, NCH, q_hi, 0))

        for cp in misc:
            cp.wait()
        st = {}
        F = wg_s.shape[1]

        def route(pieces):
            pieces = pieces[-2] + pieces[-1]
            mp = -(-M // L) * L
            cols = []
            for w_s in (wr_s, gw_s):
                w = jnp.concatenate([w_s[...].reshape(1, M).astype(F32), jnp.zeros((1, mp - M), F32)], axis=1)
                cols.append(jnp.broadcast_to(w, (L, mp)).T)
            nr, rows = 4, M // 4
            out, k, prev = ([], []), 0, None
            for ct in range(S // L):
                acc = [None, None]
                for q in range(nr):
                    link = pieces[int((FFN_TUNE[0] + FFN_TUNE[1] * k / (nr * S // L)) * len(pieces))]
                    if prev is not None:
                        link = jnp.where(never, link, prev)
                    k += 1
                    x = linked(xT_s[ct * L // RC, q * rows:(q + 1) * rows, pl.ds(ct * L % RC, L)], link)
                    for t in range(2):
                        part = fold(x * cols[t][q * rows:(q + 1) * rows], 0)
                        acc[t] = part if acc[t] is None else acc[t] + part
                    prev = acc[0] + acc[1]
                for t in range(2):
                    out[t].append(jnp.sum(acc[t], axis=0, keepdims=True))
            gate = jax.nn.sigmoid(jnp.concatenate(out[1], axis=1))
            for j in range(S // RC):
                g_s[j, 0:1, :] = gate[:, j * RC:(j + 1) * RC]
            r = jnp.concatenate(out[0], axis=1).astype(BF16).astype(F32)
            lane = jax.lax.broadcasted_iota(jnp.int32, (1, S), 1)
            m1 = jnp.max(r, axis=1, keepdims=True)
            i1 = jnp.min(jnp.where(r == m1, lane, S - 1), axis=1, keepdims=True)
            r2 = jnp.where(lane == i1, -jnp.inf, r)
            m2 = jnp.max(r2, axis=1, keepdims=True)
            i2 = jnp.min(jnp.where(jnp.logical_and(r2 == m2, lane != i1), lane, S - 1), axis=1, keepdims=True)
            ln = jax.lax.broadcasted_iota(jnp.int32, (M, L), 1)
            st["at"] = [(i[0, 0] >> 9, slice(None), pl.ds(pl.multiple_of(i[0, 0] & (RC - L), L), L))
                        for i in (i1, i2)]
            st["hit"] = [ln == (i & (L - 1)) for i in (i1, i2)]
            st["r"] = [jax.nn.sigmoid(m1), jax.nn.sigmoid(m2)]
            st["x"] = [jnp.broadcast_to(jnp.sum(jnp.where(hit, xT_s[at].astype(F32), 0.0),
                                                axis=1, keepdims=True), (M, L))
                       for at, hit in zip(st["at"], st["hit"])]

        def fold(v, axis):
            parts = [v[k * 8:(k + 1) * 8] if axis == 0 else v[:, k * L:(k + 1) * L]
                     for k in range(v.shape[axis] // (8, L)[axis])]
            while len(parts) > 1:
                parts = [parts[k] + parts[k + 1] if k + 1 < len(parts) else parts[k]
                         for k in range(0, len(parts), 2)]
            return parts[0]

        def linked(w, link):
            w = pltpu.bitcast(w, U32)
            reps = (w.shape[0] // 8, w.shape[1] // L)
            w = jnp.where(jnp.tile(never, reps), jnp.tile(pltpu.bitcast(link, U32), reps), w)
            return _as_bf16(w).astype(F32)

        def hidden(pieces):
            pieces = pieces[-3] + pieces[-2] + pieces[-1]
            nr, rows = 4, M // 4
            total = 2 * (F // L) * nr
            out, k, prev = [], 0, None
            for w_s in (wg_s, wu_s):
                cols = ([], [])
                for ct in range(F // L):
                    acc = [None, None]
                    for q in range(nr):
                        link = pieces[int((FFN_TUNE[2] + FFN_TUNE[3] * k / total) * len(pieces))]
                        if prev is not None:
                            link = jnp.where(never, link, prev)
                        k += 1
                        w = linked(w_s[q * rows:(q + 1) * rows, ct * L:(ct + 1) * L], link)
                        for t in range(2):
                            part = fold(w * st["x"][t][q * rows:(q + 1) * rows], 0)
                            acc[t] = part if acc[t] is None else acc[t] + part
                        prev = acc[0] + acc[1]
                    for t in range(2):
                        cols[t].append(jnp.sum(acc[t], axis=0, keepdims=True))
                out.append([jnp.concatenate(c, axis=1) for c in cols])
            st["h"] = [(jax.nn.silu(out[0][t]) * out[1][t]).astype(BF16).astype(F32) for t in range(2)]

        def patch(pieces):
            pieces = pieces[-2] + pieces[-1]
            half = F // 2
            ys, k, prev = ([], []), 0, None
            for rg in range(M // 16):
                acc = [None, None]
                for hf in range(2):
                    link = pieces[int((FFN_TUNE[4] + FFN_TUNE[5] * k / (M // 8)) * len(pieces))]
                    if prev is not None:
                        link = jnp.where(never, link, prev)
                    k += 1
                    w = linked(wd_s[rg * 16:(rg + 1) * 16, hf * half:(hf + 1) * half], link)
                    for t in range(2):
                        part = fold(w * st["h"][t][:, hf * half:(hf + 1) * half], 1)
                        acc[t] = part if acc[t] is None else acc[t] + part
                    prev = fold(acc[0] + acc[1], 0)
                for t in range(2):
                    ys[t].append(jnp.sum(acc[t], axis=1, keepdims=True))
            for t in range(2):
                y = jnp.concatenate(ys[t], axis=0) * st["r"][t]
                blk = xT_s[st["at"][t]].astype(F32)
                xT_s[st["at"][t]] = (blk + jnp.where(st["hit"][t], y, 0.0)).astype(BF16)

        head_program(FIRST_ORDER, None, 0, never, hooks=(route, hidden, patch))

    def phase2(x7_s, wo_ops):
        wo_copy.wait()
        tri = jax.lax.broadcasted_iota(jnp.int32, (L, L), 1) <= jax.lax.broadcasted_iota(jnp.int32, (L, L), 0)

        def head(h, _):
            head_program(LOOP_ORDER, h, h + 1, _never(h), x7_s, tri, wo_ops, LOOP_TUNE)
            return h
        last = jax.lax.fori_loop(0, H - 1, head, 0)
        head_program(LAST_ORDER, H - 1, None, _never(last), x7_s, tri, tune=LAST_TUNE)

        def out_step(j):
            m = ({}, {})
            for n in range(7):
                right = [[] for _ in range(7)]
                for pair in range(H // 2):
                    blk = [_as_bf16(x7_s[n, 2 * pair + par, pl.ds(pl.multiple_of(j * L + t * 64, 64), 64), :])
                           for par in range(2) for t in range(2)]
                    ops = list(_right(*[v.astype(F32) for v in blk]))
                    ops[1], ops[4] = blk[0], blk[3]
                    for x in range(7):
                        right[x].append(ops[x])
                mm = {x: jax.lax.dot_general(
                    jnp.concatenate([_as_bf16(wo_ops[n, x, pair, :M // 8]) for pair in range(H // 2)], axis=1),
                    jnp.concatenate(right[x], axis=1).astype(BF16), NT, preferred_element_type=F32)
                    for x in (4, 2, 1, 5, 0, 3, 6)}
                m[0][n] = jnp.concatenate([((mm[0] + mm[3]) - mm[4]) + mm[6], _c21(mm)], axis=0)
                m[1][n] = jnp.concatenate([_c12(mm), _c22(mm)], axis=0)
            gate = g_s[j, 0:1, :]
            for hf in (1, 0):
                rest = (1.0 - gate) * xT_s[j, hf * mh:(hf + 1) * mh, :].astype(F32)
                cols = []
                for t in range(RC // TQ):
                    gl, gr = gate[:, t * TQ:t * TQ + L], gate[:, t * TQ + L:(t + 1) * TQ]
                    rl, rr = rest[:, t * TQ:t * TQ + L], rest[:, t * TQ + L:(t + 1) * TQ]
                    if hf:
                        cols += [gl * _c21(m[t]) + rl, gr * _c22(m[t]) + rr]
                    else:
                        cols += [(gl * ((m[t][0] + m[t][3]) - m[t][4]) + rl) + gl * m[t][6], gr * _c12(m[t]) + rr]
                o_s[j, hf * mh:(hf + 1) * mh, :] = jnp.concatenate(cols, axis=1).astype(BF16)
                out_copy(j, hf).start()

        def out_steps(i, _):
            for k in range(O_UNROLL):
                out_step(i * O_UNROLL + k)
            return 0
        jax.lax.fori_loop(0, S // RC // O_UNROLL, out_steps, 0)
        for j in range(S // RC):
            for hf in range(2):
                out_copy(j, hf).wait()

    pl.run_scoped(
        phase1,
        *[pltpu.VMEM(r.shape, r.dtype) for r in (c_hbm, wq_hbm, wk_hbm, wv_hbm, wg_hbm, wu_hbm, wd_hbm)],
        pltpu.VMEM((7, S // 4, mh), U32),
        pltpu.VMEM((4, -(-pq // 4) * 32, L), U32),
        pltpu.VMEM((4, -(-pq // 4) * 32, L), U32),
        pltpu.VMEM((M,), BF16),
        pltpu.VMEM((M,), BF16))
    pl.run_scoped(phase2, pltpu.VMEM((7, H, S // 4, L), U32), pltpu.VMEM((7, 7, H // 2, 64, L), U32))


def _tile_view(w):
    c, h, d = w.shape
    w = w.reshape(c, h // 8, 8, d // L, L).transpose(0, 1, 3, 2, 4)
    return w.reshape(c, h // 8, 8 * (d // L), L)


@jax.jit
def pallas_gated_mix__compressed_kv_cla__moe_arch_mod__prompt_kernel(
    A_x: jax.Array,
    A_c_kv: jax.Array,
    A_w_q: jax.Array,
    A_w_uk: jax.Array,
    A_w_uv: jax.Array,
    A_w_o: jax.Array,
    B_x: jax.Array,
    B_w_r: jax.Array,
    B_w_gate: jax.Array,
    B_w_up: jax.Array,
    B_w_down: jax.Array,
    gate_w: jax.Array,
):
    _, S, M = A_x.shape
    DC = A_c_kv.shape[2]
    H, D = A_w_q.shape[1], A_w_q.shape[2]
    args = (jnp.transpose(A_x[0]), A_c_kv[0], _tile_view(A_w_q).reshape(2, M // 2, 2, 16, L),
            _tile_view(A_w_uk), _tile_view(A_w_uv),
            jnp.transpose(A_w_o, (0, 2, 1)), B_w_r, gate_w, B_w_gate, B_w_up, jnp.transpose(B_w_down))

    def kern(*refs):
        _kernel(*refs, S=S, M=M, DC=DC, H=H, D=D)

    hbm = pl.BlockSpec(memory_space=pl.ANY)
    oT = pl.pallas_call(
        kern,
        out_shape=jax.ShapeDtypeStruct((M, S), A_x.dtype),
        in_specs=[hbm] * len(args),
        out_specs=hbm,
        scratch_shapes=[
            pltpu.VMEM((S // RC, 8, RC), F32),
            pltpu.VMEM((S // RC, M, RC), BF16),
            pltpu.VMEM((H, M, D), BF16),
            pltpu.VMEM((5, S // 4, DC // 2), U32),
            pltpu.VMEM((2, 7, S // 8, DC // 4), U32),
            pltpu.VMEM((4, 4, 8 * (DC // 4 + 4), L), U32),
            pltpu.VMEM((H, S // 2, D), U32),
            pltpu.VMEM((S // 2, D), U32),
            pltpu.VMEM((S // 2, D), U32),
            pltpu.VMEM((5, S // 4, L), U32),
            pltpu.VMEM((S // RC, M, RC), BF16),
            pltpu.VMEM((5, S // 4 + PAD_V, L), U32),
            pltpu.SemaphoreType.DMA((N_SEM,)),
        ],
        compiler_params=pltpu.CompilerParams(vmem_limit_bytes=124 * 1024 * 1024, disable_bounds_checks=True,
                                             disable_semaphore_checks=True),
    )(*args)
    return jnp.transpose(oT)[None]
```

```python
import math

import jax
import jax.numpy as jnp
import jax.experimental.pallas as pl
import jax.experimental.pallas.tpu as pltpu

F32 = jnp.float32
BF16 = jnp.bfloat16
U32 = jnp.uint32
NT = (((1,), (1,)), ((), ()))

L = 128
TQ = 256
HQ = TQ // 2
RC = 512
NCH = 4

PAD_V = 16

O_UNROLL = 2

S_X, S_Q0, S_Q1, S_K, S_V, S_C, S_MISC, S_OUT = 0, 4, 12, 16, 20, 24, 28, 34
N_SEM = 42

LOOP_ORDER = ("Q0 Q7 S0 G0 S7 V0 V7 o0 Q6 G3 S6 V6 Q5 G4 S5 V5 Q4 G5 S4 V4 Q3 G6 S3 V3 Q2 g2 S2 V2 "
              "Q1 c2 G1 S1 V1 w0")
LOOP_TUNE = ((0.854, 0.969, 0.851, 0.941, 0.801, 0.94, 0.979, 0.948), (2, 4, 1, 3, 0, 6, 5), (2, 3, 4, 0, 1, 5, 6))
LAST_TUNE = ((0.8, 0.9, 0.66, 0.99, 0.9, 0.68, 0.93, 0.83), (0, 3, 4, 6, 1, 2, 5), (2, 3, 0, 4, 1, 6, 5))
FFN_TUNE = (0.03, 0.65, 0.0, 0.9, 0.1, 0.8)
FIRST_ORDER = "G0 G2 h0 G3 G4 G6 h1 G5 G1 h2 w0"
LAST_ORDER = "Q7 Q6 Q5 t7 V7 S6 Q4 V6 S5 r3 V5 S4 r2 V4 S3 r1 V3 t2 r0 V2 t1 t0 V1 V0"


def _to_u32(x_f32):
    return pltpu.bitcast(x_f32.astype(BF16), U32)


def _as_bf16(x_u32):
    return pltpu.bitcast(x_u32, BF16)


def _left(a11, a12, a21, a22):
    return (a11 + a22, a21 + a22, a11, a22, a11 + a12, a21 - a11, a12 - a22)


def _right(b11, b12, b21, b22):
    return (b11 + b22, b11, b12 - b22, b21 - b11, b22, b11 + b12, b21 + b22)


FLAT, DEEP = (0, 1, 3, 4, 6), (2, 5)
SUMS = (0, 2, 3, 5, 6)


def _c11(m):
    return (m[0] + m[3]) + (m[6] - m[4])


def _c12(m):
    return m[2] + m[4]


def _c21(m):
    return m[1] + m[3]


def _c22(m):
    return (m[0] - m[1]) + (m[2] + m[5])


def _never(i):
    return jax.lax.broadcasted_iota(jnp.int32, (8, L), 0) < (i >> 10)


def _or_all(xs):
    out = xs[0]
    for x in xs[1:]:
        out = out | x
    return out


def _split_heads(even, odd):
    return ((even & jnp.uint32(0xFFFF)) | (odd << 16), (even >> 16) | (odd & jnp.uint32(0xFFFF0000)))


def _right_one(n, blocks):
    x, y, sign = ((0, 3, 1), (0, None, 0), (1, 3, -1), (2, 0, -1), (3, None, 0), (0, 1, 1), (2, 3, 1))[n]
    if y is None:
        return blocks[x]()
    x, y = blocks[x]().astype(F32), blocks[y]().astype(F32)
    return x + y if sign > 0 else x - y


def _head_weight(ref, h, nrows, pitch):
    sel = ((h >> 3) << 1) + (h & 1)
    r = (h >> 1) & 3
    return jnp.concatenate(
        [_as_bf16(ref[sel, pl.ds((dt * 4 + r) * pitch, nrows), :]) for dt in range(2)], axis=1)


def _kernel(xT_hbm, c_hbm, wq_hbm, wk_hbm, wv_hbm, wo_hbm, wr_hbm, gw_hbm, wg_hbm, wu_hbm, wd_hbm,
            o_hbm,
            g_s, xT_s, wo_s, a_s, a2_s, b_s, q_s, k_s, v_s, k5_s, o_s, v5_s, sem, *, S, M, DC, H, D):
    nq = S // TQ
    mh = M // 2
    pq = mh // 2 + 1
    pb = DC // 4 + 1
    mq = mh // NCH
    mk = DC // NCH
    qscale = (D ** -0.5) * math.log2(math.e)
    neg = -1e9 * math.log2(math.e)
    wo_copy = pltpu.make_async_copy(wo_hbm, wo_s, sem.at[S_MISC + 5])

    def out_copy(j, hf):
        return pltpu.make_async_copy(o_s.at[j, pl.ds(hf * mh, mh)],
                                     o_hbm.at[pl.ds(hf * mh, mh), pl.ds(j * RC, RC)], sem.at[S_OUT + 2 * j + hf])

    def head_program(order, h, hn, never, x7_s=None, tri=None, wo_ops=None, tune=None, hooks=None):
        prods, held, waiting = {}, {}, []

        def spots(v, cols, rows=(0, 64, 128, 192)):
            return [v[r:r + 8, n * L:(n + 1) * L] for n in cols for r in rows]

        def tie(lhs, links, every):
            rows = []
            for rg in range(lhs.shape[0] // 8):
                blk = lhs[rg * 8:(rg + 1) * 8]
                if links and rg % every == 0:
                    blk = jnp.concatenate([jnp.where(never, links.pop(0), blk[:, :L]), blk[:, L:]], axis=1)
                rows.append(blk)
            return jnp.concatenate(rows, axis=0)

        combos = [("k", 0, _c11, (0, 3, 4, 6)), ("k", 1, _c21, (1, 3)),
                  ("v", 0, _c12, (2, 4)), ("v", 1, _c22, (0, 1, 2, 5))]

        def combine(pieces):
            ready = [c for c in combos if all(x in prods for x in c[3])]
            for e, (key, odd, comb, needs) in enumerate(ready):
                combos.remove((key, odd, comb, needs))
                for k in range(nq // 2):
                    m = {x: prods[x][k * TQ:(k + 1) * TQ] for x in needs}
                    if pieces:
                        rows = []
                        for g in range(8):
                            at = ((e * (nq // 2) + k) * 8 + g) / (len(ready) * (nq // 2) * 8)
                            rows.append(jnp.tile(pieces[int(0.95 * at * len(pieces))], (2, 2)))
                        m[needs[0]] = jnp.where(jnp.tile(never, (32, 2)), jnp.concatenate(rows + rows, axis=0),
                                                m[needs[0]])
                    c = comb(m)
                    held[2 * k + odd, key] = _to_u32(c)
                    if 2 * k + odd < nq - 1:
                        off = (c[:L, L:], c[L:, :L]) if key == "v" else (c[L:, :L], c[:L, L:])
                        ops = _right(c[:L, :L], *off, c[L:, L:])
                        held[2 * k + odd, key + "5"] = [_to_u32(ops[x]) for x in SUMS]

        def proj(n, lazy):
            w = _right_one(n, [lambda e=e: _head_weight(b_s.at[e], hn, DC // 4, pb) for e in range(4)])
            links = list(waiting)
            del waiting[:]
            if n in DEEP:
                kh = DC // 4
                right = [o.astype(BF16) for o in _right(w[:kh, :L], w[:kh, L:], w[kh:, :L], w[kh:, L:])]
                m, pieces = {}, []

                def sub(x, after):
                    lhs = a2_s[DEEP.index(n), x]
                    if after:
                        t = after[0]
                        for v in after[1:]:
                            t = jnp.maximum(t, v)
                        lhs = tie(lhs, [pltpu.bitcast(jnp.maximum(t[g * 16:g * 16 + 8], t[g * 16 + 8:g * 16 + 16]), U32)
                                        for g in range(S // 64)], 1)
                    elif links:
                        lhs = tie(lhs, links, lhs.shape[0] // 8 // len(links))
                    m[x] = jnp.dot(_as_bf16(lhs), right[x], preferred_element_type=F32)
                    pieces.extend(spots(m[x], (0,), range(0, S // 4, 64)))
                sub(1, ()), sub(3, ())
                c21 = m[1] + m[3]
                sub(2, ()), sub(4, (c21,))
                c12, c11, c22 = m[2] + m[4], m[3] - m[4], m[2] - m[1]
                sub(0, ()), sub(5, (c12, c11, c22))
                c11, c22 = c11 + m[0], c22 + (m[0] + m[5])
                sub(6, (c11, c22))
                top = jnp.concatenate([c11 + m[6], c12], axis=1)
                bot = jnp.concatenate([c21, c22], axis=1)
                prods[n] = jnp.concatenate([v[k * L:(k + 1) * L] for k in range(nq // 2) for v in (top, bot)],
                                           axis=0)
            else:
                lhs = a_s[FLAT.index(n)]
                if links:
                    lhs = tie(lhs, links, max(1, lhs.shape[0] // 8 // len(links)))
                prods[n] = jnp.dot(_as_bf16(lhs), w.astype(BF16), preferred_element_type=F32)
                pieces = spots(prods[n], (0, 1), range(0, S // 2, 32))
            if not lazy:
                combine(None)
            return pieces

        def write_kv():
            for ch in reversed(range(nq)):
                k_s[ch * HQ:(ch + 1) * HQ, :] = held[ch, "k"]
                v_s[ch * HQ:(ch + 1) * HQ, :] = held[ch, "v"]
                for key, ref in (("k5", k5_s), ("v5", v5_s)):
                    for n, o in enumerate(held.get((ch, key), ())):
                        ref[n, ch * 64:(ch + 1) * 64, :] = o

        def right_operand(n, plain, sums, c0, c1):
            if n == 1:
                return jnp.concatenate([_as_bf16(plain[c * HQ:c * HQ + 64, :L]) for c in range(c0, c1)], axis=0)
            if n == 4:
                return jnp.concatenate([_as_bf16(plain[c * HQ + 64:(c + 1) * HQ, L:]) for c in range(c0, c1)], axis=0)
            return _as_bf16(sums[SUMS.index(n), c0 * 64:c1 * 64, :])

        def qk(i, tied):
            q = qd = q_s[h, i * HQ:(i + 1) * HQ, :]
            n = len(waiting) - 8 if tied else 0
            if n > 0:
                qd = tie(q, waiting[:n], 16 // n)
                del waiting[:n]
            q, qd = _as_bf16(q), _as_bf16(qd)
            tops, bots, pieces = [], [], []
            if i:
                qf = q.astype(F32)
                left = [o.astype(BF16) for o in _left(qf[:L, :L], qf[:L, L:], qf[L:, :L], qf[L:, L:])]
                left[2], left[3] = q[:L, :L], q[L:, L:]
            done = []
            for c in range(i):
                lhs = dict(enumerate(left))
                if c >= 2:
                    u = pltpu.bitcast(left[0], U32)
                    lhs[0] = _as_bf16(jnp.concatenate(
                        [jnp.where(never, done[c - 2][g], u[g * 8:(g + 1) * 8]) for g in range(8)], axis=0))
                m = {n: jax.lax.dot_general(lhs[n], right_operand(n, k_s, k5_s, c, c + 1), NT,
                                            preferred_element_type=F32) for n in tune[1]}
                c11, c12, c21, c22 = _c11(m), _c12(m), _c21(m), _c22(m)
                tops += [c11, c12]
                bots += [c21, c22]
                t = jnp.maximum(jnp.maximum(c11, c12), jnp.maximum(c21, c22))
                done.append([pltpu.bitcast(jnp.maximum(t[g * 16:g * 16 + 8], t[g * 16 + 8:(g + 1) * 16]), U32)
                             for g in range(8)])
                for n in (0, 5):
                    pieces += spots(m[n], (0,), (0, 32, 64, 96))
            r0 = i * HQ
            s1 = jax.lax.dot_general(qd, _as_bf16(k_s[r0:r0 + 64, :]), NT, preferred_element_type=F32)
            s2 = jax.lax.dot_general(q[L:], _as_bf16(k_s[r0 + 64:r0 + HQ, :]), NT, preferred_element_type=F32)
            top = jnp.concatenate(tops + [jnp.where(tri, s1[:L], neg)], axis=1)
            bot = jnp.concatenate(bots + [s1[L:], jnp.where(tri, s2, neg)], axis=1)
            return (top, bot), pieces + spots(s1, (0,))

        def softmax(i, top, bot, pieces, again=False):
            p, sums, prev = ([], []), ([], []), None
            for k in range(TQ // 8):
                half = k % 2
                s = (top, bot)[half][(k // 2) * 8:(k // 2 + 1) * 8]
                link = pieces[int(tune[0][i] * k * 8 / TQ * len(pieces))]
                if prev is not None:
                    link = jnp.where(never, link, prev)
                m = jnp.broadcast_to(jnp.max(s, axis=1, keepdims=True), (8, L))
                m = jnp.where(never, link, m)
                e = [jnp.exp2(s[:, t:t + L] - m) for t in range(0, s.shape[1], L)]
                prev = e[0]
                for x in e[1:]:
                    prev = prev + x
                if again:
                    m = m + jnp.log2(jnp.sum(prev, axis=1, keepdims=True))
                    e = [jnp.exp2(s[:, t:t + L] - m) for t in range(0, s.shape[1], L)]
                sums[half].append(prev)
                p[half].append(jnp.concatenate(e, axis=1))
            pt, pb_ = jnp.concatenate(p[0], axis=0), jnp.concatenate(p[1], axis=0)

            def tile(x, t):
                return x[:, t * L:(t + 1) * L]
            ops = [_left(tile(pt, 2 * c), tile(pt, 2 * c + 1), tile(pb_, 2 * c), tile(pb_, 2 * c + 1))
                   for c in range(i)]
            left = [jnp.concatenate([o[n] for o in ops], axis=1).astype(BF16) for n in range(7)] if i else None
            inv = []
            for x in () if again else sums:
                l = jnp.sum(jnp.concatenate(x, axis=0), axis=1, keepdims=True)
                r = pl.reciprocal(l, approx=True)
                inv.append(r * (2.0 - l * r))
            return (left, jnp.concatenate([tile(pt, 2 * i), tile(pb_, 2 * i)], axis=0).astype(BF16),
                    tile(pb_, 2 * i + 1).astype(BF16), inv)

        def pv(i, left, p1, p2, inv):
            r0 = i * HQ
            m, pieces = {}, []
            for n in tune[2] if i else ():
                m[n] = jnp.dot(left[n], right_operand(n, v_s, v5_s, 0, i), preferred_element_type=F32)
                pieces += spots(m[n], (0,), (0, 32, 64, 96))
            c1 = jnp.dot(p1, _as_bf16(v_s[r0:r0 + 64, :]), preferred_element_type=F32)
            c2 = jnp.dot(p2, _as_bf16(v_s[r0 + 64:r0 + HQ, :]), preferred_element_type=F32)
            top, bot = c1[:L], c1[L:] + c2
            if i:
                top = top + jnp.concatenate([_c11(m), _c12(m)], axis=1)
                bot = bot + jnp.concatenate([_c21(m), _c22(m)], axis=1)
            else:
                pieces = spots(c1, (0, 1))
            if inv:
                top, bot = top * inv[0], bot * inv[1]
            us = [_to_u32(o) for o in _right(top[:, :L], bot[:, :L], top[:, L:], bot[:, L:])]
            for n in range(7):
                x7_s[n, h, i * 64:(i + 1) * 64, :] = us[n]
            waiting.extend(_or_all([us[n][g * 8:(g + 1) * 8] for n in SUMS]) for g in range(8))
            return pieces

        def wo_operands(pieces):
            groups = M // 64
            never2 = jnp.concatenate([never, never], axis=0)
            share = -(-(H // 2) * groups // (H - 1))
            for k in range(share):
                u = jnp.minimum(h * share + k, (H // 2) * groups - 1)
                pair = jax.lax.div(u, groups)
                rg = u - pair * groups
                ops = [_left(*[wo_s[2 * pair + par, pl.ds(pl.multiple_of(hf * mh + sub * (mh // 2) + rg * 16, 16), 16),
                                    ch * L:(ch + 1) * L].astype(F32) for hf in range(2) for ch in range(2)])
                       for sub in range(2) for par in range(2)]
                for n in range(7):
                    link = pieces[int(0.96 * (k * 7 + n) / (share * 7) * len(pieces))]
                    gate = jnp.concatenate([link, link], axis=0)
                    us = [_to_u32(o) for o in _left(*[jnp.where(never2, gate, o[n]) for o in ops])]
                    for x in range(7):
                        wo_ops[n, x, pair, pl.ds(pl.multiple_of(rg * 8, 8), 8), :] = us[x]
                    waiting.append(_or_all(us))

        scores, probs, pieces = {}, {}, []
        for op in order.split():
            i = int(op[1:])
            if op[0] in "Gg":
                pieces.append(proj(i, op[0] == "g"))
            elif op[0] == "c":
                combine(sum(pieces[-i:], []))
            elif op[0] == "w":
                write_kv()
            elif op[0] == "o":
                wo_operands(pieces[-1])
            elif op[0] in "Qr":
                scores[i], new = qk(i, op[0] == "r")
                pieces.append(new)
            elif op[0] == "S":
                probs[i] = softmax(i, *scores.pop(i), pieces[-1])
            elif op[0] == "t":
                probs[i] = softmax(i, *scores.pop(i), pieces[-2] + pieces[-1], again=True)
            elif op[0] == "V":
                pieces.append(pv(i, *probs.pop(i)))
            else:
                hooks[i](pieces)

    def phase1(c_s, wq_r, wk_r, wv_r, wg_s, wu_s, wd_s, xa_s, wq0_s, wq1_s, wr_s, gw_s):
        def x_copy(j):
            return pltpu.make_async_copy(xT_hbm.at[:, pl.ds(j * RC, RC)], xT_s.at[j], sem.at[S_X + j])

        def wq0_copy(kh, j):
            return pltpu.make_async_copy(wq_hbm.at[kh, pl.ds(j * mq, mq), 0], wq_r.at[kh, pl.ds(j * mq, mq), 0],
                                         sem.at[S_Q0 + kh * NCH + j])

        def wq1_copy(j):
            return pltpu.make_async_copy(wq_hbm.at[:, pl.ds(j * mq, mq), 1], wq_r.at[:, pl.ds(j * mq, mq), 1],
                                         sem.at[S_Q1 + j])

        def kv_copies(j):
            return [pltpu.make_async_copy(src.at[pl.ds(j * n, n)], dst.at[pl.ds(j * n, n)], sem.at[s0 + j])
                    for src, dst, s0, n in ((c_hbm, c_s, S_C, RC), (wk_hbm, wk_r, S_K, mk), (wv_hbm, wv_r, S_V, mk))]

        misc = [pltpu.make_async_copy(a, b, sem.at[S_MISC + i]) for i, (a, b) in enumerate(
            [(wr_hbm, wr_s), (gw_hbm, gw_s), (wg_hbm, wg_s), (wu_hbm, wu_s), (wd_hbm, wd_s)])]

        x_copy(0).start()
        for kh in range(2):
            for j in range(NCH):
                wq0_copy(kh, j).start()
        for j in range(NCH):
            if j + 1 < NCH:
                x_copy(j + 1).start()
            wq1_copy(j).start()
        misc[0].start()
        misc[1].start()
        for j in range(NCH):
            for cp in kv_copies(j):
                cp.start()
        for cp in misc[2:]:
            cp.start()
        wo_copy.start()

        def x_operands(j):
            r0 = j * HQ if isinstance(j, int) else pl.multiple_of(j * HQ, HQ)
            a = [xT_s[j, kh * mh:(kh + 1) * mh, rb * TQ:(rb + 1) * TQ].astype(F32)
                 for rb in range(2) for kh in range(2)]
            for n, o in enumerate(_left(*a)):
                xa_s[n, pl.ds(r0, HQ), :] = pltpu.bitcast(o.astype(BF16).T, U32)

        def wq_blocks(g, p, never=None, link=None, halves=(0, 1), src=None):
            for kh in halves:
                w = pltpu.bitcast(wq_r[kh, pl.ds(2 * p, 2), g if src is None else src], U32)
                w = [w[e] if link is None else jnp.where(never, link, w[e]) for e in range(2)]
                for par, u in enumerate(_split_heads(*w)):
                    (wq0_s, wq1_s)[g][2 * kh + par, pl.ds(p, 8, stride=pq), :] = u

        x_copy(0).wait()
        x_operands(0)

        def first_heads(kh):
            def chunk(j, _):
                wq0_copy(kh, j).wait()
                for k in range(mq // 2):
                    wq_blocks(0, j * (mq // 2) + k, halves=(kh,))
                return 0
            jax.lax.fori_loop(0, NCH, chunk, 0)
        first_heads(0)

        def q_step(g, j, side, early=()):
            m, count = [{} for _ in range(4)], [0]

            def product(r, n):
                w = _right_one(n, [lambda e=e: jnp.concatenate(
                    [_as_bf16((wq0_s, wq1_s)[g][e, pl.ds((dt * 4 + r) * pq, mh // 2), :]) for dt in range(2)],
                    axis=1) for e in range(4)])
                m[r][n] = jnp.dot(_as_bf16(xa_s[n, pl.ds(pl.multiple_of(j * HQ, HQ), HQ), :]), w.astype(BF16),
                                  preferred_element_type=F32)
                for k in range(5):
                    side(count[0], m[r][n][k * 48:k * 48 + 8, (k % 2) * L:(k % 2 + 1) * L])
                    count[0] += 1
            for r in range(4):
                for n in early:
                    product(r, n)
            for r in range(4):
                for n in (4, 0, 3, 6, 1, 2, 5):
                    if n not in early:
                        product(r, n)
                for par, rb, comb in ((0, 0, _c11), (0, 1, _c21), (1, 0, _c12), (1, 1, _c22)):
                    r0 = pl.multiple_of(j * TQ + rb * HQ, HQ)
                    q_s[8 * g + 2 * r + par, pl.ds(r0, HQ), :] = _to_u32(comb(m[r]) * qscale)

        def q_lo(j, _):
            never = _never(j)

            share = -(-(mh // 2) // (NCH - 1))
            p0 = jnp.clip((j - 1) * share, 0, mh // 2 - share)

            def side(k, piece):
                if k == 39:
                    pl.when(j == 0)(lambda: first_heads(1))
                    pl.when(j + 1 < NCH)(lambda: x_copy(j + 1).wait())
                    pl.when(j == 1)(lambda: wq1_copy(0).wait())
                    pl.when(j > 0)(lambda: wq1_copy(j).wait())
                if k >= 46 and k % 2 == 0 and (k - 46) // 2 < share:
                    wq_blocks(1, p0 + (k - 46) // 2, never, pltpu.bitcast(piece, U32), src=jnp.minimum(j, 1))
            q_step(0, j, side, early=(1, 5))
            x_operands((j + 1) & (NCH - 1))
            return 0
        jax.lax.fori_loop(0, NCH, q_lo, 0)

        def q_hi(j, _):
            for cp in kv_copies(j):
                cp.wait()
            never = _never(j)
            quad = []

            def side(kk, piece):
                if kk >= 128:
                    return
                k, g = kk // 2, kk % 2
                link = pltpu.bitcast(piece, U32)
                if g == 0:
                    rg, t = k // 8 + 8 * (k % 4 // 2), k // 4 % 2 + 2 * (k % 2)
                    a = []
                    for rb in range(2):
                        r0 = pl.multiple_of(j * RC + rb * TQ + rg * 16, 16)
                        for ch in range(2):
                            a.append(c_s[pl.ds(r0, 16), (2 * t + ch) * L:(2 * t + ch + 1) * L].astype(F32))
                    a[0] = jnp.where(jnp.concatenate([never, never], axis=0),
                                     jnp.concatenate([piece, piece], axis=0), a[0])
                    ops = _left(*a)
                    us = [_to_u32(ops[n]) for n in FLAT]
                    d0 = pl.multiple_of(j * HQ + rg * 8, 8)
                    for n, u in enumerate(us):
                        a_s[n, pl.ds(d0, 8), t * L:(t + 1) * L] = u
                    quad.append(ops)
                    if len(quad) == 4:
                        d0 = pl.multiple_of(j * (HQ // 2) + (rg - 8) * 8, 8)
                        for e, n in enumerate(DEEP):
                            deep = [_to_u32(o) for o in _left(*[q[n] for q in quad])]
                            for x, u in enumerate(deep):
                                a2_s[e, x, pl.ds(d0, 8), (t - 2) * L:(t - 1) * L] = u
                            us += deep
                        del quad[:]
                    link = _or_all(us)
                c0 = j * mk + 2 * k
                for e, (o, r) in enumerate((o, r) for o in (0, L) for r in (wk_r, wv_r)):
                    w = pltpu.bitcast(r[pl.ds(c0 + o, 2), g], U32)
                    for par, u in enumerate(_split_heads(jnp.where(never, link, w[0]), jnp.where(never, link, w[1]))):
                        b_s[e, 2 * g + par, pl.ds(j * (mk // 4) + k, 8, stride=pb), :] = u
            q_step(1, j, side)
            return j
        never = _never(jax.lax.fori_loop(0, NCH, q_hi, 0))

        for cp in misc:
            cp.wait()
        st = {}
        F = wg_s.shape[1]

        def route(pieces):
            pieces = pieces[-2] + pieces[-1]
            mp = -(-M // L) * L
            cols = []
            for w_s in (wr_s, gw_s):
                w = jnp.concatenate([w_s[...].reshape(1, M).astype(F32), jnp.zeros((1, mp - M), F32)], axis=1)
                cols.append(jnp.broadcast_to(w, (L, mp)).T)
            nr, rows = 4, M // 4
            out, k, prev = ([], []), 0, None
            for ct in range(S // L):
                acc = [None, None]
                for q in range(nr):
                    link = pieces[int((FFN_TUNE[0] + FFN_TUNE[1] * k / (nr * S // L)) * len(pieces))]
                    if prev is not None:
                        link = jnp.where(never, link, prev)
                    k += 1
                    x = linked(xT_s[ct * L // RC, q * rows:(q + 1) * rows, pl.ds(ct * L % RC, L)], link)
                    for t in range(2):
                        part = fold(x * cols[t][q * rows:(q + 1) * rows], 0)
                        acc[t] = part if acc[t] is None else acc[t] + part
                    prev = acc[0] + acc[1]
                for t in range(2):
                    out[t].append(jnp.sum(acc[t], axis=0, keepdims=True))
            gate = jax.nn.sigmoid(jnp.concatenate(out[1], axis=1))
            for j in range(S // RC):
                g_s[j, 0:1, :] = gate[:, j * RC:(j + 1) * RC]
            r = jnp.concatenate(out[0], axis=1).astype(BF16).astype(F32)
            lane = jax.lax.broadcasted_iota(jnp.int32, (1, S), 1)
            m1 = jnp.max(r, axis=1, keepdims=True)
            i1 = jnp.min(jnp.where(r == m1, lane, S - 1), axis=1, keepdims=True)
            r2 = jnp.where(lane == i1, -jnp.inf, r)
            m2 = jnp.max(r2, axis=1, keepdims=True)
            i2 = jnp.min(jnp.where(jnp.logical_and(r2 == m2, lane != i1), lane, S - 1), axis=1, keepdims=True)
            ln = jax.lax.broadcasted_iota(jnp.int32, (M, L), 1)
            st["at"] = [(i[0, 0] >> 9, slice(None), pl.ds(pl.multiple_of(i[0, 0] & (RC - L), L), L))
                        for i in (i1, i2)]
            st["hit"] = [ln == (i & (L - 1)) for i in (i1, i2)]
            st["r"] = [jax.nn.sigmoid(m1), jax.nn.sigmoid(m2)]
            st["x"] = [jnp.broadcast_to(jnp.sum(jnp.where(hit, xT_s[at].astype(F32), 0.0),
                                                axis=1, keepdims=True), (M, L))
                       for at, hit in zip(st["at"], st["hit"])]

        def fold(v, axis):
            parts = [v[k * 8:(k + 1) * 8] if axis == 0 else v[:, k * L:(k + 1) * L]
                     for k in range(v.shape[axis] // (8, L)[axis])]
            while len(parts) > 1:
                parts = [parts[k] + parts[k + 1] if k + 1 < len(parts) else parts[k]
                         for k in range(0, len(parts), 2)]
            return parts[0]

        def linked(w, link):
            w = pltpu.bitcast(w, U32)
            reps = (w.shape[0] // 8, w.shape[1] // L)
            w = jnp.where(jnp.tile(never, reps), jnp.tile(pltpu.bitcast(link, U32), reps), w)
            return _as_bf16(w).astype(F32)

        def hidden(pieces):
            pieces = pieces[-3] + pieces[-2] + pieces[-1]
            nr, rows = 4, M // 4
            total = 2 * (F // L) * nr
            out, k, prev = [], 0, None
            for w_s in (wg_s, wu_s):
                cols = ([], [])
                for ct in range(F // L):
                    acc = [None, None]
                    for q in range(nr):
                        link = pieces[int((FFN_TUNE[2] + FFN_TUNE[3] * k / total) * len(pieces))]
                        if prev is not None:
                            link = jnp.where(never, link, prev)
                        k += 1
                        w = linked(w_s[q * rows:(q + 1) * rows, ct * L:(ct + 1) * L], link)
                        for t in range(2):
                            part = fold(w * st["x"][t][q * rows:(q + 1) * rows], 0)
                            acc[t] = part if acc[t] is None else acc[t] + part
                        prev = acc[0] + acc[1]
                    for t in range(2):
                        cols[t].append(jnp.sum(acc[t], axis=0, keepdims=True))
                out.append([jnp.concatenate(c, axis=1) for c in cols])
            st["h"] = [(jax.nn.silu(out[0][t]) * out[1][t]).astype(BF16).astype(F32) for t in range(2)]

        def patch(pieces):
            pieces = pieces[-2] + pieces[-1]
            half = F // 2
            ys, k, prev = ([], []), 0, None
            for rg in range(M // 16):
                acc = [None, None]
                for hf in range(2):
                    link = pieces[int((FFN_TUNE[4] + FFN_TUNE[5] * k / (M // 8)) * len(pieces))]
                    if prev is not None:
                        link = jnp.where(never, link, prev)
                    k += 1
                    w = linked(wd_s[rg * 16:(rg + 1) * 16, hf * half:(hf + 1) * half], link)
                    for t in range(2):
                        part = fold(w * st["h"][t][:, hf * half:(hf + 1) * half], 1)
                        acc[t] = part if acc[t] is None else acc[t] + part
                    prev = fold(acc[0] + acc[1], 0)
                for t in range(2):
                    ys[t].append(jnp.sum(acc[t], axis=1, keepdims=True))
            for t in range(2):
                y = jnp.concatenate(ys[t], axis=0) * st["r"][t]
                blk = xT_s[st["at"][t]].astype(F32)
                xT_s[st["at"][t]] = (blk + jnp.where(st["hit"][t], y, 0.0)).astype(BF16)

        head_program(FIRST_ORDER, None, 0, never, hooks=(route, hidden, patch))

    def phase2(x7_s, wo_ops):
        wo_copy.wait()
        tri = jax.lax.broadcasted_iota(jnp.int32, (L, L), 1) <= jax.lax.broadcasted_iota(jnp.int32, (L, L), 0)

        def head(h, _):
            head_program(LOOP_ORDER, h, h + 1, _never(h), x7_s, tri, wo_ops, LOOP_TUNE)
            return h
        last = jax.lax.fori_loop(0, H - 1, head, 0)
        head_program(LAST_ORDER, H - 1, None, _never(last), x7_s, tri, tune=LAST_TUNE)

        def out_step(j):
            m = ({}, {})
            for n in range(7):
                right = [[] for _ in range(7)]
                for pair in range(H // 2):
                    blk = [_as_bf16(x7_s[n, 2 * pair + par, pl.ds(pl.multiple_of(j * L + t * 64, 64), 64), :])
                           for par in range(2) for t in range(2)]
                    ops = list(_right(*[v.astype(F32) for v in blk]))
                    ops[1], ops[4] = blk[0], blk[3]
                    for x in range(7):
                        right[x].append(ops[x])
                mm = {x: jax.lax.dot_general(
                    jnp.concatenate([_as_bf16(wo_ops[n, x, pair, :M // 8]) for pair in range(H // 2)], axis=1),
                    jnp.concatenate(right[x], axis=1).astype(BF16), NT, preferred_element_type=F32)
                    for x in (4, 2, 1, 5, 0, 3, 6)}
                m[0][n] = jnp.concatenate([((mm[0] + mm[3]) - mm[4]) + mm[6], _c21(mm)], axis=0)
                m[1][n] = jnp.concatenate([_c12(mm), _c22(mm)], axis=0)
            gate = g_s[j, 0:1, :]
            for hf in (1, 0):
                rest = (1.0 - gate) * xT_s[j, hf * mh:(hf + 1) * mh, :].astype(F32)
                cols = []
                for t in range(RC // TQ):
                    gl, gr = gate[:, t * TQ:t * TQ + L], gate[:, t * TQ + L:(t + 1) * TQ]
                    rl, rr = rest[:, t * TQ:t * TQ + L], rest[:, t * TQ + L:(t + 1) * TQ]
                    if hf:
                        cols += [gl * _c21(m[t]) + rl, gr * _c22(m[t]) + rr]
                    else:
                        cols += [(gl * ((m[t][0] + m[t][3]) - m[t][4]) + rl) + gl * m[t][6], gr * _c12(m[t]) + rr]
                o_s[j, hf * mh:(hf + 1) * mh, :] = jnp.concatenate(cols, axis=1).astype(BF16)
                out_copy(j, hf).start()

        def out_steps(i, _):
            for k in range(O_UNROLL):
                out_step(i * O_UNROLL + k)
            return 0
        jax.lax.fori_loop(0, S // RC // O_UNROLL, out_steps, 0)
        for j in range(S // RC):
            for hf in range(2):
                out_copy(j, hf).wait()

    pl.run_scoped(
        phase1,
        *[pltpu.VMEM(r.shape, r.dtype) for r in (c_hbm, wq_hbm, wk_hbm, wv_hbm, wg_hbm, wu_hbm, wd_hbm)],
        pltpu.VMEM((7, S // 4, mh), U32),
        pltpu.VMEM((4, -(-pq // 4) * 32, L), U32),
        pltpu.VMEM((4, -(-pq // 4) * 32, L), U32),
        pltpu.VMEM((M,), BF16),
        pltpu.VMEM((M,), BF16))
    pl.run_scoped(phase2, pltpu.VMEM((7, H, S // 4, L), U32), pltpu.VMEM((7, 7, H // 2, 64, L), U32))


def _tile_view(w):
    c, h, d = w.shape
    w = w.reshape(c, h // 8, 8, d // L, L).transpose(0, 1, 3, 2, 4)
    return w.reshape(c, h // 8, 8 * (d // L), L)


@jax.jit
def pallas_gated_mix__compressed_kv_cla__moe_arch_mod__prompt_kernel(
    A_x: jax.Array,
    A_c_kv: jax.Array,
    A_w_q: jax.Array,
    A_w_uk: jax.Array,
    A_w_uv: jax.Array,
    A_w_o: jax.Array,
    B_x: jax.Array,
    B_w_r: jax.Array,
    B_w_gate: jax.Array,
    B_w_up: jax.Array,
    B_w_down: jax.Array,
    gate_w: jax.Array,
):
    _, S, M = A_x.shape
    DC = A_c_kv.shape[2]
    H, D = A_w_q.shape[1], A_w_q.shape[2]
    args = (jnp.transpose(A_x[0]), A_c_kv[0], _tile_view(A_w_q).reshape(2, M // 2, 2, 16, L),
            _tile_view(A_w_uk), _tile_view(A_w_uv),
            jnp.transpose(A_w_o, (0, 2, 1)), B_w_r, gate_w, B_w_gate, B_w_up, jnp.transpose(B_w_down))

    def kern(*refs):
        _kernel(*refs, S=S, M=M, DC=DC, H=H, D=D)

    hbm = pl.BlockSpec(memory_space=pl.ANY)
    oT = pl.pallas_call(
        kern,
        out_shape=jax.ShapeDtypeStruct((M, S), A_x.dtype),
        in_specs=[hbm] * len(args),
        out_specs=hbm,
        scratch_shapes=[
            pltpu.VMEM((S // RC, 8, RC), F32),
            pltpu.VMEM((S // RC, M, RC), BF16),
            pltpu.VMEM((H, M, D), BF16),
            pltpu.VMEM((5, S // 4, DC // 2), U32),
            pltpu.VMEM((2, 7, S // 8, DC // 4), U32),
            pltpu.VMEM((4, 4, 8 * (DC // 4 + 4), L), U32),
            pltpu.VMEM((H, S // 2, D), U32),
            pltpu.VMEM((S // 2, D), U32),
            pltpu.VMEM((S // 2, D), U32),
            pltpu.VMEM((5, S // 4, L), U32),
            pltpu.VMEM((S // RC, M, RC), BF16),
            pltpu.VMEM((5, S // 4 + PAD_V, L), U32),
            pltpu.SemaphoreType.DMA((N_SEM,)),
        ],
        compiler_params=pltpu.CompilerParams(vmem_limit_bytes=124 * 1024 * 1024, disable_bounds_checks=True,
                                             disable_semaphore_checks=True),
    )(*args)
    return jnp.transpose(oT)[None]
```
